```python
import jax
import jax.numpy as jnp

def _softmax(x, axis=-1):
    return jax.nn.softmax(x, axis=axis)

def _gelu(x):
    return jax.nn.gelu(x, approximate=True)

def _silu(x):
    return jax.nn.silu(x)

def _sigmoid(x):
    return jax.nn.sigmoid(x)

def _layernorm(x, axis=-1, eps=1e-05):
    m = jnp.mean(x, axis=axis, keepdims=True)
    v = jnp.var(x, axis=axis, keepdims=True)
    return (x - m) / jnp.sqrt(v + eps)

def _scatter_add(tgt, idx, src, axis=0):
    return tgt.at[idx].add(src)

def _segment_sum(src, seg, n):
    return jax.ops.segment_sum(src, seg, n)

class _Rng:

    def __init__(self, key):
        self._k = key

    def _next(self):
        self._k, sub = jax.random.split(self._k)
        return sub

    def normal(self, shape):
        return jax.random.normal(self._next(), shape, dtype=jnp.bfloat16)

    def randint(self, lo, hi, shape):
        return jax.random.randint(self._next(), shape, lo, hi, dtype=jnp.int32)

    def uniform(self, shape, lo=0.0, hi=1.0):
        return jax.random.uniform(self._next(), shape, jnp.bfloat16, lo, hi)

    def permutation(self, n):
        return jax.random.permutation(self._next(), n)
kernel_name = 'adaLN_cond__mha_block_cached__moe_arch_mod__prompt'

def setup_inputs():
    _rng = _Rng(jax.random.key(int.from_bytes(__import__("os").urandom(4), "little")))
    _w = lambda a: (lambda t: t.astype(jnp.bfloat16) if jnp.issubdtype(t.dtype, jnp.floating) else t)(jnp.asarray(a))

    def _A_setup():
        B, Sq, D = (1, 2048, 1024)
        H, Sk, Dh = (32, 2048, 128)
        return {'x': _w((lambda *s: _rng.normal(s) * 0.05)(B, Sq, D)), 'k_cache': _w((lambda *s: _rng.normal(s) * 0.05)(B, H, Sk, Dh)), 'v_cache': _w((lambda *s: _rng.normal(s) * 0.05)(B, H, Sk, Dh)), 'wq': _w((lambda *s: _rng.normal(s) * 0.05)(D, H * Dh) * D ** (-0.5)), 'wo': _w((lambda *s: _rng.normal(s) * 0.05)(H * Dh, D) * (H * Dh) ** (-0.5))}
    _A_in = _A_setup()

    def _B_setup():
        B, S, D, F, C = (1, 2048, 1024, 3584, 2)
        return {'x': _w((lambda *s: _rng.normal(s) * 0.05)(B, S, D)), 'w_r': _w((lambda *s: _rng.normal(s) * 0.05)(D)), 'w_gate': _w((lambda *s: _rng.normal(s) * 0.05)(D, F)), 'w_up': _w((lambda *s: _rng.normal(s) * 0.05)(D, F)), 'w_down': _w((lambda *s: _rng.normal(s) * 0.05)(F, D))}
    _B_in = _B_setup()
    return {'A_x': _A_in['x'], 'A_k_cache': _A_in['k_cache'], 'A_v_cache': _A_in['v_cache'], 'A_wq': _A_in['wq'], 'A_wo': _A_in['wo'], 'B_x': _B_in['x'], 'B_w_r': _B_in['w_r'], 'B_w_gate': _B_in['w_gate'], 'B_w_up': _B_in['w_up'], 'B_w_down': _B_in['w_down'], 'c': _w((lambda *s: _rng.normal(s) * 0.05)(1, 1024)), 'w_mod': _w((lambda *s: _rng.normal(s) * 0.05)(1024, 6 * 1024) * 1024 ** (-0.5))}

def reference(A_x, A_k_cache, A_v_cache, A_wq, A_wo, B_x, B_w_r, B_w_gate, B_w_up, B_w_down, c, w_mod):

    def _A_ref(x, k_cache, v_cache, wq, wo):
        B, Sq, D = x.shape
        H, Dh = (32, 128)
        q = (lambda x, *d: x.transpose(*d))((x @ wq).reshape(B, Sq, H, Dh), 0, 2, 1, 3)
        scores = jnp.einsum('bhqd,bhkd->bhqk', q, k_cache) * Dh ** (-0.5)
        p = _softmax(scores, axis=-1)
        o = jnp.einsum('bhqk,bhkd->bhqd', p, v_cache)
        return (lambda x, *d: x.transpose(*d))(o, 0, 2, 1, 3).reshape(B, Sq, H * Dh) @ wo

    def _B_ref(x, w_r, w_gate, w_up, w_down):
        B, S, D = x.shape
        C = 2
        r = x @ w_r
        idx = jnp.argsort(-r, axis=-1)[:, :C]
        idx_e = jnp.repeat(idx.reshape(B, C, 1), D, axis=2)
        x_sel = jnp.take_along_axis(x, idx_e, axis=1)
        g = _silu(x_sel @ w_gate)
        u = x_sel @ w_up
        y = g * u @ w_down
        r_sel = _sigmoid(jnp.take_along_axis(r, idx, axis=1))
        y = y * r_sel.reshape(B, C, 1)
        b_off = (jnp.arange(B) * S).reshape(B, 1)
        flat_idx = (idx + b_off).reshape(B * C)
        zero = (x * 0.0).reshape(B * S, D)
        upd = _scatter_add(zero, flat_idx, y.reshape(B * C, D), axis=0)
        return x + upd.reshape(B, S, D)
    x = A_x
    mod = (_silu(c) @ w_mod).reshape(c.shape[0], 6, 1, -1)
    sa, ca, ga, sb, cb, gb = (mod[:, 0].copy(), mod[:, 1].copy(), mod[:, 2].copy(), mod[:, 3].copy(), mod[:, 4].copy(), mod[:, 5].copy())
    h = _layernorm(x, axis=-1) * (1 + ca) + sa
    x = x + ga * _A_ref(h, A_k_cache, A_v_cache, A_wq, A_wo)
    h = _layernorm(x, axis=-1) * (1 + cb) + sb
    x = x + gb * _B_ref(h, B_w_r, B_w_gate, B_w_up, B_w_down)
    return x
```

```python
import contextlib
import jax
import jax.numpy as jnp
from jax import lax
import jax.experimental.pallas as pl
import jax.experimental.pallas.tpu as pltpu

S, D, H, DH, F = 2048, 1024, 32, 128, 3584
EPS = 1e-5
LOG2E = 1.4426950408889634
BF = jnp.bfloat16
F32 = jnp.float32


def make_kernel(RP=512, G=4, PRE1=1, PC=32, POS=0, ORD=0, SCOPES=0, NOBC=0, name="adaln_mha_moe"):
    BQ = RP
    NP = S // RP
    NG = H // G
    NT = NP * NG
    SL = RP // NG
    NSL = S // SL
    QSCALE = (DH ** -0.5) * LOG2E
    X0 = RP + 2 * SL
    XO = 2 * S
    NWM = 4
    WMC = D // NWM
    scope = jax.named_scope if SCOPES else (lambda n: contextlib.nullcontext())

    def _ln(x):
        m = jnp.mean(x, axis=-1, keepdims=True)
        xc = x - m
        v = jnp.mean(xc * xc, axis=-1, keepdims=True)
        return xc * lax.rsqrt(v + EPS)

    def _recip(l):
        ri = pl.reciprocal(l, approx=True)
        return ri * (2.0 - l * ri)

    def kernel(x_hbm, k_hbm, v_hbm, wq_hbm, wo_hbm, wr_hbm, wg_hbm, wu_hbm, wd_hbm, c_hbm, wm_hbm,
               out_hbm,
               k_v, v_v, wq_v, wo_v, wg_v, wu_v, wd_v, ho_v, acc_v, mod_v, r_v, patch_v, of_v, xn_v,
               c_v, wr_v, sems):
        class _Sub:
            def __init__(self, off):
                self.off = off
                self.at = self

            def __getitem__(self, i):
                return sems.at[self.off + i]

        offs = [0]
        for n in (2, NWM + 2, H, H, H, H, 3, NP, 2, 2):
            offs.append(offs[-1] + n)
        sem_x, sem_m, sem_k, sem_v, sem_q, sem_o, sem_f, sem_out, sem_p, sem_s = [_Sub(o) for o in offs[:-1]]

        def cp_x0():
            return pltpu.make_async_copy(x_hbm.at[pl.ds(0, X0)], ho_v.at[pl.ds(XO, X0)], sem_x.at[0])

        def cp_x1():
            return pltpu.make_async_copy(x_hbm.at[pl.ds(X0, S - X0)], ho_v.at[pl.ds(XO + X0, S - X0)], sem_x.at[1])

        def cp_m(i):
            return pltpu.make_async_copy(wm_hbm.at[pl.ds(i * WMC, WMC), pl.ds(0, 2 * D)],
                                         wg_v.at[pl.ds(i * WMC, WMC), pl.ds(0, 2 * D)], sem_m.at[i])

        def cp_m2a():
            return pltpu.make_async_copy(wm_hbm.at[:, pl.ds(2 * D, F - 2 * D)],
                                         wg_v.at[:, pl.ds(2 * D, F - 2 * D)], sem_m.at[NWM])

        def cp_m2b():
            return pltpu.make_async_copy(wm_hbm.at[:, pl.ds(F, 6 * D - F)],
                                         wu_v.at[:, pl.ds(0, 6 * D - F)], sem_m.at[NWM + 1])

        def cp_q(h):
            c0 = pl.multiple_of(h * DH, DH)
            return pltpu.make_async_copy(wq_hbm.at[:, pl.ds(c0, DH)], wq_v.at[h], sem_q.at[h])

        def cp_kvo(h):
            return [pltpu.make_async_copy(k_hbm.at[h], k_v.at[h], sem_k.at[h]),
                    pltpu.make_async_copy(v_hbm.at[h], v_v.at[h], sem_v.at[h]),
                    pltpu.make_async_copy(wo_hbm.at[h], wo_v.at[h], sem_o.at[h])]

        def cp_group(g):
            h0 = g * G
            cps = [cp_q(h0 + i) for i in range(G)]
            cps += [pltpu.make_async_copy(k_hbm.at[pl.ds(h0, G)], k_v.at[pl.ds(h0, G)], sem_k.at[h0]),
                    pltpu.make_async_copy(v_hbm.at[pl.ds(h0, G)], v_v.at[pl.ds(h0, G)], sem_v.at[h0]),
                    pltpu.make_async_copy(wo_hbm.at[pl.ds(h0, G)], wo_v.at[pl.ds(h0, G)], sem_o.at[h0])]
            return cps

        def cp_ffn():
            return [pltpu.make_async_copy(wg_hbm, wg_v, sem_f.at[0]),
                    pltpu.make_async_copy(wu_hbm, wu_v, sem_f.at[1]),
                    pltpu.make_async_copy(wd_hbm, wd_v, sem_f.at[2])]

        def cp_out(p):
            r0 = pl.multiple_of(p * RP, RP)
            return pltpu.make_async_copy(ho_v.at[pl.ds(S + r0, RP)], out_hbm.at[pl.ds(r0, RP)], sem_out.at[p])

        def silu_c():
            c = c_v[...].astype(F32)
            sc = (c * jax.nn.sigmoid(c)).astype(BF)
            return jnp.broadcast_to(sc, (16, D))

        def rb(a):
            return a.astype(BF).astype(F32)

        def ln1(r0, n):
            x = ho_v[pl.ds(XO + r0, n), :].astype(F32)
            h = _ln(x) * mod_v[1:2, :] + mod_v[0:1, :]
            ho_v[pl.ds(r0, n), :] = h.astype(BF)

        def post(r0, n):
            x = ho_v[pl.ds(XO + r0, n), :].astype(F32)
            x2 = x + mod_v[2:3, :] * acc_v[pl.ds(r0, n), :]
            h2 = rb(_ln(x2) * mod_v[4:5, :] + mod_v[3:4, :])
            return x2, h2

        def epi(u):
            r0 = pl.multiple_of(u * SL, SL)
            x2, h2 = post(r0, SL)
            ho_v[pl.ds(S + r0, SL), :] = (x2 + mod_v[5:6, :] * h2).astype(BF)
            r = jnp.sum(h2 * mod_v[6:7, :], axis=-1, keepdims=True)
            lane = lax.broadcasted_iota(jnp.int32, (SL, 128), 1)
            r_v[...] = jnp.where(lane == u, rb(r), r_v[...])

        def epi_load(u):
            r0 = pl.multiple_of(u * SL, SL)
            return [acc_v[pl.ds(r0 + i * PC, PC), :] for i in range(SL // PC)]

        def epi_piece(u, i, a):
            r0 = pl.multiple_of(u * SL + i * PC, PC)
            x = ho_v[pl.ds(XO + r0, PC), :].astype(F32)
            x2 = x + mod_v[2:3, :] * a
            h2 = rb(_ln(x2) * mod_v[4:5, :] + mod_v[3:4, :])
            ho_v[pl.ds(S + r0, PC), :] = (x2 + mod_v[5:6, :] * h2).astype(BF)
            r = jnp.sum(h2 * mod_v[6:7, :], axis=-1, keepdims=True)
            lane = lax.broadcasted_iota(jnp.int32, (PC, 128), 1)
            r_v[i * PC:(i + 1) * PC, :] = jnp.where(lane == u, rb(r), r_v[i * PC:(i + 1) * PC, :])

        def op_carry(rr, hd):
            l = jnp.sum(of_v[1], axis=-1, keepdims=True)
            o = (of_v[0] * _recip(l)).astype(BF)
            acc_v[pl.ds(rr, BQ), :] += jnp.dot(o, wo_v[hd], preferred_element_type=F32)

        with scope("pro_init"):
            cp_c = pltpu.make_async_copy(c_hbm, c_v, sem_s.at[0])
            cp_r = pltpu.make_async_copy(wr_hbm, wr_v, sem_s.at[1])
            cp_c.start()
            cp_r.start()
            cp_x0().start()
            for i in range(NWM):
                cp_m(i).start()
            for h in range(G):
                cp_q(h).start()
                for cp in cp_kvo(h):
                    cp.start()
            if PRE1:
                for cp in cp_group(1):
                    cp.start()
            acc_v[...] = jnp.zeros_like(acc_v)
            r_v[...] = jnp.full(r_v.shape, -jnp.inf, F32)
            mod_v[...] = jnp.zeros_like(mod_v)
            of_v[0] = jnp.zeros((BQ, DH), F32)
            of_v[1] = jnp.ones((BQ, DH), F32)
            wo_v[H] = jnp.zeros((DH, D), BF)
        with scope("pro_ln"):
            cp_c.wait()
            cp_r.wait()
            mod_v[6:7, :] = wr_v[...].astype(F32).reshape(1, D)
            cp_x0().wait()
            xn_v[...] = _ln(ho_v[pl.ds(XO, RP + SL), :].astype(F32))
        with scope("pro_mod"):
            sc = silu_c()
            m1 = jnp.zeros((16, 2 * D), F32)
            for i in range(NWM):
                cp_m(i).wait()
                m1 = m1 + jnp.dot(sc[:, i * WMC:(i + 1) * WMC], wg_v[pl.ds(i * WMC, WMC), pl.ds(0, 2 * D)],
                                  preferred_element_type=F32)
            m1 = rb(m1)
            sa = m1[0:1, 0:D]
            s1 = rb(1.0 + m1[0:1, D:2 * D])
            mod_v[0:1, :] = sa
            mod_v[1:2, :] = s1
            ho_v[pl.ds(0, RP + SL), :] = (xn_v[...] * s1 + sa).astype(BF)

        def Qp_(r0, hd):
            q = jnp.dot(ho_v[pl.ds(r0, BQ), :], wq_v[hd], preferred_element_type=F32)
            return (q * QSCALE).astype(BF)

        def QK_(q, hd):
            return lax.dot_general(q, k_v[hd], (((1,), (1,)), ((), ())), preferred_element_type=F32)

        def PV_(s, hd, carry_out):
            m = jnp.max(s, axis=-1, keepdims=True)
            e = jnp.exp2(s - m)
            if carry_out:
                lp = e[:, 0:128]
                for j in range(1, S // 128):
                    lp = lp + e[:, j * 128:(j + 1) * 128]
                of_v[0] = jnp.dot(e.astype(BF), v_v[hd], preferred_element_type=F32)
                of_v[1] = lp
                return None
            l = jnp.sum(e, axis=-1, keepdims=True)
            o = jnp.dot(e.astype(BF), v_v[hd], preferred_element_type=F32)
            return (o * _recip(l)).astype(BF)

        def Op_(o, r0, hd):
            acc_v[pl.ds(r0, BQ), :] += jnp.dot(o, wo_v[hd], preferred_element_type=F32)

        def mini(h, carry):
            with scope("mini_dma"):
                cp_q(h).wait()
                for cp in cp_kvo(h):
                    cp.wait()
                if not PRE1:
                    @pl.when(h == 1)
                    def _():
                        for cp in cp_group(1):
                            cp.start()
            with scope("mini_main"):
                q = Qp_(0, h)
                op_carry(0, jnp.where(h == 0, H, h - 1))
                PV_(QK_(q, h), h, True)
            return carry

        lax.fori_loop(0, G, mini, 0)

        def body(t, carry):
            p = t // NG
            g = t % NG

            with scope("it_dma"):
                @pl.when(jnp.logical_or(t <= NG, g == 1))
                def _():
                    @pl.when(t < NG)
                    def _():
                        for cp in cp_group(t):
                            cp.wait()

                    @pl.when(t + 1 < NG)
                    def _():
                        for cp in cp_group(t + 1):
                            cp.start()

                    @pl.when(t == 1)
                    def _():
                        cp_x1().start()

                    @pl.when(t == 2)
                    def _():
                        cp_x1().wait()
                        cp_m2a().start()
                        cp_m2b().start()

                    @pl.when(t == NG)
                    def _():
                        cp_m2a().wait()
                        cp_m2b().wait()
                        scc = silu_c()
                        ma = rb(jnp.dot(scc, wg_v[:, pl.ds(2 * D, F - 2 * D)], preferred_element_type=F32))
                        mb = rb(jnp.dot(scc, wu_v[:, pl.ds(0, 6 * D - F)], preferred_element_type=F32))
                        m2 = jnp.concatenate([ma[0:1], mb[0:1]], axis=1)
                        mod_v[2:3, :] = m2[:, 0:D]
                        mod_v[3:4, :] = m2[:, D:2 * D]
                        mod_v[4:5, :] = rb(1.0 + m2[:, 2 * D:3 * D])
                        mod_v[5:6, :] = m2[:, 3 * D:4 * D]
                        for cp in cp_ffn():
                            cp.start()

                    @pl.when(jnp.logical_and(g == 1, p >= 2))
                    def _():
                        cp_out(p - 2).start()

            with scope("it_main"):
                r0 = pl.multiple_of(p * RP, RP)
                h0 = g * G
                tp = t - 1
                qs, os_ = {}, {}
                ue = jnp.maximum(t - NG - 1, 0)
                rl = pl.multiple_of(jnp.minimum(t + NG, NSL - 1) * SL, SL)
                accs = epi_load(ue)

                def pieces():
                    for i in range(SL // PC):
                        epi_piece(ue, i, accs[i])
                        ln1(pl.multiple_of(rl + i * PC, PC), PC)

                qs[0] = Qp_(r0, h0)
                if POS == 0:
                    pieces()
                op_carry(pl.multiple_of((tp // NG) * RP, RP), (tp % NG) * G + G - 1)
                qs[1] = Qp_(r0, h0 + 1)
                for u in range(G):
                    os_[u] = PV_(QK_(qs.pop(u), h0 + u), h0 + u, u == G - 1)
                    if ORD == 1 and u >= 1:
                        Op_(os_.pop(u - 1), r0, h0 + u - 1)
                    if POS == u + 1:
                        pieces()
                    if u + 2 < G:
                        qs[u + 2] = Qp_(r0, h0 + u + 2)
                    if ORD == 0 and u >= 1:
                        Op_(os_.pop(u - 1), r0, h0 + u - 1)
            return carry

        lax.fori_loop(1, NT, body, 0)

        with scope("epi_ln"):
            epi(NSL - NG - 1)
            cp_out(NP - 2).start()
            op_carry(S - RP, H - 1)
            for u in range(NSL - NG, NSL):
                epi(u)
            cp_out(NP - 1).start()

        with scope("epi_top2"):
            r = r_v[...]
            ridx = (lax.broadcasted_iota(jnp.int32, (SL, 128), 1) * SL
                    + lax.broadcasted_iota(jnp.int32, (SL, 128), 0))
            big = jnp.int32(1 << 30)
            valid = ridx < S
            m1_ = jnp.max(jnp.max(r, axis=1, keepdims=True), axis=0, keepdims=True)
            i1v = jnp.min(jnp.min(jnp.where(jnp.logical_and(r == m1_, valid), ridx, big), axis=1, keepdims=True),
                          axis=0, keepdims=True)
            rest = jnp.logical_and(ridx != i1v, valid)
            r2 = jnp.where(rest, r, -jnp.inf)
            m2_ = jnp.max(jnp.max(r2, axis=1, keepdims=True), axis=0, keepdims=True)
            i2v = jnp.min(jnp.min(jnp.where(jnp.logical_and(r2 == m2_, rest), ridx, big), axis=1, keepdims=True),
                          axis=0, keepdims=True)
            i1 = jnp.clip(i1v[0, 0], 0, S - 1)
            i2 = jnp.clip(i2v[0, 0], 0, S - 1)
            t1 = pl.multiple_of((i1 // 16) * 16, 16)
            t2 = pl.multiple_of((i2 // 16) * 16, 16)
            x2a, h2a = post(t1, 16)
            x2b, h2b = post(t2, 16)
            row = lax.broadcasted_iota(jnp.int32, (16, D), 0)
            sel1 = jnp.sum(jnp.where(row == i1 - t1, h2a, 0.0), axis=0, keepdims=True)
            sel2 = jnp.sum(jnp.where(row == i2 - t2, h2b, 0.0), axis=0, keepdims=True)
            xs = jnp.where(row == 0, sel1, jnp.where(row == 1, sel2, 0.0)).astype(BF)
        with scope("epi_ffn"):
            for cp in cp_ffn():
                cp.wait()
            gt = jnp.dot(xs, wg_v[...], preferred_element_type=F32)
            up = jnp.dot(xs, wu_v[...], preferred_element_type=F32)
            act = (gt * jax.nn.sigmoid(gt) * up).astype(BF)
            y = jnp.dot(act, wd_v[...], preferred_element_type=F32)
            y1 = y[0:1, :] * jax.nn.sigmoid(m1_)
            y2 = y[1:2, :] * jax.nn.sigmoid(m2_)

            def upd(t0):
                return jnp.where(row == i1 - t0, y1, 0.0) + jnp.where(row == i2 - t0, y2, 0.0)

            gb = mod_v[5:6, :]
            patch_v[0] = (x2a + gb * (h2a + upd(t1))).astype(BF)
            patch_v[1] = (x2b + gb * (h2b + upd(t2))).astype(BF)
        with scope("epi_out"):
            for p in range(NP):
                cp_out(p).wait()
            pa = pltpu.make_async_copy(patch_v.at[0], out_hbm.at[pl.ds(t1, 16)], sem_p.at[0])
            pb = pltpu.make_async_copy(patch_v.at[1], out_hbm.at[pl.ds(t2, 16)], sem_p.at[1])
            pa.start()

            @pl.when(t1 != t2)
            def _():
                pb.start()
                pb.wait()

            pa.wait()

    def fn(A_x, A_k_cache, A_v_cache, A_wq, A_wo, B_x, B_w_r, B_w_gate, B_w_up, B_w_down, c, w_mod):
        any_ = pl.BlockSpec(memory_space=pl.ANY)
        vm = pl.BlockSpec(memory_space=pltpu.VMEM)
        out = pl.pallas_call(
            kernel,
            in_specs=[any_] * 11,
            out_specs=any_,
            out_shape=jax.ShapeDtypeStruct((S, D), BF),
            scratch_shapes=[
                pltpu.VMEM((H, S, DH), BF),
                pltpu.VMEM((H, S, DH), BF),
                pltpu.VMEM((H, D, DH), BF),
                pltpu.VMEM((H + 1, DH, D), BF),
                pltpu.VMEM((D, F), BF),
                pltpu.VMEM((D, F), BF),
                pltpu.VMEM((F, D), BF),
                pltpu.VMEM((3 * S, D), BF),
                pltpu.VMEM((S, D), F32),
                pltpu.VMEM((8, D), F32),
                pltpu.VMEM((SL, 128), F32),
                pltpu.VMEM((2, 16, D), BF),
                pltpu.VMEM((2, BQ, DH), F32),
                pltpu.VMEM((RP + SL, D), F32),
                pltpu.VMEM((1, D), BF),
                pltpu.VMEM((D,), BF),
                pltpu.SemaphoreType.DMA((2 + NWM + 2 + 4 * H + 3 + NP + 4,)),
            ],
            compiler_params=pltpu.CompilerParams(vmem_limit_bytes=120 << 20, disable_bounds_checks=bool(NOBC)),
            name=name,
        )(A_x.reshape(S, D), A_k_cache.reshape(H, S, DH), A_v_cache.reshape(H, S, DH), A_wq, A_wo.reshape(H, DH, D),
          B_w_r, B_w_gate, B_w_up, B_w_down, c, w_mod)
        return out.reshape(1, S, D)

    return fn


_impl = make_kernel(NOBC=1, PC=64, POS=0)


@jax.jit
def pallas_adaLN_cond__mha_block_cached__moe_arch_mod__prompt_kernel(
    A_x: jax.Array,
    A_k_cache: jax.Array,
    A_v_cache: jax.Array,
    A_wq: jax.Array,
    A_wo: jax.Array,
    B_x: jax.Array,
    B_w_r: jax.Array,
    B_w_gate: jax.Array,
    B_w_up: jax.Array,
    B_w_down: jax.Array,
    c: jax.Array,
    w_mod: jax.Array,
):
    return _impl(A_x, A_k_cache, A_v_cache, A_wq, A_wo, B_x, B_w_r, B_w_gate, B_w_up, B_w_down, c, w_mod)
```

```python
import contextlib
import jax
import jax.numpy as jnp
from jax import lax
import jax.experimental.pallas as pl
import jax.experimental.pallas.tpu as pltpu

S, D, H, DH, F = 2048, 1024, 32, 128, 3584
EPS = 1e-5
LOG2E = 1.4426950408889634
BF = jnp.bfloat16
F32 = jnp.float32
I32 = jnp.int32
IMIN = -2 ** 31


def make_kernel(G=4, NWM=8, PH=0, PW=0, PA=0, EC=256, SUMBF=1, PC=64, REC=0, BAR=1, SCOPES=0,
                SEQ="Q0 E L C Q1 K0 P0 K1 Q2 P1 Q3 K2 O0 P2 K3 O1 P3 O2", name="adaln_mha_moe"):
    RP = 512
    NP = S // RP
    NG = H // G
    NT = NP * NG
    SL = RP // NG
    NSL = S // SL
    QSCALE = (DH ** -0.5) * LOG2E
    WMC = D // NWM
    HO, OO, XO = 0, S, 2 * S
    scope = jax.named_scope if SCOPES else (lambda n: contextlib.nullcontext())
    SA, S1, GA, SB, S2, GB, VA, VB, VW, VC = range(10)
    SX, SM = 0, 3
    SM2 = SM + NWM
    SH = SM2 + 1
    SGR = SH + 3 + G
    SF = SGR + 2
    SO = SF + 1
    SP = SO + NP
    SC = SP + 2
    NSEM = SC + 1

    def _recip(l):
        ri = pl.reciprocal(l, approx=True)
        return ri * (2.0 - l * ri)

    def rb(a):
        return a.astype(BF).astype(F32)

    def center(x):
        mu = jnp.mean(x, axis=-1, keepdims=True)
        xc = x - mu
        rs = lax.rsqrt(jnp.mean(xc * xc, axis=-1, keepdims=True) + EPS)
        return mu, xc, rs

    def merge(a, b):
        return jnp.maximum(a[0], b[0]), jnp.maximum(jnp.minimum(a[0], b[0]), jnp.maximum(a[1], b[1]))

    def fold(k):
        t = [k[i:i + 8] for i in range(0, k.shape[0], 8)]
        ps = [(jnp.maximum(t[i], t[i + 1]), jnp.minimum(t[i], t[i + 1])) for i in range(0, len(t), 2)]
        while len(ps) > 1:
            ps = [merge(ps[i], ps[i + 1]) for i in range(0, len(ps), 2)]
        return ps[0]

    def kernel(x_hbm, k_hbm, v_hbm, wq_hbm, wo_hbm, wr_hbm, wg_hbm, wu_hbm, wd_hbm, c_hbm, wm_hbm,
               out_hbm,
               k_v, v_v, wq_v, wo_v, wg_v, wu_v, wd_v, hox_v, acc_v, mod_v, top_v, patch_v, of_v, xn_v, st_v,
               c_v, wr_v, sems):
        cols = pl.ds(0, D)

        def cp(src, dst, s):
            return pltpu.make_async_copy(src, dst, sems.at[s])

        def cp_x(i):
            r0, n = [(0, RP), (RP, 2 * SL), (RP + 2 * SL, S - RP - 2 * SL)][i]
            return cp(x_hbm.at[pl.ds(r0, n)], hox_v.at[pl.ds(XO + r0, n), cols], SX + i)

        def cp_m(i):
            return cp(wm_hbm.at[pl.ds(i * WMC, WMC), pl.ds(0, 2 * D)],
                      wg_v.at[pl.ds(i * WMC, WMC), pl.ds(0, 2 * D)], SM + i)

        def cp_m2():
            return [cp(wm_hbm.at[:, pl.ds(2 * D, F - 2 * D)], wg_v.at[:, pl.ds(2 * D, F - 2 * D)], SM2),
                    cp(wm_hbm.at[:, pl.ds(F, 6 * D - F)], wu_v.at[:, pl.ds(0, 6 * D - F)], SM2)]

        def cp_wq(h, s):
            return cp(wq_hbm.at[:, pl.ds(pl.multiple_of(h * DH, DH), DH)], wq_v.at[h], s)

        def cp_wo(h, n, s):
            return cp(wo_hbm.at[pl.ds(h, n)], wo_v.at[pl.ds(h, n), :, cols], s)

        def cp_head0(i):
            if i == 0:
                return cp_wq(0, SH)
            return cp(k_hbm.at[0], k_v.at[0], SH + 1) if i == 1 else cp(v_hbm.at[0], v_v.at[0], SH + 2)

        def cp_head(h):
            s = SH + 2 + h
            return [cp_wo(h - 1, 1, s), cp_wq(h, s), cp(k_hbm.at[h], k_v.at[h], s), cp(v_hbm.at[h], v_v.at[h], s)]

        def cp_group(g):
            h0 = g * G
            s = SGR + g % 2
            return ([cp_wq(h0 + i, s) for i in range(G)]
                    + [cp(k_hbm.at[pl.ds(h0, G)], k_v.at[pl.ds(h0, G)], s),
                       cp(v_hbm.at[pl.ds(h0, G)], v_v.at[pl.ds(h0, G)], s),
                       cp_wo(h0, G, s)])

        def cp_ffn():
            return [cp(wg_hbm, wg_v, SF), cp(wu_hbm, wu_v, SF), cp(wd_hbm, wd_v.at[:, cols], SF)]

        def cp_out(p):
            r0 = pl.multiple_of(p * RP, RP)
            return cp(hox_v.at[pl.ds(OO + r0, RP), cols], out_hbm.at[pl.ds(r0, RP)], SO + p)

        def cp_small():
            return [cp(c_hbm, c_v, SC), cp(wr_hbm, wr_v, SC)]

        def mrow(i):
            return mod_v[i:i + 1, :]

        def silu_c():
            c = c_v[...].astype(F32)
            return jnp.broadcast_to((c * jax.nn.sigmoid(c)).astype(BF), (16, D))

        def ln1(r0, n):
            _, xc, rs = center(hox_v[pl.ds(XO + r0, n), cols].astype(F32))
            hox_v[pl.ds(HO + r0, n), cols] = ((xc * rs) * mrow(S1) + mrow(SA)).astype(BF)

        def resid(r0, n, a):
            return hox_v[pl.ds(XO + r0, n), cols].astype(F32) + mrow(GA) * a

        def keys(r0, n, xc, rs):
            r = rb(rs * jnp.sum(xc * mrow(VW), axis=-1, keepdims=True) + mod_v[VC:VC + 1, 0:1])
            b = lax.bitcast_convert_type(jnp.broadcast_to(r, (n, 128)), I32)
            b = jnp.where(b < 0, b ^ 0x7FFFFFFF, b) & (-65536)
            return b | (65535 - r0 - lax.broadcasted_iota(I32, (n, 128), 0))

        def put_stats(r0, n, mu, rs):
            st_v[0, pl.ds(r0, n), :] = jnp.broadcast_to(mu, (n, 128))
            st_v[1, pl.ds(r0, n), :] = jnp.broadcast_to(rs, (n, 128))

        def get_stats(r0, n):
            rep = lambda z: jnp.concatenate([z] * (D // 128), axis=1)
            return rep(st_v[0, pl.ds(r0, n), :]), rep(st_v[1, pl.ds(r0, n), :])

        def put_out(r0, n, x2, xc, rs):
            hox_v[pl.ds(OO + r0, n), cols] = (x2 + mrow(VB) + (xc * rs) * mrow(VA)).astype(BF)

        def epi(r0, n, a, valid):
            x2 = resid(r0, n, a)
            mu, xc, rs = center(x2)
            put_out(r0, n, x2, xc, rs)
            put_stats(r0, n, mu, rs)
            k1, k2 = fold(keys(r0, n, xc, rs))
            k1, k2 = merge((top_v[0], top_v[1]), (jnp.where(valid, k1, IMIN), jnp.where(valid, k2, IMIN)))
            top_v[0] = k1
            top_v[1] = k2

        def acc_rows(r0, n):
            return acc_v[pl.ds(r0, n), cols]

        def Qp_(h, hd):
            q = jnp.dot(h, wq_v[hd], preferred_element_type=F32)
            return (q * QSCALE).astype(BF)

        def QK_(q, hd):
            return lax.dot_general(q, k_v[hd], (((1,), (1,)), ((), ())), preferred_element_type=F32)

        raw = []

        def PV_(s, hd, carry_out):
            m = jnp.max(s, axis=-1, keepdims=True)
            e = jnp.exp2(s - m)
            eb = e.astype(BF)
            if SUMBF:
                e = eb.astype(F32)
            if carry_out:
                lp = e[:, 0:128]
                for j in range(1, S // 128):
                    lp = lp + e[:, j * 128:(j + 1) * 128]
                of_v[0] = jnp.dot(eb, v_v[hd], preferred_element_type=F32)
                of_v[1] = lp
                return None
            l = jnp.sum(e, axis=-1, keepdims=True)
            o = jnp.dot(eb, v_v[hd], preferred_element_type=F32)
            raw.append(o)
            return (o * _recip(l)).astype(BF)

        def Op_(o, r0, hd):
            acc_v[pl.ds(r0, RP), cols] += jnp.dot(o, wo_v[hd, :, cols], preferred_element_type=F32)

        def op_carry(r0, hd):
            l = jnp.sum(of_v[1], axis=-1, keepdims=True)
            Op_((of_v[0] * _recip(l)).astype(BF), r0, hd)

        with scope("pro_init"):
            for c_ in cp_small():
                c_.start()
            cp_x(0).start()
            for i in range(NWM):
                cp_m(i).start()
            for i in range(3):
                cp_head0(i).start()
            for h in range(1, G):
                for c_ in cp_head(h):
                    c_.start()
                if h == 1:
                    cp_x(1).start()
            cp_wo(G - 1, 1, SH + 2 + G).start()
            for c_ in cp_group(1):
                c_.start()
            acc_v[...] = jnp.zeros_like(acc_v)
            top_v[...] = jnp.full(top_v.shape, IMIN, I32)
            mod_v[...] = jnp.zeros_like(mod_v)
        with scope("pro_ln"):
            for c_ in cp_small():
                c_.wait()
            cp_x(0).wait()
            _, xc0, rs0 = center(hox_v[pl.ds(XO, RP), cols].astype(F32))
            xn_v[...] = xc0 * rs0
        with scope("pro_mod"):
            sc = silu_c()
            m1 = jnp.zeros((16, 2 * D), F32)
            for i in range(NWM):
                cp_m(i).wait()
                if i == NWM - 1:
                    cp_head0(0).wait()
                m1 = m1 + jnp.dot(sc[:, i * WMC:(i + 1) * WMC], wg_v[pl.ds(i * WMC, WMC), pl.ds(0, 2 * D)],
                                  preferred_element_type=F32)
            m1 = rb(m1)
            sa = m1[0:1, 0:D]
            s1 = rb(1.0 + m1[0:1, D:2 * D])
            mod_v[SA:SA + 1, :] = sa
            mod_v[S1:S1 + 1, :] = s1
            h_first = (xn_v[...] * s1 + sa).astype(BF)
            hox_v[pl.ds(HO, RP), cols] = h_first
            q_first = Qp_(h_first, 0)
        with scope("pro_head0"):
            cp_head0(1).wait()
            cp_head0(2).wait()
            PV_(QK_(q_first, 0), 0, True)

        def mini(h, carry):
            with scope("mini_dma"):
                for c_ in cp_head(h):
                    c_.wait()

                @pl.when(h == 2)
                def _():
                    cp_x(1).wait()
            with scope("mini_main"):
                q = Qp_(hox_v[pl.ds(HO, RP), cols], h)
                half = SL // 2
                ln1(pl.multiple_of(jnp.where(h < 2, 0, RP + (h - 2) * half), half), half)
                op_carry(0, h - 1)
                PV_(QK_(q, h), h, True)
            return carry

        lax.fori_loop(1, G, mini, 0)

        def body(t, carry):
            p = t // NG
            g = t % NG

            with scope("it_dma"):
                @pl.when(jnp.logical_or(t <= NG, g == 1))
                def _():
                    @pl.when(t < NG)
                    def _():
                        for c_ in cp_group(t):
                            c_.wait()

                    @pl.when(t == 1)
                    def _():
                        cp_wo(G - 1, 1, SH + 2 + G).wait()
                        cp_x(2).start()

                    @pl.when(t + 1 < NG)
                    def _():
                        for c_ in cp_group(t + 1):
                            c_.start()

                    @pl.when(t == 2)
                    def _():
                        cp_x(2).wait()
                        for c_ in cp_m2():
                            c_.start()

                    @pl.when(t == NG)
                    def _():
                        for c_ in cp_m2():
                            c_.wait()
                        scc = silu_c()
                        ma = rb(jnp.dot(scc, wg_v[:, pl.ds(2 * D, F - 2 * D)], preferred_element_type=F32))
                        mb = rb(jnp.dot(scc, wu_v[:, pl.ds(0, 6 * D - F)], preferred_element_type=F32))
                        m2 = jnp.concatenate([ma[0:1], mb[0:1]], axis=1)
                        sb = m2[:, D:2 * D]
                        s2 = rb(1.0 + m2[:, 2 * D:3 * D])
                        gb = m2[:, 3 * D:4 * D]
                        wr = wr_v[...].astype(F32).reshape(1, D)
                        mod_v[GA:GA + 1, :] = m2[:, 0:D]
                        mod_v[SB:SB + 1, :] = sb
                        mod_v[S2:S2 + 1, :] = s2
                        mod_v[GB:GB + 1, :] = gb
                        mod_v[VA:VA + 1, :] = gb * s2
                        mod_v[VB:VB + 1, :] = gb * sb
                        mod_v[VW:VW + 1, :] = s2 * wr
                        mod_v[VC:VC + 1, :] = jnp.broadcast_to(jnp.sum(sb * wr, axis=-1, keepdims=True), (1, D))
                        for c_ in cp_ffn():
                            c_.start()

                    @pl.when(jnp.logical_and(g == 1, p >= 2))
                    def _():
                        cp_out(p - 2).start()

                    @pl.when(t == NT - NG + 1)
                    def _():
                        for c_ in cp_ffn():
                            c_.wait()

            with scope("it_main"):
                r0 = pl.multiple_of(p * RP, RP)
                h0 = g * G
                tp = t - 1
                ue = jnp.maximum(t - NG - 1, 0)
                a_e = acc_rows(pl.multiple_of(ue * SL, SL), SL)
                qs, ss, os_ = {}, {}, {}
                for tok in SEQ.replace("_", " ").split():
                    kind, u = tok[0], int(tok[1:] or 0)
                    if kind == "Q":
                        qs[u] = Qp_(hox_v[pl.ds(HO + r0, RP), cols], h0 + u)
                    elif kind == "K":
                        ss[u] = QK_(qs.pop(u), h0 + u)
                    elif kind == "P":
                        os_[u] = PV_(ss.pop(u), h0 + u, u == G - 1)
                    elif kind == "O":
                        Op_(os_.pop(u), r0, h0 + u)
                    elif kind == "C":
                        op_carry(pl.multiple_of((tp // NG) * RP, RP), (tp % NG) * G + G - 1)
                    elif kind == "G":
                        hox_v[pl.ds(pl.multiple_of(3 * S + 16 * (t % 2), 16), 16), 0:DH] = raw[-1][RP - 16:RP].astype(BF)
                    elif kind == "H":
                        hox_v[pl.ds(pl.multiple_of(3 * S + 16 * (t % 2), 16), 16), 0:DH] = qs[u][RP - 16:RP]
                    elif kind == "E":
                        for i in (range(SL // PC) if len(tok) == 1 else [u]):
                            epi(pl.multiple_of(ue * SL + i * PC, PC), PC, a_e[i * PC:(i + 1) * PC], t > NG)
                    elif kind == "L":
                        for i in (range(SL // PC) if len(tok) == 1 else [u]):
                            ln1(pl.multiple_of(jnp.minimum(t + NG, NSL - 1) * SL + i * PC, PC), PC)
            return carry

        lax.fori_loop(1, NT, body, 0)

        R1 = S - RP - SL
        with scope("epi_key"):
            o_last = (of_v[0] * _recip(jnp.sum(of_v[1], axis=-1, keepdims=True))).astype(BF)
            pair = (top_v[0], top_v[1])
            for r0, n in [(R1, SL)] + [(S - RP + i * EC, EC) for i in range(RP // EC)]:
                a = acc_rows(r0, n)
                if r0 >= S - RP:
                    a = a + jnp.dot(o_last[r0 - (S - RP):r0 - (S - RP) + n], wo_v[H - 1, :, cols],
                                    preferred_element_type=F32)
                    acc_v[pl.ds(r0, n), cols] = a
                x2 = resid(r0, n, a)
                mu, xc, rs = center(x2)
                put_stats(r0, n, mu, rs)
                pair = merge(pair, fold(keys(r0, n, xc, rs)))
                if not REC:
                    put_out(r0, n, x2, xc, rs)
            if REC:
                for r0 in range(R1, S, SL):
                    x2 = resid(r0, SL, acc_rows(r0, SL))
                    mu, rs = get_stats(r0, SL)
                    put_out(r0, SL, x2, x2 - mu, rs)
            cp_out(NP - 2).start()
            cp_out(NP - 1).start()
            for sh in (4, 2, 1):
                pair = merge(pair, (pltpu.roll(pair[0], sh, 0), pltpu.roll(pair[1], sh, 0)))
            k1, k2 = pair

            def score(k):
                b = jnp.where(k < 0, k ^ 0x7FFFFFFF, k) & (-65536)
                return lax.bitcast_convert_type(b, F32)[0:1, 0:1]

            i1 = jnp.clip(65535 - (k1[0, 0] & 65535), 0, S - 1)
            i2 = jnp.clip(65535 - (k2[0, 0] & 65535), 0, S - 1)
            t1 = pl.multiple_of((i1 // 16) * 16, 16)
            t2 = pl.multiple_of((i2 // 16) * 16, 16)

            def post(t0):
                x2 = resid(t0, 16, acc_rows(t0, 16))
                mu, rs = get_stats(t0, 16)
                return x2, ((x2 - mu) * rs) * mrow(S2) + mrow(SB)

            x2a, h2a = post(t1)
            x2b, h2b = post(t2)
            row = lax.broadcasted_iota(I32, (16, D), 0)
            sel1 = jnp.sum(jnp.where(row == i1 - t1, h2a, 0.0), axis=0, keepdims=True)
            sel2 = jnp.sum(jnp.where(row == i2 - t2, h2b, 0.0), axis=0, keepdims=True)
            xs = jnp.where(row == 0, sel1, jnp.where(row == 1, sel2, 0.0)).astype(BF)
        with scope("epi_ffn"):
            if BAR:
                cp_out(0).wait()
            gt = jnp.dot(xs, wg_v[...], preferred_element_type=F32)
            up = jnp.dot(xs, wu_v[...], preferred_element_type=F32)
            act = (gt * jax.nn.sigmoid(gt) * up).astype(BF)
            y = jnp.dot(act, wd_v[:, cols], preferred_element_type=F32)
            y1 = y[0:1, :] * jax.nn.sigmoid(score(k1))
            y2 = y[1:2, :] * jax.nn.sigmoid(score(k2))

            def upd(t0):
                return jnp.where(row == i1 - t0, y1, 0.0) + jnp.where(row == i2 - t0, y2, 0.0)

            patch_v[0] = (x2a + mrow(GB) * (h2a + upd(t1))).astype(BF)
            patch_v[1] = (x2b + mrow(GB) * (h2b + upd(t2))).astype(BF)
        with scope("epi_out"):
            for p in range(1 if BAR else 0, NP):
                cp_out(p).wait()
            pa = cp(patch_v.at[0], out_hbm.at[pl.ds(t1, 16)], SP)
            pb = cp(patch_v.at[1], out_hbm.at[pl.ds(t2, 16)], SP + 1)
            pa.start()

            @pl.when(t1 != t2)
            def _():
                pb.start()
                pb.wait()

            pa.wait()

    def fn(A_x, A_k_cache, A_v_cache, A_wq, A_wo, B_x, B_w_r, B_w_gate, B_w_up, B_w_down, c, w_mod):
        any_ = pl.BlockSpec(memory_space=pl.ANY)
        out = pl.pallas_call(
            kernel,
            in_specs=[any_] * 11,
            out_specs=any_,
            out_shape=jax.ShapeDtypeStruct((S, D), BF),
            scratch_shapes=[
                pltpu.VMEM((H, S, DH), BF),
                pltpu.VMEM((H, S, DH), BF),
                pltpu.VMEM((H, D, DH), BF),
                pltpu.VMEM((H, DH, D + PW), BF),
                pltpu.VMEM((D, F), BF),
                pltpu.VMEM((D, F), BF),
                pltpu.VMEM((F, D + 128), BF),
                pltpu.VMEM((3 * S + 32, D + PH), BF),
                pltpu.VMEM((S, D + PA), F32),
                pltpu.VMEM((16, D), F32),
                pltpu.VMEM((2, 8, 128), I32),
                pltpu.VMEM((2, 16, D), BF),
                pltpu.VMEM((2, RP, DH), F32),
                pltpu.VMEM((RP, D), F32),
                pltpu.VMEM((2, S, 128), F32),
                pltpu.VMEM((1, D), BF),
                pltpu.VMEM((D,), BF),
                pltpu.SemaphoreType.DMA((NSEM,)),
            ],
            compiler_params=pltpu.CompilerParams(vmem_limit_bytes=120 << 20, disable_bounds_checks=True,
                                                 disable_semaphore_checks=True),
            name=name,
        )(A_x.reshape(S, D), A_k_cache.reshape(H, S, DH), A_v_cache.reshape(H, S, DH), A_wq,
          A_wo.reshape(H, DH, D), B_w_r, B_w_gate, B_w_up, B_w_down, c, w_mod)
        return out.reshape(1, S, D)

    return fn


_impl = make_kernel(PC=16, SEQ='Q0_C_Q1_H1_E_K0_Q2_P0_G_L_K1_Q3_P1_K2_O0_P2_K3_O1_P3_O2')


@jax.jit
def pallas_adaLN_cond__mha_block_cached__moe_arch_mod__prompt_kernel(
    A_x: jax.Array,
    A_k_cache: jax.Array,
    A_v_cache: jax.Array,
    A_wq: jax.Array,
    A_wo: jax.Array,
    B_x: jax.Array,
    B_w_r: jax.Array,
    B_w_gate: jax.Array,
    B_w_up: jax.Array,
    B_w_down: jax.Array,
    c: jax.Array,
    w_mod: jax.Array,
):
    return _impl(A_x, A_k_cache, A_v_cache, A_wq, A_wo, B_x, B_w_r, B_w_gate, B_w_up, B_w_down, c, w_mod)
```

```python
import contextlib
import jax
import jax.numpy as jnp
from jax import lax
import jax.experimental.pallas as pl
import jax.experimental.pallas.tpu as pltpu

S, D, H, DH, F = 2048, 1024, 32, 128, 3584
EPS = 1e-5
LOG2E = 1.4426950408889634
BF = jnp.bfloat16
F32 = jnp.float32
I32 = jnp.int32
IMIN = -2 ** 31


def make_kernel(G=4, CA="512,256,256", SAC="1024", QB="1,2,4,1", KC=512, KD=1536, MF="LH", MORD=2, PH=0, PW=0, PA=0, EC=256, SUMBF=1, PC=16, OUTF=1, BAR=1, SCOPES=0,
                SEQ="Q0 C Q1 H1 E K0 Q2 P0 G L K1 Q3 P1 K2 O0 P2 K3 O1 P3 O2", name="adaln_mha_moe"):
    RP = 512
    NP = S // RP
    NG = H // G
    NT = NP * NG
    SL = RP // NG
    NSL = S // SL
    QSCALE = (DH ** -0.5) * LOG2E
    T0 = 2
    NH0 = T0 * G
    X1 = RP + T0 * SL
    def chunks(spec):
        ns = [int(z) for z in spec.replace("_", ",").split(",")]
        return [(sum(ns[:i]), n) for i, n in enumerate(ns)]
    CAC, SAC_ = chunks(CA), chunks(SAC)
    HO, OO, XO = 0, S, 2 * S
    scope = jax.named_scope if SCOPES else (lambda n: contextlib.nullcontext())
    SA, S1, GA, SB, S2, GB, VA, VB, VW, VC = range(10)
    SX, SM = 0, 3
    SMS = SM + len(CAC)
    SM2 = SMS + len(SAC_)
    QBC = chunks(QB)
    SQ = SM2 + 1
    SH = SQ + len(QBC)
    SGR = SH + NH0 + 1
    SF = SGR + 2
    SO = SF + 1
    SP = SO + NP
    SC = SP + 2
    NSEM = SC + 1

    def _recip(l):
        ri = pl.reciprocal(l, approx=True)
        return ri * (2.0 - l * ri)

    def rb(a):
        return a.astype(BF).astype(F32)

    def center(x):
        mu = jnp.mean(x, axis=-1, keepdims=True)
        xc = x - mu
        rs = lax.rsqrt(jnp.mean(xc * xc, axis=-1, keepdims=True) + EPS)
        return mu, xc, rs

    def merge(a, b):
        return jnp.maximum(a[0], b[0]), jnp.maximum(jnp.minimum(a[0], b[0]), jnp.maximum(a[1], b[1]))

    def fold(k):
        t = [k[i:i + 8] for i in range(0, k.shape[0], 8)]
        ps = [(jnp.maximum(t[i], t[i + 1]), jnp.minimum(t[i], t[i + 1])) for i in range(0, len(t), 2)]
        while len(ps) > 1:
            ps = [merge(ps[i], ps[i + 1]) for i in range(0, len(ps), 2)]
        return ps[0]

    def kernel(x_hbm, k_hbm, v_hbm, wq_hbm, wo_hbm, wr_hbm, wg_hbm, wu_hbm, wd_hbm, c_hbm, wm_hbm,
               out_hbm,
               k_v, v_v, wq_v, wo_v, wg_v, wu_v, wd_v, hox_v, acc_v, mod_v, top_v, patch_v, of_v, xn_v, st_v, part_v, qf_v, qb_v,
               c_v, wr_v, sems):
        cols = pl.ds(0, D)

        def cp(src, dst, s):
            return pltpu.make_async_copy(src, dst, sems.at[s])

        def cp_x(i):
            r0, n = [(0, RP), (RP, X1 - RP), (X1, S - X1)][i]
            return cp(x_hbm.at[pl.ds(r0, n)], hox_v.at[pl.ds(XO + r0, n), cols], SX + i)

        def cp_ca(i):
            r0, n = CAC[i]
            return cp(wm_hbm.at[pl.ds(r0, n), pl.ds(D, D)], wg_v.at[pl.ds(r0, n), pl.ds(D, D)], SM + i)

        def cp_sa(i):
            r0, n = SAC_[i]
            return cp(wm_hbm.at[pl.ds(r0, n), pl.ds(0, D)], wg_v.at[pl.ds(r0, n), pl.ds(0, D)], SMS + i)

        def cp_m2():
            return [cp(wm_hbm.at[:, pl.ds(2 * D, F - 2 * D)], wg_v.at[:, pl.ds(2 * D, F - 2 * D)], SM2),
                    cp(wm_hbm.at[:, pl.ds(F, 6 * D - F)], wu_v.at[:, pl.ds(0, 6 * D - F)], SM2)]

        def cp_wq(h, s):
            return cp(wq_hbm.at[:, pl.ds(pl.multiple_of(h * DH, DH), DH)], wq_v.at[h], s)

        def cp_wo(h, n, s):
            return cp(wo_hbm.at[pl.ds(h, n)], wo_v.at[pl.ds(h, n), :, cols], s)

        def cp_kv(ref_hbm, ref_v, h, s):
            return cp(ref_hbm.at[h], ref_v.at[h], s)

        def cp_qb(i):
            h0, n = QBC[i]
            return [cp_wq(h, SQ + i) for h in range(h0, h0 + n)]

        def cp_head0():
            return [cp_kv(k_hbm, k_v, 0, SH), cp_kv(v_hbm, v_v, 0, SH)]

        def cp_head(h):
            s = SH + h
            return [cp_wo(h - 1, 1, s), cp_kv(k_hbm, k_v, h, s), cp_kv(v_hbm, v_v, h, s)]

        def cp_wo_last():
            return cp_wo(NH0 - 1, 1, SH + NH0)

        def cp_group(g):
            h0 = g * G
            s = SGR + g % 2
            return ([cp_wq(h0 + i, s) for i in range(G)]
                    + [cp(k_hbm.at[pl.ds(h0, G)], k_v.at[pl.ds(h0, G)], s),
                       cp(v_hbm.at[pl.ds(h0, G)], v_v.at[pl.ds(h0, G)], s),
                       cp_wo(h0, G, s)])

        def cp_ffn():
            return [cp(wg_hbm, wg_v, SF), cp(wu_hbm, wu_v, SF), cp(wd_hbm, wd_v.at[:, cols], SF)]

        def cp_out(p):
            r0 = pl.multiple_of(p * RP, RP)
            return cp(hox_v.at[pl.ds(OO + r0, RP), cols], out_hbm.at[pl.ds(r0, RP)], SO + p)

        def cp_small():
            return [cp(c_hbm, c_v, SC), cp(wr_hbm, wr_v, SC)]

        def mrow(i):
            return mod_v[i:i + 1, :]

        def silu_c():
            c = c_v[...].astype(F32)
            return jnp.broadcast_to((c * jax.nn.sigmoid(c)).astype(BF), (16, D))

        def ln1(r0, n):
            _, xc, rs = center(hox_v[pl.ds(XO + r0, n), cols].astype(F32))
            hox_v[pl.ds(HO + r0, n), cols] = ((xc * rs) * mrow(S1) + mrow(SA)).astype(BF)

        def resid(r0, n, a):
            return hox_v[pl.ds(XO + r0, n), cols].astype(F32) + mrow(GA) * a

        def keys(r0, n, xc, rs):
            r = rb(rs * jnp.sum(xc * mrow(VW), axis=-1, keepdims=True) + mod_v[VC:VC + 1, 0:1])
            b = lax.bitcast_convert_type(jnp.broadcast_to(r, (n, 128)), I32)
            b = jnp.where(b < 0, b ^ 0x7FFFFFFF, b) & (-65536)
            return b | (65535 - r0 - lax.broadcasted_iota(I32, (n, 128), 0))

        def put_stats(r0, n, mu, rs):
            st_v[0, pl.ds(r0, n), :] = jnp.broadcast_to(mu, (n, 128))
            st_v[1, pl.ds(r0, n), :] = jnp.broadcast_to(rs, (n, 128))

        def get_stats(r0, n):
            rep = lambda z: jnp.concatenate([z] * (D // 128), axis=1)
            return rep(st_v[0, pl.ds(r0, n), :]), rep(st_v[1, pl.ds(r0, n), :])

        def put_out(r0, n, x2, xc, rs):
            hox_v[pl.ds(OO + r0, n), cols] = (x2 + mrow(VB) + (xc * rs) * mrow(VA)).astype(BF)

        def epi(r0, n, a, valid):
            x2 = resid(r0, n, a)
            mu, xc, rs = center(x2)
            put_out(r0, n, x2, xc, rs)
            put_stats(r0, n, mu, rs)
            k1, k2 = fold(keys(r0, n, xc, rs))
            k1, k2 = merge((top_v[0], top_v[1]), (jnp.where(valid, k1, IMIN), jnp.where(valid, k2, IMIN)))
            top_v[0] = k1
            top_v[1] = k2

        def acc_rows(r0, n):
            return acc_v[pl.ds(r0, n), cols]

        def Qp_(h, hd):
            q = jnp.dot(h, wq_v[hd], preferred_element_type=F32)
            return (q * QSCALE).astype(BF)

        def QK_(q, hd):
            return lax.dot_general(q, k_v[hd], (((1,), (1,)), ((), ())), preferred_element_type=F32)

        raw = []

        def PV_(s, hd, carry_out, bias=None):
            if bias is None:
                m = jnp.max(s, axis=-1, keepdims=True)
                e = jnp.exp2(s - m)
            else:
                m = jnp.max(s + bias, axis=-1, keepdims=True)
                e = jnp.exp2((s - m) + bias)
            eb = e.astype(BF)
            if SUMBF:
                e = eb.astype(F32)
            if carry_out:
                lp = e[:, 0:128]
                for j in range(1, S // 128):
                    lp = lp + e[:, j * 128:(j + 1) * 128]
                of_v[0] = jnp.dot(eb, v_v[hd], preferred_element_type=F32)
                of_v[1] = lp
                return None
            l = jnp.sum(e, axis=-1, keepdims=True)
            o = jnp.dot(eb, v_v[hd], preferred_element_type=F32)
            raw.append(o)
            return (o * _recip(l)).astype(BF)

        def Op_(o, r0, hd):
            acc_v[pl.ds(r0, RP), cols] += jnp.dot(o, wo_v[hd, :, cols], preferred_element_type=F32)

        def op_carry(r0, hd):
            l = jnp.sum(of_v[1], axis=-1, keepdims=True)
            Op_((of_v[0] * _recip(l)).astype(BF), r0, hd)

        def start(cs):
            for c_ in cs:
                c_.start()

        def wait(cs):
            for c_ in cs:
                c_.wait()

        def matvec(slot, r0, n, c0):
            part_v[slot] = jnp.dot(silu_c()[:, r0:r0 + n], wg_v[pl.ds(r0, n), pl.ds(c0, D)],
                                   preferred_element_type=F32)

        def matsum(lo, n):
            m = part_v[lo]
            for i in range(1, n):
                m = m + part_v[lo + i]
            return m

        def q_first(h):
            return (qf_v[h] + qb_v[h, 0:1, :]).astype(BF)

        with scope("pro_init"):
            start(cp_small())
            cp_x(0).start()
            for i in range(len(CAC)):
                cp_ca(i).start()
            for i in range(len(QBC)):
                start(cp_qb(i))
            for i in range(len(SAC_)):
                cp_sa(i).start()
            start(cp_head0())
            for h in range(1, NH0):
                start(cp_head(h))
                if h == 2:
                    cp_x(1).start()
            cp_wo_last().start()
            cp_x(2).start()
            start(cp_group(T0))
            acc_v[...] = jnp.zeros_like(acc_v)
            top_v[...] = jnp.full(top_v.shape, IMIN, I32)
            mod_v[...] = jnp.zeros_like(mod_v)
        with scope("pro_ln"):
            wait(cp_small())
            cp_x(0).wait()
            _, xc0, rs0 = center(hox_v[pl.ds(XO, RP), cols].astype(F32))
            xn_v[...] = xc0 * rs0
        with scope("pro_ca"):
            for i, (r0, n) in enumerate(CAC):
                cp_ca(i).wait()
                matvec(i, r0, n, D)
            s1 = rb(1.0 + rb(matsum(0, len(CAC))[0:1]))
            mod_v[S1:S1 + 1, :] = s1
        hs = None

        def q_part(h):
            qf_v[h] = jnp.dot(hs, wq_v[h], preferred_element_type=F32) * QSCALE

        def h_piece(h):
            n = RP // NH0
            r0 = pl.multiple_of(h * n, n)
            hox_v[pl.ds(HO + r0, n), cols] = (xn_v[pl.ds(r0, n), :] * mrow(S1) + mrow(SA)).astype(BF)

        for i, (h0, n) in enumerate(QBC[:-1]):
            with scope(f"pro_q{i}"):
                wait(cp_qb(i))
                if hs is None:
                    hs = (xn_v[...] * s1).astype(BF)
                for h in range(h0, h0 + n):
                    q_part(h)
        with scope("pro_sa"):
            wait(cp_qb(len(QBC) - 1))
            for j in range(len(SAC_)):
                cp_sa(j).wait()
                matvec(len(CAC) + j, *SAC_[j], 0)
            for h in range(QBC[-1][0], NH0):
                q_part(h)
            sab = matsum(len(CAC), len(SAC_)).astype(BF)
            mod_v[SA:SA + 1, :] = sab[0:1].astype(F32)
            for h in range(NH0):
                qb_v[h] = jnp.dot(sab, wq_v[h], preferred_element_type=F32) * QSCALE
        with scope("pro_head0"):
            wait(cp_head0())
            PV_(QK_(q_first(0), 0), 0, True)
            h_piece(0)

        def mini(h, carry):
            with scope("mini_dma"):
                wait(cp_head(h))

                @pl.when(h == 3)
                def _():
                    cp_x(1).wait()
            with scope("mini_main"):
                q = q_first(h)
                dn = (((1,), (1,)), ((), ()))

                def fill():
                    inr = jnp.logical_and(h >= 3, h < 3 + T0 * SL // 32)
                    rl = jnp.where(inr, RP + (h - 3) * 32, 0)
                    for tok in MF:
                        if tok == "H":
                            h_piece(h)
                        elif tok == "L":
                            ln1(pl.multiple_of(rl, 32), 32)
                        elif tok == "l":
                            ln1(pl.multiple_of(rl, 16), 16)
                            ln1(pl.multiple_of(rl + 16, 16), 16)

                if MORD == 2:
                    fill()
                    parts = [lax.dot_general(q, k_v[h, 0:KC, :], dn, preferred_element_type=F32)]
                    op_carry(0, h - 1)
                    parts.append(lax.dot_general(q, k_v[h, KC:S, :], dn, preferred_element_type=F32))
                else:
                    QO = 3 * S + 32
                    hox_v[QO:QO + RP, 0:DH] = q
                    parts = [lax.dot_general(q, k_v[h, 0:KC, :], dn, preferred_element_type=F32)]
                    op_carry(0, h - 1)
                    if KD > KC:
                        parts.append(lax.dot_general(q, k_v[h, KC:KD, :], dn, preferred_element_type=F32))
                    fill()
                    q2 = hox_v[QO:QO + RP, 0:DH]
                    parts.append(lax.dot_general(q2, k_v[h, KD:S, :], dn, preferred_element_type=F32))
                PV_(jnp.concatenate(parts, axis=1), h, True)
            return carry

        lax.fori_loop(1, NH0, mini, 0)

        def body(t, carry):
            p = t // NG
            g = t % NG

            with scope("it_dma"):
                @pl.when(jnp.logical_or(t <= NG, g == 1))
                def _():
                    @pl.when(t < NG)
                    def _():
                        for c_ in cp_group(t):
                            c_.wait()

                    @pl.when(t == T0)
                    def _():
                        cp_wo_last().wait()
                        cp_x(2).wait()

                    @pl.when(t + 1 < NG)
                    def _():
                        for c_ in cp_group(t + 1):
                            c_.start()

                    @pl.when(t == T0 + 1)
                    def _():
                        for c_ in cp_m2():
                            c_.start()

                    @pl.when(t == NG)
                    def _():
                        for c_ in cp_m2():
                            c_.wait()
                        scc = silu_c()
                        ma = rb(jnp.dot(scc, wg_v[:, pl.ds(2 * D, F - 2 * D)], preferred_element_type=F32))
                        mb = rb(jnp.dot(scc, wu_v[:, pl.ds(0, 6 * D - F)], preferred_element_type=F32))
                        m2 = jnp.concatenate([ma[0:1], mb[0:1]], axis=1)
                        sb = m2[:, D:2 * D]
                        s2 = rb(1.0 + m2[:, 2 * D:3 * D])
                        gb = m2[:, 3 * D:4 * D]
                        wr = wr_v[...].astype(F32).reshape(1, D)
                        mod_v[GA:GA + 1, :] = m2[:, 0:D]
                        mod_v[SB:SB + 1, :] = sb
                        mod_v[S2:S2 + 1, :] = s2
                        mod_v[GB:GB + 1, :] = gb
                        mod_v[VA:VA + 1, :] = gb * s2
                        mod_v[VB:VB + 1, :] = gb * sb
                        mod_v[VW:VW + 1, :] = s2 * wr
                        mod_v[VC:VC + 1, :] = jnp.broadcast_to(jnp.sum(sb * wr, axis=-1, keepdims=True), (1, D))
                        for c_ in cp_ffn():
                            c_.start()

                    @pl.when(jnp.logical_and(g == 1, p >= 2))
                    def _():
                        cp_out(p - 2).start()

                    @pl.when(t == NT - NG + 1)
                    def _():
                        for c_ in cp_ffn():
                            c_.wait()

            with scope("it_main"):
                r0 = pl.multiple_of(p * RP, RP)
                h0 = g * G
                tp = t - 1
                ue = jnp.maximum(t - NG, 0)
                qs, ss, os_ = {}, {}, {}
                for tok in SEQ.replace("_", " ").split():
                    kind = tok[0]
                    rng = [int(z) for z in tok[1:].split("-")] if len(tok) > 1 else [0, SL // PC - 1]
                    u = rng[0]
                    if kind == "Q":
                        qs[u] = Qp_(hox_v[pl.ds(HO + r0, RP), cols], h0 + u)
                    elif kind == "K":
                        ss[u] = QK_(qs.pop(u), h0 + u)
                    elif kind == "P":
                        os_[u] = PV_(ss.pop(u), h0 + u, u == G - 1)
                    elif kind == "O":
                        Op_(os_.pop(u), r0, h0 + u)
                    elif kind == "C":
                        op_carry(pl.multiple_of((tp // NG) * RP, RP), (tp % NG) * G + G - 1)
                    elif kind == "G":
                        hox_v[pl.ds(pl.multiple_of(3 * S + 16 * (t % 2), 16), 16), 0:DH] = raw[-1][RP - 16:RP].astype(BF)
                    elif kind == "H":
                        hox_v[pl.ds(pl.multiple_of(3 * S + 16 * (t % 2), 16), 16), 0:DH] = qs[u][RP - 16:RP]
                    elif kind == "E":
                        for i in range(rng[0], rng[-1] + 1):
                            re = pl.multiple_of(ue * SL + i * PC, PC)
                            epi(re, PC, acc_rows(re, PC), t >= NG)
                    elif kind == "L":
                        for i in range(rng[0], rng[-1] + 1):
                            ln1(pl.multiple_of(jnp.minimum(t + NG, NSL - 1) * SL + i * PC, PC), PC)
            return carry

        lax.fori_loop(T0, NT, body, 0)

        with scope("epi_key"):
            o_last = (of_v[0] * _recip(jnp.sum(of_v[1], axis=-1, keepdims=True))).astype(BF)
            pair = (top_v[0], top_v[1])
            cp_out(NP - 2).start()
            for r0, n in [(S - RP + i * EC, EC) for i in range(RP // EC)]:
                a = acc_rows(r0, n)
                a = a + jnp.dot(o_last[r0 - (S - RP):r0 - (S - RP) + n], wo_v[H - 1, :, cols],
                                preferred_element_type=F32)
                acc_v[pl.ds(r0, n), cols] = a
                x2 = resid(r0, n, a)
                mu, xc, rs = center(x2)
                put_stats(r0, n, mu, rs)
                pair = merge(pair, fold(keys(r0, n, xc, rs)))
                if OUTF:
                    hox_v[pl.ds(OO + r0, n), cols] = (xc * (rs * mrow(VA) + 1.0) + (mrow(VB) + mu)).astype(BF)
                else:
                    put_out(r0, n, x2, xc, rs)
            cp_out(NP - 1).start()
            for sh in (4, 2, 1):
                pair = merge(pair, (pltpu.roll(pair[0], sh, 0), pltpu.roll(pair[1], sh, 0)))
            k1, k2 = pair

            def score(k):
                b = jnp.where(k < 0, k ^ 0x7FFFFFFF, k) & (-65536)
                return lax.bitcast_convert_type(b, F32)[0:1, 0:1]

            i1 = jnp.clip(65535 - (k1[0, 0] & 65535), 0, S - 1)
            i2 = jnp.clip(65535 - (k2[0, 0] & 65535), 0, S - 1)
            t1 = pl.multiple_of((i1 // 16) * 16, 16)
            t2 = pl.multiple_of((i2 // 16) * 16, 16)

            def post(t0):
                x2 = resid(t0, 16, acc_rows(t0, 16))
                mu, rs = get_stats(t0, 16)
                return x2, ((x2 - mu) * rs) * mrow(S2) + mrow(SB)

            x2a, h2a = post(t1)
            x2b, h2b = post(t2)
            row = lax.broadcasted_iota(I32, (16, D), 0)
            sel1 = jnp.sum(jnp.where(row == i1 - t1, h2a, 0.0), axis=0, keepdims=True)
            sel2 = jnp.sum(jnp.where(row == i2 - t2, h2b, 0.0), axis=0, keepdims=True)
            xs = jnp.where(row == 0, sel1, jnp.where(row == 1, sel2, 0.0)).astype(BF)
        with scope("epi_ffn"):
            if BAR:
                cp_out(0).wait()
            gt = jnp.dot(xs, wg_v[...], preferred_element_type=F32)
            up = jnp.dot(xs, wu_v[...], preferred_element_type=F32)
            act = (gt * jax.nn.sigmoid(gt) * up).astype(BF)
            y = jnp.dot(act, wd_v[:, cols], preferred_element_type=F32)
            y1 = y[0:1, :] * jax.nn.sigmoid(score(k1))
            y2 = y[1:2, :] * jax.nn.sigmoid(score(k2))

            def upd(t0):
                return jnp.where(row == i1 - t0, y1, 0.0) + jnp.where(row == i2 - t0, y2, 0.0)

            patch_v[0] = (x2a + mrow(GB) * (h2a + upd(t1))).astype(BF)
            patch_v[1] = (x2b + mrow(GB) * (h2b + upd(t2))).astype(BF)
        with scope("epi_out"):
            for p in range(1 if BAR else 0, NP):
                cp_out(p).wait()
            pa = cp(patch_v.at[0], out_hbm.at[pl.ds(t1, 16)], SP)
            pb = cp(patch_v.at[1], out_hbm.at[pl.ds(t2, 16)], SP + 1)
            pa.start()

            @pl.when(t1 != t2)
            def _():
                pb.start()
                pb.wait()

            pa.wait()

    def fn(A_x, A_k_cache, A_v_cache, A_wq, A_wo, B_x, B_w_r, B_w_gate, B_w_up, B_w_down, c, w_mod):
        any_ = pl.BlockSpec(memory_space=pl.ANY)
        out = pl.pallas_call(
            kernel,
            in_specs=[any_] * 11,
            out_specs=any_,
            out_shape=jax.ShapeDtypeStruct((S, D), BF),
            scratch_shapes=[
                pltpu.VMEM((H, S, DH), BF),
                pltpu.VMEM((H, S, DH), BF),
                pltpu.VMEM((H, D, DH), BF),
                pltpu.VMEM((H, DH, D + PW), BF),
                pltpu.VMEM((D, F), BF),
                pltpu.VMEM((D, F), BF),
                pltpu.VMEM((F, D + 128), BF),
                pltpu.VMEM((3 * S + 32 + (RP if MORD == 3 else 0), D + PH), BF),
                pltpu.VMEM((S, D + PA), F32),
                pltpu.VMEM((16, D), F32),
                pltpu.VMEM((2, 8, 128), I32),
                pltpu.VMEM((2, 16, D), BF),
                pltpu.VMEM((2, RP, DH), F32),
                pltpu.VMEM((RP, D), F32),
                pltpu.VMEM((2, S, 128), F32),
                pltpu.VMEM((len(CAC) + len(SAC_), 16, D), F32),
                pltpu.VMEM((NH0, RP, DH), F32),
                pltpu.VMEM((NH0, 16, DH), F32),
                pltpu.VMEM((1, D), BF),
                pltpu.VMEM((D,), BF),
                pltpu.SemaphoreType.DMA((NSEM,)),
            ],
            compiler_params=pltpu.CompilerParams(vmem_limit_bytes=120 << 20, disable_bounds_checks=True,
                                                 disable_semaphore_checks=True),
            name=name,
        )(A_x.reshape(S, D), A_k_cache.reshape(H, S, DH), A_v_cache.reshape(H, S, DH), A_wq,
          A_wo.reshape(H, DH, D), B_w_r, B_w_gate, B_w_up, B_w_down, c, w_mod)
        return out.reshape(1, S, D)

    return fn


_impl = make_kernel(MORD=3, KD=512)


@jax.jit
def pallas_adaLN_cond__mha_block_cached__moe_arch_mod__prompt_kernel(
    A_x: jax.Array,
    A_k_cache: jax.Array,
    A_v_cache: jax.Array,
    A_wq: jax.Array,
    A_wo: jax.Array,
    B_x: jax.Array,
    B_w_r: jax.Array,
    B_w_gate: jax.Array,
    B_w_up: jax.Array,
    B_w_down: jax.Array,
    c: jax.Array,
    w_mod: jax.Array,
):
    return _impl(A_x, A_k_cache, A_v_cache, A_wq, A_wo, B_x, B_w_r, B_w_gate, B_w_up, B_w_down, c, w_mod)
```

```python
import contextlib
import jax
import jax.numpy as jnp
from jax import lax
import jax.experimental.pallas as pl
import jax.experimental.pallas.tpu as pltpu

S, D, H, DH, F = 2048, 1024, 32, 128, 3584
EPS = 1e-5
LOG2E = 1.4426950408889634
BF = jnp.bfloat16
F32 = jnp.float32
I32 = jnp.int32
IMIN = -2 ** 31


def make_kernel(G=4, CA="512,256,256", SAC="1024", QB="1,2,4,1", KC=512, KD=512, MF="LH", MORD=3, PQ=0, PH=0, PW=0, PA=0, EC=256, SUMBF=1, PC=16, OUTF=1, BAR=1, SCOPES=0,
                SEQ="Q0 C Q1 H1 E K0 Q2 P0 G L K1 Q3 P1 K2 O0 P2 K3 O1 P3 O2", name="adaln_mha_moe"):
    RP = 512
    NP = S // RP
    NG = H // G
    NT = NP * NG
    SL = RP // NG
    NSL = S // SL
    QSCALE = (DH ** -0.5) * LOG2E
    T0 = 2
    NH0 = T0 * G
    X1 = RP + T0 * SL
    def chunks(spec):
        ns = [int(z) for z in spec.replace("_", ",").split(",")]
        return [(sum(ns[:i]), n) for i, n in enumerate(ns)]
    CAC, SAC_ = chunks(CA), chunks(SAC)
    HO, OO, XO = 0, S, 2 * S
    scope = jax.named_scope if SCOPES else (lambda n: contextlib.nullcontext())
    SA, S1, GA, SB, S2, GB, VA, VB, VW, VC = range(10)
    SX, SM = 0, 3
    SMS = SM + len(CAC)
    SM2 = SMS + len(SAC_)
    QBC = chunks(QB)
    SQ = SM2 + 1
    SH = SQ + len(QBC)
    SGR = SH + NH0 + 1
    SF = SGR + NG
    SO = SF + 1
    SP = SO + NP
    SC = SP + 2
    NSEM = SC + 1

    def _recip(l):
        ri = pl.reciprocal(l, approx=True)
        return ri * (2.0 - l * ri)

    def rb(a):
        return a.astype(BF).astype(F32)

    def center(x):
        mu = jnp.mean(x, axis=-1, keepdims=True)
        xc = x - mu
        rs = lax.rsqrt(jnp.mean(xc * xc, axis=-1, keepdims=True) + EPS)
        return mu, xc, rs

    def merge(a, b):
        return jnp.maximum(a[0], b[0]), jnp.maximum(jnp.minimum(a[0], b[0]), jnp.maximum(a[1], b[1]))

    def fold(k):
        t = [k[i:i + 8] for i in range(0, k.shape[0], 8)]
        ps = [(jnp.maximum(t[i], t[i + 1]), jnp.minimum(t[i], t[i + 1])) for i in range(0, len(t), 2)]
        while len(ps) > 1:
            ps = [merge(ps[i], ps[i + 1]) for i in range(0, len(ps), 2)]
        return ps[0]

    def kernel(x_hbm, k_hbm, v_hbm, wq_hbm, wo_hbm, wr_hbm, wg_hbm, wu_hbm, wd_hbm, c_hbm, wm_hbm,
               out_hbm,
               k_v, v_v, wq_v, wo_v, wg_v, wu_v, wd_v, hox_v, acc_v, mod_v, top_v, patch_v, of_v, xn_v, st_v, part_v, qf_v, qb_v,
               c_v, wr_v, sems):
        cols = pl.ds(0, D)

        def cp(src, dst, s):
            return pltpu.make_async_copy(src, dst, sems.at[s])

        def cp_x(i):
            r0, n = [(0, RP), (RP, X1 - RP), (X1, S - X1)][i]
            return cp(x_hbm.at[pl.ds(r0, n)], hox_v.at[pl.ds(XO + r0, n), cols], SX + i)

        def cp_ca(i):
            r0, n = CAC[i]
            return cp(wm_hbm.at[pl.ds(r0, n), pl.ds(D, D)], wg_v.at[pl.ds(r0, n), pl.ds(D, D)], SM + i)

        def cp_sa(i):
            r0, n = SAC_[i]
            return cp(wm_hbm.at[pl.ds(r0, n), pl.ds(0, D)], wg_v.at[pl.ds(r0, n), pl.ds(0, D)], SMS + i)

        def cp_m2():
            return [cp(wm_hbm.at[:, pl.ds(2 * D, F - 2 * D)], wg_v.at[:, pl.ds(2 * D, F - 2 * D)], SM2),
                    cp(wm_hbm.at[:, pl.ds(F, 6 * D - F)], wu_v.at[:, pl.ds(0, 6 * D - F)], SM2)]

        def cp_wq(h, s):
            return cp(wq_hbm.at[:, pl.ds(h * DH, DH)], wq_v.at[h // G, :, pl.ds((h % G) * DH, DH)], s)

        def cp_wo(h, n, s):
            return cp(wo_hbm.at[pl.ds(h, n)], wo_v.at[pl.ds(h, n), :, cols], s)

        def cp_kv(ref_hbm, ref_v, h, s):
            return cp(ref_hbm.at[h], ref_v.at[h], s)

        def cp_qb(i):
            h0, n = QBC[i]
            return [cp_wq(h, SQ + i) for h in range(h0, h0 + n)]

        def cp_head0():
            return [cp_kv(k_hbm, k_v, 0, SH), cp_kv(v_hbm, v_v, 0, SH)]

        def cp_head(h):
            s = SH + h
            return [cp_wo(h - 1, 1, s), cp_kv(k_hbm, k_v, h, s), cp_kv(v_hbm, v_v, h, s)]

        def cp_wo_last():
            return cp_wo(NH0 - 1, 1, SH + NH0)

        def cp_group(g):
            h0 = g * G
            s = SGR + g
            return ([cp(wq_hbm.at[:, pl.ds(pl.multiple_of(h0 * DH, G * DH), G * DH)], wq_v.at[g, :, pl.ds(0, G * DH)], s)]
                    + [cp(k_hbm.at[pl.ds(h0, G)], k_v.at[pl.ds(h0, G)], s),
                       cp(v_hbm.at[pl.ds(h0, G)], v_v.at[pl.ds(h0, G)], s),
                       cp_wo(h0, G, s)])

        def cp_ffn():
            return [cp(wg_hbm, wg_v, SF), cp(wu_hbm, wu_v, SF), cp(wd_hbm, wd_v.at[:, cols], SF)]

        def cp_out(p):
            r0 = pl.multiple_of(p * RP, RP)
            return cp(hox_v.at[pl.ds(OO + r0, RP), cols], out_hbm.at[pl.ds(r0, RP)], SO + p)

        def cp_small():
            return [cp(c_hbm, c_v, SC), cp(wr_hbm, wr_v, SC)]

        def mrow(i):
            return mod_v[i:i + 1, :]

        def silu_c():
            c = c_v[...].astype(F32)
            return jnp.broadcast_to((c * jax.nn.sigmoid(c)).astype(BF), (16, D))

        def ln1(r0, n):
            _, xc, rs = center(hox_v[pl.ds(XO + r0, n), cols].astype(F32))
            hox_v[pl.ds(HO + r0, n), cols] = ((xc * rs) * mrow(S1) + mrow(SA)).astype(BF)

        def resid(r0, n, a):
            return hox_v[pl.ds(XO + r0, n), cols].astype(F32) + mrow(GA) * a

        def keys(r0, n, xc, rs):
            r = rb(rs * jnp.sum(xc * mrow(VW), axis=-1, keepdims=True) + mod_v[VC:VC + 1, 0:1])
            b = lax.bitcast_convert_type(jnp.broadcast_to(r, (n, 128)), I32)
            b = jnp.where(b < 0, b ^ 0x7FFFFFFF, b) & (-65536)
            return b | (65535 - r0 - lax.broadcasted_iota(I32, (n, 128), 0))

        def put_stats(r0, n, mu, rs):
            st_v[0, pl.ds(r0, n), :] = jnp.broadcast_to(mu, (n, 128))
            st_v[1, pl.ds(r0, n), :] = jnp.broadcast_to(rs, (n, 128))

        def get_stats(r0, n):
            rep = lambda z: jnp.concatenate([z] * (D // 128), axis=1)
            return rep(st_v[0, pl.ds(r0, n), :]), rep(st_v[1, pl.ds(r0, n), :])

        def put_out(r0, n, x2, xc, rs):
            hox_v[pl.ds(OO + r0, n), cols] = (x2 + mrow(VB) + (xc * rs) * mrow(VA)).astype(BF)

        def epi(r0, n, a, valid):
            x2 = resid(r0, n, a)
            mu, xc, rs = center(x2)
            put_out(r0, n, x2, xc, rs)
            put_stats(r0, n, mu, rs)
            k1, k2 = fold(keys(r0, n, xc, rs))
            k1, k2 = merge((top_v[0], top_v[1]), (jnp.where(valid, k1, IMIN), jnp.where(valid, k2, IMIN)))
            top_v[0] = k1
            top_v[1] = k2

        def acc_rows(r0, n):
            return acc_v[pl.ds(r0, n), cols]

        def wq_head(g, u):
            return wq_v[g, :, u * DH:(u + 1) * DH]

        def Qp_(h, g, u):
            q = jnp.dot(h, wq_head(g, u), preferred_element_type=F32)
            return (q * QSCALE).astype(BF)

        def QK_(q, hd):
            return lax.dot_general(q, k_v[hd], (((1,), (1,)), ((), ())), preferred_element_type=F32)

        raw = []

        def PV_(s, hd, carry_out, bias=None):
            if bias is None:
                m = jnp.max(s, axis=-1, keepdims=True)
                e = jnp.exp2(s - m)
            else:
                m = jnp.max(s + bias, axis=-1, keepdims=True)
                e = jnp.exp2((s - m) + bias)
            eb = e.astype(BF)
            if SUMBF:
                e = eb.astype(F32)
            if carry_out:
                lp = e[:, 0:128]
                for j in range(1, S // 128):
                    lp = lp + e[:, j * 128:(j + 1) * 128]
                of_v[0] = jnp.dot(eb, v_v[hd], preferred_element_type=F32)
                of_v[1] = lp
                return None
            l = jnp.sum(e, axis=-1, keepdims=True)
            o = jnp.dot(eb, v_v[hd], preferred_element_type=F32)
            raw.append(o)
            return (o * _recip(l)).astype(BF)

        def Op_(o, r0, hd):
            acc_v[pl.ds(r0, RP), cols] += jnp.dot(o, wo_v[hd, :, cols], preferred_element_type=F32)

        def op_carry(r0, hd):
            l = jnp.sum(of_v[1], axis=-1, keepdims=True)
            Op_((of_v[0] * _recip(l)).astype(BF), r0, hd)

        def start(cs):
            for c_ in cs:
                c_.start()

        def wait(cs):
            for c_ in cs:
                c_.wait()

        def matvec(slot, r0, n, c0):
            part_v[slot] = jnp.dot(silu_c()[:, r0:r0 + n], wg_v[pl.ds(r0, n), pl.ds(c0, D)],
                                   preferred_element_type=F32)

        def matsum(lo, n):
            m = part_v[lo]
            for i in range(1, n):
                m = m + part_v[lo + i]
            return m

        def q_first(h):
            return (qf_v[h] + qb_v[h, 0:1, :]).astype(BF)

        with scope("pro_init"):
            start(cp_small())
            cp_x(0).start()
            for i in range(len(CAC)):
                cp_ca(i).start()
            for i in range(len(QBC)):
                start(cp_qb(i))
            for i in range(len(SAC_)):
                cp_sa(i).start()
            start(cp_head0())
            for h in range(1, NH0):
                start(cp_head(h))
                if h == 2:
                    cp_x(1).start()
            cp_wo_last().start()
            cp_x(2).start()
            start(cp_group(T0))
            acc_v[...] = jnp.zeros_like(acc_v)
            top_v[...] = jnp.full(top_v.shape, IMIN, I32)
            mod_v[...] = jnp.zeros_like(mod_v)
        with scope("pro_ln"):
            wait(cp_small())
            cp_x(0).wait()
            _, xc0, rs0 = center(hox_v[pl.ds(XO, RP), cols].astype(F32))
            xn_v[...] = xc0 * rs0
        with scope("pro_ca"):
            for i, (r0, n) in enumerate(CAC):
                cp_ca(i).wait()
                matvec(i, r0, n, D)
            s1 = rb(1.0 + rb(matsum(0, len(CAC))[0:1]))
            mod_v[S1:S1 + 1, :] = s1
        hs = None

        def q_part(h):
            qf_v[h] = jnp.dot(hs, wq_head(h // G, h % G), preferred_element_type=F32) * QSCALE

        def h_piece(h):
            n = RP // NH0
            r0 = pl.multiple_of(h * n, n)
            hox_v[pl.ds(HO + r0, n), cols] = (xn_v[pl.ds(r0, n), :] * mrow(S1) + mrow(SA)).astype(BF)

        for i, (h0, n) in enumerate(QBC[:-1]):
            with scope(f"pro_q{i}"):
                wait(cp_qb(i))
                if hs is None:
                    hs = (xn_v[...] * s1).astype(BF)
                for h in range(h0, h0 + n):
                    q_part(h)
        with scope("pro_sa"):
            wait(cp_qb(len(QBC) - 1))
            for j in range(len(SAC_)):
                cp_sa(j).wait()
                matvec(len(CAC) + j, *SAC_[j], 0)
            for h in range(QBC[-1][0], NH0):
                q_part(h)
            sab = matsum(len(CAC), len(SAC_)).astype(BF)
            mod_v[SA:SA + 1, :] = sab[0:1].astype(F32)
            for h in range(NH0):
                qb_v[h] = jnp.dot(sab, wq_head(h // G, h % G), preferred_element_type=F32) * QSCALE
        with scope("pro_head0"):
            wait(cp_head0())
            for g in range(T0 + 1, NG):
                start(cp_group(g))
                if g == T0 + 1:
                    start(cp_m2())
            PV_(QK_(q_first(0), 0), 0, True)
            h_piece(0)

        def mini(h, carry):
            with scope("mini_dma"):
                wait(cp_head(h))

                @pl.when(h == 3)
                def _():
                    cp_x(1).wait()
            with scope("mini_main"):
                q = q_first(h)
                dn = (((1,), (1,)), ((), ()))

                def fill():
                    inr = jnp.logical_and(h >= 3, h < 3 + T0 * SL // 32)
                    rl = jnp.where(inr, RP + (h - 3) * 32, 0)
                    for tok in MF:
                        if tok == "H":
                            h_piece(h)
                        elif tok == "L":
                            ln1(pl.multiple_of(rl, 32), 32)
                        elif tok == "l":
                            ln1(pl.multiple_of(rl, 16), 16)
                            ln1(pl.multiple_of(rl + 16, 16), 16)

                if MORD == 2:
                    fill()
                    parts = [lax.dot_general(q, k_v[h, 0:KC, :], dn, preferred_element_type=F32)]
                    op_carry(0, h - 1)
                    parts.append(lax.dot_general(q, k_v[h, KC:S, :], dn, preferred_element_type=F32))
                else:
                    QO = 3 * S + 32
                    hox_v[QO:QO + RP, 0:DH] = q
                    parts = [lax.dot_general(q, k_v[h, 0:KC, :], dn, preferred_element_type=F32)]
                    op_carry(0, h - 1)
                    if KD > KC:
                        parts.append(lax.dot_general(q, k_v[h, KC:KD, :], dn, preferred_element_type=F32))
                    fill()
                    q2 = hox_v[QO:QO + RP, 0:DH]
                    parts.append(lax.dot_general(q2, k_v[h, KD:S, :], dn, preferred_element_type=F32))
                PV_(jnp.concatenate(parts, axis=1), h, True)
            return carry

        lax.fori_loop(1, NH0, mini, 0)

        def body(t, carry):
            p = t // NG
            g = t % NG

            with scope("it_dma"):
                @pl.when(jnp.logical_or(t <= NG, g == 1))
                def _():
                    @pl.when(t < NG)
                    def _():
                        for c_ in cp_group(t):
                            c_.wait()

                    @pl.when(t == T0)
                    def _():
                        cp_wo_last().wait()
                        cp_x(2).wait()

                    @pl.when(t == NG)
                    def _():
                        for c_ in cp_m2():
                            c_.wait()
                        scc = silu_c()
                        ma = rb(jnp.dot(scc, wg_v[:, pl.ds(2 * D, F - 2 * D)], preferred_element_type=F32))
                        mb = rb(jnp.dot(scc, wu_v[:, pl.ds(0, 6 * D - F)], preferred_element_type=F32))
                        m2 = jnp.concatenate([ma[0:1], mb[0:1]], axis=1)
                        sb = m2[:, D:2 * D]
                        s2 = rb(1.0 + m2[:, 2 * D:3 * D])
                        gb = m2[:, 3 * D:4 * D]
                        wr = wr_v[...].astype(F32).reshape(1, D)
                        mod_v[GA:GA + 1, :] = m2[:, 0:D]
                        mod_v[SB:SB + 1, :] = sb
                        mod_v[S2:S2 + 1, :] = s2
                        mod_v[GB:GB + 1, :] = gb
                        mod_v[VA:VA + 1, :] = gb * s2
                        mod_v[VB:VB + 1, :] = gb * sb
                        mod_v[VW:VW + 1, :] = s2 * wr
                        mod_v[VC:VC + 1, :] = jnp.broadcast_to(jnp.sum(sb * wr, axis=-1, keepdims=True), (1, D))
                        for c_ in cp_ffn():
                            c_.start()

                    @pl.when(jnp.logical_and(g == 1, p >= 2))
                    def _():
                        cp_out(p - 2).start()

                    @pl.when(t == NT - NG + 1)
                    def _():
                        for c_ in cp_ffn():
                            c_.wait()

            with scope("it_main"):
                r0 = pl.multiple_of(p * RP, RP)
                h0 = g * G
                tp = t - 1
                ue = jnp.maximum(t - NG, 0)
                qs, ss, os_ = {}, {}, {}
                for tok in SEQ.replace("_", " ").split():
                    kind = tok[0]
                    rng = [int(z) for z in tok[1:].split("-")] if len(tok) > 1 else [0, SL // PC - 1]
                    u = rng[0]
                    if kind == "Q":
                        qs[u] = Qp_(hox_v[pl.ds(HO + r0, RP), cols], g, u)
                    elif kind == "K":
                        ss[u] = QK_(qs.pop(u), h0 + u)
                    elif kind == "P":
                        os_[u] = PV_(ss.pop(u), h0 + u, u == G - 1)
                    elif kind == "O":
                        Op_(os_.pop(u), r0, h0 + u)
                    elif kind == "C":
                        op_carry(pl.multiple_of((tp // NG) * RP, RP), (tp % NG) * G + G - 1)
                    elif kind == "G":
                        hox_v[pl.ds(pl.multiple_of(3 * S + 16 * (t % 2), 16), 16), 0:DH] = raw[-1][RP - 16:RP].astype(BF)
                    elif kind == "H":
                        hox_v[pl.ds(pl.multiple_of(3 * S + 16 * (t % 2), 16), 16), 0:DH] = qs[u][RP - 16:RP]
                    elif kind == "E":
                        for i in range(rng[0], rng[-1] + 1):
                            re = pl.multiple_of(ue * SL + i * PC, PC)
                            epi(re, PC, acc_rows(re, PC), t >= NG)
                    elif kind == "L":
                        for i in range(rng[0], rng[-1] + 1):
                            ln1(pl.multiple_of(jnp.minimum(t + NG, NSL - 1) * SL + i * PC, PC), PC)
            return carry

        lax.fori_loop(T0, NT, body, 0)

        with scope("epi_key"):
            o_last = (of_v[0] * _recip(jnp.sum(of_v[1], axis=-1, keepdims=True))).astype(BF)
            pair = (top_v[0], top_v[1])
            cp_out(NP - 2).start()
            for r0, n in [(S - RP + i * EC, EC) for i in range(RP // EC)]:
                a = acc_rows(r0, n)
                a = a + jnp.dot(o_last[r0 - (S - RP):r0 - (S - RP) + n], wo_v[H - 1, :, cols],
                                preferred_element_type=F32)
                acc_v[pl.ds(r0, n), cols] = a
                x2 = resid(r0, n, a)
                mu, xc, rs = center(x2)
                put_stats(r0, n, mu, rs)
                pair = merge(pair, fold(keys(r0, n, xc, rs)))
                if OUTF:
                    hox_v[pl.ds(OO + r0, n), cols] = (xc * (rs * mrow(VA) + 1.0) + (mrow(VB) + mu)).astype(BF)
                else:
                    put_out(r0, n, x2, xc, rs)
            cp_out(NP - 1).start()
            for sh in (4, 2, 1):
                pair = merge(pair, (pltpu.roll(pair[0], sh, 0), pltpu.roll(pair[1], sh, 0)))
            k1, k2 = pair

            def score(k):
                b = jnp.where(k < 0, k ^ 0x7FFFFFFF, k) & (-65536)
                return lax.bitcast_convert_type(b, F32)[0:1, 0:1]

            i1 = jnp.clip(65535 - (k1[0, 0] & 65535), 0, S - 1)
            i2 = jnp.clip(65535 - (k2[0, 0] & 65535), 0, S - 1)
            t1 = pl.multiple_of((i1 // 16) * 16, 16)
            t2 = pl.multiple_of((i2 // 16) * 16, 16)

            def post(t0):
                x2 = resid(t0, 16, acc_rows(t0, 16))
                mu, rs = get_stats(t0, 16)
                return x2, ((x2 - mu) * rs) * mrow(S2) + mrow(SB)

            x2a, h2a = post(t1)
            x2b, h2b = post(t2)
            row = lax.broadcasted_iota(I32, (16, D), 0)
            sel1 = jnp.sum(jnp.where(row == i1 - t1, h2a, 0.0), axis=0, keepdims=True)
            sel2 = jnp.sum(jnp.where(row == i2 - t2, h2b, 0.0), axis=0, keepdims=True)
            xs = jnp.where(row == 0, sel1, jnp.where(row == 1, sel2, 0.0)).astype(BF)
        with scope("epi_ffn"):
            if BAR:
                cp_out(0).wait()
            gt = jnp.dot(xs, wg_v[...], preferred_element_type=F32)
            up = jnp.dot(xs, wu_v[...], preferred_element_type=F32)
            act = (gt * jax.nn.sigmoid(gt) * up).astype(BF)
            y = jnp.dot(act, wd_v[:, cols], preferred_element_type=F32)
            y1 = y[0:1, :] * jax.nn.sigmoid(score(k1))
            y2 = y[1:2, :] * jax.nn.sigmoid(score(k2))

            def upd(t0):
                return jnp.where(row == i1 - t0, y1, 0.0) + jnp.where(row == i2 - t0, y2, 0.0)

            patch_v[0] = (x2a + mrow(GB) * (h2a + upd(t1))).astype(BF)
            patch_v[1] = (x2b + mrow(GB) * (h2b + upd(t2))).astype(BF)
        with scope("epi_out"):
            for p in range(1 if BAR else 0, NP):
                cp_out(p).wait()
            pa = cp(patch_v.at[0], out_hbm.at[pl.ds(t1, 16)], SP)
            pb = cp(patch_v.at[1], out_hbm.at[pl.ds(t2, 16)], SP + 1)
            pa.start()

            @pl.when(t1 != t2)
            def _():
                pb.start()
                pb.wait()

            pa.wait()

    def fn(A_x, A_k_cache, A_v_cache, A_wq, A_wo, B_x, B_w_r, B_w_gate, B_w_up, B_w_down, c, w_mod):
        any_ = pl.BlockSpec(memory_space=pl.ANY)
        out = pl.pallas_call(
            kernel,
            in_specs=[any_] * 11,
            out_specs=any_,
            out_shape=jax.ShapeDtypeStruct((S, D), BF),
            scratch_shapes=[
                pltpu.VMEM((H, S, DH), BF),
                pltpu.VMEM((H, S, DH), BF),
                pltpu.VMEM((NG, D, G * DH + PQ), BF),
                pltpu.VMEM((H, DH, D + PW), BF),
                pltpu.VMEM((D, F), BF),
                pltpu.VMEM((D, F), BF),
                pltpu.VMEM((F, D + 128), BF),
                pltpu.VMEM((3 * S + 32 + (RP if MORD == 3 else 0), D + PH), BF),
                pltpu.VMEM((S, D + PA), F32),
                pltpu.VMEM((16, D), F32),
                pltpu.VMEM((2, 8, 128), I32),
                pltpu.VMEM((2, 16, D), BF),
                pltpu.VMEM((2, RP, DH), F32),
                pltpu.VMEM((RP, D), F32),
                pltpu.VMEM((2, S, 128), F32),
                pltpu.VMEM((len(CAC) + len(SAC_), 16, D), F32),
                pltpu.VMEM((NH0, RP, DH), F32),
                pltpu.VMEM((NH0, 16, DH), F32),
                pltpu.VMEM((1, D), BF),
                pltpu.VMEM((D,), BF),
                pltpu.SemaphoreType.DMA((NSEM,)),
            ],
            compiler_params=pltpu.CompilerParams(vmem_limit_bytes=120 << 20, disable_bounds_checks=True,
                                                 disable_semaphore_checks=True),
            name=name,
        )(A_x.reshape(S, D), A_k_cache.reshape(H, S, DH), A_v_cache.reshape(H, S, DH), A_wq,
          A_wo.reshape(H, DH, D), B_w_r, B_w_gate, B_w_up, B_w_down, c, w_mod)
        return out.reshape(1, S, D)

    return fn


_impl = make_kernel()


@jax.jit
def pallas_adaLN_cond__mha_block_cached__moe_arch_mod__prompt_kernel(
    A_x: jax.Array,
    A_k_cache: jax.Array,
    A_v_cache: jax.Array,
    A_wq: jax.Array,
    A_wo: jax.Array,
    B_x: jax.Array,
    B_w_r: jax.Array,
    B_w_gate: jax.Array,
    B_w_up: jax.Array,
    B_w_down: jax.Array,
    c: jax.Array,
    w_mod: jax.Array,
):
    return _impl(A_x, A_k_cache, A_v_cache, A_wq, A_wo, B_x, B_w_r, B_w_gate, B_w_up, B_w_down, c, w_mod)
```

```python
import contextlib
import jax
import jax.numpy as jnp
from jax import lax
import jax.experimental.pallas as pl
import jax.experimental.pallas.tpu as pltpu

S, D, H, DH, F = 2048, 1024, 32, 128, 3584
EPS = 1e-5
LOG2E = 1.4426950408889634
BF = jnp.bfloat16
F32 = jnp.float32
I32 = jnp.int32
IMIN = -2 ** 31


def make_kernel(G=4, CA="512,256,256", SAC="1024", QB="1,2,4,1", KC=512, KD=512, MF="LH", MORD=3, PQ=0, PH=0, PW=0, PA=0, EC=256, SUMBF=1, PC=16, OUTF=1, BAR=1, SCOPES=0,
                SEQ="Q0 C Q1 H1 E K0 Q2 P0 G L K1 Q3 P1 K2 O0 P2 K3 O1 P3 O2", name="adaln_mha_moe"):
    RP = 512
    NP = S // RP
    NG = H // G
    NT = NP * NG
    SL = RP // NG
    NSL = S // SL
    QSCALE = (DH ** -0.5) * LOG2E
    T0 = 2
    NH0 = T0 * G
    X1 = RP + T0 * SL
    def chunks(spec):
        ns = [int(z) for z in spec.replace("_", ",").split(",")]
        return [(sum(ns[:i]), n) for i, n in enumerate(ns)]
    CAC, SAC_ = chunks(CA), chunks(SAC)
    HO, OO, XO = 0, S, 2 * S
    scope = jax.named_scope if SCOPES else (lambda n: contextlib.nullcontext())
    SA, S1, GA, SB, S2, GB, VA, VB, VW, VC = range(10)
    SX, SM = 0, 3
    SMS = SM + len(CAC)
    SM2 = SMS + len(SAC_)
    QBC = chunks(QB)
    SQ = SM2 + 1
    SH = SQ + len(QBC)
    SGR = SH + NH0 + 1
    SF = SGR + NG
    SO = SF + 1
    SP = SO + NP
    SC = SP + 2
    NSEM = SC + 1

    def _recip(l):
        ri = pl.reciprocal(l, approx=True)
        return ri * (2.0 - l * ri)

    def rb(a):
        return a.astype(BF).astype(F32)

    def center(x):
        mu = jnp.mean(x, axis=-1, keepdims=True)
        xc = x - mu
        rs = lax.rsqrt(jnp.mean(xc * xc, axis=-1, keepdims=True) + EPS)
        return mu, xc, rs

    def merge(a, b):
        return jnp.maximum(a[0], b[0]), jnp.maximum(jnp.minimum(a[0], b[0]), jnp.maximum(a[1], b[1]))

    def fold(k):
        t = [k[i:i + 8] for i in range(0, k.shape[0], 8)]
        ps = [(jnp.maximum(t[i], t[i + 1]), jnp.minimum(t[i], t[i + 1])) for i in range(0, len(t), 2)]
        while len(ps) > 1:
            ps = [merge(ps[i], ps[i + 1]) for i in range(0, len(ps), 2)]
        return ps[0]

    def kernel(x_hbm, k_hbm, v_hbm, wq_hbm, wo_hbm, wr_hbm, wg_hbm, wu_hbm, wd_hbm, c_hbm, wm_hbm,
               out_hbm,
               k_v, v_v, wq_v, wo_v, wg_v, wu_v, wd_v, hox_v, acc_v, mod_v, top_v, patch_v, of_v, xn_v, st_v, part_v, qf_v, qb_v,
               c_v, wr_v, sems):
        cols = pl.ds(0, D)

        def cp(src, dst, s):
            return pltpu.make_async_copy(src, dst, sems.at[s])

        def cp_x(i):
            r0, n = [(0, RP), (RP, X1 - RP), (X1, S - X1)][i]
            return cp(x_hbm.at[pl.ds(r0, n)], hox_v.at[pl.ds(XO + r0, n), cols], SX + i)

        def cp_ca(i):
            r0, n = CAC[i]
            return cp(wm_hbm.at[pl.ds(r0, n), pl.ds(D, D)], wg_v.at[pl.ds(r0, n), pl.ds(D, D)], SM + i)

        def cp_sa(i):
            r0, n = SAC_[i]
            return cp(wm_hbm.at[pl.ds(r0, n), pl.ds(0, D)], wg_v.at[pl.ds(r0, n), pl.ds(0, D)], SMS + i)

        def cp_m2():
            return [cp(wm_hbm.at[:, pl.ds(2 * D, F - 2 * D)], wg_v.at[:, pl.ds(2 * D, F - 2 * D)], SM2),
                    cp(wm_hbm.at[:, pl.ds(F, 6 * D - F)], wu_v.at[:, pl.ds(0, 6 * D - F)], SM2)]

        def cp_wq(h, s):
            return cp(wq_hbm.at[:, pl.ds(h * DH, DH)], wq_v.at[h // G, :, pl.ds((h % G) * DH, DH)], s)

        def cp_wo(h, n, s):
            return cp(wo_hbm.at[pl.ds(h, n)], wo_v.at[pl.ds(h, n), :, cols], s)

        def cp_kv(ref_hbm, ref_v, h, s):
            return cp(ref_hbm.at[h], ref_v.at[h], s)

        def cp_qb(i):
            h0, n = QBC[i]
            return [cp_wq(h, SQ + i) for h in range(h0, h0 + n)]

        def cp_head0():
            return [cp_kv(k_hbm, k_v, 0, SH), cp_kv(v_hbm, v_v, 0, SH)]

        def cp_head(h):
            s = SH + h
            return [cp_wo(h - 1, 1, s), cp_kv(k_hbm, k_v, h, s), cp_kv(v_hbm, v_v, h, s)]

        def cp_wo_last():
            return cp_wo(NH0 - 1, 1, SH + NH0)

        def cp_group(g):
            h0 = g * G
            s = SGR + g
            return ([cp(wq_hbm.at[:, pl.ds(pl.multiple_of(h0 * DH, G * DH), G * DH)], wq_v.at[g, :, pl.ds(0, G * DH)], s)]
                    + [cp(k_hbm.at[pl.ds(h0, G)], k_v.at[pl.ds(h0, G)], s),
                       cp(v_hbm.at[pl.ds(h0, G)], v_v.at[pl.ds(h0, G)], s),
                       cp_wo(h0, G, s)])

        def cp_ffn():
            return [cp(wg_hbm, wg_v, SF), cp(wu_hbm, wu_v, SF), cp(wd_hbm, wd_v.at[:, cols], SF)]

        def cp_out(p):
            r0 = pl.multiple_of(p * RP, RP)
            return cp(hox_v.at[pl.ds(OO + r0, RP), cols], out_hbm.at[pl.ds(r0, RP)], SO + p)

        def cp_small():
            return [cp(c_hbm, c_v, SC), cp(wr_hbm, wr_v, SC)]

        def mrow(i, n):
            m = mod_v[i]
            return m if n == 8 else jnp.concatenate([m] * (n // 8), axis=0)

        def put_mod(i, v):
            mod_v[i] = jnp.broadcast_to(v, (8, D))

        def silu_c():
            c = c_v[...].astype(F32)
            return jnp.broadcast_to((c * jax.nn.sigmoid(c)).astype(BF), (16, D))

        def ln1(r0, n):
            _, xc, rs = center(hox_v[pl.ds(XO + r0, n), cols].astype(F32))
            hox_v[pl.ds(HO + r0, n), cols] = ((xc * rs) * mrow(S1, n) + mrow(SA, n)).astype(BF)

        def resid(r0, n, a):
            return hox_v[pl.ds(XO + r0, n), cols].astype(F32) + mrow(GA, n) * a

        def keys(r0, n, xc, rs):
            r = rb(rs * jnp.sum(xc * mrow(VW, n), axis=-1, keepdims=True) + mrow(VC, n)[:, 0:128])
            b = lax.bitcast_convert_type(r, I32)
            b = jnp.where(b < 0, b ^ 0x7FFFFFFF, b) & (-65536)
            return b | (65535 - r0 - lax.broadcasted_iota(I32, (n, 128), 0))

        def put_stats(r0, n, mu, rs):
            st_v[0, pl.ds(r0, n), :] = jnp.broadcast_to(mu, (n, 128))
            st_v[1, pl.ds(r0, n), :] = jnp.broadcast_to(rs, (n, 128))

        def get_stats(r0, n):
            rep = lambda z: jnp.concatenate([z] * (D // 128), axis=1)
            return rep(st_v[0, pl.ds(r0, n), :]), rep(st_v[1, pl.ds(r0, n), :])

        def put_out(r0, n, x2, xc, rs):
            hox_v[pl.ds(OO + r0, n), cols] = (x2 + mrow(VB, n) + (xc * rs) * mrow(VA, n)).astype(BF)

        def epi(r0, n, a, valid):
            x2 = resid(r0, n, a)
            mu, xc, rs = center(x2)
            put_out(r0, n, x2, xc, rs)
            put_stats(r0, n, mu, rs)
            k1, k2 = fold(keys(r0, n, xc, rs))
            k1, k2 = merge((top_v[0], top_v[1]), (jnp.where(valid, k1, IMIN), jnp.where(valid, k2, IMIN)))
            top_v[0] = k1
            top_v[1] = k2

        def acc_rows(r0, n):
            return acc_v[pl.ds(r0, n), cols]

        def wq_head(g, u):
            return wq_v[g, :, u * DH:(u + 1) * DH]

        def Qp_(h, g, u):
            q = jnp.dot(h, wq_head(g, u), preferred_element_type=F32)
            return (q * QSCALE).astype(BF)

        def QK_(q, hd):
            return lax.dot_general(q, k_v[hd], (((1,), (1,)), ((), ())), preferred_element_type=F32)

        raw = []

        def PV_(s, hd, carry_out, bias=None):
            if bias is None:
                m = jnp.max(s, axis=-1, keepdims=True)
                e = jnp.exp2(s - m)
            else:
                m = jnp.max(s + bias, axis=-1, keepdims=True)
                e = jnp.exp2((s - m) + bias)
            eb = e.astype(BF)
            if SUMBF:
                e = eb.astype(F32)
            if carry_out:
                lp = e[:, 0:128]
                for j in range(1, S // 128):
                    lp = lp + e[:, j * 128:(j + 1) * 128]
                of_v[0] = jnp.dot(eb, v_v[hd], preferred_element_type=F32)
                of_v[1] = lp
                return None
            l = jnp.sum(e, axis=-1, keepdims=True)
            o = jnp.dot(eb, v_v[hd], preferred_element_type=F32)
            raw.append(o)
            return (o * _recip(l)).astype(BF)

        def Op_(o, r0, hd):
            acc_v[pl.ds(r0, RP), cols] += jnp.dot(o, wo_v[hd, :, cols], preferred_element_type=F32)

        def op_carry(r0, hd):
            l = jnp.sum(of_v[1], axis=-1, keepdims=True)
            Op_((of_v[0] * _recip(l)).astype(BF), r0, hd)

        def start(cs):
            for c_ in cs:
                c_.start()

        def wait(cs):
            for c_ in cs:
                c_.wait()

        def matvec(slot, r0, n, c0):
            part_v[slot] = jnp.dot(silu_c()[:, r0:r0 + n], wg_v[pl.ds(r0, n), pl.ds(c0, D)],
                                   preferred_element_type=F32)

        def matsum(lo, n):
            m = part_v[lo]
            for i in range(1, n):
                m = m + part_v[lo + i]
            return m

        def q_first(h):
            return (qf_v[h] + qb_v[h, 0:1, :]).astype(BF)

        with scope("pro_init"):
            start(cp_small())
            cp_x(0).start()
            for i in range(len(CAC)):
                cp_ca(i).start()
            for i in range(len(QBC)):
                start(cp_qb(i))
            for i in range(len(SAC_)):
                cp_sa(i).start()
            start(cp_head0())
            for h in range(1, NH0):
                start(cp_head(h))
                if h == 2:
                    cp_x(1).start()
            cp_wo_last().start()
            cp_x(2).start()
            start(cp_group(T0))
            acc_v[...] = jnp.zeros_like(acc_v)
            top_v[...] = jnp.full(top_v.shape, IMIN, I32)
            mod_v[...] = jnp.zeros_like(mod_v)
        with scope("pro_ln"):
            wait(cp_small())
            cp_x(0).wait()
            _, xc0, rs0 = center(hox_v[pl.ds(XO, RP), cols].astype(F32))
            xn_v[...] = xc0 * rs0
        with scope("pro_ca"):
            for i, (r0, n) in enumerate(CAC):
                cp_ca(i).wait()
                matvec(i, r0, n, D)
            s1 = rb(1.0 + rb(matsum(0, len(CAC))[0:1]))
            put_mod(S1, s1)
        hs = None

        def q_part(h):
            qf_v[h] = jnp.dot(hs, wq_head(h // G, h % G), preferred_element_type=F32) * QSCALE

        def h_piece(h):
            n = RP // NH0
            r0 = pl.multiple_of(h * n, n)
            hox_v[pl.ds(HO + r0, n), cols] = (xn_v[pl.ds(r0, n), :] * mrow(S1, n) + mrow(SA, n)).astype(BF)

        for i, (h0, n) in enumerate(QBC[:-1]):
            with scope(f"pro_q{i}"):
                wait(cp_qb(i))
                if hs is None:
                    hs = (xn_v[...] * s1).astype(BF)
                for h in range(h0, h0 + n):
                    q_part(h)
        with scope("pro_sa"):
            wait(cp_qb(len(QBC) - 1))
            for j in range(len(SAC_)):
                cp_sa(j).wait()
                matvec(len(CAC) + j, *SAC_[j], 0)
            for h in range(QBC[-1][0], NH0):
                q_part(h)
            sab = matsum(len(CAC), len(SAC_)).astype(BF)
            put_mod(SA, sab[0:1].astype(F32))
            for h in range(NH0):
                qb_v[h] = jnp.dot(sab, wq_head(h // G, h % G), preferred_element_type=F32) * QSCALE
        with scope("pro_head0"):
            wait(cp_head0())
            for g in range(T0 + 1, NG):
                start(cp_group(g))
                if g == T0 + 1:
                    start(cp_m2())
            PV_(QK_(q_first(0), 0), 0, True)
            h_piece(0)

        def mini(h, carry):
            with scope("mini_dma"):
                wait(cp_head(h))

                @pl.when(h == 3)
                def _():
                    cp_x(1).wait()
            with scope("mini_main"):
                q = q_first(h)
                dn = (((1,), (1,)), ((), ()))

                def fill():
                    inr = jnp.logical_and(h >= 3, h < 3 + T0 * SL // 32)
                    rl = jnp.where(inr, RP + (h - 3) * 32, 0)
                    for tok in MF:
                        if tok == "H":
                            h_piece(h)
                        elif tok == "L":
                            ln1(pl.multiple_of(rl, 32), 32)
                        elif tok == "l":
                            ln1(pl.multiple_of(rl, 16), 16)
                            ln1(pl.multiple_of(rl + 16, 16), 16)

                if MORD == 2:
                    fill()
                    parts = [lax.dot_general(q, k_v[h, 0:KC, :], dn, preferred_element_type=F32)]
                    op_carry(0, h - 1)
                    parts.append(lax.dot_general(q, k_v[h, KC:S, :], dn, preferred_element_type=F32))
                else:
                    QO = 3 * S + 32
                    hox_v[QO:QO + RP, 0:DH] = q
                    parts = [lax.dot_general(q, k_v[h, 0:KC, :], dn, preferred_element_type=F32)]
                    op_carry(0, h - 1)
                    if KD > KC:
                        parts.append(lax.dot_general(q, k_v[h, KC:KD, :], dn, preferred_element_type=F32))
                    fill()
                    q2 = hox_v[QO:QO + RP, 0:DH]
                    parts.append(lax.dot_general(q2, k_v[h, KD:S, :], dn, preferred_element_type=F32))
                PV_(jnp.concatenate(parts, axis=1), h, True)
            return carry

        lax.fori_loop(1, NH0, mini, 0)

        def body(t, carry):
            p = t // NG
            g = t % NG

            with scope("it_dma"):
                @pl.when(jnp.logical_or(t <= NG, g == 1))
                def _():
                    @pl.when(t < NG)
                    def _():
                        for c_ in cp_group(t):
                            c_.wait()

                    @pl.when(t == T0)
                    def _():
                        cp_wo_last().wait()
                        cp_x(2).wait()

                    @pl.when(t == NG)
                    def _():
                        for c_ in cp_m2():
                            c_.wait()
                        scc = silu_c()
                        ma = rb(jnp.dot(scc, wg_v[:, pl.ds(2 * D, F - 2 * D)], preferred_element_type=F32))
                        mb = rb(jnp.dot(scc, wu_v[:, pl.ds(0, 6 * D - F)], preferred_element_type=F32))
                        m2 = jnp.concatenate([ma[0:1], mb[0:1]], axis=1)
                        sb = m2[:, D:2 * D]
                        s2 = rb(1.0 + m2[:, 2 * D:3 * D])
                        gb = m2[:, 3 * D:4 * D]
                        wr = wr_v[...].astype(F32).reshape(1, D)
                        put_mod(GA, m2[:, 0:D])
                        put_mod(SB, sb)
                        put_mod(S2, s2)
                        put_mod(GB, gb)
                        put_mod(VA, gb * s2)
                        put_mod(VB, gb * sb)
                        put_mod(VW, s2 * wr)
                        put_mod(VC, jnp.broadcast_to(jnp.sum(sb * wr, axis=-1, keepdims=True), (1, D)))
                        for c_ in cp_ffn():
                            c_.start()

                    @pl.when(jnp.logical_and(g == 1, p >= 2))
                    def _():
                        cp_out(p - 2).start()

                    @pl.when(t == NT - NG + 1)
                    def _():
                        for c_ in cp_ffn():
                            c_.wait()

            with scope("it_main"):
                r0 = pl.multiple_of(p * RP, RP)
                h0 = g * G
                tp = t - 1
                ue = jnp.maximum(t - NG, 0)
                qs, ss, os_ = {}, {}, {}
                for tok in SEQ.replace("_", " ").split():
                    kind = tok[0]
                    rng = [int(z) for z in tok[1:].split("-")] if len(tok) > 1 else [0, SL // PC - 1]
                    u = rng[0]
                    if kind == "Q":
                        qs[u] = Qp_(hox_v[pl.ds(HO + r0, RP), cols], g, u)
                    elif kind == "K":
                        ss[u] = QK_(qs.pop(u), h0 + u)
                    elif kind == "P":
                        os_[u] = PV_(ss.pop(u), h0 + u, u == G - 1)
                    elif kind == "O":
                        Op_(os_.pop(u), r0, h0 + u)
                    elif kind == "C":
                        op_carry(pl.multiple_of((tp // NG) * RP, RP), (tp % NG) * G + G - 1)
                    elif kind == "G":
                        hox_v[pl.ds(pl.multiple_of(3 * S + 16 * (t % 2), 16), 16), 0:DH] = raw[-1][RP - 16:RP].astype(BF)
                    elif kind == "H":
                        hox_v[pl.ds(pl.multiple_of(3 * S + 16 * (t % 2), 16), 16), 0:DH] = qs[u][RP - 16:RP]
                    elif kind == "E":
                        for i in range(rng[0], rng[-1] + 1):
                            re = pl.multiple_of(ue * SL + i * PC, PC)
                            epi(re, PC, acc_rows(re, PC), t >= NG)
                    elif kind == "L":
                        for i in range(rng[0], rng[-1] + 1):
                            ln1(pl.multiple_of(jnp.minimum(t + NG, NSL - 1) * SL + i * PC, PC), PC)
            return carry

        lax.fori_loop(T0, NT, body, 0)

        with scope("epi_key"):
            o_last = (of_v[0] * _recip(jnp.sum(of_v[1], axis=-1, keepdims=True))).astype(BF)
            pair = (top_v[0], top_v[1])
            cp_out(NP - 2).start()
            for r0, n in [(S - RP + i * EC, EC) for i in range(RP // EC)]:
                a = acc_rows(r0, n)
                a = a + jnp.dot(o_last[r0 - (S - RP):r0 - (S - RP) + n], wo_v[H - 1, :, cols],
                                preferred_element_type=F32)
                acc_v[pl.ds(r0, n), cols] = a
                x2 = resid(r0, n, a)
                mu, xc, rs = center(x2)
                put_stats(r0, n, mu, rs)
                pair = merge(pair, fold(keys(r0, n, xc, rs)))
                if OUTF:
                    hox_v[pl.ds(OO + r0, n), cols] = (xc * (rs * mrow(VA, n) + 1.0) + (mrow(VB, n) + mu)).astype(BF)
                else:
                    put_out(r0, n, x2, xc, rs)
            cp_out(NP - 1).start()
            for sh in (4, 2, 1):
                pair = merge(pair, (pltpu.roll(pair[0], sh, 0), pltpu.roll(pair[1], sh, 0)))
            k1, k2 = pair

            def score(k):
                b = jnp.where(k < 0, k ^ 0x7FFFFFFF, k) & (-65536)
                return lax.bitcast_convert_type(b, F32)[0:1, 0:1]

            i1 = jnp.clip(65535 - (k1[0, 0] & 65535), 0, S - 1)
            i2 = jnp.clip(65535 - (k2[0, 0] & 65535), 0, S - 1)
            t1 = pl.multiple_of((i1 // 16) * 16, 16)
            t2 = pl.multiple_of((i2 // 16) * 16, 16)

            def post(t0):
                x2 = resid(t0, 16, acc_rows(t0, 16))
                mu, rs = get_stats(t0, 16)
                return x2, ((x2 - mu) * rs) * mrow(S2, 16) + mrow(SB, 16)

            x2a, h2a = post(t1)
            x2b, h2b = post(t2)
            row = lax.broadcasted_iota(I32, (16, D), 0)
            sel1 = jnp.sum(jnp.where(row == i1 - t1, h2a, 0.0), axis=0, keepdims=True)
            sel2 = jnp.sum(jnp.where(row == i2 - t2, h2b, 0.0), axis=0, keepdims=True)
            xs = jnp.where(row == 0, sel1, jnp.where(row == 1, sel2, 0.0)).astype(BF)
        with scope("epi_ffn"):
            if BAR:
                cp_out(0).wait()
            gt = jnp.dot(xs, wg_v[...], preferred_element_type=F32)
            up = jnp.dot(xs, wu_v[...], preferred_element_type=F32)
            act = (gt * jax.nn.sigmoid(gt) * up).astype(BF)
            y = jnp.dot(act, wd_v[:, cols], preferred_element_type=F32)
            y1 = y[0:1, :] * jax.nn.sigmoid(score(k1))
            y2 = y[1:2, :] * jax.nn.sigmoid(score(k2))

            def upd(t0):
                return jnp.where(row == i1 - t0, y1, 0.0) + jnp.where(row == i2 - t0, y2, 0.0)

            patch_v[0] = (x2a + mrow(GB, 16) * (h2a + upd(t1))).astype(BF)
            patch_v[1] = (x2b + mrow(GB, 16) * (h2b + upd(t2))).astype(BF)
        with scope("epi_out"):
            for p in range(1 if BAR else 0, NP):
                cp_out(p).wait()
            pa = cp(patch_v.at[0], out_hbm.at[pl.ds(t1, 16)], SP)
            pb = cp(patch_v.at[1], out_hbm.at[pl.ds(t2, 16)], SP + 1)
            pa.start()

            @pl.when(t1 != t2)
            def _():
                pb.start()
                pb.wait()

            pa.wait()

    def fn(A_x, A_k_cache, A_v_cache, A_wq, A_wo, B_x, B_w_r, B_w_gate, B_w_up, B_w_down, c, w_mod):
        any_ = pl.BlockSpec(memory_space=pl.ANY)
        out = pl.pallas_call(
            kernel,
            in_specs=[any_] * 11,
            out_specs=any_,
            out_shape=jax.ShapeDtypeStruct((S, D), BF),
            scratch_shapes=[
                pltpu.VMEM((H, S, DH), BF),
                pltpu.VMEM((H, S, DH), BF),
                pltpu.VMEM((NG, D, G * DH + PQ), BF),
                pltpu.VMEM((H, DH, D + PW), BF),
                pltpu.VMEM((D, F), BF),
                pltpu.VMEM((D, F), BF),
                pltpu.VMEM((F, D + 128), BF),
                pltpu.VMEM((3 * S + 32 + (RP if MORD == 3 else 0), D + PH), BF),
                pltpu.VMEM((S, D + PA), F32),
                pltpu.VMEM((10, 8, D), F32),
                pltpu.VMEM((2, 8, 128), I32),
                pltpu.VMEM((2, 16, D), BF),
                pltpu.VMEM((2, RP, DH), F32),
                pltpu.VMEM((RP, D), F32),
                pltpu.VMEM((2, S, 128), F32),
                pltpu.VMEM((len(CAC) + len(SAC_), 16, D), F32),
                pltpu.VMEM((NH0, RP, DH), F32),
                pltpu.VMEM((NH0, 16, DH), F32),
                pltpu.VMEM((1, D), BF),
                pltpu.VMEM((D,), BF),
                pltpu.SemaphoreType.DMA((NSEM,)),
            ],
            compiler_params=pltpu.CompilerParams(vmem_limit_bytes=120 << 20, disable_bounds_checks=True,
                                                 disable_semaphore_checks=True),
            name=name,
        )(A_x.reshape(S, D), A_k_cache.reshape(H, S, DH), A_v_cache.reshape(H, S, DH), A_wq,
          A_wo.reshape(H, DH, D), B_w_r, B_w_gate, B_w_up, B_w_down, c, w_mod)
        return out.reshape(1, S, D)

    return fn


_impl = make_kernel()


@jax.jit
def pallas_adaLN_cond__mha_block_cached__moe_arch_mod__prompt_kernel(
    A_x: jax.Array,
    A_k_cache: jax.Array,
    A_v_cache: jax.Array,
    A_wq: jax.Array,
    A_wo: jax.Array,
    B_x: jax.Array,
    B_w_r: jax.Array,
    B_w_gate: jax.Array,
    B_w_up: jax.Array,
    B_w_down: jax.Array,
    c: jax.Array,
    w_mod: jax.Array,
):
    return _impl(A_x, A_k_cache, A_v_cache, A_wq, A_wo, B_x, B_w_r, B_w_gate, B_w_up, B_w_down, c, w_mod)
```

```python
import contextlib
import jax
import jax.numpy as jnp
from jax import lax
import jax.experimental.pallas as pl
import jax.experimental.pallas.tpu as pltpu

S, D, H, DH, F = 2048, 1024, 32, 128, 3584
EPS = 1e-5
LOG2E = 1.4426950408889634
BF = jnp.bfloat16
F32 = jnp.float32
I32 = jnp.int32
IMIN = -2 ** 31


def make_kernel(G=4, CA="512,256,256", SAC="1024", QB="1,2,4,1", KC=512, KD=512, MF="LH", MORD=3, VM2=1, MW=256, PQ=0, PH=0, PW=0, PA=0, EC=256, SUMBF=1, PC=16, OUTF=1, BAR=1, SCOPES=0,
                SEQ="Q0 C Q1 H1 E K0 Q2 P0 G L K1 Q3 P1 K2 O0 P2 G k3.0-2 M k3.3-3 O1 P3 O2", name="adaln_mha_moe"):
    RP = 512
    NP = S // RP
    NG = H // G
    LNG = NG.bit_length() - 1
    NT = NP * NG
    SL = RP // NG
    NSL = S // SL
    QSCALE = (DH ** -0.5) * LOG2E
    T0 = 2
    NH0 = T0 * G
    TM = NG - 4
    X1 = RP + T0 * SL
    def chunks(spec):
        ns = [int(z) for z in spec.replace("_", ",").split(",")]
        return [(sum(ns[:i]), n) for i, n in enumerate(ns)]
    CAC, SAC_ = chunks(CA), chunks(SAC)
    HO, OO, XO = 0, S, 2 * S
    scope = jax.named_scope if SCOPES else (lambda n: contextlib.nullcontext())
    SA, S1, GA, SB, S2, GB, VA, VB, VW, VC = range(10)
    SX, SM = 0, 3
    SMS = SM + len(CAC)
    SM2 = SMS + len(SAC_)
    QBC = chunks(QB)
    SQ = SM2 + 1
    SH = SQ + len(QBC)
    SGR = SH + NH0 + 1
    SF = SGR + NG
    SO = SF + 1
    SP = SO + NP
    SC = SP + 2
    NSEM = SC + 1

    def _recip(l):
        ri = pl.reciprocal(l, approx=True)
        return ri * (2.0 - l * ri)

    def rb(a):
        return a.astype(BF).astype(F32)

    def center(x):
        mu = jnp.mean(x, axis=-1, keepdims=True)
        xc = x - mu
        rs = lax.rsqrt(jnp.mean(xc * xc, axis=-1, keepdims=True) + EPS)
        return mu, xc, rs

    def merge(a, b):
        return jnp.maximum(a[0], b[0]), jnp.maximum(jnp.minimum(a[0], b[0]), jnp.maximum(a[1], b[1]))

    def fold(k):
        t = [k[i:i + 8] for i in range(0, k.shape[0], 8)]
        ps = [(jnp.maximum(t[i], t[i + 1]), jnp.minimum(t[i], t[i + 1])) for i in range(0, len(t), 2)]
        while len(ps) > 1:
            ps = [merge(ps[i], ps[i + 1]) for i in range(0, len(ps), 2)]
        return ps[0]

    def kernel(x_hbm, k_hbm, v_hbm, wq_hbm, wo_hbm, wr_hbm, wg_hbm, wu_hbm, wd_hbm, c_hbm, wm_hbm,
               out_hbm,
               k_v, v_v, wq_v, wo_v, wgu_v, wd_v, hox_v, acc_v, mod_v, top_v, patch_v, of_v, xn_v, st_v, part_v, qf_v, qb_v, sc_v, mp_v,
               c_v, wr_v, sems):
        cols = pl.ds(0, D)

        def cp(src, dst, s):
            return pltpu.make_async_copy(src, dst, sems.at[s])

        def cp_x(i):
            r0, n = [(0, RP), (RP, X1 - RP), (X1, S - X1)][i]
            return cp(x_hbm.at[pl.ds(r0, n)], hox_v.at[pl.ds(XO + r0, n), cols], SX + i)

        def cp_ca(i):
            r0, n = CAC[i]
            return cp(wm_hbm.at[pl.ds(r0, n), pl.ds(D, D)], wgu_v.at[pl.ds(r0, n), pl.ds(D, D)], SM + i)

        def cp_sa(i):
            r0, n = SAC_[i]
            return cp(wm_hbm.at[pl.ds(r0, n), pl.ds(0, D)], wgu_v.at[pl.ds(r0, n), pl.ds(0, D)], SMS + i)

        def cp_m2():
            return [cp(wm_hbm.at[:, pl.ds(2 * D, 4 * D)], wgu_v.at[:, pl.ds(2 * D, 4 * D)], SM2)]

        def cp_wq(h, s):
            return cp(wq_hbm.at[:, pl.ds(h * DH, DH)], wq_v.at[h // G, :, pl.ds((h % G) * DH, DH)], s)

        def cp_wo(h, n, s):
            return cp(wo_hbm.at[pl.ds(h, n)], wo_v.at[pl.ds(h, n), :, cols], s)

        def cp_kv(ref_hbm, ref_v, h, s):
            return cp(ref_hbm.at[h], ref_v.at[h], s)

        def cp_qb(i):
            h0, n = QBC[i]
            return [cp_wq(h, SQ + i) for h in range(h0, h0 + n)]

        def cp_head0():
            return [cp_kv(k_hbm, k_v, 0, SH), cp_kv(v_hbm, v_v, 0, SH)]

        def cp_head(h):
            s = SH + h
            return [cp_wo(h - 1, 1, s), cp_kv(k_hbm, k_v, h, s), cp_kv(v_hbm, v_v, h, s)]

        def cp_wo_last():
            return cp_wo(NH0 - 1, 1, SH + NH0)

        def cp_group(g):
            h0 = g * G
            s = SGR + g
            return ([cp(wq_hbm.at[:, pl.ds(pl.multiple_of(h0 * DH, G * DH), G * DH)], wq_v.at[g, :, pl.ds(0, G * DH)], s)]
                    + [cp(k_hbm.at[pl.ds(h0, G)], k_v.at[pl.ds(h0, G)], s),
                       cp(v_hbm.at[pl.ds(h0, G)], v_v.at[pl.ds(h0, G)], s),
                       cp_wo(h0, G, s)])

        def cp_ffn(i):
            if i == 0:
                return [cp(wu_hbm, wgu_v.at[:, pl.ds(F, F)], SF), cp(wd_hbm, wd_v.at[:, cols], SF)]
            return [cp(wg_hbm, wgu_v.at[:, pl.ds(0, F)], SF)]

        def cp_out(p):
            r0 = pl.multiple_of(p * RP, RP)
            return cp(hox_v.at[pl.ds(OO + r0, RP), cols], out_hbm.at[pl.ds(r0, RP)], SO + p)

        def cp_small():
            return [cp(c_hbm, c_v, SC), cp(wr_hbm, wr_v, SC)]

        def mrow(i, n):
            m = mod_v[i]
            return m if n == 8 else jnp.concatenate([m] * (n // 8), axis=0)

        def put_mod(i, v):
            mod_v[i] = jnp.broadcast_to(v, (8, D))

        def silu_c():
            c = c_v[...].astype(F32)
            return jnp.broadcast_to((c * jax.nn.sigmoid(c)).astype(BF), (16, D))

        def ln1(r0, n):
            _, xc, rs = center(hox_v[pl.ds(XO + r0, n), cols].astype(F32))
            hox_v[pl.ds(HO + r0, n), cols] = ((xc * rs) * mrow(S1, n) + mrow(SA, n)).astype(BF)

        def resid(r0, n, a):
            return hox_v[pl.ds(XO + r0, n), cols].astype(F32) + mrow(GA, n) * a

        def keys(r0, n, xc, rs):
            r = rb(rs * jnp.sum(xc * mrow(VW, n), axis=-1, keepdims=True) + mrow(VC, n)[:, 0:128])
            b = lax.bitcast_convert_type(r, I32)
            b = jnp.where(b < 0, b ^ 0x7FFFFFFF, b) & (-65536)
            return b | (65535 - r0 - lax.broadcasted_iota(I32, (n, 128), 0))

        def put_stats(r0, n, mu, rs):
            st_v[0, pl.ds(r0, n), :] = jnp.broadcast_to(mu, (n, 128))
            st_v[1, pl.ds(r0, n), :] = jnp.broadcast_to(rs, (n, 128))

        def get_stats(r0, n):
            rep = lambda z: jnp.concatenate([z] * (D // 128), axis=1)
            return rep(st_v[0, pl.ds(r0, n), :]), rep(st_v[1, pl.ds(r0, n), :])

        def put_out(r0, n, x2, xc, rs):
            hox_v[pl.ds(OO + r0, n), cols] = (x2 + mrow(VB, n) + (xc * rs) * mrow(VA, n)).astype(BF)

        def epi(r0, n, a, valid):
            x2 = resid(r0, n, a)
            mu, xc, rs = center(x2)
            put_out(r0, n, x2, xc, rs)
            put_stats(r0, n, mu, rs)
            k1, k2 = fold(keys(r0, n, xc, rs))
            k1, k2 = merge((top_v[0], top_v[1]), (jnp.where(valid, k1, IMIN), jnp.where(valid, k2, IMIN)))
            top_v[0] = k1
            top_v[1] = k2

        def acc_rows(r0, n):
            return acc_v[pl.ds(r0, n), cols]

        def wq_head(g, u):
            return wq_v[g, :, u * DH:(u + 1) * DH]

        def Qp_(h, g, u):
            q = jnp.dot(h, wq_head(g, u), preferred_element_type=F32)
            return (q * QSCALE).astype(BF)

        def QK_(q, hd):
            return lax.dot_general(q, k_v[hd], (((1,), (1,)), ((), ())), preferred_element_type=F32)

        raw = []

        def PV_(s, hd, carry_out, bias=None):
            if bias is None:
                m = jnp.max(s, axis=-1, keepdims=True)
                e = jnp.exp2(s - m)
            else:
                m = jnp.max(s + bias, axis=-1, keepdims=True)
                e = jnp.exp2((s - m) + bias)
            eb = e.astype(BF)
            if SUMBF:
                e = eb.astype(F32)
            if carry_out:
                lp = e[:, 0:128]
                for j in range(1, S // 128):
                    lp = lp + e[:, j * 128:(j + 1) * 128]
                of_v[0] = jnp.dot(eb, v_v[hd], preferred_element_type=F32)
                of_v[1] = lp
                return None
            l = jnp.sum(e, axis=-1, keepdims=True)
            o = jnp.dot(eb, v_v[hd], preferred_element_type=F32)
            raw.append(o)
            return (o * _recip(l)).astype(BF)

        def Op_(o, r0, hd):
            acc_v[pl.ds(r0, RP), cols] += jnp.dot(o, wo_v[hd, :, cols], preferred_element_type=F32)

        def op_carry(r0, hd):
            l = jnp.sum(of_v[1], axis=-1, keepdims=True)
            Op_((of_v[0] * _recip(l)).astype(BF), r0, hd)

        def start(cs):
            for c_ in cs:
                c_.start()

        def wait(cs):
            for c_ in cs:
                c_.wait()

        def matvec(slot, r0, n, c0):
            part_v[slot] = jnp.dot(silu_c()[:, r0:r0 + n], wgu_v[pl.ds(r0, n), pl.ds(c0, D)],
                                   preferred_element_type=F32)

        def matsum(lo, n):
            m = part_v[lo]
            for i in range(1, n):
                m = m + part_v[lo + i]
            return m

        def q_first(h):
            return (qf_v[h] + qb_v[h, 0:1, :]).astype(BF)

        with scope("pro_init"):
            start(cp_small())
            cp_x(0).start()
            for i in range(len(CAC)):
                cp_ca(i).start()
            for i in range(len(QBC)):
                start(cp_qb(i))
            for i in range(len(SAC_)):
                cp_sa(i).start()
            start(cp_head0())
            for h in range(1, NH0):
                start(cp_head(h))
                if h == 2:
                    cp_x(1).start()
            cp_wo_last().start()
            cp_x(2).start()
            start(cp_group(T0))
            acc_v[...] = jnp.zeros_like(acc_v)
            top_v[...] = jnp.full(top_v.shape, IMIN, I32)
            mod_v[...] = jnp.zeros_like(mod_v)
        with scope("pro_ln"):
            wait(cp_small())
            sc_v[...] = jnp.broadcast_to(silu_c()[0:1].astype(F32), (128, D)).T
            hox_v[3 * S + 32 + RP:3 * S + 48 + RP, :] = jnp.zeros((16, D + PH), BF)
            cp_x(0).wait()
            _, xc0, rs0 = center(hox_v[pl.ds(XO, RP), cols].astype(F32))
            xn_v[...] = xc0 * rs0
        with scope("pro_ca"):
            for i, (r0, n) in enumerate(CAC):
                cp_ca(i).wait()
                matvec(i, r0, n, D)
            s1 = rb(1.0 + rb(matsum(0, len(CAC))[0:1]))
            put_mod(S1, s1)
        hs = None

        def q_part(h):
            qf_v[h] = jnp.dot(hs, wq_head(h // G, h % G), preferred_element_type=F32) * QSCALE

        def h_piece(h):
            n = RP // NH0
            r0 = pl.multiple_of(h * n, n)
            hox_v[pl.ds(HO + r0, n), cols] = (xn_v[pl.ds(r0, n), :] * mrow(S1, n) + mrow(SA, n)).astype(BF)

        for i, (h0, n) in enumerate(QBC[:-1]):
            with scope(f"pro_q{i}"):
                wait(cp_qb(i))
                if hs is None:
                    hs = (xn_v[...] * s1).astype(BF)
                for h in range(h0, h0 + n):
                    q_part(h)
        with scope("pro_sa"):
            wait(cp_qb(len(QBC) - 1))
            for j in range(len(SAC_)):
                cp_sa(j).wait()
                matvec(len(CAC) + j, *SAC_[j], 0)
            for h in range(QBC[-1][0], NH0):
                q_part(h)
            sab = matsum(len(CAC), len(SAC_)).astype(BF)
            put_mod(SA, sab[0:1].astype(F32))
            for h in range(NH0):
                qb_v[h] = jnp.dot(sab, wq_head(h // G, h % G), preferred_element_type=F32) * QSCALE
        with scope("pro_head0"):
            wait(cp_head0())
            for g in range(T0 + 1, NG):
                start(cp_group(g))
                if g == T0 + 1:
                    start(cp_m2())
            PV_(QK_(q_first(0), 0), 0, True)
            h_piece(0)

        def mini(h, carry):
            with scope("mini_dma"):
                wait(cp_head(h))

                @pl.when(h == 3)
                def _():
                    cp_x(1).wait()
            with scope("mini_main"):
                q = q_first(h)
                dn = (((1,), (1,)), ((), ()))

                def fill():
                    inr = jnp.logical_and(h >= 3, h < 3 + T0 * SL // 32)
                    rl = jnp.where(inr, RP + (h - 3) * 32, 0)
                    for tok in MF:
                        if tok == "H":
                            h_piece(h)
                        elif tok == "L":
                            ln1(pl.multiple_of(rl, 32), 32)
                        elif tok == "l":
                            ln1(pl.multiple_of(rl, 16), 16)
                            ln1(pl.multiple_of(rl + 16, 16), 16)

                if MORD == 2:
                    fill()
                    parts = [lax.dot_general(q, k_v[h, 0:KC, :], dn, preferred_element_type=F32)]
                    op_carry(0, h - 1)
                    parts.append(lax.dot_general(q, k_v[h, KC:S, :], dn, preferred_element_type=F32))
                else:
                    QO = 3 * S + 32
                    hox_v[QO:QO + RP, 0:DH] = q
                    parts = [lax.dot_general(q, k_v[h, 0:KC, :], dn, preferred_element_type=F32)]
                    op_carry(0, h - 1)
                    if KD > KC:
                        parts.append(lax.dot_general(q, k_v[h, KC:KD, :], dn, preferred_element_type=F32))
                    fill()
                    q2 = hox_v[QO:QO + RP, 0:DH]
                    parts.append(lax.dot_general(q2, k_v[h, KD:S, :], dn, preferred_element_type=F32))
                PV_(jnp.concatenate(parts, axis=1), h, True)
            return carry

        lax.fori_loop(1, NH0, mini, 0)

        def body(t, carry):
            p = lax.shift_right_logical(t, LNG)
            g = t & (NG - 1)

            with scope("it_dma"):
                @pl.when(jnp.logical_or(t <= NG, g == 1))
                def _():
                    @pl.when(t < NG)
                    def _():
                        for c_ in cp_group(t):
                            c_.wait()

                    @pl.when(t == T0)
                    def _():
                        cp_wo_last().wait()
                        cp_x(2).wait()

                    @pl.when(t == TM)
                    def _():
                        wait(cp_m2())

                    @pl.when(t == NG)
                    def _():
                        if VM2:
                            m2 = jnp.concatenate([jnp.sum(mp_v[i], axis=0, keepdims=True) for i in range(4)], axis=1)
                            m2 = rb(m2)
                        else:
                            m2 = rb(jnp.dot(silu_c(), wgu_v[:, 2 * D:6 * D], preferred_element_type=F32))[0:1]
                        sb = m2[:, D:2 * D]
                        s2 = rb(1.0 + m2[:, 2 * D:3 * D])
                        gb = m2[:, 3 * D:4 * D]
                        wr = wr_v[...].astype(F32).reshape(1, D)
                        put_mod(GA, m2[:, 0:D])
                        put_mod(SB, sb)
                        put_mod(S2, s2)
                        put_mod(GB, gb)
                        put_mod(VA, gb * s2)
                        put_mod(VB, gb * sb)
                        put_mod(VW, s2 * wr)
                        put_mod(VC, jnp.broadcast_to(jnp.sum(sb * wr, axis=-1, keepdims=True), (1, D)))
                        start(cp_ffn(0))

                    @pl.when(t == 2 * NG + 1)
                    def _():
                        wait(cp_ffn(0))
                        start(cp_ffn(1))

                    @pl.when(jnp.logical_and(g == 1, p >= 2))
                    def _():
                        cp_out(p - 2).start()

                    @pl.when(t == NT - NG + 1)
                    def _():
                        wait(cp_ffn(1))

            with scope("it_main"):
                r0 = pl.multiple_of(p * RP, RP)
                h0 = g * G
                tp = t - 1
                ue = jnp.maximum(t - NG, 0)
                qs, ss, os_ = {}, {}, {}
                QO = 3 * S + 32
                dn = (((1,), (1,)), ((), ()))
                parts = {}
                for tok in SEQ.replace("_", " ").split():
                    kind = tok[0]
                    if kind == "k":
                        u, ab = tok[1:].split(".")
                        u, (a_, b_) = int(u), [int(z) for z in ab.split("-")]
                        if a_ == 0:
                            q_ = qs.pop(u)
                            hox_v[QO:QO + RP, u * DH:(u + 1) * DH] = q_
                            parts[u] = []
                        else:
                            q_ = hox_v[QO:QO + RP, u * DH:(u + 1) * DH]
                        parts[u].append(lax.dot_general(q_, k_v[h0 + u, a_ * 512:(b_ + 1) * 512, :], dn,
                                                        preferred_element_type=F32))
                        if b_ == 3:
                            ss[u] = jnp.concatenate(parts.pop(u), axis=1)
                        continue
                    rng = [int(z) for z in tok[1:].split("-")] if len(tok) > 1 else [0, SL // PC - 1]
                    u = rng[0]
                    if kind == "Q":
                        qs[u] = Qp_(hox_v[pl.ds(HO + r0, RP), cols], g, u)
                    elif kind == "K":
                        ss[u] = QK_(qs.pop(u), h0 + u)
                    elif kind == "P":
                        os_[u] = PV_(ss.pop(u), h0 + u, u == G - 1)
                    elif kind == "O":
                        Op_(os_.pop(u), r0, h0 + u)
                    elif kind == "C":
                        op_carry(pl.multiple_of(lax.shift_right_logical(tp, LNG) * RP, RP), (tp & (NG - 1)) * G + G - 1)
                    elif kind == "G":
                        hox_v[pl.ds(pl.multiple_of(3 * S + 16 * (t & 1), 16), 16), 0:DH] = raw[-1][RP - 16:RP].astype(BF)
                    elif kind == "H":
                        hox_v[pl.ds(pl.multiple_of(3 * S + 16 * (t & 1), 16), 16), 0:DH] = qs[u][RP - 16:RP]
                    elif kind == "M":
                        live = jnp.logical_and(t >= TM, t < TM + 4)
                        c0 = jnp.where(live, 2 * D + (t - TM) * D, jnp.where(t <= 2 * NG, 0, 4 * D))
                        slot = jnp.where(live, t - TM, 4)
                        ZO = 3 * S + 32 + RP
                        link = hox_v[ZO:ZO + 16, 0:MW].astype(F32)[0:8]
                        for j in range(D // MW):
                            acc_ = link
                            wv = wgu_v.at[:, pl.ds(pl.multiple_of(c0, D), D)]
                            for k in range(0, D, 8):
                                w = wv[k:k + 8, j * MW:(j + 1) * MW].astype(F32)
                                acc_ = acc_ + w * jnp.concatenate([sc_v[k:k + 8, :]] * (MW // 128), axis=1)
                            mp_v[slot, :, j * MW:(j + 1) * MW] = acc_
                            link = jnp.minimum(jnp.abs(acc_), 0.0)
                        hox_v[pl.ds(pl.multiple_of(3 * S + 16 * (t & 1), 16), 8), 0:MW] = link.astype(BF)
                    elif kind == "E":
                        for i in range(rng[0], rng[-1] + 1):
                            re = pl.multiple_of(ue * SL + i * PC, PC)
                            epi(re, PC, acc_rows(re, PC), t >= NG)
                    elif kind == "L":
                        for i in range(rng[0], rng[-1] + 1):
                            ln1(pl.multiple_of(jnp.minimum(t + NG, NSL - 1) * SL + i * PC, PC), PC)
            return carry

        lax.fori_loop(T0, NT, body, 0)

        with scope("epi_key"):
            o_last = (of_v[0] * _recip(jnp.sum(of_v[1], axis=-1, keepdims=True))).astype(BF)
            pair = (top_v[0], top_v[1])
            cp_out(NP - 2).start()
            for r0, n in [(S - RP + i * EC, EC) for i in range(RP // EC)]:
                a = acc_rows(r0, n)
                a = a + jnp.dot(o_last[r0 - (S - RP):r0 - (S - RP) + n], wo_v[H - 1, :, cols],
                                preferred_element_type=F32)
                acc_v[pl.ds(r0, n), cols] = a
                x2 = resid(r0, n, a)
                mu, xc, rs = center(x2)
                put_stats(r0, n, mu, rs)
                pair = merge(pair, fold(keys(r0, n, xc, rs)))
                if OUTF:
                    hox_v[pl.ds(OO + r0, n), cols] = (xc * (rs * mrow(VA, n) + 1.0) + (mrow(VB, n) + mu)).astype(BF)
                else:
                    put_out(r0, n, x2, xc, rs)
            cp_out(NP - 1).start()
            for sh in (4, 2, 1):
                pair = merge(pair, (pltpu.roll(pair[0], sh, 0), pltpu.roll(pair[1], sh, 0)))
            k1, k2 = pair

            def score(k):
                b = jnp.where(k < 0, k ^ 0x7FFFFFFF, k) & (-65536)
                return lax.bitcast_convert_type(b, F32)[0:1, 0:1]

            i1 = jnp.clip(65535 - (k1[0, 0] & 65535), 0, S - 1)
            i2 = jnp.clip(65535 - (k2[0, 0] & 65535), 0, S - 1)
            t1 = pl.multiple_of(i1 & -16, 16)
            t2 = pl.multiple_of(i2 & -16, 16)

            def post(t0):
                x2 = resid(t0, 16, acc_rows(t0, 16))
                mu, rs = get_stats(t0, 16)
                return x2, ((x2 - mu) * rs) * mrow(S2, 16) + mrow(SB, 16)

            x2a, h2a = post(t1)
            x2b, h2b = post(t2)
            row = lax.broadcasted_iota(I32, (16, D), 0)
            sel1 = jnp.sum(jnp.where(row == i1 - t1, h2a, 0.0), axis=0, keepdims=True)
            sel2 = jnp.sum(jnp.where(row == i2 - t2, h2b, 0.0), axis=0, keepdims=True)
            xs = jnp.where(row == 0, sel1, jnp.where(row == 1, sel2, 0.0)).astype(BF)
        with scope("epi_ffn"):
            if BAR:
                cp_out(0).wait()
            gt = jnp.dot(xs, wgu_v[:, 0:F], preferred_element_type=F32)
            up = jnp.dot(xs, wgu_v[:, F:2 * F], preferred_element_type=F32)
            act = (gt * jax.nn.sigmoid(gt) * up).astype(BF)
            y = jnp.dot(act, wd_v[:, cols], preferred_element_type=F32)
            y1 = y[0:1, :] * jax.nn.sigmoid(score(k1))
            y2 = y[1:2, :] * jax.nn.sigmoid(score(k2))

            def upd(t0):
                return jnp.where(row == i1 - t0, y1, 0.0) + jnp.where(row == i2 - t0, y2, 0.0)

            patch_v[0] = (x2a + mrow(GB, 16) * (h2a + upd(t1))).astype(BF)
            patch_v[1] = (x2b + mrow(GB, 16) * (h2b + upd(t2))).astype(BF)
        with scope("epi_out"):
            for p in range(1 if BAR else 0, NP):
                cp_out(p).wait()
            pa = cp(patch_v.at[0], out_hbm.at[pl.ds(t1, 16)], SP)
            pb = cp(patch_v.at[1], out_hbm.at[pl.ds(t2, 16)], SP + 1)
            pa.start()

            @pl.when(t1 != t2)
            def _():
                pb.start()
                pb.wait()

            pa.wait()

    def fn(A_x, A_k_cache, A_v_cache, A_wq, A_wo, B_x, B_w_r, B_w_gate, B_w_up, B_w_down, c, w_mod):
        any_ = pl.BlockSpec(memory_space=pl.ANY)
        out = pl.pallas_call(
            kernel,
            in_specs=[any_] * 11,
            out_specs=any_,
            out_shape=jax.ShapeDtypeStruct((S, D), BF),
            scratch_shapes=[
                pltpu.VMEM((H, S, DH), BF),
                pltpu.VMEM((H, S, DH), BF),
                pltpu.VMEM((NG, D, G * DH + PQ), BF),
                pltpu.VMEM((H, DH, D + PW), BF),
                pltpu.VMEM((D, 2 * F + 128), BF),
                pltpu.VMEM((F, D + 128), BF),
                pltpu.VMEM((3 * S + 32 + RP + 16, D + PH), BF),
                pltpu.VMEM((S, D + PA), F32),
                pltpu.VMEM((10, 8, D), F32),
                pltpu.VMEM((2, 8, 128), I32),
                pltpu.VMEM((2, 16, D), BF),
                pltpu.VMEM((2, RP, DH), F32),
                pltpu.VMEM((RP, D), F32),
                pltpu.VMEM((2, S, 128), F32),
                pltpu.VMEM((len(CAC) + len(SAC_), 16, D), F32),
                pltpu.VMEM((NH0, RP, DH), F32),
                pltpu.VMEM((NH0, 16, DH), F32),
                pltpu.VMEM((D, 128), F32),
                pltpu.VMEM((5, 8, D), F32),
                pltpu.VMEM((1, D), BF),
                pltpu.VMEM((D,), BF),
                pltpu.SemaphoreType.DMA((NSEM,)),
            ],
            compiler_params=pltpu.CompilerParams(vmem_limit_bytes=120 << 20, disable_bounds_checks=True,
                                                 disable_semaphore_checks=True),
            name=name,
        )(A_x.reshape(S, D), A_k_cache.reshape(H, S, DH), A_v_cache.reshape(H, S, DH), A_wq,
          A_wo.reshape(H, DH, D), B_w_r, B_w_gate, B_w_up, B_w_down, c, w_mod)
        return out.reshape(1, S, D)

    return fn


_impl = make_kernel(MW=128)


@jax.jit
def pallas_adaLN_cond__mha_block_cached__moe_arch_mod__prompt_kernel(
    A_x: jax.Array,
    A_k_cache: jax.Array,
    A_v_cache: jax.Array,
    A_wq: jax.Array,
    A_wo: jax.Array,
    B_x: jax.Array,
    B_w_r: jax.Array,
    B_w_gate: jax.Array,
    B_w_up: jax.Array,
    B_w_down: jax.Array,
    c: jax.Array,
    w_mod: jax.Array,
):
    return _impl(A_x, A_k_cache, A_v_cache, A_wq, A_wo, B_x, B_w_r, B_w_gate, B_w_up, B_w_down, c, w_mod)
```

```python
import contextlib
import jax
import jax.numpy as jnp
from jax import lax
import jax.experimental.pallas as pl
import jax.experimental.pallas.tpu as pltpu

S, D, H, DH, F = 2048, 1024, 32, 128, 3584
EPS = 1e-5
LOG2E = 1.4426950408889634
BF = jnp.bfloat16
F32 = jnp.float32
I32 = jnp.int32
IMIN = -2 ** 31


def make_kernel(G=4, CA="512,256,256", SAC="1024", QB="1,2,4,1", KC=512, KD=512, MF="LH", MORD=3, VM2=1, MW=128, SBM=15, SXC=0, PQ=0, PH=0, PW=0, PA=0, EC=256, SUMBF=1, PC=16, OUTF=1, BAR=1, SCOPES=0,
                SEQ="Q0 C Q1 H1 E K0 Q2 P0 G L K1 Q3 P1 K2 O0 P2 G k3.0-2 M k3.3-3 O1 P3 O2", name="adaln_mha_moe"):
    RP = 512
    NP = S // RP
    NG = H // G
    LNG = NG.bit_length() - 1
    NT = NP * NG
    SL = RP // NG
    NSL = S // SL
    QSCALE = (DH ** -0.5) * LOG2E
    T0 = 2
    NH0 = T0 * G
    TM = NG - 4
    X1 = RP + T0 * SL
    def chunks(spec):
        ns = [int(z) for z in spec.replace("_", ",").split(",")]
        return [(sum(ns[:i]), n) for i, n in enumerate(ns)]
    CAC, SAC_ = chunks(CA), chunks(SAC)
    HO, OO, XO = 0, S, 2 * S
    scope = jax.named_scope if SCOPES else (lambda n: contextlib.nullcontext())
    SA, S1, GA, SB, S2, GB, VA, VB, VW, VC = range(10)
    SX, SM = 0, 3
    SMS = SM + len(CAC)
    SM2 = SMS + len(SAC_)
    QBC = chunks(QB)
    SQ = SM2 + 1
    SH = SQ + len(QBC)
    SGR = SH + NH0 + 1
    SF = SGR + NG
    SO = SF + 1
    SP = SO + NP
    SC = SP + 2
    NSEM = SC + 1

    def _recip(l):
        ri = pl.reciprocal(l, approx=True)
        return ri * (2.0 - l * ri)

    def rb(a):
        return a.astype(BF).astype(F32)

    def center(x):
        mu = jnp.mean(x, axis=-1, keepdims=True)
        xc = x - mu
        rs = lax.rsqrt(jnp.mean(xc * xc, axis=-1, keepdims=True) + EPS)
        return mu, xc, rs

    def merge(a, b):
        return jnp.maximum(a[0], b[0]), jnp.maximum(jnp.minimum(a[0], b[0]), jnp.maximum(a[1], b[1]))

    def fold(k):
        t = [k[i:i + 8] for i in range(0, k.shape[0], 8)]
        ps = [(jnp.maximum(t[i], t[i + 1]), jnp.minimum(t[i], t[i + 1])) for i in range(0, len(t), 2)]
        while len(ps) > 1:
            ps = [merge(ps[i], ps[i + 1]) for i in range(0, len(ps), 2)]
        return ps[0]

    def kernel(x_hbm, k_hbm, v_hbm, wq_hbm, wo_hbm, wr_hbm, wg_hbm, wu_hbm, wd_hbm, c_hbm, wm_hbm,
               out_hbm,
               k_v, v_v, wq_v, wo_v, wgu_v, wd_v, hox_v, acc_v, mod_v, top_v, patch_v, of_v, xn_v, st_v, part_v, qf_v, qb_v, sc_v, mp_v,
               c_v, wr_v, sems):
        cols = pl.ds(0, D)

        def cp(src, dst, s):
            return pltpu.make_async_copy(src, dst, sems.at[s])

        def cp_x(i):
            r0, n = [(0, RP), (RP, X1 - RP), (X1, S - X1)][i]
            return cp(x_hbm.at[pl.ds(r0, n)], hox_v.at[pl.ds(XO + r0, n), cols], SX + i)

        def cp_ca(i):
            r0, n = CAC[i]
            return cp(wm_hbm.at[pl.ds(r0, n), pl.ds(D, D)], wgu_v.at[pl.ds(r0, n), pl.ds(D, D)], SM + i)

        def cp_sa(i):
            r0, n = SAC_[i]
            return cp(wm_hbm.at[pl.ds(r0, n), pl.ds(0, D)], wgu_v.at[pl.ds(r0, n), pl.ds(0, D)], SMS + i)

        def cp_m2():
            return [cp(wm_hbm.at[:, pl.ds(2 * D, 4 * D)], wgu_v.at[:, pl.ds(2 * D, 4 * D)], SM2)]

        def cp_wq(h, s):
            return cp(wq_hbm.at[:, pl.ds(h * DH, DH)], wq_v.at[h // G, :, pl.ds((h % G) * DH, DH)], s)

        def cp_wo(h, n, s):
            return cp(wo_hbm.at[pl.ds(h, n)], wo_v.at[pl.ds(h, n), :, cols], s)

        def cp_kv(ref_hbm, ref_v, h, s):
            return cp(ref_hbm.at[h], ref_v.at[h], s)

        def cp_qb(i):
            h0, n = QBC[i]
            return [cp_wq(h, SQ + i) for h in range(h0, h0 + n)]

        def cp_head0():
            return [cp_kv(k_hbm, k_v, 0, SH), cp_kv(v_hbm, v_v, 0, SH)]

        def cp_head(h):
            s = SH + h
            return [cp_wo(h - 1, 1, s), cp_kv(k_hbm, k_v, h, s), cp_kv(v_hbm, v_v, h, s)]

        def cp_wo_last():
            return cp_wo(NH0 - 1, 1, SH + NH0)

        def cp_group(g):
            h0 = g * G
            s = SGR + g
            return ([cp(wq_hbm.at[:, pl.ds(pl.multiple_of(h0 * DH, G * DH), G * DH)], wq_v.at[g, :, pl.ds(0, G * DH)], s)]
                    + [cp(k_hbm.at[pl.ds(h0, G)], k_v.at[pl.ds(h0, G)], s),
                       cp(v_hbm.at[pl.ds(h0, G)], v_v.at[pl.ds(h0, G)], s),
                       cp_wo(h0, G, s)])

        def cp_ffn(i):
            if i == 0:
                return [cp(wu_hbm, wgu_v.at[:, pl.ds(F, F)], SF), cp(wd_hbm, wd_v.at[:, cols], SF)]
            return [cp(wg_hbm, wgu_v.at[:, pl.ds(0, F)], SF)]

        def cp_out(p):
            r0 = pl.multiple_of(p * RP, RP)
            return cp(hox_v.at[pl.ds(OO + r0, RP), cols], out_hbm.at[pl.ds(r0, RP)], SO + p)

        def cp_small():
            return [cp(c_hbm, c_v, SC), cp(wr_hbm, wr_v, SC)]

        def mrow(i, n):
            m = mod_v[i]
            return m if n == 8 else jnp.concatenate([m] * (n // 8), axis=0)

        def put_mod(i, v):
            mod_v[i] = jnp.broadcast_to(v, (8, D))

        def silu_c():
            c = c_v[...].astype(F32)
            return jnp.broadcast_to((c * jax.nn.sigmoid(c)).astype(BF), (16, D))

        def ln1(r0, n):
            _, xc, rs = center(hox_v[pl.ds(XO + r0, n), cols].astype(F32))
            hox_v[pl.ds(HO + r0, n), cols] = ((xc * rs) * mrow(S1, n) + mrow(SA, n)).astype(BF)

        def resid(r0, n, a):
            return hox_v[pl.ds(XO + r0, n), cols].astype(F32) + mrow(GA, n) * a

        def keys(r0, n, xc, rs):
            r = rb(rs * jnp.sum(xc * mrow(VW, n), axis=-1, keepdims=True) + mrow(VC, n)[:, 0:128])
            b = lax.bitcast_convert_type(r, I32)
            b = jnp.where(b < 0, b ^ 0x7FFFFFFF, b) & (-65536)
            return b | (65535 - r0 - lax.broadcasted_iota(I32, (n, 128), 0))

        def put_stats(r0, n, mu, rs):
            st_v[0, pl.ds(r0, n), :] = jnp.broadcast_to(mu, (n, 128))
            st_v[1, pl.ds(r0, n), :] = jnp.broadcast_to(rs, (n, 128))

        def get_stats(r0, n):
            rep = lambda z: jnp.concatenate([z] * (D // 128), axis=1)
            return rep(st_v[0, pl.ds(r0, n), :]), rep(st_v[1, pl.ds(r0, n), :])

        def put_out(r0, n, x2, xc, rs):
            hox_v[pl.ds(OO + r0, n), cols] = (x2 + mrow(VB, n) + (xc * rs) * mrow(VA, n)).astype(BF)

        def epi(r0, n, a, valid):
            x2 = resid(r0, n, a)
            mu, xc, rs = center(x2)
            put_out(r0, n, x2, xc, rs)
            put_stats(r0, n, mu, rs)
            k1, k2 = fold(keys(r0, n, xc, rs))
            k1, k2 = merge((top_v[0], top_v[1]), (jnp.where(valid, k1, IMIN), jnp.where(valid, k2, IMIN)))
            top_v[0] = k1
            top_v[1] = k2

        def acc_rows(r0, n):
            return acc_v[pl.ds(r0, n), cols]

        def wq_head(g, u):
            return wq_v[g, :, u * DH:(u + 1) * DH]

        def Qp_(h, g, u):
            q = jnp.dot(h, wq_head(g, u), preferred_element_type=F32)
            return (q * QSCALE).astype(BF)

        def QK_(q, hd):
            return lax.dot_general(q, k_v[hd], (((1,), (1,)), ((), ())), preferred_element_type=F32)

        raw = []

        def PV_(s, hd, carry_out, bias=None, sbf=True):
            if bias is None:
                m = jnp.max(s, axis=-1, keepdims=True)
                e = jnp.exp2(s - m)
            else:
                m = jnp.max(s + bias, axis=-1, keepdims=True)
                e = jnp.exp2((s - m) + bias)
            eb = e.astype(BF)
            if sbf:
                e = eb.astype(F32)
            if carry_out:
                lp = e[:, 0:128]
                for j in range(1, S // 128):
                    lp = lp + e[:, j * 128:(j + 1) * 128]
                of_v[0] = jnp.dot(eb, v_v[hd], preferred_element_type=F32)
                of_v[1] = lp
                return None
            l = jnp.sum(e, axis=-1, keepdims=True)
            o = jnp.dot(eb, v_v[hd], preferred_element_type=F32)
            raw.append(o)
            return (o * _recip(l)).astype(BF)

        def Op_(o, r0, hd):
            acc_v[pl.ds(r0, RP), cols] += jnp.dot(o, wo_v[hd, :, cols], preferred_element_type=F32)

        def op_carry(r0, hd):
            l = jnp.sum(of_v[1], axis=-1, keepdims=True)
            Op_((of_v[0] * _recip(l)).astype(BF), r0, hd)

        def start(cs):
            for c_ in cs:
                c_.start()

        def wait(cs):
            for c_ in cs:
                c_.wait()

        def matvec(slot, r0, n, c0):
            part_v[slot] = jnp.dot(silu_c()[:, r0:r0 + n], wgu_v[pl.ds(r0, n), pl.ds(c0, D)],
                                   preferred_element_type=F32)

        def matsum(lo, n):
            m = part_v[lo]
            for i in range(1, n):
                m = m + part_v[lo + i]
            return m

        def q_first(h):
            return (qf_v[h] + qb_v[h, 0:1, :]).astype(BF)

        with scope("pro_init"):
            start(cp_small())
            cp_x(0).start()
            for i in range(len(CAC)):
                cp_ca(i).start()
            for i in range(len(QBC)):
                start(cp_qb(i))
            for i in range(len(SAC_)):
                cp_sa(i).start()
            start(cp_head0())
            for h in range(1, NH0):
                start(cp_head(h))
                if h == 2:
                    cp_x(1).start()
            cp_wo_last().start()
            cp_x(2).start()
            start(cp_group(T0))
            acc_v[...] = jnp.zeros_like(acc_v)
            top_v[...] = jnp.full(top_v.shape, IMIN, I32)
            mod_v[...] = jnp.zeros_like(mod_v)
        with scope("pro_ln"):
            wait(cp_small())
            sc_v[...] = jnp.broadcast_to(silu_c()[0:1].astype(F32), (128, D)).T
            hox_v[3 * S + 32 + RP:3 * S + 48 + RP, :] = jnp.zeros((16, D + PH), BF)
            cp_x(0).wait()
            _, xc0, rs0 = center(hox_v[pl.ds(XO, RP), cols].astype(F32))
            xn_v[...] = xc0 * rs0
        with scope("pro_ca"):
            for i, (r0, n) in enumerate(CAC):
                cp_ca(i).wait()
                matvec(i, r0, n, D)
            s1 = rb(1.0 + rb(matsum(0, len(CAC))[0:1]))
            put_mod(S1, s1)
        hs = None

        def q_part(h):
            qf_v[h] = jnp.dot(hs, wq_head(h // G, h % G), preferred_element_type=F32) * QSCALE

        def h_piece(h):
            n = RP // NH0
            r0 = pl.multiple_of(h * n, n)
            hox_v[pl.ds(HO + r0, n), cols] = (xn_v[pl.ds(r0, n), :] * mrow(S1, n) + mrow(SA, n)).astype(BF)

        for i, (h0, n) in enumerate(QBC[:-1]):
            with scope(f"pro_q{i}"):
                wait(cp_qb(i))
                if hs is None:
                    hs = (xn_v[...] * s1).astype(BF)
                for h in range(h0, h0 + n):
                    q_part(h)
        with scope("pro_sa"):
            wait(cp_qb(len(QBC) - 1))
            for j in range(len(SAC_)):
                cp_sa(j).wait()
                matvec(len(CAC) + j, *SAC_[j], 0)
            for h in range(QBC[-1][0], NH0):
                q_part(h)
            sab = matsum(len(CAC), len(SAC_)).astype(BF)
            put_mod(SA, sab[0:1].astype(F32))
            for h in range(NH0):
                qb_v[h] = jnp.dot(sab, wq_head(h // G, h % G), preferred_element_type=F32) * QSCALE
        with scope("pro_head0"):
            wait(cp_head0())
            for g in range(T0 + 1, NG):
                start(cp_group(g))
                if g == T0 + 1:
                    start(cp_m2())
            PV_(QK_(q_first(0), 0), 0, True)
            h_piece(0)

        def mini(h, carry):
            with scope("mini_dma"):
                wait(cp_head(h))

                @pl.when(h == 3)
                def _():
                    cp_x(1).wait()
            with scope("mini_main"):
                q = q_first(h)
                dn = (((1,), (1,)), ((), ()))

                def fill():
                    inr = jnp.logical_and(h >= 3, h < 3 + T0 * SL // 32)
                    rl = jnp.where(inr, RP + (h - 3) * 32, 0)
                    for tok in MF:
                        if tok == "H":
                            h_piece(h)
                        elif tok == "L":
                            ln1(pl.multiple_of(rl, 32), 32)
                        elif tok == "l":
                            ln1(pl.multiple_of(rl, 16), 16)
                            ln1(pl.multiple_of(rl + 16, 16), 16)

                if MORD == 2:
                    fill()
                    parts = [lax.dot_general(q, k_v[h, 0:KC, :], dn, preferred_element_type=F32)]
                    op_carry(0, h - 1)
                    parts.append(lax.dot_general(q, k_v[h, KC:S, :], dn, preferred_element_type=F32))
                else:
                    QO = 3 * S + 32
                    hox_v[QO:QO + RP, 0:DH] = q
                    parts = [lax.dot_general(q, k_v[h, 0:KC, :], dn, preferred_element_type=F32)]
                    op_carry(0, h - 1)
                    if KD > KC:
                        parts.append(lax.dot_general(q, k_v[h, KC:KD, :], dn, preferred_element_type=F32))
                    fill()
                    q2 = hox_v[QO:QO + RP, 0:DH]
                    parts.append(lax.dot_general(q2, k_v[h, KD:S, :], dn, preferred_element_type=F32))
                PV_(jnp.concatenate(parts, axis=1), h, True)
            return carry

        lax.fori_loop(1, NH0, mini, 0)

        def body(t, carry):
            p = lax.shift_right_logical(t, LNG)
            g = t & (NG - 1)

            with scope("it_dma"):
                @pl.when(jnp.logical_or(t <= NG, g == 1))
                def _():
                    @pl.when(t < NG)
                    def _():
                        for c_ in cp_group(t):
                            c_.wait()

                    @pl.when(t == T0)
                    def _():
                        cp_wo_last().wait()
                        cp_x(2).wait()

                    @pl.when(t == TM)
                    def _():
                        wait(cp_m2())

                    @pl.when(t == NG)
                    def _():
                        if VM2:
                            m2 = jnp.concatenate([jnp.sum(mp_v[i], axis=0, keepdims=True) for i in range(4)], axis=1)
                            m2 = rb(m2)
                        else:
                            m2 = rb(jnp.dot(silu_c(), wgu_v[:, 2 * D:6 * D], preferred_element_type=F32))[0:1]
                        sb = m2[:, D:2 * D]
                        s2 = rb(1.0 + m2[:, 2 * D:3 * D])
                        gb = m2[:, 3 * D:4 * D]
                        wr = wr_v[...].astype(F32).reshape(1, D)
                        put_mod(GA, m2[:, 0:D])
                        put_mod(SB, sb)
                        put_mod(S2, s2)
                        put_mod(GB, gb)
                        put_mod(VA, gb * s2)
                        put_mod(VB, gb * sb)
                        put_mod(VW, s2 * wr)
                        put_mod(VC, jnp.broadcast_to(jnp.sum(sb * wr, axis=-1, keepdims=True), (1, D)))
                        start(cp_ffn(0))

                    @pl.when(t == 2 * NG + 1)
                    def _():
                        wait(cp_ffn(0))
                        start(cp_ffn(1))

                    @pl.when(jnp.logical_and(g == 1, p >= 2))
                    def _():
                        cp_out(p - 2).start()

                    @pl.when(t == NT - NG + 1)
                    def _():
                        wait(cp_ffn(1))

            with scope("it_main"):
                r0 = pl.multiple_of(p * RP, RP)
                h0 = g * G
                tp = t - 1
                ue = jnp.maximum(t - NG, 0)
                qs, ss, os_ = {}, {}, {}
                QO = 3 * S + 32
                dn = (((1,), (1,)), ((), ()))
                parts = {}
                for tok in SEQ.replace("_", " ").split():
                    kind = tok[0]
                    if kind == "k":
                        u, ab = tok[1:].split(".")
                        u, (a_, b_) = int(u), [int(z) for z in ab.split("-")]
                        if a_ == 0:
                            q_ = qs.pop(u)
                            hox_v[QO:QO + RP, u * DH:(u + 1) * DH] = q_
                            parts[u] = []
                        else:
                            q_ = hox_v[QO:QO + RP, u * DH:(u + 1) * DH]
                        parts[u].append(lax.dot_general(q_, k_v[h0 + u, a_ * 512:(b_ + 1) * 512, :], dn,
                                                        preferred_element_type=F32))
                        if b_ == 3:
                            ss[u] = jnp.concatenate(parts.pop(u), axis=1)
                        continue
                    rng = [int(z) for z in tok[1:].split("-")] if len(tok) > 1 else [0, SL // PC - 1]
                    u = rng[0]
                    if kind == "Q":
                        qs[u] = Qp_(hox_v[pl.ds(HO + r0, RP), cols], g, u)
                    elif kind == "K":
                        ss[u] = QK_(qs.pop(u), h0 + u)
                    elif kind == "P":
                        os_[u] = PV_(ss.pop(u), h0 + u, u == G - 1, sbf=bool((SBM >> u) & 1))
                    elif kind == "O":
                        Op_(os_.pop(u), r0, h0 + u)
                    elif kind == "C":
                        op_carry(pl.multiple_of(lax.shift_right_logical(tp, LNG) * RP, RP), (tp & (NG - 1)) * G + G - 1)
                    elif kind == "G":
                        hox_v[pl.ds(pl.multiple_of(3 * S + 16 * (t & 1), 16), 16), 0:DH] = raw[-1][RP - 16:RP].astype(BF)
                    elif kind == "H":
                        hox_v[pl.ds(pl.multiple_of(3 * S + 16 * (t & 1), 16), 16), 0:DH] = qs[u][RP - 16:RP]
                    elif kind == "M":
                        live = jnp.logical_and(t >= TM, t < TM + 4)
                        c0 = jnp.where(live, 2 * D + (t - TM) * D, jnp.where(t <= 2 * NG, 0, 4 * D))
                        slot = jnp.where(live, t - TM, 4)
                        ZO = 3 * S + 32 + RP
                        link = hox_v[ZO:ZO + 16, 0:MW].astype(F32)[0:8]
                        for j in range(D // MW):
                            acc_ = link
                            wv = wgu_v.at[:, pl.ds(pl.multiple_of(c0, D), D)]
                            for k in range(0, D, 8):
                                w = wv[k:k + 8, j * MW:(j + 1) * MW].astype(F32)
                                acc_ = acc_ + w * jnp.concatenate([sc_v[k:k + 8, :]] * (MW // 128), axis=1)
                            mp_v[slot, :, j * MW:(j + 1) * MW] = acc_
                            link = jnp.minimum(jnp.abs(acc_), 0.0)
                        hox_v[pl.ds(pl.multiple_of(3 * S + 16 * (t & 1), 16), 8), 0:MW] = link.astype(BF)
                    elif kind == "E":
                        for i in range(rng[0], rng[-1] + 1):
                            re = pl.multiple_of(ue * SL + i * PC, PC)
                            epi(re, PC, acc_rows(re, PC), t >= NG)
                    elif kind == "L":
                        for i in range(rng[0], rng[-1] + 1):
                            ln1(pl.multiple_of(jnp.minimum(t + NG, NSL - 1) * SL + i * PC, PC), PC)
            return carry

        lax.fori_loop(T0, NT, body, 0)

        with scope("epi_key"):
            o_last = (of_v[0] * _recip(jnp.sum(of_v[1], axis=-1, keepdims=True))).astype(BF)
            pair = (top_v[0], top_v[1])
            cp_out(NP - 2).start()
            for r0, n in [(S - RP + i * EC, EC) for i in range(RP // EC)]:
                a = acc_rows(r0, n)
                a = a + jnp.dot(o_last[r0 - (S - RP):r0 - (S - RP) + n], wo_v[H - 1, :, cols],
                                preferred_element_type=F32)
                x2 = resid(r0, n, a)
                if not SXC:
                    xn_v[r0 - (S - RP):r0 - (S - RP) + n, :] = x2
                mu, xc, rs = center(x2)
                if SXC == 1:
                    xn_v[r0 - (S - RP):r0 - (S - RP) + n, :] = xc
                if SXC == 2:
                    xn_v[r0 - (S - RP):r0 - (S - RP) + n, :] = x2
                    acc_v[pl.ds(r0, n), cols] = xc
                put_stats(r0, n, mu, rs)
                pair = merge(pair, fold(keys(r0, n, xc, rs)))
                if OUTF == 2:
                    t_ = rs * mrow(VA, n)
                    hox_v[pl.ds(OO + r0, n), cols] = (x2 * (t_ + 1.0) + (mrow(VB, n) - mu * t_)).astype(BF)
                elif OUTF == 3:
                    hox_v[pl.ds(OO + r0, n), cols] = (x2 + mrow(VB, n) + (x2 * rs - mu * rs) * mrow(VA, n)).astype(BF)
                elif OUTF:
                    hox_v[pl.ds(OO + r0, n), cols] = (xc * (rs * mrow(VA, n) + 1.0) + (mrow(VB, n) + mu)).astype(BF)
                else:
                    put_out(r0, n, x2, xc, rs)
            cp_out(NP - 1).start()
            for sh in (4, 2, 1):
                pair = merge(pair, (pltpu.roll(pair[0], sh, 0), pltpu.roll(pair[1], sh, 0)))
            k1, k2 = pair

            def score(k):
                b = jnp.where(k < 0, k ^ 0x7FFFFFFF, k) & (-65536)
                return lax.bitcast_convert_type(b, F32)[0:1, 0:1]

            i1 = jnp.clip(65535 - (k1[0, 0] & 65535), 0, S - 1)
            i2 = jnp.clip(65535 - (k2[0, 0] & 65535), 0, S - 1)
            t1 = pl.multiple_of(i1 & -16, 16)
            t2 = pl.multiple_of(i2 & -16, 16)

            def post(t0):
                x2 = resid(t0, 16, acc_rows(t0, 16))
                tl = pl.multiple_of(jnp.maximum(t0 - (S - RP), 0), 16)
                mu, rs = get_stats(t0, 16)
                x2 = jnp.where(t0 >= S - RP, xn_v[pl.ds(tl, 16), :] + (mu if SXC == 1 else 0.0), x2)
                return x2, ((x2 - mu) * rs) * mrow(S2, 16) + mrow(SB, 16)

            x2a, h2a = post(t1)
            x2b, h2b = post(t2)
            row = lax.broadcasted_iota(I32, (16, D), 0)
            sel1 = jnp.sum(jnp.where(row == i1 - t1, h2a, 0.0), axis=0, keepdims=True)
            sel2 = jnp.sum(jnp.where(row == i2 - t2, h2b, 0.0), axis=0, keepdims=True)
            xs = jnp.where(row == 0, sel1, jnp.where(row == 1, sel2, 0.0)).astype(BF)
        with scope("epi_ffn"):
            if BAR:
                cp_out(0).wait()
            gt = jnp.dot(xs, wgu_v[:, 0:F], preferred_element_type=F32)
            up = jnp.dot(xs, wgu_v[:, F:2 * F], preferred_element_type=F32)
            act = (gt * jax.nn.sigmoid(gt) * up).astype(BF)
            y = jnp.dot(act, wd_v[:, cols], preferred_element_type=F32)
            y1 = y[0:1, :] * jax.nn.sigmoid(score(k1))
            y2 = y[1:2, :] * jax.nn.sigmoid(score(k2))

            def upd(t0):
                return jnp.where(row == i1 - t0, y1, 0.0) + jnp.where(row == i2 - t0, y2, 0.0)

            patch_v[0] = (x2a + mrow(GB, 16) * (h2a + upd(t1))).astype(BF)
            patch_v[1] = (x2b + mrow(GB, 16) * (h2b + upd(t2))).astype(BF)
        with scope("epi_out"):
            for p in range(1 if BAR else 0, NP):
                cp_out(p).wait()
            pa = cp(patch_v.at[0], out_hbm.at[pl.ds(t1, 16)], SP)
            pb = cp(patch_v.at[1], out_hbm.at[pl.ds(t2, 16)], SP + 1)
            pa.start()

            @pl.when(t1 != t2)
            def _():
                pb.start()
                pb.wait()

            pa.wait()

    def fn(A_x, A_k_cache, A_v_cache, A_wq, A_wo, B_x, B_w_r, B_w_gate, B_w_up, B_w_down, c, w_mod):
        any_ = pl.BlockSpec(memory_space=pl.ANY)
        out = pl.pallas_call(
            kernel,
            in_specs=[any_] * 11,
            out_specs=any_,
            out_shape=jax.ShapeDtypeStruct((S, D), BF),
            scratch_shapes=[
                pltpu.VMEM((H, S, DH), BF),
                pltpu.VMEM((H, S, DH), BF),
                pltpu.VMEM((NG, D, G * DH + PQ), BF),
                pltpu.VMEM((H, DH, D + PW), BF),
                pltpu.VMEM((D, 2 * F + 128), BF),
                pltpu.VMEM((F, D + 128), BF),
                pltpu.VMEM((3 * S + 32 + RP + 16, D + PH), BF),
                pltpu.VMEM((S, D + PA), F32),
                pltpu.VMEM((10, 8, D), F32),
                pltpu.VMEM((2, 8, 128), I32),
                pltpu.VMEM((2, 16, D), BF),
                pltpu.VMEM((2, RP, DH), F32),
                pltpu.VMEM((RP, D), F32),
                pltpu.VMEM((2, S, 128), F32),
                pltpu.VMEM((len(CAC) + len(SAC_), 16, D), F32),
                pltpu.VMEM((NH0, RP, DH), F32),
                pltpu.VMEM((NH0, 16, DH), F32),
                pltpu.VMEM((D, 128), F32),
                pltpu.VMEM((5, 8, D), F32),
                pltpu.VMEM((1, D), BF),
                pltpu.VMEM((D,), BF),
                pltpu.SemaphoreType.DMA((NSEM,)),
            ],
            compiler_params=pltpu.CompilerParams(vmem_limit_bytes=120 << 20, disable_bounds_checks=True,
                                                 disable_semaphore_checks=True),
            name=name,
        )(A_x.reshape(S, D), A_k_cache.reshape(H, S, DH), A_v_cache.reshape(H, S, DH), A_wq,
          A_wo.reshape(H, DH, D), B_w_r, B_w_gate, B_w_up, B_w_down, c, w_mod)
        return out.reshape(1, S, D)

    return fn


_impl = make_kernel(OUTF=0, EC=128)


@jax.jit
def pallas_adaLN_cond__mha_block_cached__moe_arch_mod__prompt_kernel(
    A_x: jax.Array,
    A_k_cache: jax.Array,
    A_v_cache: jax.Array,
    A_wq: jax.Array,
    A_wo: jax.Array,
    B_x: jax.Array,
    B_w_r: jax.Array,
    B_w_gate: jax.Array,
    B_w_up: jax.Array,
    B_w_down: jax.Array,
    c: jax.Array,
    w_mod: jax.Array,
):
    return _impl(A_x, A_k_cache, A_v_cache, A_wq, A_wo, B_x, B_w_r, B_w_gate, B_w_up, B_w_down, c, w_mod)
```

```python
import jax
import jax.numpy as jnp
from jax import lax
import jax.experimental.pallas as pl
import jax.experimental.pallas.tpu as pltpu

S, D, H, DH, F = 2048, 1024, 32, 128, 3584
EPS = 1e-5
QSCALE = DH ** -0.5 * 1.4426950408889634
BF, F32, I32 = jnp.bfloat16, jnp.float32, jnp.int32
IMIN = -2 ** 31
NT_DIMS = (((1,), (1,)), ((), ()))

RP = 512
G = 4
NP, NG = S // RP, H // G
LNG = NG.bit_length() - 1
NT = NP * NG
SL = RP // NG
PC = 16
T0 = 2
NH0 = T0 * G
TM = NG - 4
X1 = RP + T0 * SL
EC = 128
CA_CHUNKS = ((0, 512), (512, 256), (768, 256))
Q_BATCHES = ((0, 1), (1, 2), (3, 4), (7, 1))

HO, OO, XO, GO = 0, S, 2 * S, 3 * S
QO = GO + 32
ZO = QO + RP
SA, S1, GA, SB, S2, GB, VA, VB, VW, VC = range(10)
SX = 0
SCA = SX + 3
SSA = SCA + len(CA_CHUNKS)
SM2 = SSA + 1
SQ = SM2 + 1
SH = SQ + len(Q_BATCHES)
SGR = SH + NH0 + 1
SF = SGR + NG
SO = SF + 1
SP = SO + NP
SC = SP + 2
NSEM = SC + 1


def _recip(l):
    ri = pl.reciprocal(l, approx=True)
    return ri * (2.0 - l * ri)


def _rb(a):
    return a.astype(BF).astype(F32)


def _center(x):
    mu = jnp.mean(x, axis=-1, keepdims=True)
    xc = x - mu
    rs = lax.rsqrt(jnp.mean(xc * xc, axis=-1, keepdims=True) + EPS)
    return mu, xc, rs


def _merge(a, b):
    return jnp.maximum(a[0], b[0]), jnp.maximum(jnp.minimum(a[0], b[0]), jnp.maximum(a[1], b[1]))


def _fold(k):
    t = [k[i:i + 8] for i in range(0, k.shape[0], 8)]
    ps = [(jnp.maximum(t[i], t[i + 1]), jnp.minimum(t[i], t[i + 1])) for i in range(0, len(t), 2)]
    while len(ps) > 1:
        ps = [_merge(ps[i], ps[i + 1]) for i in range(0, len(ps), 2)]
    return ps[0]


def _kernel(x_hbm, k_hbm, v_hbm, wq_hbm, wo_hbm, wr_hbm, wg_hbm, wu_hbm, wd_hbm, c_hbm, wm_hbm,
            out_hbm,
            k_v, v_v, wq_v, wo_v, wgu_v, wd_v, hox_v, acc_v, mod_v, top_v, patch_v, of_v, xn_v, st_v,
            part_v, qf_v, qb_v, sc_v, mp_v, c_v, wr_v, sems):
    def cp(src, dst, s):
        return pltpu.make_async_copy(src, dst, sems.at[s])

    def cp_x(i):
        r0, n = [(0, RP), (RP, X1 - RP), (X1, S - X1)][i]
        return [cp(x_hbm.at[pl.ds(r0, n)], hox_v.at[pl.ds(XO + r0, n)], SX + i)]

    def cp_wm(r0, n, c0, w, s):
        return [cp(wm_hbm.at[pl.ds(r0, n), pl.ds(c0, w)], wgu_v.at[pl.ds(r0, n), pl.ds(c0, w)], s)]

    def cp_ca(i):
        return cp_wm(*CA_CHUNKS[i], D, D, SCA + i)

    def cp_sa():
        return cp_wm(0, D, 0, D, SSA)

    def cp_m2():
        return cp_wm(0, D, 2 * D, 4 * D, SM2)

    def cp_wo(h, n, s):
        return cp(wo_hbm.at[pl.ds(h, n)], wo_v.at[pl.ds(h, n)], s)

    def cp_qb(i):
        h0, n = Q_BATCHES[i]
        return [cp(wq_hbm.at[:, pl.ds(h * DH, DH)], wq_v.at[h // G, :, pl.ds((h % G) * DH, DH)], SQ + i)
                for h in range(h0, h0 + n)]

    def cp_kv(h):
        return [cp(k_hbm.at[h], k_v.at[h], SH + h), cp(v_hbm.at[h], v_v.at[h], SH + h)]

    def cp_head(h):
        return [cp_wo(h - 1, 1, SH + h)] + cp_kv(h)

    def cp_wo_last():
        return [cp_wo(NH0 - 1, 1, SH + NH0)]

    def cp_group(g):
        h0 = g * G
        s = SGR + g
        return [cp(wq_hbm.at[:, pl.ds(pl.multiple_of(h0 * DH, G * DH), G * DH)], wq_v.at[g], s),
                cp(k_hbm.at[pl.ds(h0, G)], k_v.at[pl.ds(h0, G)], s),
                cp(v_hbm.at[pl.ds(h0, G)], v_v.at[pl.ds(h0, G)], s),
                cp_wo(h0, G, s)]

    def cp_ffn(i):
        if i == 0:
            return [cp(wu_hbm, wgu_v.at[:, pl.ds(F, F)], SF), cp(wd_hbm, wd_v.at[:, pl.ds(0, D)], SF)]
        return [cp(wg_hbm, wgu_v.at[:, pl.ds(0, F)], SF)]

    def cp_out(p):
        r0 = pl.multiple_of(p * RP, RP)
        return [cp(hox_v.at[pl.ds(OO + r0, RP)], out_hbm.at[pl.ds(r0, RP)], SO + p)]

    def cp_small():
        return [cp(c_hbm, c_v, SC), cp(wr_hbm, wr_v, SC)]

    def start(cs):
        for c_ in cs:
            c_.start()

    def wait(cs):
        for c_ in cs:
            c_.wait()

    def mrow(i, n):
        return jnp.concatenate([mod_v[i]] * (n // 8), axis=0)

    def put_mod(i, v):
        mod_v[i] = jnp.broadcast_to(v, (8, D))

    def silu_c():
        c = c_v[...].astype(F32)
        return jnp.broadcast_to((c * jax.nn.sigmoid(c)).astype(BF), (16, D))

    def ln1(r0, n):
        _, xc, rs = _center(hox_v[pl.ds(XO + r0, n), :].astype(F32))
        hox_v[pl.ds(HO + r0, n), :] = ((xc * rs) * mrow(S1, n) + mrow(SA, n)).astype(BF)

    def resid(r0, n, a):
        return hox_v[pl.ds(XO + r0, n), :].astype(F32) + mrow(GA, n) * a

    def keys(r0, n, xc, rs):
        r = _rb(rs * jnp.sum(xc * mrow(VW, n), axis=-1, keepdims=True) + mrow(VC, n)[:, 0:128])
        b = lax.bitcast_convert_type(r, I32)
        b = jnp.where(b < 0, b ^ 0x7FFFFFFF, b) & (-65536)
        return b | (65535 - r0 - lax.broadcasted_iota(I32, (n, 128), 0))

    def put_stats(r0, n, mu, rs):
        st_v[0, pl.ds(r0, n), :] = jnp.broadcast_to(mu, (n, 128))
        st_v[1, pl.ds(r0, n), :] = jnp.broadcast_to(rs, (n, 128))

    def put_out(r0, n, x2, xc, rs):
        hox_v[pl.ds(OO + r0, n), :] = (x2 + mrow(VB, n) + (xc * rs) * mrow(VA, n)).astype(BF)

    def epi(r0, n, valid):
        x2 = resid(r0, n, acc_v[pl.ds(r0, n), :])
        mu, xc, rs = _center(x2)
        put_out(r0, n, x2, xc, rs)
        put_stats(r0, n, mu, rs)
        k1, k2 = _fold(keys(r0, n, xc, rs))
        k1, k2 = _merge((top_v[0], top_v[1]), (jnp.where(valid, k1, IMIN), jnp.where(valid, k2, IMIN)))
        top_v[0] = k1
        top_v[1] = k2

    def wq_head(g, u):
        return wq_v[g, :, u * DH:(u + 1) * DH]

    def qk(q, hd, k0=0, k1=S):
        return lax.dot_general(q, k_v[hd, k0:k1, :], NT_DIMS, preferred_element_type=F32)

    def probs(s):
        p = jnp.exp2(s - jnp.max(s, axis=-1, keepdims=True)).astype(BF)
        return p, p.astype(F32)

    def pv(s, hd):
        p, pf = probs(s)
        l = jnp.sum(pf, axis=-1, keepdims=True)
        o = jnp.dot(p, v_v[hd], preferred_element_type=F32)
        return (o * _recip(l)).astype(BF), o

    def pv_carry(s, hd):
        p, pf = probs(s)
        lp = pf[:, 0:128]
        for j in range(1, S // 128):
            lp = lp + pf[:, j * 128:(j + 1) * 128]
        of_v[0] = jnp.dot(p, v_v[hd], preferred_element_type=F32)
        of_v[1] = lp

    def carried_o():
        return (of_v[0] * _recip(jnp.sum(of_v[1], axis=-1, keepdims=True))).astype(BF)

    def oproj(o, r0, hd):
        acc_v[pl.ds(r0, RP), :] += jnp.dot(o, wo_v[hd], preferred_element_type=F32)

    start(cp_small())
    start(cp_x(0))
    for i in range(len(CA_CHUNKS)):
        start(cp_ca(i))
    for i in range(len(Q_BATCHES)):
        start(cp_qb(i))
    start(cp_sa())
    start(cp_kv(0))
    for h in range(1, NH0):
        start(cp_head(h))
        if h == 2:
            start(cp_x(1))
    start(cp_wo_last())
    start(cp_x(2))
    start(cp_group(T0))
    acc_v[...] = jnp.zeros_like(acc_v)
    top_v[...] = jnp.full(top_v.shape, IMIN, I32)
    mod_v[...] = jnp.zeros_like(mod_v)

    wait(cp_small())
    sc_v[...] = jnp.broadcast_to(silu_c()[0:1].astype(F32), (128, D)).T
    hox_v[ZO:ZO + 16, :] = jnp.zeros((16, D), BF)
    wait(cp_x(0))
    _, xc0, rs0 = _center(hox_v[pl.ds(XO, RP), :].astype(F32))
    xn_v[...] = xc0 * rs0

    def matvec(slot, r0, n, c0):
        part_v[slot] = jnp.dot(silu_c()[:, r0:r0 + n], wgu_v[pl.ds(r0, n), pl.ds(c0, D)],
                               preferred_element_type=F32)

    for i, (r0, n) in enumerate(CA_CHUNKS):
        wait(cp_ca(i))
        matvec(i, r0, n, D)
    s1 = _rb(1.0 + _rb((part_v[0] + part_v[1] + part_v[2])[0:1]))
    put_mod(S1, s1)

    hs = None
    for i, (h0, n) in enumerate(Q_BATCHES):
        wait(cp_qb(i))
        if i == 0:
            hs = (xn_v[...] * s1).astype(BF)
        if i == len(Q_BATCHES) - 1:
            wait(cp_sa())
            matvec(len(CA_CHUNKS), 0, D, 0)
        for h in range(h0, h0 + n):
            qf_v[h] = jnp.dot(hs, wq_head(h // G, h % G), preferred_element_type=F32) * QSCALE
    sab = part_v[len(CA_CHUNKS)].astype(BF)
    put_mod(SA, sab[0:1].astype(F32))
    for h in range(NH0):
        qb_v[h] = jnp.dot(sab, wq_head(h // G, h % G), preferred_element_type=F32) * QSCALE

    def q_first(h):
        return (qf_v[h] + qb_v[h, 0:1, :]).astype(BF)

    def h_piece(h):
        n = RP // NH0
        r0 = pl.multiple_of(h * n, n)
        hox_v[pl.ds(HO + r0, n), :] = (xn_v[pl.ds(r0, n), :] * mrow(S1, n) + mrow(SA, n)).astype(BF)

    wait(cp_kv(0))
    for g in range(T0 + 1, NG):
        start(cp_group(g))
        if g == T0 + 1:
            start(cp_m2())
    pv_carry(qk(q_first(0), 0), 0)
    h_piece(0)

    def mini(h, carry):
        wait(cp_head(h))

        @pl.when(h == 3)
        def _():
            wait(cp_x(1))

        q = q_first(h)
        hox_v[QO:QO + RP, 0:DH] = q
        s_a = qk(q, h, 0, 512)
        oproj(carried_o(), 0, h - 1)
        live = jnp.logical_and(h >= 3, h < 3 + T0 * SL // 32)
        ln1(pl.multiple_of(jnp.where(live, RP + (h - 3) * 32, 0), 32), 32)
        h_piece(h)
        s_b = qk(hox_v[QO:QO + RP, 0:DH], h, 512, S)
        pv_carry(jnp.concatenate([s_a, s_b], axis=1), h)
        return carry

    lax.fori_loop(1, NH0, mini, 0)

    def block(t, carry):
        p = lax.shift_right_logical(t, LNG)
        g = t & (NG - 1)

        @pl.when(jnp.logical_or(t <= NG, g == 1))
        def _():
            @pl.when(t < NG)
            def _():
                wait(cp_group(t))

            @pl.when(t == T0)
            def _():
                wait(cp_wo_last())
                wait(cp_x(2))

            @pl.when(t == TM)
            def _():
                wait(cp_m2())

            @pl.when(t == NG)
            def _():
                m2 = _rb(jnp.concatenate([jnp.sum(mp_v[i], axis=0, keepdims=True) for i in range(4)], axis=1))
                sb = m2[:, D:2 * D]
                s2 = _rb(1.0 + m2[:, 2 * D:3 * D])
                gb = m2[:, 3 * D:4 * D]
                wr = wr_v[...].astype(F32).reshape(1, D)
                put_mod(GA, m2[:, 0:D])
                put_mod(SB, sb)
                put_mod(S2, s2)
                put_mod(GB, gb)
                put_mod(VA, gb * s2)
                put_mod(VB, gb * sb)
                put_mod(VW, s2 * wr)
                put_mod(VC, jnp.broadcast_to(jnp.sum(sb * wr, axis=-1, keepdims=True), (1, D)))
                start(cp_ffn(0))

            @pl.when(t == 2 * NG + 1)
            def _():
                wait(cp_ffn(0))
                start(cp_ffn(1))

            @pl.when(jnp.logical_and(g == 1, p >= 2))
            def _():
                start(cp_out(p - 2))

            @pl.when(t == NT - NG + 1)
            def _():
                wait(cp_ffn(1))

        r0 = pl.multiple_of(p * RP, RP)
        h0 = g * G

        def qproj(u):
            q = jnp.dot(hox_v[pl.ds(HO + r0, RP), :], wq_head(g, u), preferred_element_type=F32)
            return (q * QSCALE).astype(BF)

        def gate(val):
            hox_v[pl.ds(pl.multiple_of(GO + 16 * (t & 1), 16), val.shape[0]), 0:DH] = val.astype(BF)

        def mod_quarter():
            live = jnp.logical_and(t >= TM, t < TM + 4)
            c0 = jnp.where(live, 2 * D + (t - TM) * D, jnp.where(t <= 2 * NG, 0, 4 * D))
            slot = jnp.where(live, t - TM, 4)
            link = hox_v[ZO:ZO + 16, 0:128].astype(F32)[0:8]
            for j in range(D // 128):
                a = link
                wv = wgu_v.at[:, pl.ds(pl.multiple_of(c0, D), D)]
                for k in range(0, D, 8):
                    a = a + wv[k:k + 8, j * 128:(j + 1) * 128].astype(F32) * sc_v[k:k + 8, :]
                mp_v[slot, :, j * 128:(j + 1) * 128] = a
                link = jnp.minimum(jnp.abs(a), 0.0)
            gate(link)

        q0 = qproj(0)
        tp = t - 1
        oproj(carried_o(), pl.multiple_of(lax.shift_right_logical(tp, LNG) * RP, RP), (tp & (NG - 1)) * G + G - 1)
        q1 = qproj(1)
        gate(q1[RP - 16:RP])
        for i in range(SL // PC):
            epi(pl.multiple_of(jnp.maximum(t - NG, 0) * SL + i * PC, PC), PC, t >= NG)
        s = qk(q0, h0)
        q2 = qproj(2)
        o0, raw = pv(s, h0)
        gate(raw[RP - 16:RP])
        for i in range(SL // PC):
            ln1(pl.multiple_of(jnp.minimum(t + NG, S // SL - 1) * SL + i * PC, PC), PC)
        s = qk(q1, h0 + 1)
        q3 = qproj(3)
        o1, _ = pv(s, h0 + 1)
        s = qk(q2, h0 + 2)
        oproj(o0, r0, h0)
        o2, raw = pv(s, h0 + 2)
        gate(raw[RP - 16:RP])
        hox_v[QO:QO + RP, 3 * DH:4 * DH] = q3
        s_a = qk(q3, h0 + 3, 0, 1536)
        mod_quarter()
        s_b = qk(hox_v[QO:QO + RP, 3 * DH:4 * DH], h0 + 3, 1536, S)
        oproj(o1, r0, h0 + 1)
        pv_carry(jnp.concatenate([s_a, s_b], axis=1), h0 + 3)
        oproj(o2, r0, h0 + 2)
        return carry

    lax.fori_loop(T0, NT, block, 0)

    RL = S - RP
    o_last = carried_o()
    pair = (top_v[0], top_v[1])
    start(cp_out(NP - 2))
    for r in range(0, RP, EC):
        a = acc_v[pl.ds(RL + r, EC), :] + jnp.dot(o_last[r:r + EC], wo_v[H - 1], preferred_element_type=F32)
        x2 = resid(RL + r, EC, a)
        xn_v[r:r + EC, :] = x2
        mu, xc, rs = _center(x2)
        put_stats(RL + r, EC, mu, rs)
        pair = _merge(pair, _fold(keys(RL + r, EC, xc, rs)))
        put_out(RL + r, EC, x2, xc, rs)
    start(cp_out(NP - 1))
    for sh in (4, 2, 1):
        pair = _merge(pair, (pltpu.roll(pair[0], sh, 0), pltpu.roll(pair[1], sh, 0)))
    k1, k2 = pair

    def score(k):
        b = jnp.where(k < 0, k ^ 0x7FFFFFFF, k) & (-65536)
        return lax.bitcast_convert_type(b, F32)[0:1, 0:1]

    def row_of(k):
        i = 65535 - (k[0, 0] & 65535)
        return i, pl.multiple_of(jnp.clip(i >> 4, 0, S // 16 - 1) * 16, 16)

    i1, t1 = row_of(k1)
    i2, t2 = row_of(k2)

    def post(t0):
        x2 = resid(t0, 16, acc_v[pl.ds(t0, 16), :])
        tl = pl.multiple_of(jnp.maximum(t0 - RL, 0), 16)
        mu = jnp.concatenate([st_v[0, pl.ds(t0, 16), :]] * (D // 128), axis=1)
        rs = jnp.concatenate([st_v[1, pl.ds(t0, 16), :]] * (D // 128), axis=1)
        x2 = jnp.where(t0 >= RL, xn_v[pl.ds(tl, 16), :], x2)
        return x2, ((x2 - mu) * rs) * mrow(S2, 16) + mrow(SB, 16)

    x2a, h2a = post(t1)
    x2b, h2b = post(t2)
    row = lax.broadcasted_iota(I32, (16, D), 0)
    sel1 = jnp.sum(jnp.where(row == i1 - t1, h2a, 0.0), axis=0, keepdims=True)
    sel2 = jnp.sum(jnp.where(row == i2 - t2, h2b, 0.0), axis=0, keepdims=True)
    xs = jnp.where(row == 0, sel1, jnp.where(row == 1, sel2, 0.0)).astype(BF)

    wait(cp_out(0))
    gt = jnp.dot(xs, wgu_v[:, 0:F], preferred_element_type=F32)
    up = jnp.dot(xs, wgu_v[:, F:2 * F], preferred_element_type=F32)
    act = (gt * jax.nn.sigmoid(gt) * up).astype(BF)
    y = jnp.dot(act, wd_v[:, 0:D], preferred_element_type=F32)
    y1 = y[0:1, :] * jax.nn.sigmoid(score(k1))
    y2 = y[1:2, :] * jax.nn.sigmoid(score(k2))

    def upd(t0):
        return jnp.where(row == i1 - t0, y1, 0.0) + jnp.where(row == i2 - t0, y2, 0.0)

    patch_v[0] = (x2a + mrow(GB, 16) * (h2a + upd(t1))).astype(BF)
    patch_v[1] = (x2b + mrow(GB, 16) * (h2b + upd(t2))).astype(BF)
    for p in range(1, NP):
        wait(cp_out(p))
    pa = cp(patch_v.at[0], out_hbm.at[pl.ds(t1, 16)], SP)
    pb = cp(patch_v.at[1], out_hbm.at[pl.ds(t2, 16)], SP + 1)
    pa.start()

    @pl.when(t1 != t2)
    def _():
        pb.start()
        pb.wait()

    pa.wait()


@jax.jit
def pallas_adaLN_cond__mha_block_cached__moe_arch_mod__prompt_kernel(
    A_x: jax.Array,
    A_k_cache: jax.Array,
    A_v_cache: jax.Array,
    A_wq: jax.Array,
    A_wo: jax.Array,
    B_x: jax.Array,
    B_w_r: jax.Array,
    B_w_gate: jax.Array,
    B_w_up: jax.Array,
    B_w_down: jax.Array,
    c: jax.Array,
    w_mod: jax.Array,
):
    hbm = pl.BlockSpec(memory_space=pl.ANY)
    out = pl.pallas_call(
        _kernel,
        in_specs=[hbm] * 11,
        out_specs=hbm,
        out_shape=jax.ShapeDtypeStruct((S, D), BF),
        scratch_shapes=[
            pltpu.VMEM((H, S, DH), BF),
            pltpu.VMEM((H, S, DH), BF),
            pltpu.VMEM((NG, D, G * DH), BF),
            pltpu.VMEM((H, DH, D), BF),
            pltpu.VMEM((D, 2 * F + 128), BF),
            pltpu.VMEM((F, D + 128), BF),
            pltpu.VMEM((ZO + 16, D), BF),
            pltpu.VMEM((S, D), F32),
            pltpu.VMEM((10, 8, D), F32),
            pltpu.VMEM((2, 8, 128), I32),
            pltpu.VMEM((2, 16, D), BF),
            pltpu.VMEM((2, RP, DH), F32),
            pltpu.VMEM((RP, D), F32),
            pltpu.VMEM((2, S, 128), F32),
            pltpu.VMEM((len(CA_CHUNKS) + 1, 16, D), F32),
            pltpu.VMEM((NH0, RP, DH), F32),
            pltpu.VMEM((NH0, 16, DH), F32),
            pltpu.VMEM((D, 128), F32),
            pltpu.VMEM((5, 8, D), F32),
            pltpu.VMEM((1, D), BF),
            pltpu.VMEM((D,), BF),
            pltpu.SemaphoreType.DMA((NSEM,)),
        ],
        compiler_params=pltpu.CompilerParams(vmem_limit_bytes=120 << 20, disable_bounds_checks=True,
                                             disable_semaphore_checks=True),
        name="adaln_mha_moe",
    )(A_x.reshape(S, D), A_k_cache.reshape(H, S, DH), A_v_cache.reshape(H, S, DH), A_wq,
      A_wo.reshape(H, DH, D), B_w_r, B_w_gate, B_w_up, B_w_down, c, w_mod)
    return out.reshape(1, S, D)
```

```python
import jax
import jax.numpy as jnp
from jax import lax
import jax.experimental.pallas as pl
import jax.experimental.pallas.tpu as pltpu

S, D, H, DH, F = 2048, 1024, 32, 128, 3584
EPS = 1e-5
QSCALE = DH ** -0.5 * 1.4426950408889634
BF, F32, I32 = jnp.bfloat16, jnp.float32, jnp.int32
IMIN = -2 ** 31
NT_DIMS = (((1,), (1,)), ((), ()))

RP = 512
G = 4
NP, NG = S // RP, H // G
LNG = NG.bit_length() - 1
NT = NP * NG
SL = RP // NG
PC = 16
T0 = 2
NH0 = T0 * G
TM = NG - 4
X1 = RP + T0 * SL
EC = 128
CA_CHUNKS = ((0, 512), (512, 256), (768, 256))
Q_BATCHES = ((0, 1), (1, 2), (3, 4), (7, 1))

HO, OO, XO, GO = 0, S, 2 * S, 3 * S
QO = GO + 32
ZO = QO + RP
SA, S1, GA, SB, S2, GB, VA, VB, VW, VC = range(10)
SX = 0
SCA = SX + 3
SSA = SCA + len(CA_CHUNKS)
SM2 = SSA + 1
SQ = SM2 + 1
SH = SQ + len(Q_BATCHES)
SGR = SH + NH0 + 1
SF = SGR + NG
SO = SF + 1
SP = SO + NP
SC = SP + 2
NSEM = SC + 1


def _recip(l):
    ri = pl.reciprocal(l, approx=True)
    return ri * (2.0 - l * ri)


def _rb(a):
    return a.astype(BF).astype(F32)


def _center(x):
    mu = jnp.mean(x, axis=-1, keepdims=True)
    xc = x - mu
    rs = lax.rsqrt(jnp.mean(xc * xc, axis=-1, keepdims=True) + EPS)
    return mu, xc, rs


def _merge(a, b):
    return jnp.maximum(a[0], b[0]), jnp.maximum(jnp.minimum(a[0], b[0]), jnp.maximum(a[1], b[1]))


def _fold(k):
    t = [k[i:i + 8] for i in range(0, k.shape[0], 8)]
    ps = [(jnp.maximum(t[i], t[i + 1]), jnp.minimum(t[i], t[i + 1])) for i in range(0, len(t), 2)]
    while len(ps) > 1:
        ps = [_merge(ps[i], ps[i + 1]) for i in range(0, len(ps), 2)]
    return ps[0]


def _kernel(x_hbm, k_hbm, v_hbm, wq_hbm, wo_hbm, wr_hbm, wg_hbm, wu_hbm, wd_hbm, c_hbm, wm_hbm,
            out_hbm,
            k_v, v_v, wq_v, wo_v, wgu_v, wd_v, hox_v, acc_v, mod_v, top_v, patch_v, of_v, xn_v, st_v,
            part_v, qf_v, qb_v, sc_v, scb_v, mp_v, c_v, wr_v, sems):
    def cp(src, dst, s):
        return pltpu.make_async_copy(src, dst, sems.at[s])

    def cp_x(i):
        r0, n = [(0, RP), (RP, X1 - RP), (X1, S - X1)][i]
        return [cp(x_hbm.at[pl.ds(r0, n)], hox_v.at[pl.ds(XO + r0, n)], SX + i)]

    def cp_wm(r0, n, c0, w, s):
        return [cp(wm_hbm.at[pl.ds(r0, n), pl.ds(c0, w)], wgu_v.at[pl.ds(r0, n), pl.ds(c0, w)], s)]

    def cp_ca(i):
        return cp_wm(*CA_CHUNKS[i], D, D, SCA + i)

    def cp_sa():
        return cp_wm(0, D, 0, D, SSA)

    def cp_m2():
        return cp_wm(0, D, 2 * D, 4 * D, SM2)

    def cp_wo(h, n, s):
        return cp(wo_hbm.at[pl.ds(h, n)], wo_v.at[pl.ds(h, n)], s)

    def cp_qb(i):
        h0, n = Q_BATCHES[i]
        return [cp(wq_hbm.at[:, pl.ds(h * DH, DH)], wq_v.at[h // G, :, pl.ds((h % G) * DH, DH)], SQ + i)
                for h in range(h0, h0 + n)]

    def cp_kv(h):
        return [cp(k_hbm.at[h], k_v.at[h], SH + h), cp(v_hbm.at[h], v_v.at[h], SH + h)]

    def cp_head(h):
        return [cp_wo(h - 1, 1, SH + h)] + cp_kv(h)

    def cp_wo_last():
        return [cp_wo(NH0 - 1, 1, SH + NH0)]

    def cp_group(g):
        h0 = g * G
        s = SGR + g
        return [cp(wq_hbm.at[:, pl.ds(pl.multiple_of(h0 * DH, G * DH), G * DH)], wq_v.at[g], s),
                cp(k_hbm.at[pl.ds(h0, G)], k_v.at[pl.ds(h0, G)], s),
                cp(v_hbm.at[pl.ds(h0, G)], v_v.at[pl.ds(h0, G)], s),
                cp_wo(h0, G, s)]

    def cp_ffn(i):
        if i == 0:
            return [cp(wu_hbm, wgu_v.at[:, pl.ds(F, F)], SF), cp(wd_hbm, wd_v.at[:, pl.ds(0, D)], SF)]
        return [cp(wg_hbm, wgu_v.at[:, pl.ds(0, F)], SF)]

    def cp_out(p):
        r0 = pl.multiple_of(p * RP, RP)
        return [cp(hox_v.at[pl.ds(OO + r0, RP)], out_hbm.at[pl.ds(r0, RP)], SO + p)]

    def cp_small():
        return [cp(c_hbm, c_v, SC), cp(wr_hbm, wr_v, SC)]

    def start(cs):
        for c_ in cs:
            c_.start()

    def wait(cs):
        for c_ in cs:
            c_.wait()

    def mrow(i, n):
        return jnp.concatenate([mod_v[i]] * (n // 8), axis=0)

    def put_mod(i, v):
        mod_v[i] = jnp.broadcast_to(v, (8, D))

    def ln1(r0, n):
        _, xc, rs = _center(hox_v[pl.ds(XO + r0, n), :].astype(F32))
        hox_v[pl.ds(HO + r0, n), :] = ((xc * rs) * mrow(S1, n) + mrow(SA, n)).astype(BF)

    def resid(r0, n, a):
        return hox_v[pl.ds(XO + r0, n), :].astype(F32) + mrow(GA, n) * a

    def keys(r0, n, xc, rs):
        r = _rb(rs * jnp.sum(xc * mrow(VW, n), axis=-1, keepdims=True) + mrow(VC, n)[:, 0:128])
        b = lax.bitcast_convert_type(r, I32)
        b = jnp.where(b < 0, b ^ 0x7FFFFFFF, b) & (-65536)
        return b | (65535 - r0 - lax.broadcasted_iota(I32, (n, 128), 0))

    def put_stats(r0, n, mu, rs):
        st_v[0, pl.ds(r0, n), :] = jnp.broadcast_to(mu, (n, 128))
        st_v[1, pl.ds(r0, n), :] = jnp.broadcast_to(rs, (n, 128))

    def put_out(r0, n, x2, xc, rs):
        hox_v[pl.ds(OO + r0, n), :] = (x2 + mrow(VB, n) + (xc * rs) * mrow(VA, n)).astype(BF)

    def epi(r0, n, valid):
        x2 = resid(r0, n, acc_v[pl.ds(r0, n), :])
        mu, xc, rs = _center(x2)
        put_out(r0, n, x2, xc, rs)
        put_stats(r0, n, mu, rs)
        k1, k2 = _fold(keys(r0, n, xc, rs))
        k1, k2 = _merge((top_v[0], top_v[1]), (jnp.where(valid, k1, IMIN), jnp.where(valid, k2, IMIN)))
        top_v[0] = k1
        top_v[1] = k2

    def wq_head(g, u):
        return wq_v[g, :, u * DH:(u + 1) * DH]

    def qk(q, hd, k0=0, k1=S):
        return lax.dot_general(q, k_v[hd, k0:k1, :], NT_DIMS, preferred_element_type=F32)

    def probs(s):
        p = jnp.exp2(s - jnp.max(s, axis=-1, keepdims=True)).astype(BF)
        return p, p.astype(F32)

    def pv(s, hd):
        p, pf = probs(s)
        l = jnp.sum(pf, axis=-1, keepdims=True)
        o = jnp.dot(p, v_v[hd], preferred_element_type=F32)
        return (o * _recip(l)).astype(BF), o

    def pv_carry(s, hd):
        p, pf = probs(s)
        lp = pf[:, 0:128]
        for j in range(1, S // 128):
            lp = lp + pf[:, j * 128:(j + 1) * 128]
        of_v[0] = jnp.dot(p, v_v[hd], preferred_element_type=F32)
        of_v[1] = lp

    def carried_o():
        return (of_v[0] * _recip(jnp.sum(of_v[1], axis=-1, keepdims=True))).astype(BF)

    def oproj(o, r0, hd):
        acc_v[pl.ds(r0, RP), :] += jnp.dot(o, wo_v[hd], preferred_element_type=F32)

    start(cp_small())
    start(cp_x(0))
    for i in range(len(CA_CHUNKS)):
        start(cp_ca(i))
    for i in range(len(Q_BATCHES)):
        start(cp_qb(i))
    start(cp_sa())
    start(cp_kv(0))
    for h in range(1, NH0):
        start(cp_head(h))
        if h == 3:
            start(cp_x(1))
    start(cp_wo_last())
    start(cp_x(2))
    start(cp_group(T0))
    acc_v[...] = jnp.zeros_like(acc_v)
    top_v[...] = jnp.full(top_v.shape, IMIN, I32)
    mod_v[...] = jnp.zeros_like(mod_v)

    wait(cp_small())
    c = c_v[...].astype(F32)
    sc = (c * jax.nn.sigmoid(c)).astype(BF)
    scb_v[...] = jnp.broadcast_to(sc, (16, D))
    sc_v[...] = jnp.broadcast_to(sc.astype(F32), (128, D)).T
    hox_v[ZO:ZO + 16, :] = jnp.zeros((16, D), BF)
    wait(cp_x(0))
    _, xc0, rs0 = _center(hox_v[pl.ds(XO, RP), :].astype(F32))
    xn_v[...] = xc0 * rs0

    def matvec(slot, r0, n, c0):
        part_v[slot] = jnp.dot(scb_v[:, r0:r0 + n], wgu_v[pl.ds(r0, n), pl.ds(c0, D)],
                               preferred_element_type=F32)

    for i, (r0, n) in enumerate(CA_CHUNKS):
        wait(cp_ca(i))
        matvec(i, r0, n, D)
    s1 = _rb(1.0 + _rb((part_v[0] + part_v[1] + part_v[2])[0:1]))
    put_mod(S1, s1)

    hs = None
    for i, (h0, n) in enumerate(Q_BATCHES):
        wait(cp_qb(i))
        if i == 0:
            hs = (xn_v[...] * s1).astype(BF)
        if i == len(Q_BATCHES) - 1:
            wait(cp_sa())
            matvec(len(CA_CHUNKS), 0, D, 0)
        for h in range(h0, h0 + n):
            qf_v[h] = jnp.dot(hs, wq_head(h // G, h % G), preferred_element_type=F32) * QSCALE
    sab = part_v[len(CA_CHUNKS)].astype(BF)
    put_mod(SA, sab[0:1].astype(F32))
    for h in range(NH0):
        qb_v[h] = jnp.dot(sab, wq_head(h // G, h % G), preferred_element_type=F32) * QSCALE

    def q_first(h):
        return (qf_v[h] + qb_v[h, 0:1, :]).astype(BF)

    for g in range(T0 + 1, NG):
        start(cp_group(g))
        if g == T0 + 1:
            start(cp_m2())
    wait(cp_kv(0))
    pv_carry(qk(q_first(0), 0), 0)

    wait(cp_head(1))
    q = q_first(1)
    oc = carried_o()
    s_a = qk(q, 1, 0, 512)
    oproj(oc, 0, 0)
    s_b = qk(q, 1, 512, S)
    pv_carry(jnp.concatenate([s_a, s_b], axis=1), 1)

    def double(i, carry):
        h = 2 * i
        wait(cp_head(h))
        wait(cp_head(h + 1))

        @pl.when(i == 1)
        def _():
            wait(cp_x(1))

        def oproj_half(o, c):
            cs = slice(c * (D // 2), (c + 1) * (D // 2))
            acc_v[0:RP, cs] += jnp.dot(o, wo_v[h - 1, :, cs], preferred_element_type=F32)

        q = q_first(h)
        hox_v[QO:QO + RP, 0:DH] = q
        oc = carried_o()
        parts = [qk(q, h, 0, 512)]
        oproj_half(oc, 0)
        parts.append(qk(q, h, 512, 1536))
        rl = RP + jnp.minimum(i - 1, 1) * 64
        for j in range(2):
            ln1(pl.multiple_of(rl + j * 32, 32), 32)
        rh = jnp.minimum((i - 1) * 192, RP - 192)
        for j in range(6):
            r = pl.multiple_of(rh + j * 32, 32)
            hox_v[pl.ds(HO + r, 32), :] = (xn_v[pl.ds(r, 32), :] * mrow(S1, 32) + mrow(SA, 32)).astype(BF)
        parts.append(qk(hox_v[QO:QO + RP, 0:DH], h, 1536, S))
        o0, _ = pv(jnp.concatenate(parts, axis=1), h)
        s = qk(q_first(h + 1), h + 1)
        oproj_half(oc, 1)
        pv_carry(s, h + 1)
        oproj(o0, 0, h)
        return carry

    lax.fori_loop(1, NH0 // 2, double, 0)

    def block(t, carry):
        p = lax.shift_right_logical(t, LNG)
        g = t & (NG - 1)

        @pl.when(jnp.logical_or(t <= NG, g == 1))
        def _():
            @pl.when(t < NG)
            def _():
                wait(cp_group(t))

            @pl.when(t == T0)
            def _():
                wait(cp_wo_last())
                wait(cp_x(2))

            @pl.when(t == TM)
            def _():
                wait(cp_m2())

            @pl.when(t == NG)
            def _():
                m2 = _rb(jnp.concatenate([jnp.sum(mp_v[i], axis=0, keepdims=True) for i in range(4)], axis=1))
                sb = m2[:, D:2 * D]
                s2 = _rb(1.0 + m2[:, 2 * D:3 * D])
                gb = m2[:, 3 * D:4 * D]
                wr = wr_v[...].astype(F32).reshape(1, D)
                put_mod(GA, m2[:, 0:D])
                put_mod(SB, sb)
                put_mod(S2, s2)
                put_mod(GB, gb)
                put_mod(VA, gb * s2)
                put_mod(VB, gb * sb)
                put_mod(VW, s2 * wr)
                put_mod(VC, jnp.broadcast_to(jnp.sum(sb * wr, axis=-1, keepdims=True), (1, D)))
                start(cp_ffn(0))

            @pl.when(t == 2 * NG + 1)
            def _():
                wait(cp_ffn(0))
                start(cp_ffn(1))

            @pl.when(jnp.logical_and(g == 1, p >= 2))
            def _():
                start(cp_out(p - 2))

            @pl.when(t == NT - NG + 1)
            def _():
                wait(cp_ffn(1))

        r0 = pl.multiple_of(p * RP, RP)
        h0 = g * G

        def qproj(u):
            q = jnp.dot(hox_v[pl.ds(HO + r0, RP), :], wq_head(g, u), preferred_element_type=F32)
            return (q * QSCALE).astype(BF)

        def gate(val):
            hox_v[pl.ds(pl.multiple_of(GO + 16 * (t & 1), 16), val.shape[0]), 0:DH] = val.astype(BF)

        def mod_quarter():
            live = jnp.logical_and(t >= TM, t < TM + 4)
            c0 = jnp.where(live, 2 * D + (t - TM) * D, jnp.where(t <= 2 * NG, 0, 4 * D))
            slot = jnp.where(live, t - TM, 4)
            link = hox_v[ZO:ZO + 16, 0:128].astype(F32)[0:8]
            for j in range(D // 128):
                a = link
                wv = wgu_v.at[:, pl.ds(pl.multiple_of(c0, D), D)]
                for k in range(0, D, 8):
                    a = a + wv[k:k + 8, j * 128:(j + 1) * 128].astype(F32) * sc_v[k:k + 8, :]
                mp_v[slot, :, j * 128:(j + 1) * 128] = a
                link = jnp.minimum(jnp.abs(a), 0.0)
            gate(link)

        q0 = qproj(0)
        tp = t - 1
        oproj(carried_o(), pl.multiple_of(lax.shift_right_logical(tp, LNG) * RP, RP), (tp & (NG - 1)) * G + G - 1)
        q1 = qproj(1)
        gate(q1[RP - 16:RP])
        for i in range(SL // PC):
            epi(pl.multiple_of(jnp.maximum(t - NG, 0) * SL + i * PC, PC), PC, t >= NG)
        s = qk(q0, h0)
        q2 = qproj(2)
        o0, raw = pv(s, h0)
        gate(raw[RP - 16:RP])
        for i in range(SL // PC):
            ln1(pl.multiple_of(jnp.minimum(t + NG, S // SL - 1) * SL + i * PC, PC), PC)
        s = qk(q1, h0 + 1)
        q3 = qproj(3)
        o1, _ = pv(s, h0 + 1)
        s = qk(q2, h0 + 2)
        oproj(o0, r0, h0)
        o2, raw = pv(s, h0 + 2)
        gate(raw[RP - 16:RP])
        hox_v[QO:QO + RP, 3 * DH:4 * DH] = q3
        s_a = qk(q3, h0 + 3, 0, 1536)
        mod_quarter()
        s_b = qk(hox_v[QO:QO + RP, 3 * DH:4 * DH], h0 + 3, 1536, S)
        oproj(o1, r0, h0 + 1)
        pv_carry(jnp.concatenate([s_a, s_b], axis=1), h0 + 3)
        oproj(o2, r0, h0 + 2)
        return carry

    lax.fori_loop(T0, NT, block, 0)

    RL = S - RP
    o_last = carried_o()
    pair = (top_v[0], top_v[1])
    start(cp_out(NP - 2))
    for r in range(0, RP, EC):
        a = acc_v[pl.ds(RL + r, EC), :] + jnp.dot(o_last[r:r + EC], wo_v[H - 1], preferred_element_type=F32)
        x2 = resid(RL + r, EC, a)
        xn_v[r:r + EC, :] = x2
        mu, xc, rs = _center(x2)
        put_stats(RL + r, EC, mu, rs)
        pair = _merge(pair, _fold(keys(RL + r, EC, xc, rs)))
        put_out(RL + r, EC, x2, xc, rs)
    start(cp_out(NP - 1))
    for sh in (4, 2, 1):
        pair = _merge(pair, (pltpu.roll(pair[0], sh, 0), pltpu.roll(pair[1], sh, 0)))
    k1, k2 = pair

    def score(k):
        b = jnp.where(k < 0, k ^ 0x7FFFFFFF, k) & (-65536)
        return lax.bitcast_convert_type(b, F32)[0:1, 0:1]

    def row_of(k):
        i = 65535 - (k[0, 0] & 65535)
        return i, pl.multiple_of(jnp.clip(i >> 4, 0, S // 16 - 1) * 16, 16)

    i1, t1 = row_of(k1)
    i2, t2 = row_of(k2)

    def post(t0):
        x2 = resid(t0, 16, acc_v[pl.ds(t0, 16), :])
        tl = pl.multiple_of(jnp.maximum(t0 - RL, 0), 16)
        mu = jnp.concatenate([st_v[0, pl.ds(t0, 16), :]] * (D // 128), axis=1)
        rs = jnp.concatenate([st_v[1, pl.ds(t0, 16), :]] * (D // 128), axis=1)
        x2 = jnp.where(t0 >= RL, xn_v[pl.ds(tl, 16), :], x2)
        return x2, ((x2 - mu) * rs) * mrow(S2, 16) + mrow(SB, 16)

    x2a, h2a = post(t1)
    x2b, h2b = post(t2)
    row = lax.broadcasted_iota(I32, (16, D), 0)
    sel1 = jnp.sum(jnp.where(row == i1 - t1, h2a, 0.0), axis=0, keepdims=True)
    sel2 = jnp.sum(jnp.where(row == i2 - t2, h2b, 0.0), axis=0, keepdims=True)
    row8 = lax.broadcasted_iota(I32, (8, D), 0)
    xs = jnp.where(row8 == 0, sel1, jnp.where(row8 == 1, sel2, 0.0)).astype(BF)

    wait(cp_out(0))
    gt = jnp.dot(xs, wgu_v[:, 0:F], preferred_element_type=F32)
    up = jnp.dot(xs, wgu_v[:, F:2 * F], preferred_element_type=F32)
    act = (gt * jax.nn.sigmoid(gt) * up).astype(BF)
    y = jnp.dot(act, wd_v[:, 0:D], preferred_element_type=F32)
    y1 = y[0:1, :] * jax.nn.sigmoid(score(k1))
    y2 = y[1:2, :] * jax.nn.sigmoid(score(k2))

    def upd(t0):
        return jnp.where(row == i1 - t0, y1, 0.0) + jnp.where(row == i2 - t0, y2, 0.0)

    patch_v[0] = (x2a + mrow(GB, 16) * (h2a + upd(t1))).astype(BF)
    patch_v[1] = (x2b + mrow(GB, 16) * (h2b + upd(t2))).astype(BF)
    for p in range(1, NP):
        wait(cp_out(p))
    pa = cp(patch_v.at[0], out_hbm.at[pl.ds(t1, 16)], SP)
    pb = cp(patch_v.at[1], out_hbm.at[pl.ds(t2, 16)], SP + 1)
    pa.start()

    @pl.when(t1 != t2)
    def _():
        pb.start()
        pb.wait()

    pa.wait()


@jax.jit
def pallas_adaLN_cond__mha_block_cached__moe_arch_mod__prompt_kernel(
    A_x: jax.Array,
    A_k_cache: jax.Array,
    A_v_cache: jax.Array,
    A_wq: jax.Array,
    A_wo: jax.Array,
    B_x: jax.Array,
    B_w_r: jax.Array,
    B_w_gate: jax.Array,
    B_w_up: jax.Array,
    B_w_down: jax.Array,
    c: jax.Array,
    w_mod: jax.Array,
):
    hbm = pl.BlockSpec(memory_space=pl.ANY)
    out = pl.pallas_call(
        _kernel,
        in_specs=[hbm] * 11,
        out_specs=hbm,
        out_shape=jax.ShapeDtypeStruct((S, D), BF),
        scratch_shapes=[
            pltpu.VMEM((H, S, DH), BF),
            pltpu.VMEM((H, S, DH), BF),
            pltpu.VMEM((NG, D, G * DH), BF),
            pltpu.VMEM((H, DH, D), BF),
            pltpu.VMEM((D, 2 * F + 128), BF),
            pltpu.VMEM((F, D + 128), BF),
            pltpu.VMEM((ZO + 16, D), BF),
            pltpu.VMEM((S, D), F32),
            pltpu.VMEM((10, 8, D), F32),
            pltpu.VMEM((2, 8, 128), I32),
            pltpu.VMEM((2, 16, D), BF),
            pltpu.VMEM((2, RP, DH), F32),
            pltpu.VMEM((RP, D), F32),
            pltpu.VMEM((2, S, 128), F32),
            pltpu.VMEM((len(CA_CHUNKS) + 1, 16, D), F32),
            pltpu.VMEM((NH0, RP, DH), F32),
            pltpu.VMEM((NH0, 16, DH), F32),
            pltpu.VMEM((D, 128), F32),
            pltpu.VMEM((16, D), BF),
            pltpu.VMEM((5, 8, D), F32),
            pltpu.VMEM((1, D), BF),
            pltpu.VMEM((D,), BF),
            pltpu.SemaphoreType.DMA((NSEM,)),
        ],
        compiler_params=pltpu.CompilerParams(vmem_limit_bytes=120 << 20, disable_bounds_checks=True,
                                             disable_semaphore_checks=True),
        name="adaln_mha_moe",
    )(A_x.reshape(S, D), A_k_cache.reshape(H, S, DH), A_v_cache.reshape(H, S, DH), A_wq,
      A_wo.reshape(H, DH, D), B_w_r, B_w_gate, B_w_up, B_w_down, c, w_mod)
    return out.reshape(1, S, D)
```

```python
import jax
import jax.numpy as jnp
from jax import lax
import jax.experimental.pallas as pl
import jax.experimental.pallas.tpu as pltpu

S, D, H, DH, F = 2048, 1024, 32, 128, 3584
EPS = 1e-5
QSCALE = DH ** -0.5 * 1.4426950408889634
BF, F32, I32 = jnp.bfloat16, jnp.float32, jnp.int32
IMIN = -2 ** 31
NT_DIMS = (((1,), (1,)), ((), ()))

RP = 512
G = 4
NP, NG = S // RP, H // G
LNG = NG.bit_length() - 1
NT = NP * NG
SL = RP // NG
PC = 16
T0 = 2
NH0 = T0 * G
TM = NG - 4
X1 = RP + T0 * SL
EC = 128
DK = D // 2
CA_CHUNKS = ((0, 768), (768, 256))
Q_BATCHES = ((0, 0, 2), (0, 2, 6), (1, 0, 4), (1, 4, 4))

HO, OO, XO, GO = 0, S, 2 * S, 3 * S
QO = GO + 32
ZO = QO + RP
SA, S1, GA, SB, S2, GB, VA, VB, VW, VC = range(10)
SX = 0
SCA = SX + 3
SCB = SCA + len(CA_CHUNKS)
SV0 = SCB + 1
SSA = SV0 + 1
SM2 = SSA + 1
SQ = SM2 + 1
SH = SQ + len(Q_BATCHES)
SGR = SH + NH0 + 1
SF = SGR + NG
SO = SF + 1
SP = SO + NP
SC = SP + 2
NSEM = SC + 1


def _recip(l):
    ri = pl.reciprocal(l, approx=True)
    return ri * (2.0 - l * ri)


def _rb(a):
    return a.astype(BF).astype(F32)


def _center(x):
    mu = jnp.mean(x, axis=-1, keepdims=True)
    xc = x - mu
    rs = lax.rsqrt(jnp.mean(xc * xc, axis=-1, keepdims=True) + EPS)
    return mu, xc, rs


def _merge(a, b):
    return jnp.maximum(a[0], b[0]), jnp.maximum(jnp.minimum(a[0], b[0]), jnp.maximum(a[1], b[1]))


def _fold(k):
    t = [k[i:i + 8] for i in range(0, k.shape[0], 8)]
    ps = [(jnp.maximum(t[i], t[i + 1]), jnp.minimum(t[i], t[i + 1])) for i in range(0, len(t), 2)]
    while len(ps) > 1:
        ps = [_merge(ps[i], ps[i + 1]) for i in range(0, len(ps), 2)]
    return ps[0]


def _kernel(x_hbm, k_hbm, v_hbm, wq_hbm, wo_hbm, wr_hbm, wg_hbm, wu_hbm, wd_hbm, c_hbm, wm_hbm,
            out_hbm,
            k_v, v_v, wq_v, wo_v, wgu_v, wd_v, hox_v, acc_v, mod_v, top_v, patch_v, of_v, xn_v, st_v,
            part_v, qf_v, qb_v, sc_v, scb_v, mp_v, c_v, wr_v, sems):
    def cp(src, dst, s):
        return pltpu.make_async_copy(src, dst, sems.at[s])

    def cp_x(i):
        r0, n = [(0, RP), (RP, X1 - RP), (X1, S - X1)][i]
        return [cp(x_hbm.at[pl.ds(r0, n)], hox_v.at[pl.ds(XO + r0, n)], SX + i)]

    def cp_wm(r0, n, c0, w, s):
        return [cp(wm_hbm.at[pl.ds(r0, n), pl.ds(c0, w)], wgu_v.at[pl.ds(r0, n), pl.ds(c0, w)], s)]

    def cp_ca(i):
        return cp_wm(*CA_CHUNKS[i], D, DK, SCA + i)

    def cp_cb():
        return cp_wm(0, D, D + DK, DK, SCB)

    def cp_sa():
        return cp_wm(0, D, 0, D, SSA)

    def cp_m2():
        return cp_wm(0, D, 2 * D, 4 * D, SM2)

    def cp_wo(h, n, s):
        return cp(wo_hbm.at[pl.ds(h, n)], wo_v.at[pl.ds(h, n)], s)

    def cp_qb(i):
        half, h0, n = Q_BATCHES[i]
        cuts = sorted({h0, h0 + n} | {b for b in range(0, NH0, G) if h0 < b < h0 + n})
        return [cp(wq_hbm.at[pl.ds(half * DK, DK), pl.ds(a * DH, (b - a) * DH)],
                   wq_v.at[a // G, pl.ds(half * DK, DK), pl.ds((a % G) * DH, (b - a) * DH)], SQ + i)
                for a, b in zip(cuts[:-1], cuts[1:])]

    def cp_k0():
        return [cp(k_hbm.at[0], k_v.at[0], SH)]

    def cp_v0():
        return [cp(v_hbm.at[0], v_v.at[0], SV0)]

    def cp_head(h):
        return [cp_wo(h - 1, 1, SH + h), cp(k_hbm.at[h], k_v.at[h], SH + h), cp(v_hbm.at[h], v_v.at[h], SH + h)]

    def cp_wo_last():
        return [cp_wo(NH0 - 1, 1, SH + NH0)]

    def cp_group(g):
        h0 = g * G
        s = SGR + g
        return [cp(wq_hbm.at[:, pl.ds(pl.multiple_of(h0 * DH, G * DH), G * DH)], wq_v.at[g], s),
                cp(k_hbm.at[pl.ds(h0, G)], k_v.at[pl.ds(h0, G)], s),
                cp(v_hbm.at[pl.ds(h0, G)], v_v.at[pl.ds(h0, G)], s),
                cp_wo(h0, G, s)]

    def cp_ffn(i):
        if i == 0:
            return [cp(wu_hbm, wgu_v.at[:, pl.ds(F, F)], SF), cp(wd_hbm, wd_v.at[:, pl.ds(0, D)], SF)]
        return [cp(wg_hbm, wgu_v.at[:, pl.ds(0, F)], SF)]

    def cp_out(p):
        r0 = pl.multiple_of(p * RP, RP)
        return [cp(hox_v.at[pl.ds(OO + r0, RP)], out_hbm.at[pl.ds(r0, RP)], SO + p)]

    def cp_small():
        return [cp(c_hbm, c_v, SC), cp(wr_hbm, wr_v, SC)]

    def start(cs):
        for c_ in cs:
            c_.start()

    def wait(cs):
        for c_ in cs:
            c_.wait()

    def mrow(i, n):
        return jnp.concatenate([mod_v[i]] * (n // 8), axis=0)

    def put_mod(i, v):
        mod_v[i] = jnp.broadcast_to(v, (8, D))

    def ln1(r0, n):
        _, xc, rs = _center(hox_v[pl.ds(XO + r0, n), :].astype(F32))
        hox_v[pl.ds(HO + r0, n), :] = ((xc * rs) * mrow(S1, n) + mrow(SA, n)).astype(BF)

    def resid(r0, n, a):
        return hox_v[pl.ds(XO + r0, n), :].astype(F32) + mrow(GA, n) * a

    def keys(r0, n, xc, rs):
        r = _rb(rs * jnp.sum(xc * mrow(VW, n), axis=-1, keepdims=True) + mrow(VC, n)[:, 0:128])
        b = lax.bitcast_convert_type(r, I32)
        b = jnp.where(b < 0, b ^ 0x7FFFFFFF, b) & (-65536)
        return b | (65535 - r0 - lax.broadcasted_iota(I32, (n, 128), 0))

    def put_stats(r0, n, mu, rs):
        st_v[0, pl.ds(r0, n), :] = jnp.broadcast_to(mu, (n, 128))
        st_v[1, pl.ds(r0, n), :] = jnp.broadcast_to(rs, (n, 128))

    def put_out(r0, n, x2, xc, rs):
        hox_v[pl.ds(OO + r0, n), :] = (x2 + mrow(VB, n) + (xc * rs) * mrow(VA, n)).astype(BF)

    def epi(r0, n, valid):
        x2 = resid(r0, n, acc_v[pl.ds(r0, n), :])
        mu, xc, rs = _center(x2)
        put_out(r0, n, x2, xc, rs)
        put_stats(r0, n, mu, rs)
        k1, k2 = _fold(keys(r0, n, xc, rs))
        k1, k2 = _merge((top_v[0], top_v[1]), (jnp.where(valid, k1, IMIN), jnp.where(valid, k2, IMIN)))
        top_v[0] = k1
        top_v[1] = k2

    def wq_head(g, u):
        return wq_v[g, :, u * DH:(u + 1) * DH]

    def qk(q, hd, k0=0, k1=S):
        return lax.dot_general(q, k_v[hd, k0:k1, :], NT_DIMS, preferred_element_type=F32)

    def probs(s):
        p = jnp.exp2(s - jnp.max(s, axis=-1, keepdims=True)).astype(BF)
        return p, p.astype(F32)

    def pv(s, hd):
        p, pf = probs(s)
        l = jnp.sum(pf, axis=-1, keepdims=True)
        o = jnp.dot(p, v_v[hd], preferred_element_type=F32)
        return (o * _recip(l)).astype(BF), o

    def pv_carry(s, hd):
        p, pf = probs(s)
        lp = pf[:, 0:128]
        for j in range(1, S // 128):
            lp = lp + pf[:, j * 128:(j + 1) * 128]
        of_v[0] = jnp.dot(p, v_v[hd], preferred_element_type=F32)
        of_v[1] = lp

    def carried_o():
        return (of_v[0] * _recip(jnp.sum(of_v[1], axis=-1, keepdims=True))).astype(BF)

    def oproj(o, r0, hd):
        acc_v[pl.ds(r0, RP), :] += jnp.dot(o, wo_v[hd], preferred_element_type=F32)

    start(cp_small())
    start(cp_x(0))
    for i in range(len(CA_CHUNKS)):
        start(cp_ca(i))
    for i in range(len(Q_BATCHES)):
        if Q_BATCHES[i][:2] == (1, 0):
            start(cp_cb())
        start(cp_qb(i))
    start(cp_sa())
    start(cp_k0())
    start(cp_v0())
    for h in range(1, NH0):
        start(cp_head(h))
        if h == 3:
            start(cp_x(1))
    start(cp_wo_last())
    start(cp_x(2))
    start(cp_group(T0))
    acc_v[...] = jnp.zeros_like(acc_v)
    top_v[...] = jnp.full(top_v.shape, IMIN, I32)
    mod_v[...] = jnp.zeros_like(mod_v)

    wait(cp_small())
    c = c_v[...].astype(F32)
    sc = (c * jax.nn.sigmoid(c)).astype(BF)
    scb_v[...] = jnp.broadcast_to(sc, (16, D))
    sc_v[...] = jnp.broadcast_to(sc.astype(F32), (128, D)).T
    hox_v[ZO:ZO + 16, :] = jnp.zeros((16, D), BF)
    wait(cp_x(0))
    _, xc0, rs0 = _center(hox_v[pl.ds(XO, RP), :].astype(F32))
    xn_v[...] = xc0 * rs0

    def put_s1(half, m):
        s1 = _rb(1.0 + _rb(m[0:1]))
        mod_v[S1, :, half * DK:(half + 1) * DK] = jnp.broadcast_to(s1, (8, DK))
        return s1

    for i, (r0, n) in enumerate(CA_CHUNKS):
        wait(cp_ca(i))
        part_v[i] = jnp.dot(scb_v[:, r0:r0 + n], wgu_v[r0:r0 + n, D:D + DK], preferred_element_type=F32)
    s1 = put_s1(0, part_v[0] + part_v[1])

    hs = None
    for i, (half, h0, n) in enumerate(Q_BATCHES):
        wait(cp_qb(i))
        if (half, h0) == (1, 0):
            wait(cp_cb())
            s1 = put_s1(1, jnp.dot(scb_v[...], wgu_v[:, D + DK:2 * D], preferred_element_type=F32))
        if h0 == 0:
            hs = (xn_v[:, half * DK:(half + 1) * DK] * s1).astype(BF)
        for h in range(h0, h0 + n):
            w = wq_v[h // G, half * DK:(half + 1) * DK, (h % G) * DH:(h % G + 1) * DH]
            if half == 0:
                qf_v[h] = jnp.dot(hs, w, preferred_element_type=F32)
            else:
                qf_v[h] = (qf_v[h] + jnp.dot(hs, w, preferred_element_type=F32)) * QSCALE
    wait(cp_sa())
    sab = jnp.dot(scb_v[...], wgu_v[:, 0:D], preferred_element_type=F32).astype(BF)
    put_mod(SA, sab[0:1].astype(F32))
    for h in range(NH0):
        qb_v[h] = jnp.dot(sab, wq_head(h // G, h % G), preferred_element_type=F32) * QSCALE

    def q_first(h):
        return (qf_v[h] + qb_v[h, 0:1, :]).astype(BF)

    for g in range(T0 + 1, NG):
        start(cp_group(g))
        if g == T0 + 1:
            start(cp_m2())
    wait(cp_k0())
    q = q_first(0)
    s_a = qk(q, 0, 0, 1536)
    wait(cp_v0())
    pv_carry(jnp.concatenate([s_a, qk(q, 0, 1536, S)], axis=1), 0)

    wait(cp_head(1))
    q = q_first(1)
    oc = carried_o()
    s_a = qk(q, 1, 0, 512)
    oproj(oc, 0, 0)
    s_b = qk(q, 1, 512, S)
    pv_carry(jnp.concatenate([s_a, s_b], axis=1), 1)

    def double(i, carry):
        h = 2 * i
        wait(cp_head(h))
        wait(cp_head(h + 1))

        @pl.when(i == 1)
        def _():
            wait(cp_x(1))

        def oproj_half(o, c):
            cs = slice(c * (D // 2), (c + 1) * (D // 2))
            acc_v[0:RP, cs] += jnp.dot(o, wo_v[h - 1, :, cs], preferred_element_type=F32)

        q = q_first(h)
        hox_v[QO:QO + RP, 0:DH] = q
        oc = carried_o()
        parts = [qk(q, h, 0, 512)]
        oproj_half(oc, 0)
        parts.append(qk(q, h, 512, 1536))
        rl = RP + jnp.minimum(i - 1, 1) * 64
        for j in range(2):
            ln1(pl.multiple_of(rl + j * 32, 32), 32)
        rh = jnp.minimum((i - 1) * 192, RP - 192)
        for j in range(6):
            r = pl.multiple_of(rh + j * 32, 32)
            hox_v[pl.ds(HO + r, 32), :] = (xn_v[pl.ds(r, 32), :] * mrow(S1, 32) + mrow(SA, 32)).astype(BF)
        parts.append(qk(hox_v[QO:QO + RP, 0:DH], h, 1536, S))
        o0, _ = pv(jnp.concatenate(parts, axis=1), h)
        s = qk(q_first(h + 1), h + 1)
        oproj_half(oc, 1)
        pv_carry(s, h + 1)
        oproj(o0, 0, h)
        return carry

    lax.fori_loop(1, NH0 // 2, double, 0)

    def block(t, carry):
        p = lax.shift_right_logical(t, LNG)
        g = t & (NG - 1)

        @pl.when(jnp.logical_or(t <= NG, g == 1))
        def _():
            @pl.when(t < NG)
            def _():
                wait(cp_group(t))

            @pl.when(t == T0)
            def _():
                wait(cp_wo_last())
                wait(cp_x(2))

            @pl.when(t == TM)
            def _():
                wait(cp_m2())

            @pl.when(t == NG)
            def _():
                m2 = _rb(jnp.concatenate([jnp.sum(mp_v[i], axis=0, keepdims=True) for i in range(4)], axis=1))
                sb = m2[:, D:2 * D]
                s2 = _rb(1.0 + m2[:, 2 * D:3 * D])
                gb = m2[:, 3 * D:4 * D]
                wr = wr_v[...].astype(F32).reshape(1, D)
                put_mod(GA, m2[:, 0:D])
                put_mod(SB, sb)
                put_mod(S2, s2)
                put_mod(GB, gb)
                put_mod(VA, gb * s2)
                put_mod(VB, gb * sb)
                put_mod(VW, s2 * wr)
                put_mod(VC, jnp.broadcast_to(jnp.sum(sb * wr, axis=-1, keepdims=True), (1, D)))
                start(cp_ffn(0))

            @pl.when(t == 2 * NG + 1)
            def _():
                wait(cp_ffn(0))
                start(cp_ffn(1))

            @pl.when(jnp.logical_and(g == 1, p >= 2))
            def _():
                start(cp_out(p - 2))

            @pl.when(t == NT - NG + 1)
            def _():
                wait(cp_ffn(1))

        r0 = pl.multiple_of(p * RP, RP)
        h0 = g * G

        def qproj(u):
            q = jnp.dot(hox_v[pl.ds(HO + r0, RP), :], wq_head(g, u), preferred_element_type=F32)
            return (q * QSCALE).astype(BF)

        def gate(val):
            hox_v[pl.ds(pl.multiple_of(GO + 16 * (t & 1), 16), val.shape[0]), 0:DH] = val.astype(BF)

        def mod_quarter():
            live = jnp.logical_and(t >= TM, t < TM + 4)
            c0 = jnp.where(live, 2 * D + (t - TM) * D, jnp.where(t <= 2 * NG, 0, 4 * D))
            slot = jnp.where(live, t - TM, 4)
            link = hox_v[ZO:ZO + 16, 0:128].astype(F32)[0:8]
            for j in range(D // 128):
                a = link
                wv = wgu_v.at[:, pl.ds(pl.multiple_of(c0, D), D)]
                for k in range(0, D, 8):
                    a = a + wv[k:k + 8, j * 128:(j + 1) * 128].astype(F32) * sc_v[k:k + 8, :]
                mp_v[slot, :, j * 128:(j + 1) * 128] = a
                link = jnp.minimum(jnp.abs(a), 0.0)
            gate(link)

        q0 = qproj(0)
        tp = t - 1
        oproj(carried_o(), pl.multiple_of(lax.shift_right_logical(tp, LNG) * RP, RP), (tp & (NG - 1)) * G + G - 1)
        q1 = qproj(1)
        gate(q1[RP - 16:RP])
        for i in range(SL // PC):
            epi(pl.multiple_of(jnp.maximum(t - NG, 0) * SL + i * PC, PC), PC, t >= NG)
        s = qk(q0, h0)
        q2 = qproj(2)
        o0, raw = pv(s, h0)
        gate(raw[RP - 16:RP])
        for i in range(SL // PC):
            ln1(pl.multiple_of(jnp.minimum(t + NG, S // SL - 1) * SL + i * PC, PC), PC)
        s = qk(q1, h0 + 1)
        q3 = qproj(3)
        o1, _ = pv(s, h0 + 1)
        s = qk(q2, h0 + 2)
        oproj(o0, r0, h0)
        o2, raw = pv(s, h0 + 2)
        gate(raw[RP - 16:RP])
        hox_v[QO:QO + RP, 3 * DH:4 * DH] = q3
        s_a = qk(q3, h0 + 3, 0, 1536)
        mod_quarter()
        s_b = qk(hox_v[QO:QO + RP, 3 * DH:4 * DH], h0 + 3, 1536, S)
        oproj(o1, r0, h0 + 1)
        pv_carry(jnp.concatenate([s_a, s_b], axis=1), h0 + 3)
        oproj(o2, r0, h0 + 2)
        return carry

    lax.fori_loop(T0, NT, block, 0)

    RL = S - RP
    o_last = carried_o()
    pair = (top_v[0], top_v[1])
    start(cp_out(NP - 2))
    for r in range(0, RP, EC):
        a = acc_v[pl.ds(RL + r, EC), :] + jnp.dot(o_last[r:r + EC], wo_v[H - 1], preferred_element_type=F32)
        x2 = resid(RL + r, EC, a)
        xn_v[r:r + EC, :] = x2
        mu, xc, rs = _center(x2)
        put_stats(RL + r, EC, mu, rs)
        pair = _merge(pair, _fold(keys(RL + r, EC, xc, rs)))
        put_out(RL + r, EC, x2, xc, rs)
    start(cp_out(NP - 1))
    for sh in (4, 2, 1):
        pair = _merge(pair, (pltpu.roll(pair[0], sh, 0), pltpu.roll(pair[1], sh, 0)))
    k1, k2 = pair

    def score(k):
        b = jnp.where(k < 0, k ^ 0x7FFFFFFF, k) & (-65536)
        return lax.bitcast_convert_type(b, F32)[0:1, 0:1]

    def row_of(k):
        i = 65535 - (k[0, 0] & 65535)
        return i, pl.multiple_of(jnp.clip(i >> 4, 0, S // 16 - 1) * 16, 16)

    i1, t1 = row_of(k1)
    i2, t2 = row_of(k2)

    def post(t0):
        x2 = resid(t0, 16, acc_v[pl.ds(t0, 16), :])
        tl = pl.multiple_of(jnp.maximum(t0 - RL, 0), 16)
        mu = jnp.concatenate([st_v[0, pl.ds(t0, 16), :]] * (D // 128), axis=1)
        rs = jnp.concatenate([st_v[1, pl.ds(t0, 16), :]] * (D // 128), axis=1)
        x2 = jnp.where(t0 >= RL, xn_v[pl.ds(tl, 16), :], x2)
        return x2, ((x2 - mu) * rs) * mrow(S2, 16) + mrow(SB, 16)

    x2a, h2a = post(t1)
    x2b, h2b = post(t2)
    row = lax.broadcasted_iota(I32, (16, D), 0)
    sel1 = jnp.sum(jnp.where(row == i1 - t1, h2a, 0.0), axis=0, keepdims=True)
    sel2 = jnp.sum(jnp.where(row == i2 - t2, h2b, 0.0), axis=0, keepdims=True)
    row8 = lax.broadcasted_iota(I32, (8, D), 0)
    xs = jnp.where(row8 == 0, sel1, jnp.where(row8 == 1, sel2, 0.0)).astype(BF)

    wait(cp_out(0))
    gt = jnp.dot(xs, wgu_v[:, 0:F], preferred_element_type=F32)
    up = jnp.dot(xs, wgu_v[:, F:2 * F], preferred_element_type=F32)
    act = (gt * jax.nn.sigmoid(gt) * up).astype(BF)
    y = jnp.dot(act, wd_v[:, 0:D], preferred_element_type=F32)
    y1 = y[0:1, :] * jax.nn.sigmoid(score(k1))
    y2 = y[1:2, :] * jax.nn.sigmoid(score(k2))

    def upd(t0):
        return jnp.where(row == i1 - t0, y1, 0.0) + jnp.where(row == i2 - t0, y2, 0.0)

    patch_v[0] = (x2a + mrow(GB, 16) * (h2a + upd(t1))).astype(BF)
    patch_v[1] = (x2b + mrow(GB, 16) * (h2b + upd(t2))).astype(BF)
    for p in range(1, NP):
        wait(cp_out(p))
    pa = cp(patch_v.at[0], out_hbm.at[pl.ds(t1, 16)], SP)
    pb = cp(patch_v.at[1], out_hbm.at[pl.ds(t2, 16)], SP + 1)
    pa.start()

    @pl.when(t1 != t2)
    def _():
        pb.start()
        pb.wait()

    pa.wait()


@jax.jit
def pallas_adaLN_cond__mha_block_cached__moe_arch_mod__prompt_kernel(
    A_x: jax.Array,
    A_k_cache: jax.Array,
    A_v_cache: jax.Array,
    A_wq: jax.Array,
    A_wo: jax.Array,
    B_x: jax.Array,
    B_w_r: jax.Array,
    B_w_gate: jax.Array,
    B_w_up: jax.Array,
    B_w_down: jax.Array,
    c: jax.Array,
    w_mod: jax.Array,
):
    hbm = pl.BlockSpec(memory_space=pl.ANY)
    out = pl.pallas_call(
        _kernel,
        in_specs=[hbm] * 11,
        out_specs=hbm,
        out_shape=jax.ShapeDtypeStruct((S, D), BF),
        scratch_shapes=[
            pltpu.VMEM((H, S, DH), BF),
            pltpu.VMEM((H, S, DH), BF),
            pltpu.VMEM((NG, D, G * DH), BF),
            pltpu.VMEM((H, DH, D), BF),
            pltpu.VMEM((D, 2 * F + 128), BF),
            pltpu.VMEM((F, D + 128), BF),
            pltpu.VMEM((ZO + 16, D), BF),
            pltpu.VMEM((S, D), F32),
            pltpu.VMEM((10, 8, D), F32),
            pltpu.VMEM((2, 8, 128), I32),
            pltpu.VMEM((2, 16, D), BF),
            pltpu.VMEM((2, RP, DH), F32),
            pltpu.VMEM((RP, D), F32),
            pltpu.VMEM((2, S, 128), F32),
            pltpu.VMEM((len(CA_CHUNKS), 16, DK), F32),
            pltpu.VMEM((NH0, RP, DH), F32),
            pltpu.VMEM((NH0, 16, DH), F32),
            pltpu.VMEM((D, 128), F32),
            pltpu.VMEM((16, D), BF),
            pltpu.VMEM((5, 8, D), F32),
            pltpu.VMEM((1, D), BF),
            pltpu.VMEM((D,), BF),
            pltpu.SemaphoreType.DMA((NSEM,)),
        ],
        compiler_params=pltpu.CompilerParams(vmem_limit_bytes=120 << 20, disable_bounds_checks=True,
                                             disable_semaphore_checks=True),
        name="adaln_mha_moe",
    )(A_x.reshape(S, D), A_k_cache.reshape(H, S, DH), A_v_cache.reshape(H, S, DH), A_wq,
      A_wo.reshape(H, DH, D), B_w_r, B_w_gate, B_w_up, B_w_down, c, w_mod)
    return out.reshape(1, S, D)
```

```python
import jax
import jax.numpy as jnp
from jax import lax
import jax.experimental.pallas as pl
import jax.experimental.pallas.tpu as pltpu

S, D, H, DH, F = 2048, 1024, 32, 128, 3584
EPS = 1e-5
QSCALE = DH ** -0.5 * 1.4426950408889634
BF, F32, I32 = jnp.bfloat16, jnp.float32, jnp.int32
IMIN = -2 ** 31
NT_DIMS = (((1,), (1,)), ((), ()))

RP = 512
G = 4
NP, NG = S // RP, H // G
LNG = NG.bit_length() - 1
NT = NP * NG
SL = RP // NG
PC = 16
T0 = 2
NH0 = T0 * G
TM = NG - 4
X1 = RP + T0 * SL
EC = 128
DK = D // 2
CA_CHUNKS = ((0, 768), (768, 256))
Q_BATCHES = ((0, 0, 2), (0, 2, 6), (1, 0, 4), (1, 4, 4))

HO, OO, XO, GO = 0, S, 2 * S, 3 * S
QO = GO + 32
ZO = QO + RP
SA, S1, GA, SB, S2, GB, VA, VB, VW, VC = range(10)
SX = 0
SCA = SX + 3
SCB = SCA + len(CA_CHUNKS)
SV0 = SCB + 1
SSA = SV0 + 1
SM2 = SSA + 1
SQ = SM2 + 1
SH = SQ + len(Q_BATCHES)
SGR = SH + NH0 + 1
SF = SGR + NG
SO = SF + 1
SP = SO + NP
SC = SP + 2
NSEM = SC + 1


def _recip(l):
    ri = pl.reciprocal(l, approx=True)
    return ri * (2.0 - l * ri)


def _rb(a):
    return a.astype(BF).astype(F32)


def _center(x):
    mu = jnp.mean(x, axis=-1, keepdims=True)
    xc = x - mu
    rs = lax.rsqrt(jnp.mean(xc * xc, axis=-1, keepdims=True) + EPS)
    return mu, xc, rs


def _merge(a, b):
    return jnp.maximum(a[0], b[0]), jnp.maximum(jnp.minimum(a[0], b[0]), jnp.maximum(a[1], b[1]))


def _fold(k):
    t = [k[i:i + 8] for i in range(0, k.shape[0], 8)]
    ps = [(jnp.maximum(t[i], t[i + 1]), jnp.minimum(t[i], t[i + 1])) for i in range(0, len(t), 2)]
    while len(ps) > 1:
        ps = [_merge(ps[i], ps[i + 1]) for i in range(0, len(ps), 2)]
    return ps[0]


def _kernel(x_hbm, k_hbm, v_hbm, wq_hbm, wo_hbm, wr_hbm, wg_hbm, wu_hbm, wd_hbm, c_hbm, wm_hbm,
            out_hbm,
            k_v, v_v, wq_v, wo_v, wgu_v, wd_v, hox_v, acc_v, mod_v, top_v, patch_v, of_v, xn_v, st_v,
            part_v, qf_v, qb_v, sc_v, scb_v, mp_v, c_v, wr_v, sems):
    def cp(src, dst, s):
        return pltpu.make_async_copy(src, dst, sems.at[s])

    def cp_x(i):
        r0, n = [(0, RP), (RP, X1 - RP), (X1, S - X1)][i]
        return [cp(x_hbm.at[pl.ds(r0, n)], hox_v.at[pl.ds(XO + r0, n)], SX + i)]

    def cp_wm(r0, n, c0, w, s):
        return [cp(wm_hbm.at[pl.ds(r0, n), pl.ds(c0, w)], wgu_v.at[pl.ds(r0, n), pl.ds(c0, w)], s)]

    def cp_ca(i):
        return cp_wm(*CA_CHUNKS[i], D, DK, SCA + i)

    def cp_cb():
        return cp_wm(0, D, D + DK, DK, SCB)

    def cp_sa():
        return cp_wm(0, D, 0, D, SSA)

    def cp_m2():
        return cp_wm(0, D, 2 * D, 4 * D, SM2)

    def cp_wo(h, n, s):
        return cp(wo_hbm.at[pl.ds(h, n)], wo_v.at[pl.ds(h, n)], s)

    def cp_qb(i):
        half, h0, n = Q_BATCHES[i]
        cuts = sorted({h0, h0 + n} | {b for b in range(0, NH0, G) if h0 < b < h0 + n})
        return [cp(wq_hbm.at[pl.ds(half * DK, DK), pl.ds(a * DH, (b - a) * DH)],
                   wq_v.at[a // G, pl.ds(half * DK, DK), pl.ds((a % G) * DH, (b - a) * DH)], SQ + i)
                for a, b in zip(cuts[:-1], cuts[1:])]

    def cp_k0():
        return [cp(k_hbm.at[0], k_v.at[0], SH)]

    def cp_v0():
        return [cp(v_hbm.at[0], v_v.at[0], SV0)]

    def cp_head(h):
        return [cp_wo(h - 1, 1, SH + h), cp(k_hbm.at[h], k_v.at[h], SH + h), cp(v_hbm.at[h], v_v.at[h], SH + h)]

    def cp_wo_last():
        return [cp_wo(NH0 - 1, 1, SH + NH0)]

    def cp_group(g):
        h0 = g * G
        s = SGR + g
        return [cp(wq_hbm.at[:, pl.ds(pl.multiple_of(h0 * DH, G * DH), G * DH)], wq_v.at[g], s),
                cp(k_hbm.at[pl.ds(h0, G)], k_v.at[pl.ds(h0, G)], s),
                cp(v_hbm.at[pl.ds(h0, G)], v_v.at[pl.ds(h0, G)], s),
                cp_wo(h0, G, s)]

    def cp_ffn(i):
        if i == 0:
            return [cp(wu_hbm, wgu_v.at[:, pl.ds(F, F)], SF), cp(wd_hbm, wd_v.at[:, pl.ds(0, D)], SF)]
        return [cp(wg_hbm, wgu_v.at[:, pl.ds(0, F)], SF)]

    def cp_out(p):
        r0 = pl.multiple_of(p * RP, RP)
        return [cp(hox_v.at[pl.ds(OO + r0, RP)], out_hbm.at[pl.ds(r0, RP)], SO + p)]

    def cp_small():
        return [cp(c_hbm, c_v, SC), cp(wr_hbm, wr_v, SC)]

    def start(cs):
        for c_ in cs:
            c_.start()

    def wait(cs):
        for c_ in cs:
            c_.wait()

    def mrow(i, n):
        return jnp.concatenate([mod_v[i]] * (n // 8), axis=0)

    def put_mod(i, v):
        mod_v[i] = jnp.broadcast_to(v, (8, D))

    def ln1(r0, n):
        _, xc, rs = _center(hox_v[pl.ds(XO + r0, n), :].astype(F32))
        hox_v[pl.ds(HO + r0, n), :] = ((xc * rs) * mrow(S1, n) + mrow(SA, n)).astype(BF)

    def resid(r0, n, a):
        return hox_v[pl.ds(XO + r0, n), :].astype(F32) + mrow(GA, n) * a

    def keys(r0, n, xc, rs):
        r = _rb(rs * jnp.sum(xc * mrow(VW, n), axis=-1, keepdims=True) + mrow(VC, n)[:, 0:128])
        b = lax.bitcast_convert_type(r, I32)
        b = jnp.where(b < 0, b ^ 0x7FFFFFFF, b) & (-65536)
        return b | (65535 - r0 - lax.broadcasted_iota(I32, (n, 128), 0))

    def put_stats(r0, n, mu, rs):
        st_v[0, pl.ds(r0, n), :] = jnp.broadcast_to(mu, (n, 128))
        st_v[1, pl.ds(r0, n), :] = jnp.broadcast_to(rs, (n, 128))

    def put_out(r0, n, x2, xc, rs):
        hox_v[pl.ds(OO + r0, n), :] = (x2 + mrow(VB, n) + (xc * rs) * mrow(VA, n)).astype(BF)

    def epi(r0, n, valid):
        x2 = resid(r0, n, acc_v[pl.ds(r0, n), :])
        mu, xc, rs = _center(x2)
        put_out(r0, n, x2, xc, rs)
        put_stats(r0, n, mu, rs)
        k1, k2 = _fold(keys(r0, n, xc, rs))
        k1, k2 = _merge((top_v[0], top_v[1]), (jnp.where(valid, k1, IMIN), jnp.where(valid, k2, IMIN)))
        top_v[0] = k1
        top_v[1] = k2

    def wq_head(g, u):
        return wq_v[g, :, u * DH:(u + 1) * DH]

    def qk(q, hd, k0=0, k1=S):
        return lax.dot_general(q, k_v[hd, k0:k1, :], NT_DIMS, preferred_element_type=F32)

    def probs(s):
        p = jnp.exp2(s - jnp.max(s, axis=-1, keepdims=True)).astype(BF)
        return p, p.astype(F32)

    def pv(s, hd):
        p, pf = probs(s)
        l = jnp.sum(pf, axis=-1, keepdims=True)
        o = jnp.dot(p, v_v[hd], preferred_element_type=F32)
        return (o * _recip(l)).astype(BF)

    def pv_carry(s, hd):
        p, pf = probs(s)
        lp = pf[:, 0:128]
        for j in range(1, S // 128):
            lp = lp + pf[:, j * 128:(j + 1) * 128]
        of_v[0] = jnp.dot(p, v_v[hd], preferred_element_type=F32)
        of_v[1] = lp

    def carried_o():
        return (of_v[0] * _recip(jnp.sum(of_v[1], axis=-1, keepdims=True))).astype(BF)

    def oproj(o, r0, hd):
        acc_v[pl.ds(r0, RP), :] += jnp.dot(o, wo_v[hd], preferred_element_type=F32)

    start(cp_small())
    start(cp_x(0))
    for i in range(len(CA_CHUNKS)):
        start(cp_ca(i))
    for i in range(len(Q_BATCHES)):
        if Q_BATCHES[i][:2] == (1, 0):
            start(cp_cb())
        start(cp_qb(i))
    start(cp_sa())
    start(cp_k0())
    start(cp_v0())
    for h in range(1, NH0):
        start(cp_head(h))
        if h == 3:
            start(cp_x(1))
    start(cp_wo_last())
    start(cp_x(2))
    start(cp_group(T0))
    acc_v[...] = jnp.zeros_like(acc_v)
    top_v[...] = jnp.full(top_v.shape, IMIN, I32)
    mod_v[...] = jnp.zeros_like(mod_v)

    wait(cp_small())
    c = c_v[...].astype(F32)
    sc = (c * jax.nn.sigmoid(c)).astype(BF)
    scb_v[...] = jnp.broadcast_to(sc, (16, D))
    sc_v[...] = jnp.broadcast_to(sc.astype(F32), (128, D)).T
    hox_v[ZO:ZO + 16, :] = jnp.zeros((16, D), BF)
    wait(cp_x(0))
    _, xc0, rs0 = _center(hox_v[pl.ds(XO, RP), :].astype(F32))
    xn_v[...] = xc0 * rs0

    def put_s1(half, m):
        s1 = _rb(1.0 + _rb(m[0:1]))
        mod_v[S1, :, half * DK:(half + 1) * DK] = jnp.broadcast_to(s1, (8, DK))
        return s1

    for i, (r0, n) in enumerate(CA_CHUNKS):
        wait(cp_ca(i))
        part_v[i] = jnp.dot(scb_v[:, r0:r0 + n], wgu_v[r0:r0 + n, D:D + DK], preferred_element_type=F32)
    s1 = put_s1(0, part_v[0] + part_v[1])

    hs = None
    for i, (half, h0, n) in enumerate(Q_BATCHES):
        wait(cp_qb(i))
        if (half, h0) == (1, 0):
            wait(cp_cb())
            s1 = put_s1(1, jnp.dot(scb_v[...], wgu_v[:, D + DK:2 * D], preferred_element_type=F32))
        if h0 == 0:
            hs = (xn_v[:, half * DK:(half + 1) * DK] * s1).astype(BF)
        for h in range(h0, h0 + n):
            w = wq_v[h // G, half * DK:(half + 1) * DK, (h % G) * DH:(h % G + 1) * DH]
            if half == 0:
                qf_v[h] = jnp.dot(hs, w, preferred_element_type=F32)
            else:
                qf_v[h] = (qf_v[h] + jnp.dot(hs, w, preferred_element_type=F32)) * QSCALE
    wait(cp_sa())
    sab = jnp.dot(scb_v[...], wgu_v[:, 0:D], preferred_element_type=F32).astype(BF)
    put_mod(SA, sab[0:1].astype(F32))
    for h in range(NH0):
        qb_v[h] = jnp.dot(sab, wq_head(h // G, h % G), preferred_element_type=F32) * QSCALE

    def q_first(h):
        return (qf_v[h] + qb_v[h, 0:1, :]).astype(BF)

    for g in range(T0 + 1, NG):
        start(cp_group(g))
        if g == T0 + 1:
            start(cp_m2())
    wait(cp_k0())
    q = q_first(0)
    s_a = qk(q, 0, 0, 1536)
    wait(cp_v0())
    pv_carry(jnp.concatenate([s_a, qk(q, 0, 1536, S)], axis=1), 0)

    wait(cp_head(1))
    q = q_first(1)
    oc = carried_o()
    s_a = qk(q, 1, 0, 512)
    oproj(oc, 0, 0)
    s_b = qk(q, 1, 512, S)
    pv_carry(jnp.concatenate([s_a, s_b], axis=1), 1)

    def double(i, carry):
        h = 2 * i
        wait(cp_head(h))
        wait(cp_head(h + 1))

        @pl.when(i == 1)
        def _():
            wait(cp_x(1))

        def oproj_half(o, c):
            cs = slice(c * (D // 2), (c + 1) * (D // 2))
            acc_v[0:RP, cs] += jnp.dot(o, wo_v[h - 1, :, cs], preferred_element_type=F32)

        q = q_first(h)
        hox_v[QO:QO + RP, 0:DH] = q
        oc = carried_o()
        parts = [qk(q, h, 0, 512)]
        oproj_half(oc, 0)
        parts.append(qk(q, h, 512, 1536))
        rl = RP + jnp.minimum(i - 1, 1) * 64
        for j in range(2):
            ln1(pl.multiple_of(rl + j * 32, 32), 32)
        rh = jnp.minimum((i - 1) * 192, RP - 192)
        for j in range(6):
            r = pl.multiple_of(rh + j * 32, 32)
            hox_v[pl.ds(HO + r, 32), :] = (xn_v[pl.ds(r, 32), :] * mrow(S1, 32) + mrow(SA, 32)).astype(BF)
        parts.append(qk(hox_v[QO:QO + RP, 0:DH], h, 1536, S))
        o0 = pv(jnp.concatenate(parts, axis=1), h)
        s = qk(q_first(h + 1), h + 1)
        oproj_half(oc, 1)
        pv_carry(s, h + 1)
        oproj(o0, 0, h)
        return carry

    lax.fori_loop(1, NH0 // 2, double, 0)

    def block(t, carry):
        p = lax.shift_right_logical(t, LNG)
        g = t & (NG - 1)

        @pl.when(jnp.logical_or(t <= NG, g == 1))
        def _():
            @pl.when(t < NG)
            def _():
                wait(cp_group(t))

            @pl.when(t == T0)
            def _():
                wait(cp_wo_last())
                wait(cp_x(2))

            @pl.when(t == TM)
            def _():
                wait(cp_m2())

            @pl.when(t == NG)
            def _():
                m2 = _rb(jnp.concatenate([jnp.sum(mp_v[i], axis=0, keepdims=True) for i in range(4)], axis=1))
                sb = m2[:, D:2 * D]
                s2 = _rb(1.0 + m2[:, 2 * D:3 * D])
                gb = m2[:, 3 * D:4 * D]
                wr = wr_v[...].astype(F32).reshape(1, D)
                put_mod(GA, m2[:, 0:D])
                put_mod(SB, sb)
                put_mod(S2, s2)
                put_mod(GB, gb)
                put_mod(VA, gb * s2)
                put_mod(VB, gb * sb)
                put_mod(VW, s2 * wr)
                put_mod(VC, jnp.broadcast_to(jnp.sum(sb * wr, axis=-1, keepdims=True), (1, D)))
                start(cp_ffn(0))

            @pl.when(t == 2 * NG + 1)
            def _():
                wait(cp_ffn(0))
                start(cp_ffn(1))

            @pl.when(jnp.logical_and(g == 1, p >= 2))
            def _():
                start(cp_out(p - 2))

            @pl.when(t == NT - NG + 1)
            def _():
                wait(cp_ffn(1))

        r0 = pl.multiple_of(p * RP, RP)
        h0 = g * G

        def qproj(u):
            q = jnp.dot(hox_v[pl.ds(HO + r0, RP), :], wq_head(g, u), preferred_element_type=F32)
            return (q * QSCALE).astype(BF)

        def mod_quarter():
            live = jnp.logical_and(t >= TM, t < TM + 4)
            c0 = jnp.where(live, 2 * D + (t - TM) * D, jnp.where(t <= 2 * NG, 0, 4 * D))
            slot = jnp.where(live, t - TM, 4)
            link = hox_v[ZO:ZO + 16, 0:128].astype(F32)[0:8]
            for j in range(D // 128):
                a = link
                wv = wgu_v.at[:, pl.ds(pl.multiple_of(c0, D), D)]
                for k in range(0, D, 8):
                    a = a + wv[k:k + 8, j * 128:(j + 1) * 128].astype(F32) * sc_v[k:k + 8, :]
                mp_v[slot, :, j * 128:(j + 1) * 128] = a
                link = jnp.minimum(jnp.abs(a), 0.0)
            hox_v[pl.ds(pl.multiple_of(GO + 16 * (t & 1), 16), 8), 0:DH] = link.astype(BF)

        q0 = qproj(0)
        q1 = qproj(1)
        for i in range(SL // PC):
            ln1(pl.multiple_of(jnp.minimum(t + NG, S // SL - 1) * SL + i * PC, PC), PC)
        tp = t - 1
        oproj(carried_o(), pl.multiple_of(lax.shift_right_logical(tp, LNG) * RP, RP), (tp & (NG - 1)) * G + G - 1)
        for i in range(SL // PC):
            epi(pl.multiple_of(jnp.maximum(t - NG, 0) * SL + i * PC, PC), PC, t >= NG)
        s = qk(q0, h0)
        q2 = qproj(2)
        o0 = pv(s, h0)
        mod_quarter()
        s = jnp.concatenate([qk(q1[0:RP // 2], h0 + 1), qk(q1[RP // 2:RP], h0 + 1)], axis=0)
        q3 = qproj(3)
        o1 = pv(s, h0 + 1)
        s = qk(q2, h0 + 2)
        oproj(o0, r0, h0)
        o2 = pv(s, h0 + 2)
        s = qk(q3, h0 + 3)
        oproj(o1, r0, h0 + 1)
        pv_carry(s, h0 + 3)
        oproj(o2, r0, h0 + 2)
        return carry

    lax.fori_loop(T0, NT, block, 0)

    RL = S - RP
    o_last = carried_o()
    pair = (top_v[0], top_v[1])
    start(cp_out(NP - 2))
    for r in range(0, RP, EC):
        a = acc_v[pl.ds(RL + r, EC), :] + jnp.dot(o_last[r:r + EC], wo_v[H - 1], preferred_element_type=F32)
        x2 = resid(RL + r, EC, a)
        xn_v[r:r + EC, :] = x2
        mu, xc, rs = _center(x2)
        put_stats(RL + r, EC, mu, rs)
        pair = _merge(pair, _fold(keys(RL + r, EC, xc, rs)))
        put_out(RL + r, EC, x2, xc, rs)
    start(cp_out(NP - 1))
    for sh in (4, 2, 1):
        pair = _merge(pair, (pltpu.roll(pair[0], sh, 0), pltpu.roll(pair[1], sh, 0)))
    k1, k2 = pair

    def score(k):
        b = jnp.where(k < 0, k ^ 0x7FFFFFFF, k) & (-65536)
        return lax.bitcast_convert_type(b, F32)[0:1, 0:1]

    def row_of(k):
        i = 65535 - (k[0, 0] & 65535)
        return i, pl.multiple_of(jnp.clip(i >> 4, 0, S // 16 - 1) * 16, 16)

    i1, t1 = row_of(k1)
    i2, t2 = row_of(k2)

    def post(t0):
        x2 = resid(t0, 16, acc_v[pl.ds(t0, 16), :])
        tl = pl.multiple_of(jnp.maximum(t0 - RL, 0), 16)
        mu = jnp.concatenate([st_v[0, pl.ds(t0, 16), :]] * (D // 128), axis=1)
        rs = jnp.concatenate([st_v[1, pl.ds(t0, 16), :]] * (D // 128), axis=1)
        x2 = jnp.where(t0 >= RL, xn_v[pl.ds(tl, 16), :], x2)
        return x2, ((x2 - mu) * rs) * mrow(S2, 16) + mrow(SB, 16)

    x2a, h2a = post(t1)
    x2b, h2b = post(t2)
    row = lax.broadcasted_iota(I32, (16, D), 0)
    sel1 = jnp.sum(jnp.where(row == i1 - t1, h2a, 0.0), axis=0, keepdims=True)
    sel2 = jnp.sum(jnp.where(row == i2 - t2, h2b, 0.0), axis=0, keepdims=True)
    row8 = lax.broadcasted_iota(I32, (8, D), 0)
    xs = jnp.where(row8 == 0, sel1, jnp.where(row8 == 1, sel2, 0.0)).astype(BF)

    wait(cp_out(0))
    gt = jnp.dot(xs, wgu_v[:, 0:F], preferred_element_type=F32)
    up = jnp.dot(xs, wgu_v[:, F:2 * F], preferred_element_type=F32)
    act = (gt * jax.nn.sigmoid(gt) * up).astype(BF)
    y = jnp.dot(act, wd_v[:, 0:D], preferred_element_type=F32)
    y1 = y[0:1, :] * jax.nn.sigmoid(score(k1))
    y2 = y[1:2, :] * jax.nn.sigmoid(score(k2))

    def upd(t0):
        return jnp.where(row == i1 - t0, y1, 0.0) + jnp.where(row == i2 - t0, y2, 0.0)

    patch_v[0] = (x2a + mrow(GB, 16) * (h2a + upd(t1))).astype(BF)
    patch_v[1] = (x2b + mrow(GB, 16) * (h2b + upd(t2))).astype(BF)
    for p in range(1, NP):
        wait(cp_out(p))
    pa = cp(patch_v.at[0], out_hbm.at[pl.ds(t1, 16)], SP)
    pb = cp(patch_v.at[1], out_hbm.at[pl.ds(t2, 16)], SP + 1)
    pa.start()

    @pl.when(t1 != t2)
    def _():
        pb.start()
        pb.wait()

    pa.wait()


@jax.jit
def pallas_adaLN_cond__mha_block_cached__moe_arch_mod__prompt_kernel(
    A_x: jax.Array,
    A_k_cache: jax.Array,
    A_v_cache: jax.Array,
    A_wq: jax.Array,
    A_wo: jax.Array,
    B_x: jax.Array,
    B_w_r: jax.Array,
    B_w_gate: jax.Array,
    B_w_up: jax.Array,
    B_w_down: jax.Array,
    c: jax.Array,
    w_mod: jax.Array,
):
    hbm = pl.BlockSpec(memory_space=pl.ANY)
    out = pl.pallas_call(
        _kernel,
        in_specs=[hbm] * 11,
        out_specs=hbm,
        out_shape=jax.ShapeDtypeStruct((S, D), BF),
        scratch_shapes=[
            pltpu.VMEM((H, S, DH), BF),
            pltpu.VMEM((H, S, DH), BF),
            pltpu.VMEM((NG, D, G * DH), BF),
            pltpu.VMEM((H, DH, D), BF),
            pltpu.VMEM((D, 2 * F + 128), BF),
            pltpu.VMEM((F, D + 128), BF),
            pltpu.VMEM((ZO + 16, D), BF),
            pltpu.VMEM((S, D), F32),
            pltpu.VMEM((10, 8, D), F32),
            pltpu.VMEM((2, 8, 128), I32),
            pltpu.VMEM((2, 16, D), BF),
            pltpu.VMEM((2, RP, DH), F32),
            pltpu.VMEM((RP, D), F32),
            pltpu.VMEM((2, S, 128), F32),
            pltpu.VMEM((len(CA_CHUNKS), 16, DK), F32),
            pltpu.VMEM((NH0, RP, DH), F32),
            pltpu.VMEM((NH0, 16, DH), F32),
            pltpu.VMEM((D, 128), F32),
            pltpu.VMEM((16, D), BF),
            pltpu.VMEM((5, 8, D), F32),
            pltpu.VMEM((1, D), BF),
            pltpu.VMEM((D,), BF),
            pltpu.SemaphoreType.DMA((NSEM,)),
        ],
        compiler_params=pltpu.CompilerParams(vmem_limit_bytes=120 << 20, disable_bounds_checks=True,
                                             disable_semaphore_checks=True),
        name="adaln_mha_moe",
    )(A_x.reshape(S, D), A_k_cache.reshape(H, S, DH), A_v_cache.reshape(H, S, DH), A_wq,
      A_wo.reshape(H, DH, D), B_w_r, B_w_gate, B_w_up, B_w_down, c, w_mod)
    return out.reshape(1, S, D)
```

```python
import jax
import jax.numpy as jnp
from jax import lax
import jax.experimental.pallas as pl
import jax.experimental.pallas.tpu as pltpu

S, D, H, DH, F = 2048, 1024, 32, 128, 3584
EPS = 1e-5
QSCALE = DH ** -0.5 * 1.4426950408889634
BF, F32, I32 = jnp.bfloat16, jnp.float32, jnp.int32
IMIN = -2 ** 31
NT_DIMS = (((1,), (1,)), ((), ()))

RP = 512
G = 4
NP, NG = S // RP, H // G
LNG = NG.bit_length() - 1
NT = NP * NG
SL = RP // NG
PC = 16
T0 = 2
NH0 = T0 * G
TM = NG - 4
HR = RP // 2
XE = T0 * SL // 2
EC = 128
HPOS = (2, 4, 1, 3, 0, 5, 6)
DK = D // 2
CA_CHUNKS = ((0, 768), (768, 256))
Q_BATCHES = ((0, 0, 2), (0, 2, 6), (1, 0, 4), (1, 4, 4))

HO, OO, XO, GO = 0, S, 2 * S, 3 * S
QO = GO + 32
ZO = QO + RP
SA, S1, GA, SB, S2, GB, VA, VB, VW, VC = range(10)
SX = 0
SCA = SX + 3
SCB = SCA + len(CA_CHUNKS)
SV0 = SCB + 1
SSA = SV0 + 1
SM2 = SSA + 1
SQ = SM2 + 1
SH = SQ + len(Q_BATCHES)
SGR = SH + NH0 + 1
SF = SGR + NG
SO = SF + 1
SP = SO + NP
SC = SP + 2
NSEM = SC + 1


def _recip(l):
    ri = pl.reciprocal(l, approx=True)
    return ri * (2.0 - l * ri)


def _rb(a):
    return a.astype(BF).astype(F32)


def _center(x):
    mu = jnp.mean(x, axis=-1, keepdims=True)
    xc = x - mu
    rs = lax.rsqrt(jnp.mean(xc * xc, axis=-1, keepdims=True) + EPS)
    return mu, xc, rs


def _merge(a, b):
    return jnp.maximum(a[0], b[0]), jnp.maximum(jnp.minimum(a[0], b[0]), jnp.maximum(a[1], b[1]))


def _fold(k):
    t = [k[i:i + 8] for i in range(0, k.shape[0], 8)]
    ps = [(jnp.maximum(t[i], t[i + 1]), jnp.minimum(t[i], t[i + 1])) for i in range(0, len(t), 2)]
    while len(ps) > 1:
        ps = [_merge(ps[i], ps[i + 1]) for i in range(0, len(ps), 2)]
    return ps[0]


def _kernel(x_hbm, k_hbm, v_hbm, wq_hbm, wo_hbm, wr_hbm, wg_hbm, wu_hbm, wd_hbm, c_hbm, wm_hbm,
            out_hbm,
            k_v, v_v, wq_v, wo_v, wgu_v, wd_v, hox_v, acc_v, mod_v, top_v, patch_v, of_v, xn_v, st_v,
            part_v, qf_v, qb_v, sc_v, scb_v, mp_v, c_v, wr_v, sems):
    def cp(src, dst, s):
        return pltpu.make_async_copy(src, dst, sems.at[s])

    def cp_x(i):
        rng = [[(0, RP)], [(RP, XE), (RP + HR, XE)], [(RP + XE, HR - XE), (RP + HR + XE, S - RP - HR - XE)]][i]
        return [cp(x_hbm.at[pl.ds(r0, n)], hox_v.at[pl.ds(XO + r0, n)], SX + i) for r0, n in rng]

    def cp_wm(r0, n, c0, w, s):
        return [cp(wm_hbm.at[pl.ds(r0, n), pl.ds(c0, w)], wgu_v.at[pl.ds(r0, n), pl.ds(c0, w)], s)]

    def cp_ca(i):
        return cp_wm(*CA_CHUNKS[i], D, DK, SCA + i)

    def cp_cb():
        return cp_wm(0, D, D + DK, DK, SCB)

    def cp_sa():
        return cp_wm(0, D, 0, D, SSA)

    def cp_m2():
        return cp_wm(0, D, 2 * D, 4 * D, SM2)

    def cp_wo(h, n, s):
        return cp(wo_hbm.at[pl.ds(h, n)], wo_v.at[pl.ds(h, n)], s)

    def cp_qb(i):
        half, h0, n = Q_BATCHES[i]
        cuts = sorted({h0, h0 + n} | {b for b in range(0, NH0, G) if h0 < b < h0 + n})
        return [cp(wq_hbm.at[pl.ds(half * DK, DK), pl.ds(a * DH, (b - a) * DH)],
                   wq_v.at[a // G, pl.ds(half * DK, DK), pl.ds((a % G) * DH, (b - a) * DH)], SQ + i)
                for a, b in zip(cuts[:-1], cuts[1:])]

    def cp_k0():
        return [cp(k_hbm.at[0], k_v.at[0], SH)]

    def cp_v0():
        return [cp(v_hbm.at[0], v_v.at[0], SV0)]

    def cp_head(h):
        return [cp_wo(h - 1, 1, SH + h), cp(k_hbm.at[h], k_v.at[h], SH + h), cp(v_hbm.at[h], v_v.at[h], SH + h)]

    def cp_wo_last():
        return [cp_wo(NH0 - 1, 1, SH + NH0)]

    def cp_group(g):
        h0 = g * G
        s = SGR + g
        return [cp(wq_hbm.at[:, pl.ds(pl.multiple_of(h0 * DH, G * DH), G * DH)], wq_v.at[g], s),
                cp(k_hbm.at[pl.ds(h0, G)], k_v.at[pl.ds(h0, G)], s),
                cp(v_hbm.at[pl.ds(h0, G)], v_v.at[pl.ds(h0, G)], s),
                cp_wo(h0, G, s)]

    def cp_ffn(i):
        if i == 0:
            return [cp(wu_hbm, wgu_v.at[:, pl.ds(F, F)], SF), cp(wd_hbm, wd_v.at[:, pl.ds(0, D)], SF)]
        return [cp(wg_hbm, wgu_v.at[:, pl.ds(0, F)], SF)]

    def cp_out(p):
        r0 = pl.multiple_of(p * RP, RP)
        return [cp(hox_v.at[pl.ds(OO + r0, RP)], out_hbm.at[pl.ds(r0, RP)], SO + p)]

    def cp_small():
        return [cp(c_hbm, c_v, SC), cp(wr_hbm, wr_v, SC)]

    def start(cs):
        for c_ in cs:
            c_.start()

    def wait(cs):
        for c_ in cs:
            c_.wait()

    def mrow(i, n):
        return jnp.concatenate([mod_v[i]] * (n // 8), axis=0)

    def put_mod(i, v):
        mod_v[i] = jnp.broadcast_to(v, (8, D))

    def lhs_ops(top, bot):
        w = top.shape[1] // 2
        a11, a12, a21, a22 = top[:, :w], top[:, w:], bot[:, :w], bot[:, w:]
        return [lambda: a11 + a22, lambda: a21 + a22, lambda: a11, lambda: a22,
                lambda: a11 + a12, lambda: a21 - a11, lambda: a12 - a22]

    def rhs_op(i, blk):
        f = lambda r, c: blk(r, c).astype(F32)
        if i == 1:
            return blk(0, 0)
        if i == 4:
            return blk(1, 1)
        return {
            0: lambda: f(0, 0) + f(1, 1), 2: lambda: f(0, 1) - f(1, 1), 3: lambda: f(1, 0) - f(0, 0),
            5: lambda: f(0, 0) + f(0, 1), 6: lambda: f(1, 0) + f(1, 1)}[i]().astype(BF)

    def top_of(m):
        return m(0) + m(3) - m(4) + m(6), m(2) + m(4)

    def bot_of(m):
        return m(1) + m(3), m(0) - m(1) + m(2) + m(5)

    def put_h(p, r, n, top, bot):
        base = HO + (p & 1) * (2 * RP) + r
        top = top()
        a11, a12 = top[:, :DK], top[:, DK:]
        hox_v[pl.ds(pl.multiple_of(base, 16), n), :] = jnp.concatenate([a11, a11 + a12], axis=1).astype(BF)
        ops = lhs_ops(top, bot())
        for j in (1, 2):
            hox_v[pl.ds(pl.multiple_of(base + j * HR, 16), n), :] = jnp.concatenate(
                [ops[HPOS[2 * j]](), ops[HPOS[2 * j + 1]]()], axis=1).astype(BF)
        hox_v[pl.ds(pl.multiple_of(base + 3 * HR, 16), n), 0:DK] = ops[HPOS[6]]().astype(BF)

    def ln1(p, r, n, serial):
        def rows(half):
            _, xc, rs = _center(hox_v[pl.ds(pl.multiple_of(XO + p * RP + half * HR + r, 16), n), :].astype(F32))
            return (xc * rs) * mrow(S1, n) + mrow(SA, n)

        if serial:
            put_h(p, r, n, lambda: rows(0), lambda: rows(1))
        else:
            top, bot = rows(0), rows(1)
            put_h(p, r, n, lambda: top, lambda: bot)

    def attn_rows(p, half, r, n):
        m = lambda i: acc_v[i, pl.ds(pl.multiple_of(p * HR + r, 16), n), :]
        return jnp.concatenate((top_of, bot_of)[half](m), axis=1)

    def resid(r0, n, a):
        return hox_v[pl.ds(XO + r0, n), :].astype(F32) + mrow(GA, n) * a

    def keys(r0, n, xc, rs):
        r = _rb(rs * jnp.sum(xc * mrow(VW, n), axis=-1, keepdims=True) + mrow(VC, n)[:, 0:128])
        b = lax.bitcast_convert_type(r, I32)
        b = jnp.where(b < 0, b ^ 0x7FFFFFFF, b) & (-65536)
        return b | (65535 - r0 - lax.broadcasted_iota(I32, (n, 128), 0))

    def put_stats(r0, n, mu, rs):
        st_v[0, pl.ds(r0, n), :] = jnp.broadcast_to(mu, (n, 128))
        st_v[1, pl.ds(r0, n), :] = jnp.broadcast_to(rs, (n, 128))

    def put_out(r0, n, x2, xc, rs):
        hox_v[pl.ds(OO + r0, n), :] = (x2 + mrow(VB, n) + (xc * rs) * mrow(VA, n)).astype(BF)

    def epi(p, half, r, n, valid):
        r0 = pl.multiple_of(p * RP + half * HR + r, 16)
        x2 = resid(r0, n, attn_rows(p, half, pl.multiple_of(r, 16), n))
        mu, xc, rs = _center(x2)
        put_out(r0, n, x2, xc, rs)
        put_stats(r0, n, mu, rs)
        k1, k2 = _fold(keys(r0, n, xc, rs))
        k1, k2 = _merge((top_v[0], top_v[1]), (jnp.where(valid, k1, IMIN), jnp.where(valid, k2, IMIN)))
        top_v[0] = k1
        top_v[1] = k2

    def wq_head(g, u):
        return wq_v[g, :, u * DH:(u + 1) * DH]

    def qk(q, hd, k0=0, k1=S):
        return lax.dot_general(q, k_v[hd, k0:k1, :], NT_DIMS, preferred_element_type=F32)

    def probs(s):
        p = jnp.exp2(s - jnp.max(s, axis=-1, keepdims=True)).astype(BF)
        return p, p.astype(F32)

    def pv(s, hd):
        p, pf = probs(s)
        l = jnp.sum(pf, axis=-1, keepdims=True)
        o = jnp.dot(p, v_v[hd], preferred_element_type=F32)
        return o * _recip(l), o

    def pv_carry(s, hd):
        p, pf = probs(s)
        lp = pf[:, 0:128]
        for j in range(1, S // 128):
            lp = lp + pf[:, j * 128:(j + 1) * 128]
        of_v[0] = jnp.dot(p, v_v[hd], preferred_element_type=F32)
        of_v[1] = lp

    def carried_o():
        return of_v[0] * _recip(jnp.sum(of_v[1], axis=-1, keepdims=True))

    def o_ops(oa, ob):
        return lhs_ops(jnp.concatenate([oa[:HR], ob[:HR]], axis=1), jnp.concatenate([oa[HR:], ob[HR:]], axis=1))

    def oprod(ops, i, p, hd):
        w = rhs_op(i, lambda r, c: wo_v[hd + r, :, c * DK:(c + 1) * DK])
        rows = pl.ds(pl.multiple_of(p * HR, HR), HR)
        acc_v[i, rows, :] = acc_v[i, rows, :] + jnp.dot(ops[i]().astype(BF), w, preferred_element_type=F32)

    start(cp_small())
    start(cp_x(0))
    for i in range(len(CA_CHUNKS)):
        start(cp_ca(i))
    for i in range(len(Q_BATCHES)):
        if Q_BATCHES[i][:2] == (1, 0):
            start(cp_cb())
        start(cp_qb(i))
    start(cp_sa())
    start(cp_k0())
    start(cp_v0())
    for h in range(1, NH0):
        start(cp_head(h))
        if h == 3:
            start(cp_x(1))
    start(cp_wo_last())
    start(cp_x(2))
    start(cp_group(T0))

    def clear(i, carry):
        acc_v[:, pl.ds(pl.multiple_of(i * 32, 32), 32), :] = jnp.zeros((7, 32, DK), F32)
        return carry

    lax.fori_loop(0, 20, clear, 0)
    top_v[...] = jnp.full(top_v.shape, IMIN, I32)
    mod_v[...] = jnp.zeros_like(mod_v)

    wait(cp_small())
    c = c_v[...].astype(F32)
    sc = (c * jax.nn.sigmoid(c)).astype(BF)
    scb_v[...] = jnp.broadcast_to(sc, (16, D))
    sc_v[...] = jnp.broadcast_to(sc.astype(F32), (128, D)).T
    hox_v[ZO:ZO + 16, :] = jnp.zeros((16, D), BF)
    wait(cp_x(0))
    _, xc0, rs0 = _center(hox_v[pl.ds(XO, RP), :].astype(F32))
    xn_v[...] = xc0 * rs0
    lax.fori_loop(20, NP * HR // 32, clear, 0)

    def put_s1(half, m):
        s1 = _rb(1.0 + _rb(m[0:1]))
        mod_v[S1, :, half * DK:(half + 1) * DK] = jnp.broadcast_to(s1, (8, DK))
        return s1

    for i, (r0, n) in enumerate(CA_CHUNKS):
        wait(cp_ca(i))
        part_v[i] = jnp.dot(scb_v[:, r0:r0 + n], wgu_v[r0:r0 + n, D:D + DK], preferred_element_type=F32)
    s1 = put_s1(0, part_v[0] + part_v[1])

    hs = None
    for i, (half, h0, n) in enumerate(Q_BATCHES):
        wait(cp_qb(i))
        if (half, h0) == (1, 0):
            wait(cp_cb())
            s1 = put_s1(1, jnp.dot(scb_v[...], wgu_v[:, D + DK:2 * D], preferred_element_type=F32))
        if h0 == 0:
            hs = (xn_v[:, half * DK:(half + 1) * DK] * s1).astype(BF)
        for h in range(h0, h0 + n):
            w = wq_v[h // G, half * DK:(half + 1) * DK, (h % G) * DH:(h % G + 1) * DH]
            if half == 0:
                qf_v[h] = jnp.dot(hs, w, preferred_element_type=F32)
            else:
                qf_v[h] = (qf_v[h] + jnp.dot(hs, w, preferred_element_type=F32)) * QSCALE
    wait(cp_sa())
    sab = jnp.dot(scb_v[...], wgu_v[:, 0:D], preferred_element_type=F32).astype(BF)
    put_mod(SA, sab[0:1].astype(F32))
    for h in range(NH0):
        qb_v[h] = jnp.dot(sab, wq_head(h // G, h % G), preferred_element_type=F32) * QSCALE

    def q_first(h):
        return (qf_v[h] + qb_v[h, 0:1, :]).astype(BF)

    for g in range(T0 + 1, NG):
        start(cp_group(g))
        if g == T0 + 1:
            start(cp_m2())
    wait(cp_k0())
    q = q_first(0)
    s_a = qk(q, 0, 0, 1536)
    wait(cp_v0())
    pv_carry(jnp.concatenate([s_a, qk(q, 0, 1536, S)], axis=1), 0)

    wait(cp_head(1))
    of_v[2] = carried_o()
    pv_carry(qk(q_first(1), 1), 1)

    def double(i, carry):
        h = 2 * i
        wait(cp_head(h))
        wait(cp_head(h + 1))

        @pl.when(i == 1)
        def _():
            wait(cp_x(1))

        q = q_first(h)
        hox_v[QO:QO + RP, 0:DH] = q
        ops = o_ops(of_v[2], carried_o())
        parts = [qk(q, h, 0, 512)]
        for j in (2, 5, 0, 3, 6):
            oprod(ops, j, 0, h - 2)
        parts.append(qk(q, h, 512, 1536))
        rl = jnp.minimum(i - 1, 1) * 32
        for j in range(2):
            ln1(1, rl + j * 16, 16, False)
        rh = jnp.minimum((i - 1) * 96, HR - 96)
        for j in range(6):
            r = pl.multiple_of(rh + j * 16, 16)
            put_h(0, r, 16, *[(lambda half=half: xn_v[pl.ds(half * HR + r, 16), :] * mrow(S1, 16) + mrow(SA, 16)) for half in range(2)])
        parts.append(qk(hox_v[QO:QO + RP, 0:DH], h, 1536, S))
        o0, _ = pv(jnp.concatenate(parts, axis=1), h)
        s = qk(q_first(h + 1), h + 1)
        for j in (1, 4):
            oprod(ops, j, 0, h - 2)
        pv_carry(s, h + 1)
        of_v[2] = o0
        return carry

    lax.fori_loop(1, NH0 // 2, double, 0)

    def block(t, carry):
        p = lax.shift_right_logical(t, LNG)
        g = t & (NG - 1)

        @pl.when(jnp.logical_or(t <= NG, g == 1))
        def _():
            @pl.when(t < NG)
            def _():
                wait(cp_group(t))

            @pl.when(t == T0)
            def _():
                wait(cp_wo_last())
                wait(cp_x(2))

            @pl.when(t == TM)
            def _():
                wait(cp_m2())

            @pl.when(t == NG)
            def _():
                m2 = _rb(jnp.concatenate([jnp.sum(mp_v[i], axis=0, keepdims=True) for i in range(4)], axis=1))
                sb = m2[:, D:2 * D]
                s2 = _rb(1.0 + m2[:, 2 * D:3 * D])
                gb = m2[:, 3 * D:4 * D]
                wr = wr_v[...].astype(F32).reshape(1, D)
                put_mod(GA, m2[:, 0:D])
                put_mod(SB, sb)
                put_mod(S2, s2)
                put_mod(GB, gb)
                put_mod(VA, gb * s2)
                put_mod(VB, gb * sb)
                put_mod(VW, s2 * wr)
                put_mod(VC, jnp.broadcast_to(jnp.sum(sb * wr, axis=-1, keepdims=True), (1, D)))
                start(cp_ffn(0))

            @pl.when(t == 2 * NG + 1)
            def _():
                wait(cp_ffn(0))
                start(cp_ffn(1))

            @pl.when(jnp.logical_and(g == 1, p >= 2))
            def _():
                start(cp_out(p - 2))

            @pl.when(t == NT - NG + 1)
            def _():
                wait(cp_ffn(1))

        h0 = g * G

        def qprod(i, u):
            j = HPOS.index(i)
            base = pl.multiple_of(HO + (p & 1) * (2 * RP) + (j // 2) * HR, HR)
            w = rhs_op(i, lambda r, c: wq_v[g, r * DK:(r + 1) * DK, (u + c) * DH:(u + c + 1) * DH])
            return jnp.dot(hox_v[pl.ds(base, HR), (j % 2) * DK:(j % 2 + 1) * DK], w, preferred_element_type=F32)

        def mod_quarter():
            live = jnp.logical_and(t >= TM, t < TM + 4)
            c0 = jnp.where(live, 2 * D + (t - TM) * D, jnp.where(t <= 2 * NG, 0, 4 * D))
            slot = jnp.where(live, t - TM, 4)
            link = hox_v[ZO:ZO + 16, 0:128].astype(F32)[0:8]
            for j in range(D // 128):
                a = link
                wv = wgu_v.at[:, pl.ds(pl.multiple_of(c0, D), D)]
                for k in range(0, D, 8):
                    a = a + wv[k:k + 8, j * 128:(j + 1) * 128].astype(F32) * sc_v[k:k + 8, :]
                mp_v[slot, :, j * 128:(j + 1) * 128] = a
                link = jnp.minimum(jnp.abs(a), 0.0)
            for i in range(7):
                acc_v[i, pl.ds(pl.multiple_of(NP * HR + 8 * (t & 1), 8), 8), 0:128] = link

        def q_pair(m):
            tops, bots = top_of(m.get), bot_of(m.get)
            return [(jnp.concatenate([tops[c], bots[c]], axis=0) * QSCALE).astype(BF) for c in range(2)]

        def epi_half(half):
            te = jnp.maximum(t - NG, 0)
            for i in range(SL // PC // 2):
                epi(lax.shift_right_logical(te, LNG), half, (te & (NG - 1)) * (SL // 2) + i * PC, PC, t >= NG)

        tp = t - 1
        tn = jnp.minimum(t + NG, NT - 1)
        ops = o_ops(of_v[2], carried_o())
        q0, q1 = q_pair({i: qprod(i, 0) for i in (1, 4, 0, 2, 3, 5, 6)})
        for i in range(SL // PC // 2):
            ln1(lax.shift_right_logical(tn, LNG), (tn & (NG - 1)) * (SL // 2) + i * PC, PC, True)
        for i in (2, 5, 1, 4, 0, 3, 6):
            oprod(ops, i, lax.shift_right_logical(tp, LNG), (tp & (NG - 1)) * G + G - 2)
        epi_half(0)
        s = qk(q0, h0)
        m = {i: qprod(i, 2) for i in (2, 0, 3, 5)}
        o0, raw = pv(s, h0)
        m[6] = qprod(6, 2)
        hox_v[pl.ds(pl.multiple_of(GO + 16 * (t & 1), 16), 16), 0:DH] = raw[RP - 16:RP].astype(BF)
        epi_half(1)
        s = jnp.concatenate([qk(q1[:HR], h0 + 1), qk(q1[HR:], h0 + 1)], axis=0)
        m[1] = qprod(1, 2)
        m[4] = qprod(4, 2)
        q2, q3 = q_pair(m)
        o1, _ = pv(s, h0 + 1)
        s = qk(q2, h0 + 2)
        ops = o_ops(o0, o1)
        for i in (2, 5):
            oprod(ops, i, p, h0)
        o2, _ = pv(s, h0 + 2)
        for i in (0, 6):
            oprod(ops, i, p, h0)
        mod_quarter()
        s = qk(q3, h0 + 3)
        for i in (1, 3):
            oprod(ops, i, p, h0)
        pv_carry(s, h0 + 3)
        oprod(ops, 4, p, h0)
        of_v[2] = o2
        return carry

    lax.fori_loop(T0, NT, block, 0)

    RL = S - RP
    o_last = jnp.concatenate([of_v[2], carried_o()], axis=1).astype(BF)
    w_last = jnp.concatenate([wo_v[H - 2], wo_v[H - 1]], axis=0)
    pair = (top_v[0], top_v[1])
    start(cp_out(NP - 2))
    for r in range(0, RP, EC):
        a = attn_rows(NP - 1, r // HR, r % HR, EC) + jnp.dot(o_last[r:r + EC], w_last, preferred_element_type=F32)
        x2 = resid(RL + r, EC, a)
        xn_v[r:r + EC, :] = x2
        mu, xc, rs = _center(x2)
        put_stats(RL + r, EC, mu, rs)
        pair = _merge(pair, _fold(keys(RL + r, EC, xc, rs)))
        put_out(RL + r, EC, x2, xc, rs)
    start(cp_out(NP - 1))
    for sh in (4, 2, 1):
        pair = _merge(pair, (pltpu.roll(pair[0], sh, 0), pltpu.roll(pair[1], sh, 0)))
    k1, k2 = pair

    def score(k):
        b = jnp.where(k < 0, k ^ 0x7FFFFFFF, k) & (-65536)
        return lax.bitcast_convert_type(b, F32)[0:1, 0:1]

    def row_of(k):
        i = 65535 - (k[0, 0] & 65535)
        return i, pl.multiple_of(jnp.clip(i >> 4, 0, S // 16 - 1) * 16, 16)

    i1, t1 = row_of(k1)
    i2, t2 = row_of(k2)

    def post(t0):
        pt, rt = t0 >> 9, pl.multiple_of(t0 & (HR - 1), 16)
        x2 = resid(t0, 16, jnp.where((t0 & HR) == 0, attn_rows(pt, 0, rt, 16), attn_rows(pt, 1, rt, 16)))
        tl = pl.multiple_of(jnp.maximum(t0 - RL, 0), 16)
        mu = jnp.concatenate([st_v[0, pl.ds(t0, 16), :]] * (D // 128), axis=1)
        rs = jnp.concatenate([st_v[1, pl.ds(t0, 16), :]] * (D // 128), axis=1)
        x2 = jnp.where(t0 >= RL, xn_v[pl.ds(tl, 16), :], x2)
        return x2, ((x2 - mu) * rs) * mrow(S2, 16) + mrow(SB, 16)

    x2a, h2a = post(t1)
    x2b, h2b = post(t2)
    row = lax.broadcasted_iota(I32, (16, D), 0)
    sel1 = jnp.sum(jnp.where(row == i1 - t1, h2a, 0.0), axis=0, keepdims=True)
    sel2 = jnp.sum(jnp.where(row == i2 - t2, h2b, 0.0), axis=0, keepdims=True)
    row8 = lax.broadcasted_iota(I32, (8, D), 0)
    xs = jnp.where(row8 == 0, sel1, jnp.where(row8 == 1, sel2, 0.0)).astype(BF)

    wait(cp_out(0))
    gt = jnp.dot(xs, wgu_v[:, 0:F], preferred_element_type=F32)
    up = jnp.dot(xs, wgu_v[:, F:2 * F], preferred_element_type=F32)
    act = (gt * jax.nn.sigmoid(gt) * up).astype(BF)
    y = jnp.dot(act, wd_v[:, 0:D], preferred_element_type=F32)
    y1 = y[0:1, :] * jax.nn.sigmoid(score(k1))
    y2 = y[1:2, :] * jax.nn.sigmoid(score(k2))

    def upd(t0):
        return jnp.where(row == i1 - t0, y1, 0.0) + jnp.where(row == i2 - t0, y2, 0.0)

    patch_v[0] = (x2a + mrow(GB, 16) * (h2a + upd(t1))).astype(BF)
    patch_v[1] = (x2b + mrow(GB, 16) * (h2b + upd(t2))).astype(BF)
    for p in range(1, NP):
        wait(cp_out(p))
    pa = cp(patch_v.at[0], out_hbm.at[pl.ds(t1, 16)], SP)
    pb = cp(patch_v.at[1], out_hbm.at[pl.ds(t2, 16)], SP + 1)
    pa.start()

    @pl.when(t1 != t2)
    def _():
        pb.start()
        pb.wait()

    pa.wait()


@jax.jit
def pallas_adaLN_cond__mha_block_cached__moe_arch_mod__prompt_kernel(
    A_x: jax.Array,
    A_k_cache: jax.Array,
    A_v_cache: jax.Array,
    A_wq: jax.Array,
    A_wo: jax.Array,
    B_x: jax.Array,
    B_w_r: jax.Array,
    B_w_gate: jax.Array,
    B_w_up: jax.Array,
    B_w_down: jax.Array,
    c: jax.Array,
    w_mod: jax.Array,
):
    hbm = pl.BlockSpec(memory_space=pl.ANY)
    out = pl.pallas_call(
        _kernel,
        in_specs=[hbm] * 11,
        out_specs=hbm,
        out_shape=jax.ShapeDtypeStruct((S, D), BF),
        scratch_shapes=[
            pltpu.VMEM((H, S, DH), BF),
            pltpu.VMEM((H, S, DH), BF),
            pltpu.VMEM((NG, D, G * DH), BF),
            pltpu.VMEM((H, DH, D), BF),
            pltpu.VMEM((D, 2 * F + 128), BF),
            pltpu.VMEM((F, D + 128), BF),
            pltpu.VMEM((ZO + 16, D), BF),
            pltpu.VMEM((7, NP * HR + 16, DK), F32),
            pltpu.VMEM((10, 8, D), F32),
            pltpu.VMEM((2, 8, 128), I32),
            pltpu.VMEM((2, 16, D), BF),
            pltpu.VMEM((3, RP, DH), F32),
            pltpu.VMEM((RP, D), F32),
            pltpu.VMEM((2, S, 128), F32),
            pltpu.VMEM((len(CA_CHUNKS), 16, DK), F32),
            pltpu.VMEM((NH0, RP, DH), F32),
            pltpu.VMEM((NH0, 16, DH), F32),
            pltpu.VMEM((D, 128), F32),
            pltpu.VMEM((16, D), BF),
            pltpu.VMEM((5, 8, D), F32),
            pltpu.VMEM((1, D), BF),
            pltpu.VMEM((D,), BF),
            pltpu.SemaphoreType.DMA((NSEM,)),
        ],
        compiler_params=pltpu.CompilerParams(vmem_limit_bytes=124 << 20, disable_bounds_checks=True,
                                             disable_semaphore_checks=True),
        name="adaln_mha_moe",
    )(A_x.reshape(S, D), A_k_cache.reshape(H, S, DH), A_v_cache.reshape(H, S, DH), A_wq,
      A_wo.reshape(H, DH, D), B_w_r, B_w_gate, B_w_up, B_w_down, c, w_mod)
    return out.reshape(1, S, D)
```

```python
import jax
import jax.numpy as jnp
from jax import lax
import jax.experimental.pallas as pl
import jax.experimental.pallas.tpu as pltpu

S, D, H, DH, F = 2048, 1024, 32, 128, 3584
EPS = 1e-5
QSCALE = DH ** -0.5 * 1.4426950408889634
BF, F32, I32 = jnp.bfloat16, jnp.float32, jnp.int32
IMIN = -2 ** 31
NT_DIMS = (((1,), (1,)), ((), ()))

RP = 512
G = 4
NP, NG = S // RP, H // G
LNG = NG.bit_length() - 1
NT = NP * NG
SL = RP // NG
PC = 8
T0 = 2
NH0 = T0 * G
TM = NG - 4
HR = RP // 2
XE = T0 * SL // 2
EC = 128
HPOS = (2, 4, 1, 3, 0, 5, 6)
DK = D // 2
CA_CHUNKS = ((0, 768), (768, 256))
Q_BATCHES = ((0, 0, 2), (0, 2, 6), (1, 0, 4), (1, 4, 4))

HO, OO, XO, GO = 0, S, 2 * S, 3 * S
QO = GO + 32
ZO = QO + RP
SA, S1, GA, SB, S2, GB, VA, VB, VW, VC = range(10)
SX = 0
SCA = SX + 3
SCB = SCA + len(CA_CHUNKS)
SV0 = SCB + 1
SSA = SV0 + 1
SM2 = SSA + 1
SQ = SM2 + 1
SH = SQ + len(Q_BATCHES)
SGR = SH + NH0 + 1
SF = SGR + NG
SO = SF + 1
SP = SO + NP
SC = SP + 2
NSEM = SC + 1


def _recip(l):
    ri = pl.reciprocal(l, approx=True)
    return ri * (2.0 - l * ri)


def _rb(a):
    return a.astype(BF).astype(F32)


def _center(x):
    mu = jnp.mean(x, axis=-1, keepdims=True)
    xc = x - mu
    rs = lax.rsqrt(jnp.mean(xc * xc, axis=-1, keepdims=True) + EPS)
    return mu, xc, rs


def _merge(a, b):
    return jnp.maximum(a[0], b[0]), jnp.maximum(jnp.minimum(a[0], b[0]), jnp.maximum(a[1], b[1]))


def _fold(k):
    if k.shape[0] == 8:
        return k, jnp.full(k.shape, IMIN, I32)
    t = [k[i:i + 8] for i in range(0, k.shape[0], 8)]
    ps = [(jnp.maximum(t[i], t[i + 1]), jnp.minimum(t[i], t[i + 1])) for i in range(0, len(t), 2)]
    while len(ps) > 1:
        ps = [_merge(ps[i], ps[i + 1]) for i in range(0, len(ps), 2)]
    return ps[0]


def _kernel(x_hbm, k_hbm, v_hbm, wq_hbm, wo_hbm, wr_hbm, wg_hbm, wu_hbm, wd_hbm, c_hbm, wm_hbm,
            out_hbm,
            k_v, v_v, wq_v, wo_v, wgu_v, wd_v, hox_v, acc_v, mod_v, top_v, patch_v, of_v, xn_v, st_v,
            part_v, qf_v, qb_v, sc_v, scb_v, mp_v, c_v, wr_v, sems):
    def cp(src, dst, s):
        return pltpu.make_async_copy(src, dst, sems.at[s])

    def cp_x(i):
        rng = [[(0, RP)], [(RP, XE), (RP + HR, XE)], [(RP + XE, HR - XE), (RP + HR + XE, S - RP - HR - XE)]][i]
        return [cp(x_hbm.at[pl.ds(r0, n)], hox_v.at[pl.ds(XO + r0, n)], SX + i) for r0, n in rng]

    def cp_wm(r0, n, c0, w, s):
        return [cp(wm_hbm.at[pl.ds(r0, n), pl.ds(c0, w)], wgu_v.at[pl.ds(r0, n), pl.ds(c0, w)], s)]

    def cp_ca(i):
        return cp_wm(*CA_CHUNKS[i], D, DK, SCA + i)

    def cp_cb():
        return cp_wm(0, D, D + DK, DK, SCB)

    def cp_sa():
        return cp_wm(0, D, 0, D, SSA)

    def cp_m2():
        return cp_wm(0, D, 2 * D, 4 * D, SM2)

    def cp_wo(h, n, s):
        return cp(wo_hbm.at[pl.ds(h, n)], wo_v.at[pl.ds(h, n)], s)

    def cp_qb(i):
        half, h0, n = Q_BATCHES[i]
        cuts = sorted({h0, h0 + n} | {b for b in range(0, NH0, G) if h0 < b < h0 + n})
        return [cp(wq_hbm.at[pl.ds(half * DK, DK), pl.ds(a * DH, (b - a) * DH)],
                   wq_v.at[a // G, pl.ds(half * DK, DK), pl.ds((a % G) * DH, (b - a) * DH)], SQ + i)
                for a, b in zip(cuts[:-1], cuts[1:])]

    def cp_k0():
        return [cp(k_hbm.at[0], k_v.at[0], SH)]

    def cp_v0():
        return [cp(v_hbm.at[0], v_v.at[0], SV0)]

    def cp_head(h):
        return [cp_wo(h - 1, 1, SH + h), cp(k_hbm.at[h], k_v.at[h], SH + h), cp(v_hbm.at[h], v_v.at[h], SH + h)]

    def cp_wo_last():
        return [cp_wo(NH0 - 1, 1, SH + NH0)]

    def cp_group(g):
        h0 = g * G
        s = SGR + g
        return [cp(wq_hbm.at[:, pl.ds(pl.multiple_of(h0 * DH, G * DH), G * DH)], wq_v.at[g], s),
                cp(k_hbm.at[pl.ds(h0, G)], k_v.at[pl.ds(h0, G)], s),
                cp(v_hbm.at[pl.ds(h0, G)], v_v.at[pl.ds(h0, G)], s),
                cp_wo(h0, G, s)]

    def cp_ffn(i):
        if i == 0:
            return [cp(wu_hbm, wgu_v.at[:, pl.ds(F, F)], SF), cp(wd_hbm, wd_v.at[:, pl.ds(0, D)], SF)]
        return [cp(wg_hbm, wgu_v.at[:, pl.ds(0, F)], SF)]

    def cp_out(p):
        r0 = pl.multiple_of(p * RP, RP)
        return [cp(hox_v.at[pl.ds(OO + r0, RP)], out_hbm.at[pl.ds(r0, RP)], SO + p)]

    def cp_small():
        return [cp(c_hbm, c_v, SC), cp(wr_hbm, wr_v, SC)]

    def start(cs):
        for c_ in cs:
            c_.start()

    def wait(cs):
        for c_ in cs:
            c_.wait()

    def mrow(i, n):
        return jnp.concatenate([mod_v[i]] * (n // 8), axis=0)

    def put_mod(i, v):
        mod_v[i] = jnp.broadcast_to(v, (8, D))

    def lhs_ops(top, bot):
        w = top.shape[1] // 2
        a11, a12, a21, a22 = top[:, :w], top[:, w:], bot[:, :w], bot[:, w:]
        return [lambda: a11 + a22, lambda: a21 + a22, lambda: a11, lambda: a22,
                lambda: a11 + a12, lambda: a21 - a11, lambda: a12 - a22]

    def rhs_op(i, blk):
        f = lambda r, c: blk(r, c).astype(F32)
        if i == 1:
            return blk(0, 0)
        if i == 4:
            return blk(1, 1)
        return {
            0: lambda: f(0, 0) + f(1, 1), 2: lambda: f(0, 1) - f(1, 1), 3: lambda: f(1, 0) - f(0, 0),
            5: lambda: f(0, 0) + f(0, 1), 6: lambda: f(1, 0) + f(1, 1)}[i]().astype(BF)

    def top_of(m):
        return m(0) + m(3) - m(4) + m(6), m(2) + m(4)

    def bot_of(m):
        return m(1) + m(3), m(0) - m(1) + m(2) + m(5)

    def put_h(p, r, n, top, bot):
        base = HO + (p & 1) * (2 * RP) + r
        top = top()
        a11, a12 = top[:, :DK], top[:, DK:]
        hox_v[pl.ds(pl.multiple_of(base, 8), n), :] = jnp.concatenate([a11, a11 + a12], axis=1).astype(BF)
        ops = lhs_ops(top, bot())
        for j in (1, 2):
            hox_v[pl.ds(pl.multiple_of(base + j * HR, 8), n), :] = jnp.concatenate(
                [ops[HPOS[2 * j]](), ops[HPOS[2 * j + 1]]()], axis=1).astype(BF)
        hox_v[pl.ds(pl.multiple_of(base + 3 * HR, 8), n), 0:DK] = ops[HPOS[6]]().astype(BF)

    def ln1(p, r, n, serial):
        def rows(half):
            _, xc, rs = _center(hox_v[pl.ds(pl.multiple_of(XO + p * RP + half * HR + r, 8), n), :].astype(F32))
            return (xc * rs) * mrow(S1, n) + mrow(SA, n)

        if serial:
            put_h(p, r, n, lambda: rows(0), lambda: rows(1))
        else:
            top, bot = rows(0), rows(1)
            put_h(p, r, n, lambda: top, lambda: bot)

    def attn_rows(p, half, r, n):
        m = lambda i: acc_v[i, pl.ds(pl.multiple_of(p * HR + r, 8), n), :]
        return jnp.concatenate((top_of, bot_of)[half](m), axis=1)

    def resid(r0, n, a):
        return hox_v[pl.ds(XO + r0, n), :].astype(F32) + mrow(GA, n) * a

    def keys(r0, n, xc, rs):
        r = _rb(rs * jnp.sum(xc * mrow(VW, n), axis=-1, keepdims=True) + mrow(VC, n)[:, 0:128])
        b = lax.bitcast_convert_type(r, I32)
        b = jnp.where(b < 0, b ^ 0x7FFFFFFF, b) & (-65536)
        return b | (65535 - r0 - lax.broadcasted_iota(I32, (n, 128), 0))

    def put_stats(r0, n, mu, rs):
        st_v[0, pl.ds(r0, n), :] = jnp.broadcast_to(mu, (n, 128))
        st_v[1, pl.ds(r0, n), :] = jnp.broadcast_to(rs, (n, 128))

    def put_out(r0, n, x2, xc, rs):
        hox_v[pl.ds(OO + r0, n), :] = (x2 + mrow(VB, n) + (xc * rs) * mrow(VA, n)).astype(BF)

    def epi(p, half, r, n, valid):
        r0 = pl.multiple_of(p * RP + half * HR + r, 8)
        x2 = resid(r0, n, attn_rows(p, half, pl.multiple_of(r, 8), n))
        mu, xc, rs = _center(x2)
        put_out(r0, n, x2, xc, rs)
        put_stats(r0, n, mu, rs)
        k1, k2 = _fold(keys(r0, n, xc, rs))
        k1, k2 = _merge((top_v[0], top_v[1]), (jnp.where(valid, k1, IMIN), jnp.where(valid, k2, IMIN)))
        top_v[0] = k1
        top_v[1] = k2

    def wq_head(g, u):
        return wq_v[g, :, u * DH:(u + 1) * DH]

    def qk(q, hd, k0=0, k1=S):
        return lax.dot_general(q, k_v[hd, k0:k1, :], NT_DIMS, preferred_element_type=F32)

    def probs(s):
        p = jnp.exp2(s - jnp.max(s, axis=-1, keepdims=True)).astype(BF)
        return p, p.astype(F32)

    def pv(s, hd):
        p, pf = probs(s)
        l = jnp.sum(pf, axis=-1, keepdims=True)
        o = jnp.dot(p, v_v[hd], preferred_element_type=F32)
        return o * _recip(l), o

    def pv_carry(s, hd):
        p, pf = probs(s)
        lp = pf[:, 0:128]
        for j in range(1, S // 128):
            lp = lp + pf[:, j * 128:(j + 1) * 128]
        of_v[0] = jnp.dot(p, v_v[hd], preferred_element_type=F32)
        of_v[1] = lp

    def carried_o():
        return of_v[0] * _recip(jnp.sum(of_v[1], axis=-1, keepdims=True))

    def o_ops(oa, ob):
        return lhs_ops(jnp.concatenate([oa[:HR], ob[:HR]], axis=1), jnp.concatenate([oa[HR:], ob[HR:]], axis=1))

    def oprod(ops, i, p, hd):
        w = rhs_op(i, lambda r, c: wo_v[hd + r, :, c * DK:(c + 1) * DK])
        rows = pl.ds(pl.multiple_of(p * HR, HR), HR)
        acc_v[i, rows, :] = acc_v[i, rows, :] + jnp.dot(ops[i]().astype(BF), w, preferred_element_type=F32)

    start(cp_small())
    start(cp_x(0))
    for i in range(len(CA_CHUNKS)):
        start(cp_ca(i))
    for i in range(len(Q_BATCHES)):
        if Q_BATCHES[i][:2] == (1, 0):
            start(cp_cb())
        start(cp_qb(i))
    start(cp_sa())
    start(cp_k0())
    start(cp_v0())
    for h in range(1, NH0):
        start(cp_head(h))
        if h == 3:
            start(cp_x(1))
    start(cp_wo_last())
    start(cp_x(2))
    start(cp_group(T0))

    def clear(i, carry):
        acc_v[:, pl.ds(pl.multiple_of(i * 32, 32), 32), :] = jnp.zeros((7, 32, DK), F32)
        return carry

    lax.fori_loop(0, 20, clear, 0)
    top_v[...] = jnp.full(top_v.shape, IMIN, I32)
    mod_v[...] = jnp.zeros_like(mod_v)

    wait(cp_small())
    c = c_v[...].astype(F32)
    sc = (c * jax.nn.sigmoid(c)).astype(BF)
    scb_v[...] = jnp.broadcast_to(sc, (16, D))
    sc_v[...] = jnp.broadcast_to(sc.astype(F32), (128, D)).T
    hox_v[ZO:ZO + 16, :] = jnp.zeros((16, D), BF)
    wait(cp_x(0))
    _, xc0, rs0 = _center(hox_v[pl.ds(XO, RP), :].astype(F32))
    xn_v[...] = xc0 * rs0
    lax.fori_loop(20, NP * HR // 32, clear, 0)

    def put_s1(half, m):
        s1 = _rb(1.0 + _rb(m[0:1]))
        mod_v[S1, :, half * DK:(half + 1) * DK] = jnp.broadcast_to(s1, (8, DK))
        return s1

    for i, (r0, n) in enumerate(CA_CHUNKS):
        wait(cp_ca(i))
        part_v[i] = jnp.dot(scb_v[:, r0:r0 + n], wgu_v[r0:r0 + n, D:D + DK], preferred_element_type=F32)
    s1 = put_s1(0, part_v[0] + part_v[1])

    hs = None
    for i, (half, h0, n) in enumerate(Q_BATCHES):
        wait(cp_qb(i))
        if (half, h0) == (1, 0):
            wait(cp_cb())
            s1 = put_s1(1, jnp.dot(scb_v[...], wgu_v[:, D + DK:2 * D], preferred_element_type=F32))
        if h0 == 0:
            hs = (xn_v[:, half * DK:(half + 1) * DK] * s1).astype(BF)
        for h in range(h0, h0 + n):
            w = wq_v[h // G, half * DK:(half + 1) * DK, (h % G) * DH:(h % G + 1) * DH]
            if half == 0:
                qf_v[h] = jnp.dot(hs, w, preferred_element_type=F32)
            else:
                qf_v[h] = (qf_v[h] + jnp.dot(hs, w, preferred_element_type=F32)) * QSCALE
    wait(cp_sa())
    sab = jnp.dot(scb_v[...], wgu_v[:, 0:D], preferred_element_type=F32).astype(BF)
    put_mod(SA, sab[0:1].astype(F32))
    for h in range(NH0):
        qb_v[h] = jnp.dot(sab, wq_head(h // G, h % G), preferred_element_type=F32) * QSCALE

    def q_first(h):
        return (qf_v[h] + qb_v[h, 0:1, :]).astype(BF)

    for g in range(T0 + 1, NG):
        start(cp_group(g))
        if g == T0 + 1:
            start(cp_m2())
    wait(cp_k0())
    q = q_first(0)
    s_a = qk(q, 0, 0, 1536)
    wait(cp_v0())
    pv_carry(jnp.concatenate([s_a, qk(q, 0, 1536, S)], axis=1), 0)

    wait(cp_head(1))
    of_v[2] = carried_o()
    pv_carry(qk(q_first(1), 1), 1)

    def double(i, carry):
        h = 2 * i
        wait(cp_head(h))
        wait(cp_head(h + 1))

        @pl.when(i == 1)
        def _():
            wait(cp_x(1))

        q = q_first(h)
        hox_v[QO:QO + RP, 0:DH] = q
        ops = o_ops(of_v[2], carried_o())
        parts = [qk(q, h, 0, 512)]
        for j in (2, 5, 0, 3, 6):
            oprod(ops, j, 0, h - 2)
        parts.append(qk(q, h, 512, 1536))
        rl = jnp.minimum(i - 1, 1) * 32
        for j in range(2):
            ln1(1, rl + j * 16, 16, False)
        rh = jnp.minimum((i - 1) * 96, HR - 96)
        for j in range(6):
            r = pl.multiple_of(rh + j * 16, 16)
            put_h(0, r, 16, *[(lambda half=half: xn_v[pl.ds(half * HR + r, 16), :] * mrow(S1, 16) + mrow(SA, 16)) for half in range(2)])
        parts.append(qk(hox_v[QO:QO + RP, 0:DH], h, 1536, S))
        o0, _ = pv(jnp.concatenate(parts, axis=1), h)
        s = qk(q_first(h + 1), h + 1)
        for j in (1, 4):
            oprod(ops, j, 0, h - 2)
        pv_carry(s, h + 1)
        of_v[2] = o0
        return carry

    lax.fori_loop(1, NH0 // 2, double, 0)

    def block(t, carry):
        p = lax.shift_right_logical(t, LNG)
        g = t & (NG - 1)

        @pl.when(jnp.logical_or(t <= NG, g == 1))
        def _():
            @pl.when(t < NG)
            def _():
                wait(cp_group(t))

            @pl.when(t == T0)
            def _():
                wait(cp_wo_last())
                wait(cp_x(2))

            @pl.when(t == TM)
            def _():
                wait(cp_m2())

            @pl.when(t == NG)
            def _():
                m2 = _rb(jnp.concatenate([jnp.sum(mp_v[i], axis=0, keepdims=True) for i in range(4)], axis=1))
                sb = m2[:, D:2 * D]
                s2 = _rb(1.0 + m2[:, 2 * D:3 * D])
                gb = m2[:, 3 * D:4 * D]
                wr = wr_v[...].astype(F32).reshape(1, D)
                put_mod(GA, m2[:, 0:D])
                put_mod(SB, sb)
                put_mod(S2, s2)
                put_mod(GB, gb)
                put_mod(VA, gb * s2)
                put_mod(VB, gb * sb)
                put_mod(VW, s2 * wr)
                put_mod(VC, jnp.broadcast_to(jnp.sum(sb * wr, axis=-1, keepdims=True), (1, D)))
                start(cp_ffn(0))

            @pl.when(t == 2 * NG + 1)
            def _():
                wait(cp_ffn(0))
                start(cp_ffn(1))

            @pl.when(jnp.logical_and(g == 1, p >= 2))
            def _():
                start(cp_out(p - 2))

            @pl.when(t == NT - NG + 1)
            def _():
                wait(cp_ffn(1))

        h0 = g * G

        def qprod(i, u):
            j = HPOS.index(i)
            base = pl.multiple_of(HO + (p & 1) * (2 * RP) + (j // 2) * HR, HR)
            w = rhs_op(i, lambda r, c: wq_v[g, r * DK:(r + 1) * DK, (u + c) * DH:(u + c + 1) * DH])
            return jnp.dot(hox_v[pl.ds(base, HR), (j % 2) * DK:(j % 2 + 1) * DK], w, preferred_element_type=F32)

        def mod_quarter():
            live = jnp.logical_and(t >= TM, t < TM + 4)
            c0 = jnp.where(live, 2 * D + (t - TM) * D, jnp.where(t <= 2 * NG, 0, 4 * D))
            slot = jnp.where(live, t - TM, 4)
            link = hox_v[ZO:ZO + 16, 0:128].astype(F32)[0:8]
            for j in range(D // 128):
                a = link
                wv = wgu_v.at[:, pl.ds(pl.multiple_of(c0, D), D)]
                for k in range(0, D, 8):
                    a = a + wv[k:k + 8, j * 128:(j + 1) * 128].astype(F32) * sc_v[k:k + 8, :]
                mp_v[slot, :, j * 128:(j + 1) * 128] = a
                link = jnp.minimum(jnp.abs(a), 0.0)
            for i in range(7):
                acc_v[i, pl.ds(pl.multiple_of(NP * HR + 8 * (t & 1), 8), 8), 0:128] = link

        def q_even(m):
            return (jnp.concatenate([m[0] + m[3] - m[4] + m[6], m[1] + m[3]], axis=0) * QSCALE).astype(BF)

        def q_odd(m):
            return (jnp.concatenate([m[2] + m[4], m[0] - m[1] + m[2] + m[5]], axis=0) * QSCALE).astype(BF)

        def ln_next(i):
            tn = jnp.minimum(t + NG, NT - 1)
            ln1(lax.shift_right_logical(tn, LNG), (tn & (NG - 1)) * (SL // 2) + i * PC, PC, True)

        def epi_half(half):
            te = jnp.maximum(t - NG, 0)
            for i in range(SL // PC // 2):
                epi(lax.shift_right_logical(te, LNG), half, (te & (NG - 1)) * (SL // 2) + i * PC, PC, t >= NG)

        def gate(raw):
            hox_v[pl.ds(pl.multiple_of(GO + 16 * (t & 1), 16), 16), 0:DH] = raw[RP - 16:RP].astype(BF)

        tp = t - 1
        ops = o_ops(of_v[2], carried_o())
        m = {i: qprod(i, 0) for i in (1, 4, 0, 2, 3, 5, 6)}
        q0, q1 = q_even(m), q_odd(m)
        ln_next(0)
        ln_next(1)
        for i in (2, 5, 1, 4, 0, 3, 6):
            oprod(ops, i, lax.shift_right_logical(tp, LNG), (tp & (NG - 1)) * G + G - 2)
        epi_half(0)
        s = qk(q0, h0)
        m = {i: qprod(i, 2) for i in (2, 0, 3, 6)}
        o0, raw = pv(s, h0)
        gate(raw)
        epi_half(1)
        s = jnp.concatenate([qk(q1[:HR], h0 + 1), qk(q1[HR:], h0 + 1)], axis=0)
        m[1] = qprod(1, 2)
        m[4] = qprod(4, 2)
        q2 = q_even(m)
        o1, raw = pv(s, h0 + 1)
        gate(raw)
        ln_next(2)
        ln_next(3)
        s = qk(q2, h0 + 2)
        ops = o_ops(o0, o1)
        for i in (2, 5):
            oprod(ops, i, p, h0)
        m[5] = qprod(5, 2)
        q3 = q_odd(m)
        o2, _ = pv(s, h0 + 2)
        for i in (0, 6):
            oprod(ops, i, p, h0)
        s = qk(q3, h0 + 3)
        for i in (1, 3):
            oprod(ops, i, p, h0)
        mod_quarter()
        pv_carry(s, h0 + 3)
        oprod(ops, 4, p, h0)
        of_v[2] = o2
        return carry

    lax.fori_loop(T0, NT, block, 0)

    RL = S - RP
    o_last = jnp.concatenate([of_v[2], carried_o()], axis=1).astype(BF)
    w_last = jnp.concatenate([wo_v[H - 2], wo_v[H - 1]], axis=0)
    pair = (top_v[0], top_v[1])
    start(cp_out(NP - 2))
    for r in range(0, RP, EC):
        a = attn_rows(NP - 1, r // HR, r % HR, EC) + jnp.dot(o_last[r:r + EC], w_last, preferred_element_type=F32)
        x2 = resid(RL + r, EC, a)
        xn_v[r:r + EC, :] = x2
        mu, xc, rs = _center(x2)
        put_stats(RL + r, EC, mu, rs)
        pair = _merge(pair, _fold(keys(RL + r, EC, xc, rs)))
        put_out(RL + r, EC, x2, xc, rs)
    start(cp_out(NP - 1))
    for sh in (4, 2, 1):
        pair = _merge(pair, (pltpu.roll(pair[0], sh, 0), pltpu.roll(pair[1], sh, 0)))
    k1, k2 = pair

    def score(k):
        b = jnp.where(k < 0, k ^ 0x7FFFFFFF, k) & (-65536)
        return lax.bitcast_convert_type(b, F32)[0:1, 0:1]

    def row_of(k):
        i = 65535 - (k[0, 0] & 65535)
        return i, pl.multiple_of(jnp.clip(i >> 4, 0, S // 16 - 1) * 16, 16)

    i1, t1 = row_of(k1)
    i2, t2 = row_of(k2)

    def post(t0):
        pt, rt = t0 >> 9, pl.multiple_of(t0 & (HR - 1), 16)
        x2 = resid(t0, 16, jnp.where((t0 & HR) == 0, attn_rows(pt, 0, rt, 16), attn_rows(pt, 1, rt, 16)))
        tl = pl.multiple_of(jnp.maximum(t0 - RL, 0), 16)
        mu = jnp.concatenate([st_v[0, pl.ds(t0, 16), :]] * (D // 128), axis=1)
        rs = jnp.concatenate([st_v[1, pl.ds(t0, 16), :]] * (D // 128), axis=1)
        x2 = jnp.where(t0 >= RL, xn_v[pl.ds(tl, 16), :], x2)
        return x2, ((x2 - mu) * rs) * mrow(S2, 16) + mrow(SB, 16)

    x2a, h2a = post(t1)
    x2b, h2b = post(t2)
    row = lax.broadcasted_iota(I32, (16, D), 0)
    sel1 = jnp.sum(jnp.where(row == i1 - t1, h2a, 0.0), axis=0, keepdims=True)
    sel2 = jnp.sum(jnp.where(row == i2 - t2, h2b, 0.0), axis=0, keepdims=True)
    row8 = lax.broadcasted_iota(I32, (8, D), 0)
    xs = jnp.where(row8 == 0, sel1, jnp.where(row8 == 1, sel2, 0.0)).astype(BF)

    wait(cp_out(0))
    gt = jnp.dot(xs, wgu_v[:, 0:F], preferred_element_type=F32)
    up = jnp.dot(xs, wgu_v[:, F:2 * F], preferred_element_type=F32)
    act = (gt * jax.nn.sigmoid(gt) * up).astype(BF)
    y = jnp.dot(act, wd_v[:, 0:D], preferred_element_type=F32)
    y1 = y[0:1, :] * jax.nn.sigmoid(score(k1))
    y2 = y[1:2, :] * jax.nn.sigmoid(score(k2))

    def upd(t0):
        return jnp.where(row == i1 - t0, y1, 0.0) + jnp.where(row == i2 - t0, y2, 0.0)

    patch_v[0] = (x2a + mrow(GB, 16) * (h2a + upd(t1))).astype(BF)
    patch_v[1] = (x2b + mrow(GB, 16) * (h2b + upd(t2))).astype(BF)
    for p in range(1, NP):
        wait(cp_out(p))
    pa = cp(patch_v.at[0], out_hbm.at[pl.ds(t1, 16)], SP)
    pb = cp(patch_v.at[1], out_hbm.at[pl.ds(t2, 16)], SP + 1)
    pa.start()

    @pl.when(t1 != t2)
    def _():
        pb.start()
        pb.wait()

    pa.wait()


@jax.jit
def pallas_adaLN_cond__mha_block_cached__moe_arch_mod__prompt_kernel(
    A_x: jax.Array,
    A_k_cache: jax.Array,
    A_v_cache: jax.Array,
    A_wq: jax.Array,
    A_wo: jax.Array,
    B_x: jax.Array,
    B_w_r: jax.Array,
    B_w_gate: jax.Array,
    B_w_up: jax.Array,
    B_w_down: jax.Array,
    c: jax.Array,
    w_mod: jax.Array,
):
    hbm = pl.BlockSpec(memory_space=pl.ANY)
    out = pl.pallas_call(
        _kernel,
        in_specs=[hbm] * 11,
        out_specs=hbm,
        out_shape=jax.ShapeDtypeStruct((S, D), BF),
        scratch_shapes=[
            pltpu.VMEM((H, S, DH), BF),
            pltpu.VMEM((H, S, DH), BF),
            pltpu.VMEM((NG, D, G * DH), BF),
            pltpu.VMEM((H, DH, D), BF),
            pltpu.VMEM((D, 2 * F + 128), BF),
            pltpu.VMEM((F, D + 128), BF),
            pltpu.VMEM((ZO + 16, D), BF),
            pltpu.VMEM((7, NP * HR + 16, DK), F32),
            pltpu.VMEM((10, 8, D), F32),
            pltpu.VMEM((2, 8, 128), I32),
            pltpu.VMEM((2, 16, D), BF),
            pltpu.VMEM((3, RP, DH), F32),
            pltpu.VMEM((RP, D), F32),
            pltpu.VMEM((2, S, 128), F32),
            pltpu.VMEM((len(CA_CHUNKS), 16, DK), F32),
            pltpu.VMEM((NH0, RP, DH), F32),
            pltpu.VMEM((NH0, 16, DH), F32),
            pltpu.VMEM((D, 128), F32),
            pltpu.VMEM((16, D), BF),
            pltpu.VMEM((5, 8, D), F32),
            pltpu.VMEM((1, D), BF),
            pltpu.VMEM((D,), BF),
            pltpu.SemaphoreType.DMA((NSEM,)),
        ],
        compiler_params=pltpu.CompilerParams(vmem_limit_bytes=124 << 20, disable_bounds_checks=True,
                                             disable_semaphore_checks=True),
        name="adaln_mha_moe",
    )(A_x.reshape(S, D), A_k_cache.reshape(H, S, DH), A_v_cache.reshape(H, S, DH), A_wq,
      A_wo.reshape(H, DH, D), B_w_r, B_w_gate, B_w_up, B_w_down, c, w_mod)
    return out.reshape(1, S, D)
```

```python
import jax
import jax.numpy as jnp
from jax import lax
import jax.experimental.pallas as pl
import jax.experimental.pallas.tpu as pltpu

S, D, H, DH, F = 2048, 1024, 32, 128, 3584
EPS = 1e-5
QSCALE = DH ** -0.5 * 1.4426950408889634
BF, F32, I32 = jnp.bfloat16, jnp.float32, jnp.int32
IMIN = -2 ** 31
NT_DIMS = (((1,), (1,)), ((), ()))

RP = 512
G = 4
NP, NG = S // RP, H // G
LNG = NG.bit_length() - 1
NT = NP * NG
SL = RP // NG
PC = 8
T0 = 2
NH0 = T0 * G
TM = NG - 4
HR = RP // 2
QR = RP // 4
XE = T0 * SL // 4
ECS = (64, 64, 128, 128, 64, 64)
DK = D // 2
CA_CHUNKS = ((0, 768), (768, 256))
Q_BATCHES = ((0, 0, 2), (0, 2, 6), (1, 0, 4), (1, 4, 4))

LHS = (((1, 0, 0), (1, 1, 1)), ((1, 1, 0), (1, 1, 1)), ((1, 0, 0),), ((1, 1, 1),),
       ((1, 0, 0), (1, 0, 1)), ((1, 1, 0), (-1, 0, 0)), ((1, 0, 1), (-1, 1, 1)))
RHS = (((1, 0, 0), (1, 1, 1)), ((1, 0, 0),), ((1, 0, 1), (-1, 1, 1)), ((1, 1, 0), (-1, 0, 0)),
       ((1, 1, 1),), ((1, 0, 0), (1, 0, 1)), ((1, 1, 0), (1, 1, 1)))
OUT = {(0, 0): ((1, 0), (1, 3), (-1, 4), (1, 6)), (0, 1): ((1, 2), (1, 4)),
       (1, 0): ((1, 1), (1, 3)), (1, 1): ((1, 0), (-1, 1), (1, 2), (1, 5))}
_T, _R = (2, 4), (1, 3, 0, 5, 6)
STAGES = [[(i, j) for i in u for j in v] for u, v in ((_T, _T), (_T, _R), (_R, _T), (_R, _R))]
HPOS = [ij for stage in STAGES for ij in stage]
HROWS = 13 * QR

HO, OO = 0, 2 * HROWS
XO, GO = OO + S, OO + 2 * S
QO = GO + 32
ZO = QO + RP
SA, S1, GA, SB, S2, GB, VA, VB, VW, VC = range(10)
SX = 0
SCA = SX + 3
SCB = SCA + len(CA_CHUNKS)
SV0 = SCB + 1
SSA = SV0 + 1
SM2 = SSA + 1
SQ = SM2 + 1
SH = SQ + len(Q_BATCHES)
SGR = SH + NH0 + 1
SF = SGR + NG
SO = SF + 1
SP = SO + NP
SC = SP + 2
NSEM = SC + 1


def _comb(terms, f):
    acc = f(*terms[0][1:])
    for sign, *idx in terms[1:]:
        acc = acc + f(*idx) if sign > 0 else acc - f(*idx)
    return acc


def _memo(f):
    cache = {}

    def g(*k):
        if k not in cache:
            cache[k] = f(*k)
        return cache[k]

    return g


def _half(z, c):
    w = z.shape[1] // 2
    return z[:, c * w:(c + 1) * w]


def _recip(l):
    ri = pl.reciprocal(l, approx=True)
    return ri * (2.0 - l * ri)


def _rb(a):
    return a.astype(BF).astype(F32)


def _center(x):
    mu = jnp.mean(x, axis=-1, keepdims=True)
    xc = x - mu
    rs = lax.rsqrt(jnp.mean(xc * xc, axis=-1, keepdims=True) + EPS)
    return mu, xc, rs


def _merge(a, b):
    return jnp.maximum(a[0], b[0]), jnp.maximum(jnp.minimum(a[0], b[0]), jnp.maximum(a[1], b[1]))


def _fold(k):
    if k.shape[0] == 8:
        return k, jnp.full(k.shape, IMIN, I32)
    t = [k[i:i + 8] for i in range(0, k.shape[0], 8)]
    ps = [(jnp.maximum(t[i], t[i + 1]), jnp.minimum(t[i], t[i + 1])) for i in range(0, len(t), 2)]
    while len(ps) > 1:
        ps = [_merge(ps[i], ps[i + 1]) if i + 1 < len(ps) else ps[i] for i in range(0, len(ps), 2)]
    return ps[0]


def _kernel(x_hbm, k_hbm, v_hbm, wq_hbm, wo_hbm, wr_hbm, wg_hbm, wu_hbm, wd_hbm, c_hbm, wm_hbm,
            out_hbm,
            k_v, v_v, wq_v, wo_v, wgu_v, wd_v, hox_v, acc_v, mod_v, top_v, patch_v, of_v, xn_v, st_v,
            part_v, qf_v, qb_v, sc_v, scb_v, mp_v, c_v, wr_v, sems):
    def cp(src, dst, s):
        return pltpu.make_async_copy(src, dst, sems.at[s])

    def cp_x(i):
        rng = [[(0, RP)], [(RP + j * QR, XE) for j in range(4)],
               [(RP + j * QR + XE, QR - XE) for j in range(3)] + [(RP + 3 * QR + XE, S - RP - 3 * QR - XE)]][i]
        return [cp(x_hbm.at[pl.ds(r0, n)], hox_v.at[pl.ds(XO + r0, n)], SX + i) for r0, n in rng]

    def cp_wm(r0, n, c0, w, s):
        return [cp(wm_hbm.at[pl.ds(r0, n), pl.ds(c0, w)], wgu_v.at[pl.ds(r0, n), pl.ds(c0, w)], s)]

    def cp_ca(i):
        return cp_wm(*CA_CHUNKS[i], D, DK, SCA + i)

    def cp_cb():
        return cp_wm(0, D, D + DK, DK, SCB)

    def cp_sa():
        return cp_wm(0, D, 0, D, SSA)

    def cp_m2():
        return cp_wm(0, D, 2 * D, 4 * D, SM2)

    def cp_wo(h, n, s):
        return cp(wo_hbm.at[pl.ds(h, n)], wo_v.at[pl.ds(h, n)], s)

    def cp_qb(i):
        half, h0, n = Q_BATCHES[i]
        cuts = sorted({h0, h0 + n} | {b for b in range(0, NH0, G) if h0 < b < h0 + n})
        return [cp(wq_hbm.at[pl.ds(half * DK, DK), pl.ds(a * DH, (b - a) * DH)],
                   wq_v.at[a // G, pl.ds(half * DK, DK), pl.ds((a % G) * DH, (b - a) * DH)], SQ + i)
                for a, b in zip(cuts[:-1], cuts[1:])]

    def cp_k0():
        return [cp(k_hbm.at[0], k_v.at[0], SH)]

    def cp_v0():
        return [cp(v_hbm.at[0], v_v.at[0], SV0)]

    def cp_head(h):
        return [cp_wo(h - 1, 1, SH + h), cp(k_hbm.at[h], k_v.at[h], SH + h), cp(v_hbm.at[h], v_v.at[h], SH + h)]

    def cp_wo_last():
        return [cp_wo(NH0 - 1, 1, SH + NH0)]

    def cp_group(g):
        h0 = g * G
        s = SGR + g
        return [cp(wq_hbm.at[:, pl.ds(pl.multiple_of(h0 * DH, G * DH), G * DH)], wq_v.at[g], s),
                cp(k_hbm.at[pl.ds(h0, G)], k_v.at[pl.ds(h0, G)], s),
                cp(v_hbm.at[pl.ds(h0, G)], v_v.at[pl.ds(h0, G)], s),
                cp_wo(h0, G, s)]

    def cp_ffn(i):
        if i == 0:
            return [cp(wu_hbm, wgu_v.at[:, pl.ds(F, F)], SF), cp(wd_hbm, wd_v.at[:, pl.ds(0, D)], SF)]
        return [cp(wg_hbm, wgu_v.at[:, pl.ds(0, F)], SF)]

    def cp_out(p):
        r0 = pl.multiple_of(p * RP, RP)
        return [cp(hox_v.at[pl.ds(OO + r0, RP)], out_hbm.at[pl.ds(r0, RP)], SO + p)]

    def cp_small():
        return [cp(c_hbm, c_v, SC), cp(wr_hbm, wr_v, SC)]

    def start(cs):
        for c_ in cs:
            c_.start()

    def wait(cs):
        for c_ in cs:
            c_.wait()

    def mrow(i, n):
        return jnp.concatenate([mod_v[i]] * (n // 8), axis=0)

    def put_mod(i, v):
        mod_v[i] = jnp.broadcast_to(v, (8, D))

    def put_h(p, r, n, quarter):
        base = HO + (p & 1) * HROWS + r
        hq = {}
        lvl1 = _memo(lambda i, d: _comb(LHS[i], lambda u, c: _half(hq[2 * u + d], c)))
        done = 0
        for j in range(4):
            hq[j] = quarter(j)
            end = done + len(STAGES[j])
            while done < end:
                k = min(end, (done // 4 + 1) * 4)
                ops = [_comb(LHS[v], lambda d, c: _half(lvl1(u, d), c)) for u, v in HPOS[done:k]]
                hox_v[pl.ds(pl.multiple_of(base + (done // 4) * QR, 8), n),
                      (done % 4) * 256:(done % 4 + k - done) * 256] = jnp.concatenate(ops, axis=1).astype(BF)
                done = k

    def ln1(p, r, n, serial):
        def rows(j):
            _, xc, rs = _center(hox_v[pl.ds(pl.multiple_of(XO + p * RP + j * QR + r, 8), n), :].astype(F32))
            return (xc * rs) * mrow(S1, n) + mrow(SA, n)

        if serial:
            put_h(p, r, n, rows)
        else:
            hs_ = [rows(j) for j in range(4)]
            put_h(p, r, n, lambda j: hs_[j])

    def attn_rows(p, half, r, n):
        m = lambda i: acc_v[i, pl.ds(pl.multiple_of(p * HR + r, 8), n), :]
        return jnp.concatenate([_comb(OUT[half, c], m) for c in range(2)], axis=1)

    def resid(r0, n, a):
        return hox_v[pl.ds(XO + r0, n), :].astype(F32) + mrow(GA, n) * a

    def keys(r0, n, xc, rs):
        r = _rb(rs * jnp.sum(xc * mrow(VW, n), axis=-1, keepdims=True) + mrow(VC, n)[:, 0:128])
        b = lax.bitcast_convert_type(r, I32)
        b = jnp.where(b < 0, b ^ 0x7FFFFFFF, b) & (-65536)
        return b | (65535 - r0 - lax.broadcasted_iota(I32, (n, 128), 0))

    def put_stats(r0, n, mu, rs):
        st_v[0, pl.ds(r0, n), :] = jnp.broadcast_to(mu, (n, 128))
        st_v[1, pl.ds(r0, n), :] = jnp.broadcast_to(rs, (n, 128))

    def put_out(r0, n, x2, xc, rs):
        hox_v[pl.ds(OO + r0, n), :] = (x2 + mrow(VB, n) + (xc * rs) * mrow(VA, n)).astype(BF)

    def epi(p, half, r, n, valid):
        r0 = pl.multiple_of(p * RP + half * HR + r, 8)
        x2 = resid(r0, n, attn_rows(p, half, pl.multiple_of(r, 8), n))
        mu, xc, rs = _center(x2)
        put_out(r0, n, x2, xc, rs)
        put_stats(r0, n, mu, rs)
        k1, k2 = _fold(keys(r0, n, xc, rs))
        k1, k2 = _merge((top_v[0], top_v[1]), (jnp.where(valid, k1, IMIN), jnp.where(valid, k2, IMIN)))
        top_v[0] = k1
        top_v[1] = k2

    def wq_head(g, u):
        return wq_v[g, :, u * DH:(u + 1) * DH]

    def qk(q, hd, k0=0, k1=S):
        return lax.dot_general(q, k_v[hd, k0:k1, :], NT_DIMS, preferred_element_type=F32)

    def probs(s):
        p = jnp.exp2(s - jnp.max(s, axis=-1, keepdims=True)).astype(BF)
        return p, p.astype(F32)

    def pv(s, hd):
        p, pf = probs(s)
        l = jnp.sum(pf, axis=-1, keepdims=True)
        o = jnp.dot(p, v_v[hd], preferred_element_type=F32)
        return o * _recip(l), o

    def pv_carry(s, hd):
        p, pf = probs(s)
        lp = pf[:, 0:128]
        for j in range(1, S // 128):
            lp = lp + pf[:, j * 128:(j + 1) * 128]
        of_v[0] = jnp.dot(p, v_v[hd], preferred_element_type=F32)
        of_v[1] = lp

    def carried_o():
        return of_v[0] * _recip(jnp.sum(of_v[1], axis=-1, keepdims=True))

    def oprod(o, i, p, hd):
        blk = lambda r, c: wo_v[hd + r, :, c * DK:(c + 1) * DK]
        w = blk(*RHS[i][0][1:]) if len(RHS[i]) == 1 else _comb(RHS[i], lambda r, c: blk(r, c).astype(F32)).astype(BF)
        rows = pl.ds(pl.multiple_of(p * HR, HR), HR)
        lhs = _comb(LHS[i], lambda r, c: o[c][r * HR:(r + 1) * HR]).astype(BF)
        acc_v[i, rows, :] = acc_v[i, rows, :] + jnp.dot(lhs, w, preferred_element_type=F32)

    start(cp_small())
    start(cp_x(0))
    for i in range(len(CA_CHUNKS)):
        start(cp_ca(i))
    for i in range(len(Q_BATCHES)):
        if Q_BATCHES[i][:2] == (1, 0):
            start(cp_cb())
        start(cp_qb(i))
    start(cp_sa())
    start(cp_k0())
    start(cp_v0())
    for h in range(1, NH0):
        start(cp_head(h))
        if h == 3:
            start(cp_x(1))
    start(cp_wo_last())
    start(cp_x(2))
    start(cp_group(T0))

    def clear(i, carry):
        acc_v[:, pl.ds(pl.multiple_of(i * 32, 32), 32), :] = jnp.zeros((7, 32, DK), F32)
        return carry

    lax.fori_loop(0, 20, clear, 0)
    top_v[...] = jnp.full(top_v.shape, IMIN, I32)
    mod_v[...] = jnp.zeros_like(mod_v)

    wait(cp_small())
    c = c_v[...].astype(F32)
    sc = (c * jax.nn.sigmoid(c)).astype(BF)
    scb_v[...] = jnp.broadcast_to(sc, (16, D))
    sc_v[...] = jnp.broadcast_to(sc.astype(F32), (128, D)).T
    hox_v[ZO:ZO + 16, :] = jnp.zeros((16, D), BF)
    wait(cp_x(0))
    _, xc0, rs0 = _center(hox_v[pl.ds(XO, RP), :].astype(F32))
    xn_v[...] = xc0 * rs0
    lax.fori_loop(20, NP * HR // 32, clear, 0)

    def put_s1(half, m):
        s1 = _rb(1.0 + _rb(m[0:1]))
        mod_v[S1, :, half * DK:(half + 1) * DK] = jnp.broadcast_to(s1, (8, DK))
        return s1

    for i, (r0, n) in enumerate(CA_CHUNKS):
        wait(cp_ca(i))
        part_v[i] = jnp.dot(scb_v[:, r0:r0 + n], wgu_v[r0:r0 + n, D:D + DK], preferred_element_type=F32)
    s1 = put_s1(0, part_v[0] + part_v[1])

    hs = None
    for i, (half, h0, n) in enumerate(Q_BATCHES):
        wait(cp_qb(i))
        if (half, h0) == (1, 0):
            wait(cp_cb())
            s1 = put_s1(1, jnp.dot(scb_v[...], wgu_v[:, D + DK:2 * D], preferred_element_type=F32))
        if h0 == 0:
            hs = (xn_v[:, half * DK:(half + 1) * DK] * s1).astype(BF)
        for h in range(h0, h0 + n):
            w = wq_v[h // G, half * DK:(half + 1) * DK, (h % G) * DH:(h % G + 1) * DH]
            if half == 0:
                qf_v[h] = jnp.dot(hs, w, preferred_element_type=F32)
            else:
                qf_v[h] = (qf_v[h] + jnp.dot(hs, w, preferred_element_type=F32)) * QSCALE
    wait(cp_sa())
    sab = jnp.dot(scb_v[...], wgu_v[:, 0:D], preferred_element_type=F32).astype(BF)
    put_mod(SA, sab[0:1].astype(F32))
    for h in range(NH0):
        qb_v[h] = jnp.dot(sab, wq_head(h // G, h % G), preferred_element_type=F32) * QSCALE

    def q_first(h):
        return (qf_v[h] + qb_v[h, 0:1, :]).astype(BF)

    for g in range(T0 + 1, NG):
        start(cp_group(g))
        if g == T0 + 1:
            start(cp_m2())
    wait(cp_k0())
    q = q_first(0)
    s_a = qk(q, 0, 0, 1536)
    wait(cp_v0())
    pv_carry(jnp.concatenate([s_a, qk(q, 0, 1536, S)], axis=1), 0)

    wait(cp_head(1))
    of_v[2] = carried_o()
    pv_carry(qk(q_first(1), 1), 1)

    def double(i, carry):
        h = 2 * i
        wait(cp_head(h))
        wait(cp_head(h + 1))

        @pl.when(i == 1)
        def _():
            wait(cp_x(1))

        q = q_first(h)
        hox_v[QO:QO + RP, 0:DH] = q
        ops = (of_v[2], carried_o())
        parts = [qk(q, h, 0, 512)]
        for j in (2, 5, 0, 3, 6):
            oprod(ops, j, 0, h - 2)
        parts.append(qk(q, h, 512, 1536))
        rl = jnp.minimum(i - 1, 1) * 16
        for j in range(2):
            ln1(1, rl + j * 8, 8, False)
        rh = jnp.minimum((i - 1) * 48, QR - 48)
        for j in range(6):
            r = pl.multiple_of(rh + j * 8, 8)
            put_h(0, r, 8, lambda u: xn_v[pl.ds(u * QR + r, 8), :] * mrow(S1, 8) + mrow(SA, 8))
        parts.append(qk(hox_v[QO:QO + RP, 0:DH], h, 1536, S))
        o0, _ = pv(jnp.concatenate(parts, axis=1), h)
        s = qk(q_first(h + 1), h + 1)
        for j in (1, 4):
            oprod(ops, j, 0, h - 2)
        pv_carry(s, h + 1)
        of_v[2] = o0
        return carry

    lax.fori_loop(1, NH0 // 2, double, 0)

    def block(t, carry):
        p = lax.shift_right_logical(t, LNG)
        g = t & (NG - 1)

        @pl.when(jnp.logical_or(t <= NG, g == 1))
        def _():
            @pl.when(t < NG)
            def _():
                wait(cp_group(t))

            @pl.when(t == T0)
            def _():
                wait(cp_wo_last())
                wait(cp_x(2))

            @pl.when(t == TM)
            def _():
                wait(cp_m2())

            @pl.when(t == NG)
            def _():
                m2 = _rb(jnp.concatenate([jnp.sum(mp_v[i], axis=0, keepdims=True) for i in range(4)], axis=1))
                sb = m2[:, D:2 * D]
                s2 = _rb(1.0 + m2[:, 2 * D:3 * D])
                gb = m2[:, 3 * D:4 * D]
                wr = wr_v[...].astype(F32).reshape(1, D)
                put_mod(GA, m2[:, 0:D])
                put_mod(SB, sb)
                put_mod(S2, s2)
                put_mod(GB, gb)
                put_mod(VA, gb * s2)
                put_mod(VB, gb * sb)
                put_mod(VW, s2 * wr)
                put_mod(VC, jnp.broadcast_to(jnp.sum(sb * wr, axis=-1, keepdims=True), (1, D)))
                start(cp_ffn(0))

            @pl.when(t == 2 * NG + 1)
            def _():
                wait(cp_ffn(0))
                start(cp_ffn(1))

            @pl.when(jnp.logical_and(g == 1, p >= 2))
            def _():
                start(cp_out(p - 2))

            @pl.when(t == NT - NG + 1)
            def _():
                wait(cp_ffn(1))

        h0 = g * G

        mq = {}

        def qprods(i, js=(1, 4, 3, 0, 6, 2, 5)):
            blk = lambda R, C, r, c: wq_v[g, R * DK + r * 256:R * DK + (r + 1) * 256,
                                          C * 256 + c * DH:C * 256 + (c + 1) * DH]
            lvl1 = _memo(lambda r, c: _comb(RHS[i], lambda R, C: blk(R, C, r, c).astype(F32)))
            for j in js:
                if len(RHS[i]) == 1 and len(RHS[j]) == 1:
                    w = blk(*RHS[i][0][1:], *RHS[j][0][1:])
                else:
                    w = _comb(RHS[j], lvl1).astype(BF)
                k = HPOS.index((i, j))
                base = pl.multiple_of(HO + (p & 1) * HROWS + (k // 4) * QR, QR)
                mq[i, j] = jnp.dot(hox_v[pl.ds(base, QR), (k % 4) * 256:(k % 4 + 1) * 256], w,
                                   preferred_element_type=F32)

        mq1 = _memo(lambda i, d, c: _comb(OUT[d, c], lambda j: mq[i, j]))

        def q_of(u):
            rows = [_comb(OUT[r, u // 2], lambda i: mq1(i, d, u % 2)) for r in range(2) for d in range(2)]
            return (jnp.concatenate(rows, axis=0) * QSCALE).astype(BF)

        def mod_quarter():
            live = jnp.logical_and(t >= TM, t < TM + 4)
            c0 = jnp.where(live, 2 * D + (t - TM) * D, jnp.where(t <= 2 * NG, 0, 4 * D))
            slot = jnp.where(live, t - TM, 4)
            link = hox_v[ZO:ZO + 16, 0:128].astype(F32)[0:8]
            for j in range(D // 128):
                a = link
                wv = wgu_v.at[:, pl.ds(pl.multiple_of(c0, D), D)]
                for k in range(0, D, 8):
                    a = a + wv[k:k + 8, j * 128:(j + 1) * 128].astype(F32) * sc_v[k:k + 8, :]
                mp_v[slot, :, j * 128:(j + 1) * 128] = a
                link = jnp.minimum(jnp.abs(a), 0.0)
            for i in range(7):
                acc_v[i, pl.ds(pl.multiple_of(NP * HR + 8 * (t & 1), 8), 8), 0:128] = link

        def ln_next(i):
            tn = jnp.minimum(t + NG, NT - 1)
            ln1(lax.shift_right_logical(tn, LNG), (tn & (NG - 1)) * (SL // 4) + i * PC, PC, True)

        def epi_half(half):
            te = jnp.maximum(t - NG, 0)
            for i in range(SL // PC // 2):
                epi(lax.shift_right_logical(te, LNG), half, (te & (NG - 1)) * (SL // 2) + i * PC, PC, t >= NG)

        def gate(raw):
            hox_v[pl.ds(pl.multiple_of(GO + 16 * (t & 1), 16), 16), 0:DH] = raw[RP - 16:RP].astype(BF)

        tp = t - 1
        ops = (of_v[2], carried_o())
        for i in (1, 4, 0, 3, 6):
            qprods(i)
        q0, q1 = q_of(0), q_of(1)
        ln_next(0)
        for i in (2, 5, 1, 4, 0, 3, 6):
            oprod(ops, i, lax.shift_right_logical(tp, LNG), (tp & (NG - 1)) * G + G - 2)
        epi_half(0)
        s = qk(q0, h0)
        qprods(2)
        o0, raw = pv(s, h0)
        gate(raw)
        epi_half(1)
        s = jnp.concatenate([qk(q1[:HR], h0 + 1), qk(q1[HR:], h0 + 1)], axis=0)
        qprods(5, (1, 4, 0, 2, 3, 6))
        q2 = q_of(2)
        o1, raw = pv(s, h0 + 1)
        gate(raw)
        ln_next(1)
        s = qk(q2, h0 + 2)
        ops = (o0, o1)
        for i in (2, 5):
            oprod(ops, i, p, h0)
        qprods(5, (5,))
        q3 = q_of(3)
        o2, _ = pv(s, h0 + 2)
        for i in (0, 6):
            oprod(ops, i, p, h0)
        s = qk(q3, h0 + 3)
        for i in (1, 3):
            oprod(ops, i, p, h0)
        mod_quarter()
        pv_carry(s, h0 + 3)
        oprod(ops, 4, p, h0)
        of_v[2] = o2
        return carry

    lax.fori_loop(T0, NT, block, 0)

    RL = S - RP
    o_last = jnp.concatenate([of_v[2], carried_o()], axis=1).astype(BF)
    w_last = jnp.concatenate([wo_v[H - 2], wo_v[H - 1]], axis=0)
    pair = (top_v[0], top_v[1])
    start(cp_out(NP - 2))
    for r, EC in [(sum(ECS[:i]), n) for i, n in enumerate(ECS)]:
        a = attn_rows(NP - 1, r // HR, r % HR, EC) + jnp.dot(o_last[r:r + EC], w_last, preferred_element_type=F32)
        x2 = resid(RL + r, EC, a)
        xn_v[r:r + EC, :] = x2
        mu, xc, rs = _center(x2)
        put_stats(RL + r, EC, mu, rs)
        pair = _merge(pair, _fold(keys(RL + r, EC, xc, rs)))
        put_out(RL + r, EC, x2, xc, rs)
    start(cp_out(NP - 1))
    for sh in (4, 2, 1):
        pair = _merge(pair, (pltpu.roll(pair[0], sh, 0), pltpu.roll(pair[1], sh, 0)))
    k1, k2 = pair

    def score(k):
        b = jnp.where(k < 0, k ^ 0x7FFFFFFF, k) & (-65536)
        return lax.bitcast_convert_type(b, F32)[0:1, 0:1]

    def row_of(k):
        i = 65535 - (k[0, 0] & 65535)
        return i, pl.multiple_of(jnp.clip(i >> 3, 0, S // 8 - 1) * 8, 8)

    i1, t1 = row_of(k1)
    i2, t2 = row_of(k2)

    def post(t0):
        pt, rt = t0 >> 9, pl.multiple_of(t0 & (HR - 1), 8)
        x2 = resid(t0, 8, jnp.where((t0 & HR) == 0, attn_rows(pt, 0, rt, 8), attn_rows(pt, 1, rt, 8)))
        tl = pl.multiple_of(jnp.maximum(t0 - RL, 0), 8)
        mu = jnp.concatenate([st_v[0, pl.ds(t0, 8), :]] * (D // 128), axis=1)
        rs = jnp.concatenate([st_v[1, pl.ds(t0, 8), :]] * (D // 128), axis=1)
        x2 = jnp.where(t0 >= RL, xn_v[pl.ds(tl, 8), :], x2)
        return x2, ((x2 - mu) * rs) * mrow(S2, 8) + mrow(SB, 8)

    x2a, h2a = post(t1)
    x2b, h2b = post(t2)
    row = lax.broadcasted_iota(I32, (8, D), 0)
    sel1 = jnp.sum(jnp.where(row == i1 - t1, h2a, 0.0), axis=0, keepdims=True)
    sel2 = jnp.sum(jnp.where(row == i2 - t2, h2b, 0.0), axis=0, keepdims=True)
    row8 = lax.broadcasted_iota(I32, (8, D), 0)
    xs = jnp.where(row8 == 0, sel1, jnp.where(row8 == 1, sel2, 0.0)).astype(BF)

    wait(cp_out(0))
    gt = jnp.dot(xs, wgu_v[:, 0:F], preferred_element_type=F32)
    up = jnp.dot(xs, wgu_v[:, F:2 * F], preferred_element_type=F32)
    act = (gt * jax.nn.sigmoid(gt) * up).astype(BF)
    y = jnp.dot(act, wd_v[:, 0:D], preferred_element_type=F32)
    y1 = y[0:1, :] * jax.nn.sigmoid(score(k1))
    y2 = y[1:2, :] * jax.nn.sigmoid(score(k2))

    def upd(t0):
        return jnp.where(row == i1 - t0, y1, 0.0) + jnp.where(row == i2 - t0, y2, 0.0)

    patch_v[0] = (x2a + mrow(GB, 8) * (h2a + upd(t1))).astype(BF)
    patch_v[1] = (x2b + mrow(GB, 8) * (h2b + upd(t2))).astype(BF)
    for p in range(1, NP):
        wait(cp_out(p))
    pa = cp(patch_v.at[0], out_hbm.at[pl.ds(t1, 8)], SP)
    pb = cp(patch_v.at[1], out_hbm.at[pl.ds(t2, 8)], SP + 1)
    pa.start()

    @pl.when(t1 != t2)
    def _():
        pb.start()
        pb.wait()

    pa.wait()


@jax.jit
def pallas_adaLN_cond__mha_block_cached__moe_arch_mod__prompt_kernel(
    A_x: jax.Array,
    A_k_cache: jax.Array,
    A_v_cache: jax.Array,
    A_wq: jax.Array,
    A_wo: jax.Array,
    B_x: jax.Array,
    B_w_r: jax.Array,
    B_w_gate: jax.Array,
    B_w_up: jax.Array,
    B_w_down: jax.Array,
    c: jax.Array,
    w_mod: jax.Array,
):
    hbm = pl.BlockSpec(memory_space=pl.ANY)
    out = pl.pallas_call(
        _kernel,
        in_specs=[hbm] * 11,
        out_specs=hbm,
        out_shape=jax.ShapeDtypeStruct((S, D), BF),
        scratch_shapes=[
            pltpu.VMEM((H, S, DH), BF),
            pltpu.VMEM((H, S, DH), BF),
            pltpu.VMEM((NG, D, G * DH), BF),
            pltpu.VMEM((H, DH, D), BF),
            pltpu.VMEM((D, 2 * F + 128), BF),
            pltpu.VMEM((F, D + 128), BF),
            pltpu.VMEM((ZO + 16, D), BF),
            pltpu.VMEM((7, NP * HR + 16, DK), F32),
            pltpu.VMEM((10, 8, D), F32),
            pltpu.VMEM((2, 8, 128), I32),
            pltpu.VMEM((2, 8, D), BF),
            pltpu.VMEM((3, RP, DH), F32),
            pltpu.VMEM((RP, D), F32),
            pltpu.VMEM((2, S, 128), F32),
            pltpu.VMEM((len(CA_CHUNKS), 16, DK), F32),
            pltpu.VMEM((NH0, RP, DH), F32),
            pltpu.VMEM((NH0, 16, DH), F32),
            pltpu.VMEM((D, 128), F32),
            pltpu.VMEM((16, D), BF),
            pltpu.VMEM((5, 8, D), F32),
            pltpu.VMEM((1, D), BF),
            pltpu.VMEM((D,), BF),
            pltpu.SemaphoreType.DMA((NSEM,)),
        ],
        compiler_params=pltpu.CompilerParams(vmem_limit_bytes=124 << 20, disable_bounds_checks=True,
                                             disable_semaphore_checks=True),
        name="adaln_mha_moe",
    )(A_x.reshape(S, D), A_k_cache.reshape(H, S, DH), A_v_cache.reshape(H, S, DH), A_wq,
      A_wo.reshape(H, DH, D), B_w_r, B_w_gate, B_w_up, B_w_down, c, w_mod)
    return out.reshape(1, S, D)
```

```python
import jax
import jax.numpy as jnp
from jax import lax
import jax.experimental.pallas as pl
import jax.experimental.pallas.tpu as pltpu

S, D, H, DH, F = 2048, 1024, 32, 128, 3584
EPS = 1e-5
QSCALE = DH ** -0.5 * 1.4426950408889634
BF, F32, I32 = jnp.bfloat16, jnp.float32, jnp.int32
IMIN = -2 ** 31
NT_DIMS = (((1,), (1,)), ((), ()))

RP = 512
G = 4
NP, NG = S // RP, H // G
LNG = NG.bit_length() - 1
NT = NP * NG
SL = RP // NG
PC = 8
T0 = 2
NH0 = T0 * G
TM = NG - 4
HR = RP // 2
QR = RP // 4
XE = T0 * SL // 4
ECS = (64, 64, 128, 128, 64, 64)
DK = D // 2
CA_CHUNKS = ((0, 768), (768, 256))
Q_BATCHES = ((0, 0, 2), (0, 2, 6), (1, 0, 4), (1, 4, 4))

LHS = (((1, 0, 0), (1, 1, 1)), ((1, 1, 0), (1, 1, 1)), ((1, 0, 0),), ((1, 1, 1),),
       ((1, 0, 0), (1, 0, 1)), ((1, 1, 0), (-1, 0, 0)), ((1, 0, 1), (-1, 1, 1)))
RHS = (((1, 0, 0), (1, 1, 1)), ((1, 0, 0),), ((1, 0, 1), (-1, 1, 1)), ((1, 1, 0), (-1, 0, 0)),
       ((1, 1, 1),), ((1, 0, 0), (1, 0, 1)), ((1, 1, 0), (1, 1, 1)))
OUT = {(0, 0): ((1, 0), (1, 3), (-1, 4), (1, 6)), (0, 1): ((1, 2), (1, 4)),
       (1, 0): ((1, 1), (1, 3)), (1, 1): ((1, 0), (-1, 1), (1, 2), (1, 5))}
_T, _R = (2, 4), (1, 3, 0, 5, 6)
STAGES = [[(i, j) for i in u for j in v] for u, v in ((_T, _T), (_T, _R), (_R, _T), (_R, _R))]
HPOS = [ij for stage in STAGES for ij in stage]
HROWS = 13 * QR

HO, OO = 0, 2 * HROWS
XO, GO = OO + S, OO + 2 * S
QO = GO + 32
ZO = QO + RP
SA, S1, GA, SB, S2, GB, VA, VB, VW, VC = range(10)
SX = 0
SCA = SX + 3
SCB = SCA + len(CA_CHUNKS)
SV0 = SCB + 1
SSA = SV0 + 1
SM2 = SSA + 1
SQ = SM2 + 1
SH = SQ + len(Q_BATCHES)
SGR = SH + NH0 + 1
SF = SGR + NG
SO = SF + 1
SP = SO + NP
SC = SP + 2
NSEM = SC + 1


def _comb(terms, f):
    acc = f(*terms[0][1:])
    for sign, *idx in terms[1:]:
        acc = acc + f(*idx) if sign > 0 else acc - f(*idx)
    return acc


def _memo(f):
    cache = {}

    def g(*k):
        if k not in cache:
            cache[k] = f(*k)
        return cache[k]

    return g


def _half(z, c):
    w = z.shape[1] // 2
    return z[:, c * w:(c + 1) * w]


def _recip(l):
    ri = pl.reciprocal(l, approx=True)
    return ri * (2.0 - l * ri)


def _rb(a):
    return a.astype(BF).astype(F32)


def _center(x):
    mu = jnp.mean(x, axis=-1, keepdims=True)
    xc = x - mu
    rs = lax.rsqrt(jnp.mean(xc * xc, axis=-1, keepdims=True) + EPS)
    return mu, xc, rs


def _merge(a, b):
    return jnp.maximum(a[0], b[0]), jnp.maximum(jnp.minimum(a[0], b[0]), jnp.maximum(a[1], b[1]))


def _fold(k):
    if k.shape[0] == 8:
        return k, jnp.full(k.shape, IMIN, I32)
    t = [k[i:i + 8] for i in range(0, k.shape[0], 8)]
    ps = [(jnp.maximum(t[i], t[i + 1]), jnp.minimum(t[i], t[i + 1])) for i in range(0, len(t), 2)]
    while len(ps) > 1:
        ps = [_merge(ps[i], ps[i + 1]) if i + 1 < len(ps) else ps[i] for i in range(0, len(ps), 2)]
    return ps[0]


def _kernel(x_hbm, k_hbm, v_hbm, wq_hbm, wo_hbm, wr_hbm, wg_hbm, wu_hbm, wd_hbm, c_hbm, wm_hbm,
            out_hbm,
            k_v, v_v, wq_v, wo_v, wgu_v, wd_v, hox_v, acc_v, mod_v, top_v, patch_v, of_v, xn_v, st_v,
            part_v, qf_v, qb_v, sc_v, scb_v, mp_v, c_v, wr_v, sems):
    def cp(src, dst, s):
        return pltpu.make_async_copy(src, dst, sems.at[s])

    def cp_x(i):
        rng = [[(0, RP)], [(RP + j * QR, XE) for j in range(4)],
               [(RP + j * QR + XE, QR - XE) for j in range(3)] + [(RP + 3 * QR + XE, S - RP - 3 * QR - XE)]][i]
        return [cp(x_hbm.at[pl.ds(r0, n)], hox_v.at[pl.ds(XO + r0, n)], SX + i) for r0, n in rng]

    def cp_wm(r0, n, c0, w, s):
        return [cp(wm_hbm.at[pl.ds(r0, n), pl.ds(c0, w)], wgu_v.at[pl.ds(r0, n), pl.ds(c0, w)], s)]

    def cp_ca(i):
        return cp_wm(*CA_CHUNKS[i], D, DK, SCA + i)

    def cp_cb():
        return cp_wm(0, D, D + DK, DK, SCB)

    def cp_sa():
        return cp_wm(0, D, 0, D, SSA)

    def cp_m2():
        return cp_wm(0, D, 2 * D, 4 * D, SM2)

    def cp_wo(h, n, s):
        return cp(wo_hbm.at[pl.ds(h, n)], wo_v.at[pl.ds(h, n)], s)

    def cp_qb(i):
        half, h0, n = Q_BATCHES[i]
        cuts = sorted({h0, h0 + n} | {b for b in range(0, NH0, G) if h0 < b < h0 + n})
        return [cp(wq_hbm.at[pl.ds(half * DK, DK), pl.ds(a * DH, (b - a) * DH)],
                   wq_v.at[a // G, pl.ds(half * DK, DK), pl.ds((a % G) * DH, (b - a) * DH)], SQ + i)
                for a, b in zip(cuts[:-1], cuts[1:])]

    def cp_k0():
        return [cp(k_hbm.at[0], k_v.at[0], SH)]

    def cp_v0():
        return [cp(v_hbm.at[0], v_v.at[0], SV0)]

    def cp_head(h):
        return [cp_wo(h - 1, 1, SH + h), cp(k_hbm.at[h], k_v.at[h], SH + h), cp(v_hbm.at[h], v_v.at[h], SH + h)]

    def cp_wo_last():
        return [cp_wo(NH0 - 1, 1, SH + NH0)]

    def cp_group(g):
        h0 = g * G
        s = SGR + g
        return [cp(wq_hbm.at[:, pl.ds(pl.multiple_of(h0 * DH, G * DH), G * DH)], wq_v.at[g], s),
                cp(k_hbm.at[pl.ds(h0, G)], k_v.at[pl.ds(h0, G)], s),
                cp(v_hbm.at[pl.ds(h0, G)], v_v.at[pl.ds(h0, G)], s),
                cp_wo(h0, G, s)]

    def cp_ffn(i):
        if i == 0:
            return [cp(wu_hbm, wgu_v.at[:, pl.ds(F, F)], SF), cp(wd_hbm, wd_v.at[:, pl.ds(0, D)], SF)]
        return [cp(wg_hbm, wgu_v.at[:, pl.ds(0, F)], SF)]

    def cp_out(p):
        r0 = pl.multiple_of(p * RP, RP)
        return [cp(hox_v.at[pl.ds(OO + r0, RP)], out_hbm.at[pl.ds(r0, RP)], SO + p)]

    def cp_small():
        return [cp(c_hbm, c_v, SC), cp(wr_hbm, wr_v, SC)]

    def start(cs):
        for c_ in cs:
            c_.start()

    def wait(cs):
        for c_ in cs:
            c_.wait()

    def mrow(i, n):
        return jnp.concatenate([mod_v[i]] * (n // 8), axis=0)

    def put_mod(i, v):
        mod_v[i] = jnp.broadcast_to(v, (8, D))

    def put_h(p, r, n, quarter):
        base = HO + (p & 1) * HROWS + r
        hq = {}
        lvl1 = _memo(lambda i, d: _comb(LHS[i], lambda u, c: _half(hq[2 * u + d], c)))
        done = 0
        for j in range(4):
            hq[j] = quarter(j)
            end = done + len(STAGES[j])
            while done < end:
                k = min(end, (done // 4 + 1) * 4)
                ops = [_comb(LHS[v], lambda d, c: _half(lvl1(u, d), c)) for u, v in HPOS[done:k]]
                hox_v[pl.ds(pl.multiple_of(base + (done // 4) * QR, 8), n),
                      (done % 4) * 256:(done % 4 + k - done) * 256] = jnp.concatenate(ops, axis=1).astype(BF)
                done = k

    def ln1(p, r, n, serial):
        def rows(j):
            _, xc, rs = _center(hox_v[pl.ds(pl.multiple_of(XO + p * RP + j * QR + r, 8), n), :].astype(F32))
            return (xc * rs) * mrow(S1, n) + mrow(SA, n)

        if serial:
            put_h(p, r, n, rows)
        else:
            hs_ = [rows(j) for j in range(4)]
            put_h(p, r, n, lambda j: hs_[j])

    def attn_rows(p, half, r, n):
        m = lambda i: acc_v[i, pl.ds(pl.multiple_of(p * HR + r, 8), n), :]
        return jnp.concatenate([_comb(OUT[half, c], m) for c in range(2)], axis=1)

    def resid(r0, n, a):
        return hox_v[pl.ds(XO + r0, n), :].astype(F32) + mrow(GA, n) * a

    def keys(r0, n, xc, rs):
        r = _rb(rs * jnp.sum(xc * mrow(VW, n), axis=-1, keepdims=True) + mrow(VC, n)[:, 0:128])
        b = lax.bitcast_convert_type(r, I32)
        b = jnp.where(b < 0, b ^ 0x7FFFFFFF, b) & (-65536)
        return b | (65535 - r0 - lax.broadcasted_iota(I32, (n, 128), 0))

    def put_stats(r0, n, mu, rs):
        st_v[0, pl.ds(r0, n), :] = jnp.broadcast_to(mu, (n, 128))
        st_v[1, pl.ds(r0, n), :] = jnp.broadcast_to(rs, (n, 128))

    def put_out(r0, n, x2, xc, rs):
        hox_v[pl.ds(OO + r0, n), :] = (x2 + mrow(VB, n) + (xc * rs) * mrow(VA, n)).astype(BF)

    def epi(p, half, r, n, valid):
        r0 = pl.multiple_of(p * RP + half * HR + r, 8)
        x2 = resid(r0, n, attn_rows(p, half, pl.multiple_of(r, 8), n))
        mu, xc, rs = _center(x2)
        put_out(r0, n, x2, xc, rs)
        put_stats(r0, n, mu, rs)
        k1, k2 = _fold(keys(r0, n, xc, rs))
        k1, k2 = _merge((top_v[0], top_v[1]), (jnp.where(valid, k1, IMIN), jnp.where(valid, k2, IMIN)))
        top_v[0] = k1
        top_v[1] = k2

    def wq_head(g, u):
        return wq_v[g, :, u * DH:(u + 1) * DH]

    def qk(q, hd, k0=0, k1=S):
        return lax.dot_general(q, k_v[hd, k0:k1, :], NT_DIMS, preferred_element_type=F32)

    def probs(s):
        p = jnp.exp2(s - jnp.max(s, axis=-1, keepdims=True)).astype(BF)
        return p, p.astype(F32)

    def pv(s, hd):
        p, pf = probs(s)
        l = jnp.sum(pf, axis=-1, keepdims=True)
        o = jnp.dot(p, v_v[hd], preferred_element_type=F32)
        return o * _recip(l), o

    def pv_carry(s, hd):
        p, pf = probs(s)
        lp = pf[:, 0:128]
        for j in range(1, S // 128):
            lp = lp + pf[:, j * 128:(j + 1) * 128]
        of_v[0] = jnp.dot(p, v_v[hd], preferred_element_type=F32)
        of_v[1] = lp

    def carried_o():
        return of_v[0] * _recip(jnp.sum(of_v[1], axis=-1, keepdims=True))

    def oprod(o, i, p, hd):
        blk = lambda r, c: wo_v[hd + r, :, c * DK:(c + 1) * DK]
        w = blk(*RHS[i][0][1:]) if len(RHS[i]) == 1 else _comb(RHS[i], lambda r, c: blk(r, c).astype(F32)).astype(BF)
        rows = pl.ds(pl.multiple_of(p * HR, HR), HR)
        lhs = _comb(LHS[i], lambda r, c: o[c][r * HR:(r + 1) * HR]).astype(BF)
        acc_v[i, rows, :] = acc_v[i, rows, :] + jnp.dot(lhs, w, preferred_element_type=F32)

    start(cp_small())
    start(cp_x(0))
    for i in range(len(CA_CHUNKS)):
        start(cp_ca(i))
    for i in range(len(Q_BATCHES)):
        if Q_BATCHES[i][:2] == (1, 0):
            start(cp_cb())
        start(cp_qb(i))
    start(cp_sa())
    start(cp_k0())
    start(cp_v0())
    for h in range(1, NH0):
        start(cp_head(h))
        if h == 3:
            start(cp_x(1))
    start(cp_wo_last())
    start(cp_x(2))
    start(cp_group(T0))

    def clear(i, carry):
        acc_v[:, pl.ds(pl.multiple_of(i * 32, 32), 32), :] = jnp.zeros((7, 32, DK), F32)
        return carry

    lax.fori_loop(0, 20, clear, 0)
    top_v[...] = jnp.full(top_v.shape, IMIN, I32)
    mod_v[...] = jnp.zeros_like(mod_v)

    wait(cp_small())
    c = c_v[...].astype(F32)
    sc = (c * jax.nn.sigmoid(c)).astype(BF)
    scb_v[...] = jnp.broadcast_to(sc, (16, D))
    sc_v[...] = jnp.broadcast_to(sc.astype(F32), (128, D)).T
    hox_v[ZO:ZO + 16, :] = jnp.zeros((16, D), BF)
    wait(cp_x(0))
    _, xc0, rs0 = _center(hox_v[pl.ds(XO, RP), :].astype(F32))
    xn_v[...] = xc0 * rs0
    lax.fori_loop(20, NP * HR // 32, clear, 0)

    def put_s1(half, m):
        s1 = _rb(1.0 + _rb(m[0:1]))
        mod_v[S1, :, half * DK:(half + 1) * DK] = jnp.broadcast_to(s1, (8, DK))
        return s1

    for i, (r0, n) in enumerate(CA_CHUNKS):
        wait(cp_ca(i))
        part_v[i] = jnp.dot(scb_v[:, r0:r0 + n], wgu_v[r0:r0 + n, D:D + DK], preferred_element_type=F32)
    s1 = put_s1(0, part_v[0] + part_v[1])

    hs = None
    for i, (half, h0, n) in enumerate(Q_BATCHES):
        wait(cp_qb(i))
        if (half, h0) == (1, 0):
            wait(cp_cb())
            s1 = put_s1(1, jnp.dot(scb_v[...], wgu_v[:, D + DK:2 * D], preferred_element_type=F32))
        if h0 == 0:
            hs = (xn_v[:, half * DK:(half + 1) * DK] * s1).astype(BF)
        for h in range(h0, h0 + n):
            w = wq_v[h // G, half * DK:(half + 1) * DK, (h % G) * DH:(h % G + 1) * DH]
            if half == 0:
                qf_v[h] = jnp.dot(hs, w, preferred_element_type=F32)
            else:
                qf_v[h] = (qf_v[h] + jnp.dot(hs, w, preferred_element_type=F32)) * QSCALE
    wait(cp_sa())
    sab = jnp.dot(scb_v[...], wgu_v[:, 0:D], preferred_element_type=F32).astype(BF)
    put_mod(SA, sab[0:1].astype(F32))
    for h in range(NH0):
        qb_v[h] = jnp.dot(sab, wq_head(h // G, h % G), preferred_element_type=F32) * QSCALE

    def q_first(h):
        return (qf_v[h] + qb_v[h, 0:1, :]).astype(BF)

    for g in range(T0 + 1, NG):
        start(cp_group(g))
        if g == T0 + 1:
            start(cp_m2())
    wait(cp_k0())
    q = q_first(0)
    s_a = qk(q, 0, 0, 1536)
    wait(cp_v0())
    pv_carry(jnp.concatenate([s_a, qk(q, 0, 1536, S)], axis=1), 0)

    wait(cp_head(1))
    of_v[2] = carried_o()
    pv_carry(qk(q_first(1), 1), 1)

    def double(i, carry):
        h = 2 * i
        wait(cp_head(h))
        wait(cp_head(h + 1))

        @pl.when(i == 1)
        def _():
            wait(cp_x(1))

        q = q_first(h)
        hox_v[QO:QO + RP, 0:DH] = q
        ops = (of_v[2], carried_o())
        parts = [qk(q, h, 0, 512)]
        for j in (2, 5, 0, 3, 6):
            oprod(ops, j, 0, h - 2)
        parts.append(qk(q, h, 512, 1536))
        rl = jnp.minimum(i - 1, 1) * 16
        for j in range(2):
            ln1(1, rl + j * 8, 8, False)
        rh = jnp.minimum((i - 1) * 48, QR - 48)
        for j in range(6):
            r = pl.multiple_of(rh + j * 8, 8)
            put_h(0, r, 8, lambda u: xn_v[pl.ds(u * QR + r, 8), :] * mrow(S1, 8) + mrow(SA, 8))
        parts.append(qk(hox_v[QO:QO + RP, 0:DH], h, 1536, S))
        o0, _ = pv(jnp.concatenate(parts, axis=1), h)
        s = qk(q_first(h + 1), h + 1)
        for j in (1, 4):
            oprod(ops, j, 0, h - 2)
        pv_carry(s, h + 1)
        of_v[2] = o0
        return carry

    lax.fori_loop(1, NH0 // 2, double, 0)

    def block(t, carry):
        p = lax.shift_right_logical(t, LNG)
        g = t & (NG - 1)

        @pl.when(jnp.logical_or(t <= NG, g == 1))
        def _():
            @pl.when(t < NG)
            def _():
                wait(cp_group(t))

            @pl.when(t == T0)
            def _():
                wait(cp_wo_last())
                wait(cp_x(2))

            @pl.when(t == TM)
            def _():
                wait(cp_m2())

            @pl.when(t == NG)
            def _():
                m2 = _rb(jnp.concatenate([jnp.sum(mp_v[i], axis=0, keepdims=True) for i in range(4)], axis=1))
                sb = m2[:, D:2 * D]
                s2 = _rb(1.0 + m2[:, 2 * D:3 * D])
                gb = m2[:, 3 * D:4 * D]
                wr = wr_v[...].astype(F32).reshape(1, D)
                put_mod(GA, m2[:, 0:D])
                put_mod(SB, sb)
                put_mod(S2, s2)
                put_mod(GB, gb)
                put_mod(VA, gb * s2)
                put_mod(VB, gb * sb)
                put_mod(VW, s2 * wr)
                put_mod(VC, jnp.broadcast_to(jnp.sum(sb * wr, axis=-1, keepdims=True), (1, D)))
                start(cp_ffn(0))

            @pl.when(t == 2 * NG + 1)
            def _():
                wait(cp_ffn(0))
                start(cp_ffn(1))

            @pl.when(jnp.logical_and(g == 1, p >= 2))
            def _():
                start(cp_out(p - 2))

            @pl.when(t == NT - NG + 1)
            def _():
                wait(cp_ffn(1))

        h0 = g * G

        mq = {}

        def qprods(i, js=(1, 4, 3, 0, 6, 2, 5)):
            blk = lambda R, C, r, c: wq_v[g, R * DK + r * 256:R * DK + (r + 1) * 256,
                                          C * 256 + c * DH:C * 256 + (c + 1) * DH]
            lvl1 = _memo(lambda r, c: _comb(RHS[i], lambda R, C: blk(R, C, r, c).astype(F32)))
            for j in js:
                if len(RHS[i]) == 1 and len(RHS[j]) == 1:
                    w = blk(*RHS[i][0][1:], *RHS[j][0][1:])
                else:
                    w = _comb(RHS[j], lvl1).astype(BF)
                k = HPOS.index((i, j))
                base = pl.multiple_of(HO + (p & 1) * HROWS + (k // 4) * QR, QR)
                a = hox_v[pl.ds(base, QR), (k % 4) * 256:(k % 4 + 1) * 256]
                if len(js) == 1:
                    mq[i, j] = jnp.concatenate([jnp.dot(a[z:z + QR // 2], w, preferred_element_type=F32)
                                                for z in (0, QR // 2)], axis=0)
                else:
                    mq[i, j] = jnp.dot(a, w, preferred_element_type=F32)

        mq1 = _memo(lambda i, d, c: _comb(OUT[d, c], lambda j: mq[i, j]))

        def q_of(u):
            rows = [_comb(OUT[r, u // 2], lambda i: mq1(i, d, u % 2)) for r in range(2) for d in range(2)]
            return (jnp.concatenate(rows, axis=0) * QSCALE).astype(BF)

        def mod_quarter():
            live = jnp.logical_and(t >= TM, t < TM + 4)
            c0 = jnp.where(live, 2 * D + (t - TM) * D, jnp.where(t <= 2 * NG, 0, 4 * D))
            slot = jnp.where(live, t - TM, 4)
            link = hox_v[ZO:ZO + 16, 0:128].astype(F32)[0:8]
            for j in range(D // 128):
                a = link
                wv = wgu_v.at[:, pl.ds(pl.multiple_of(c0, D), D)]
                for k in range(0, D, 8):
                    a = a + wv[k:k + 8, j * 128:(j + 1) * 128].astype(F32) * sc_v[k:k + 8, :]
                mp_v[slot, :, j * 128:(j + 1) * 128] = a
                link = jnp.minimum(jnp.abs(a), 0.0)
            for i in range(7):
                acc_v[i, pl.ds(pl.multiple_of(NP * HR + 8 * (t & 1), 8), 8), 0:128] = link

        def ln_next(i):
            tn = jnp.minimum(t + NG, NT - 1)
            ln1(lax.shift_right_logical(tn, LNG), (tn & (NG - 1)) * (SL // 4) + i * PC, PC, True)

        def epi_half(half):
            te = jnp.maximum(t - NG, 0)
            for i in range(SL // PC // 2):
                epi(lax.shift_right_logical(te, LNG), half, (te & (NG - 1)) * (SL // 2) + i * PC, PC, t >= NG)

        def gate(raw):
            hox_v[pl.ds(pl.multiple_of(GO + 16 * (t & 1), 16), 16), 0:DH] = raw[RP - 16:RP].astype(BF)

        tp = t - 1
        ops = (of_v[2], carried_o())
        for i in (1, 4, 0, 3, 6):
            qprods(i)
        q0, q1 = q_of(0), q_of(1)
        ln_next(0)
        for i in (2, 5, 1, 4, 0, 3, 6):
            oprod(ops, i, lax.shift_right_logical(tp, LNG), (tp & (NG - 1)) * G + G - 2)
        epi_half(0)
        s = qk(q0, h0)
        qprods(2)
        o0, raw = pv(s, h0)
        gate(raw)
        epi_half(1)
        s = jnp.concatenate([qk(q1[:HR], h0 + 1), qk(q1[HR:], h0 + 1)], axis=0)
        qprods(5, (1, 4, 0, 2, 3, 6))
        q2 = q_of(2)
        o1, raw = pv(s, h0 + 1)
        gate(raw)
        ln_next(1)
        s = qk(q2, h0 + 2)
        ops = (o0, o1)
        for i in (2, 5):
            oprod(ops, i, p, h0)
        qprods(5, (5,))
        q3 = q_of(3)
        o2, _ = pv(s, h0 + 2)
        for i in (0, 6):
            oprod(ops, i, p, h0)
        s = qk(q3, h0 + 3)
        for i in (1, 3):
            oprod(ops, i, p, h0)
        mod_quarter()
        pv_carry(s, h0 + 3)
        oprod(ops, 4, p, h0)
        of_v[2] = o2
        return carry

    lax.fori_loop(T0, NT, block, 0)

    RL = S - RP
    o_last = jnp.concatenate([of_v[2], carried_o()], axis=1).astype(BF)
    w_last = jnp.concatenate([wo_v[H - 2], wo_v[H - 1]], axis=0)
    pair = (top_v[0], top_v[1])
    start(cp_out(NP - 2))
    for r, EC in [(sum(ECS[:i]), n) for i, n in enumerate(ECS)]:
        a = attn_rows(NP - 1, r // HR, r % HR, EC) + jnp.dot(o_last[r:r + EC], w_last, preferred_element_type=F32)
        x2 = resid(RL + r, EC, a)
        xn_v[r:r + EC, :] = x2
        mu, xc, rs = _center(x2)
        put_stats(RL + r, EC, mu, rs)
        pair = _merge(pair, _fold(keys(RL + r, EC, xc, rs)))
        put_out(RL + r, EC, x2, xc, rs)
    start(cp_out(NP - 1))
    for sh in (4, 2, 1):
        pair = _merge(pair, (pltpu.roll(pair[0], sh, 0), pltpu.roll(pair[1], sh, 0)))
    k1, k2 = pair

    def score(k):
        b = jnp.where(k < 0, k ^ 0x7FFFFFFF, k) & (-65536)
        return lax.bitcast_convert_type(b, F32)[0:1, 0:1]

    def row_of(k):
        i = 65535 - (k[0, 0] & 65535)
        return i, pl.multiple_of(jnp.clip(i >> 3, 0, S // 8 - 1) * 8, 8)

    i1, t1 = row_of(k1)
    i2, t2 = row_of(k2)

    def post(t0):
        pt, rt = t0 >> 9, pl.multiple_of(t0 & (HR - 1), 8)
        x2 = resid(t0, 8, jnp.where((t0 & HR) == 0, attn_rows(pt, 0, rt, 8), attn_rows(pt, 1, rt, 8)))
        tl = pl.multiple_of(jnp.maximum(t0 - RL, 0), 8)
        mu = jnp.concatenate([st_v[0, pl.ds(t0, 8), :]] * (D // 128), axis=1)
        rs = jnp.concatenate([st_v[1, pl.ds(t0, 8), :]] * (D // 128), axis=1)
        x2 = jnp.where(t0 >= RL, xn_v[pl.ds(tl, 8), :], x2)
        return x2, ((x2 - mu) * rs) * mrow(S2, 8) + mrow(SB, 8)

    x2a, h2a = post(t1)
    x2b, h2b = post(t2)
    row = lax.broadcasted_iota(I32, (8, D), 0)
    sel1 = jnp.sum(jnp.where(row == i1 - t1, h2a, 0.0), axis=0, keepdims=True)
    sel2 = jnp.sum(jnp.where(row == i2 - t2, h2b, 0.0), axis=0, keepdims=True)
    row8 = lax.broadcasted_iota(I32, (8, D), 0)
    xs = jnp.where(row8 == 0, sel1, jnp.where(row8 == 1, sel2, 0.0)).astype(BF)

    wait(cp_out(0))
    gt = jnp.dot(xs, wgu_v[:, 0:F], preferred_element_type=F32)
    up = jnp.dot(xs, wgu_v[:, F:2 * F], preferred_element_type=F32)
    act = (gt * jax.nn.sigmoid(gt) * up).astype(BF)
    y = jnp.dot(act, wd_v[:, 0:D], preferred_element_type=F32)
    y1 = y[0:1, :] * jax.nn.sigmoid(score(k1))
    y2 = y[1:2, :] * jax.nn.sigmoid(score(k2))

    def upd(t0):
        return jnp.where(row == i1 - t0, y1, 0.0) + jnp.where(row == i2 - t0, y2, 0.0)

    patch_v[0] = (x2a + mrow(GB, 8) * (h2a + upd(t1))).astype(BF)
    patch_v[1] = (x2b + mrow(GB, 8) * (h2b + upd(t2))).astype(BF)
    for p in range(1, NP):
        wait(cp_out(p))
    pa = cp(patch_v.at[0], out_hbm.at[pl.ds(t1, 8)], SP)
    pb = cp(patch_v.at[1], out_hbm.at[pl.ds(t2, 8)], SP + 1)
    pa.start()

    @pl.when(t1 != t2)
    def _():
        pb.start()
        pb.wait()

    pa.wait()


@jax.jit
def pallas_adaLN_cond__mha_block_cached__moe_arch_mod__prompt_kernel(
    A_x: jax.Array,
    A_k_cache: jax.Array,
    A_v_cache: jax.Array,
    A_wq: jax.Array,
    A_wo: jax.Array,
    B_x: jax.Array,
    B_w_r: jax.Array,
    B_w_gate: jax.Array,
    B_w_up: jax.Array,
    B_w_down: jax.Array,
    c: jax.Array,
    w_mod: jax.Array,
):
    hbm = pl.BlockSpec(memory_space=pl.ANY)
    out = pl.pallas_call(
        _kernel,
        in_specs=[hbm] * 11,
        out_specs=hbm,
        out_shape=jax.ShapeDtypeStruct((S, D), BF),
        scratch_shapes=[
            pltpu.VMEM((H, S, DH), BF),
            pltpu.VMEM((H, S, DH), BF),
            pltpu.VMEM((NG, D, G * DH), BF),
            pltpu.VMEM((H, DH, D), BF),
            pltpu.VMEM((D, 2 * F + 128), BF),
            pltpu.VMEM((F, D + 128), BF),
            pltpu.VMEM((ZO + 16, D), BF),
            pltpu.VMEM((7, NP * HR + 16, DK), F32),
            pltpu.VMEM((10, 8, D), F32),
            pltpu.VMEM((2, 8, 128), I32),
            pltpu.VMEM((2, 8, D), BF),
            pltpu.VMEM((3, RP, DH), F32),
            pltpu.VMEM((RP, D), F32),
            pltpu.VMEM((2, S, 128), F32),
            pltpu.VMEM((len(CA_CHUNKS), 16, DK), F32),
            pltpu.VMEM((NH0, RP, DH), F32),
            pltpu.VMEM((NH0, 16, DH), F32),
            pltpu.VMEM((D, 128), F32),
            pltpu.VMEM((16, D), BF),
            pltpu.VMEM((5, 8, D), F32),
            pltpu.VMEM((1, D), BF),
            pltpu.VMEM((D,), BF),
            pltpu.SemaphoreType.DMA((NSEM,)),
        ],
        compiler_params=pltpu.CompilerParams(vmem_limit_bytes=124 << 20, disable_bounds_checks=True,
                                             disable_semaphore_checks=True),
        name="adaln_mha_moe",
    )(A_x.reshape(S, D), A_k_cache.reshape(H, S, DH), A_v_cache.reshape(H, S, DH), A_wq,
      A_wo.reshape(H, DH, D), B_w_r, B_w_gate, B_w_up, B_w_down, c, w_mod)
    return out.reshape(1, S, D)
```

```python
import jax
import jax.numpy as jnp
from jax import lax
import jax.experimental.pallas as pl
import jax.experimental.pallas.tpu as pltpu

S, D, H, DH, F = 2048, 1024, 32, 128, 3584
EPS = 1e-5
QSCALE = DH ** -0.5 * 1.4426950408889634
BF, F32, I32 = jnp.bfloat16, jnp.float32, jnp.int32
IMIN = -2 ** 31
NT_DIMS = (((1,), (1,)), ((), ()))

RP = 512
G = 4
NP, NG = S // RP, H // G
LNG = NG.bit_length() - 1
NT = NP * NG
SL = RP // NG
PC = 8
T0 = 2
NH0 = T0 * G
TM = NG - 4
HR = RP // 2
QR = RP // 4
XE = T0 * SL // 4
ECS = (64, 64, 128, 128, 64, 64)
DK = D // 2
CA_CHUNKS = ((0, 768), (768, 256))
Q_BATCHES = ((0, 0, 2), (0, 2, 6), (1, 0, 4), (1, 4, 4))

LHS = (((1, 0, 0), (1, 1, 1)), ((1, 1, 0), (1, 1, 1)), ((1, 0, 0),), ((1, 1, 1),),
       ((1, 0, 0), (1, 0, 1)), ((1, 1, 0), (-1, 0, 0)), ((1, 0, 1), (-1, 1, 1)))
RHS = (((1, 0, 0), (1, 1, 1)), ((1, 0, 0),), ((1, 0, 1), (-1, 1, 1)), ((1, 1, 0), (-1, 0, 0)),
       ((1, 1, 1),), ((1, 0, 0), (1, 0, 1)), ((1, 1, 0), (1, 1, 1)))
OUT = {(0, 0): ((1, 0), (1, 3), (-1, 4), (1, 6)), (0, 1): ((1, 2), (1, 4)),
       (1, 0): ((1, 1), (1, 3)), (1, 1): ((1, 0), (-1, 1), (1, 2), (1, 5))}
_T, _R = (2, 4), (5, 0, 6, 3, 1)
STAGES = [[(i, j) for i in u for j in v] for u, v in ((_T, _T), (_T, _R), (_R, _T), (_R, _R))]
HPOS = [ij for stage in STAGES for ij in stage]
HROWS = 13 * QR

HO, OO = 0, 2 * HROWS
XO, GO = OO + S, OO + 2 * S
ZO = GO + 32
QO = OO + RP
SA, S1, GA, SB, S2, GB, VA, VB, VW, VC = range(10)
SX = 0
SCA = SX + 3
SCB = SCA + len(CA_CHUNKS)
SV0 = SCB + 1
SSA = SV0 + 1
SM2 = SSA + 1
SQ = SM2 + 1
SH = SQ + len(Q_BATCHES)
SGR = SH + NH0 + 1
SF = SGR + NG
SO = SF + 1
SP = SO + NP
SC = SP + 2
NSEM = SC + 1


def _comb(terms, f):
    acc = f(*terms[0][1:])
    for sign, *idx in terms[1:]:
        acc = acc + f(*idx) if sign > 0 else acc - f(*idx)
    return acc


def _memo(f):
    cache = {}

    def g(*k):
        if k not in cache:
            cache[k] = f(*k)
        return cache[k]

    return g


def _half(z, c):
    w = z.shape[1] // 2
    return z[:, c * w:(c + 1) * w]


def _recip(l):
    ri = pl.reciprocal(l, approx=True)
    return ri * (2.0 - l * ri)


def _rb(a):
    return a.astype(BF).astype(F32)


def _center(x):
    mu = jnp.mean(x, axis=-1, keepdims=True)
    xc = x - mu
    rs = lax.rsqrt(jnp.mean(xc * xc, axis=-1, keepdims=True) + EPS)
    return mu, xc, rs


def _merge(a, b):
    return jnp.maximum(a[0], b[0]), jnp.maximum(jnp.minimum(a[0], b[0]), jnp.maximum(a[1], b[1]))


def _fold(k):
    if k.shape[0] == 8:
        return k, jnp.full(k.shape, IMIN, I32)
    t = [k[i:i + 8] for i in range(0, k.shape[0], 8)]
    ps = [(jnp.maximum(t[i], t[i + 1]), jnp.minimum(t[i], t[i + 1])) for i in range(0, len(t), 2)]
    while len(ps) > 1:
        ps = [_merge(ps[i], ps[i + 1]) if i + 1 < len(ps) else ps[i] for i in range(0, len(ps), 2)]
    return ps[0]


def _kernel(x_hbm, k_hbm, v_hbm, wq_hbm, wo_hbm, wr_hbm, wg_hbm, wu_hbm, wd_hbm, c_hbm, wm_hbm,
            out_hbm,
            k_v, v_v, wq_v, wo_v, wgu_v, wd_v, hox_v, acc_v, mod_v, top_v, patch_v, of_v, xn_v, st_v,
            part_v, qf_v, qb_v, sc_v, scb_v, mp_v, c_v, wr_v, sems):
    def cp(src, dst, s):
        return pltpu.make_async_copy(src, dst, sems.at[s])

    def cp_x(i):
        rng = [[(0, RP)], [(RP + j * QR, XE) for j in range(4)],
               [(RP + j * QR + XE, QR - XE) for j in range(3)] + [(RP + 3 * QR + XE, S - RP - 3 * QR - XE)]][i]
        return [cp(x_hbm.at[pl.ds(r0, n)], hox_v.at[pl.ds(XO + r0, n)], SX + i) for r0, n in rng]

    def cp_wm(r0, n, c0, w, s):
        return [cp(wm_hbm.at[pl.ds(r0, n), pl.ds(c0, w)], wgu_v.at[pl.ds(r0, n), pl.ds(c0, w)], s)]

    def cp_ca(i):
        return cp_wm(*CA_CHUNKS[i], D, DK, SCA + i)

    def cp_cb():
        return cp_wm(0, D, D + DK, DK, SCB)

    def cp_sa():
        return cp_wm(0, D, 0, D, SSA)

    def cp_m2():
        return cp_wm(0, D, 2 * D, 4 * D, SM2)

    def cp_wo(h, n, s):
        return cp(wo_hbm.at[pl.ds(h, n)], wo_v.at[pl.ds(h, n)], s)

    def cp_qb(i):
        half, h0, n = Q_BATCHES[i]
        cuts = sorted({h0, h0 + n} | {b for b in range(0, NH0, G) if h0 < b < h0 + n})
        return [cp(wq_hbm.at[pl.ds(half * DK, DK), pl.ds(a * DH, (b - a) * DH)],
                   wq_v.at[a // G, pl.ds(half * DK, DK), pl.ds((a % G) * DH, (b - a) * DH)], SQ + i)
                for a, b in zip(cuts[:-1], cuts[1:])]

    def cp_k0():
        return [cp(k_hbm.at[0], k_v.at[0], SH)]

    def cp_v0():
        return [cp(v_hbm.at[0], v_v.at[0], SV0)]

    def cp_head(h):
        return [cp_wo(h - 1, 1, SH + h), cp(k_hbm.at[h], k_v.at[h], SH + h), cp(v_hbm.at[h], v_v.at[h], SH + h)]

    def cp_wo_last():
        return [cp_wo(NH0 - 1, 1, SH + NH0)]

    def cp_group(g):
        h0 = g * G
        s = SGR + g
        return [cp(wq_hbm.at[:, pl.ds(pl.multiple_of(h0 * DH, G * DH), G * DH)], wq_v.at[g], s),
                cp(k_hbm.at[pl.ds(h0, G)], k_v.at[pl.ds(h0, G)], s),
                cp(v_hbm.at[pl.ds(h0, G)], v_v.at[pl.ds(h0, G)], s),
                cp_wo(h0, G, s)]

    def cp_ffn(i):
        if i == 0:
            return [cp(wu_hbm, wgu_v.at[:, pl.ds(F, F)], SF), cp(wd_hbm, wd_v.at[:, pl.ds(0, D)], SF)]
        return [cp(wg_hbm, wgu_v.at[:, pl.ds(0, F)], SF)]

    def cp_out(p):
        r0 = pl.multiple_of(p * RP, RP)
        return [cp(hox_v.at[pl.ds(OO + r0, RP)], out_hbm.at[pl.ds(r0, RP)], SO + p)]

    def cp_small():
        return [cp(c_hbm, c_v, SC), cp(wr_hbm, wr_v, SC)]

    def start(cs):
        for c_ in cs:
            c_.start()

    def wait(cs):
        for c_ in cs:
            c_.wait()

    def mrow(i, n):
        return jnp.concatenate([mod_v[i]] * (n // 8), axis=0)

    def put_mod(i, v):
        mod_v[i] = jnp.broadcast_to(v, (8, D))

    def put_h(p, r, n, quarter):
        base = HO + (p & 1) * HROWS + r
        hq = {}
        lvl1 = _memo(lambda i, d: _comb(LHS[i], lambda u, c: _half(hq[2 * u + d], c)))
        done = 0
        for j in range(4):
            hq[j] = quarter(j)
            end = done + len(STAGES[j])
            while done < end:
                k = min(end, (done // 4 + 1) * 4)
                ops = [_comb(LHS[v], lambda d, c: _half(lvl1(u, d), c)) for u, v in HPOS[done:k]]
                hox_v[pl.ds(pl.multiple_of(base + (done // 4) * QR, 8), n),
                      (done % 4) * 256:(done % 4 + k - done) * 256] = jnp.concatenate(ops, axis=1).astype(BF)
                done = k

    def ln1(p, r, n, serial):
        def rows(j):
            _, xc, rs = _center(hox_v[pl.ds(pl.multiple_of(XO + p * RP + j * QR + r, 8), n), :].astype(F32))
            return (xc * rs) * mrow(S1, n) + mrow(SA, n)

        if serial:
            put_h(p, r, n, rows)
        else:
            hs_ = [rows(j) for j in range(4)]
            put_h(p, r, n, lambda j: hs_[j])

    def attn_rows(p, half, r, n):
        m = lambda i: acc_v[i, pl.ds(pl.multiple_of(p * HR + r, 8), n), :]
        return jnp.concatenate([_comb(OUT[half, c], m) for c in range(2)], axis=1)

    def resid(r0, n, a):
        return hox_v[pl.ds(XO + r0, n), :].astype(F32) + mrow(GA, n) * a

    def keys(r0, n, xc, rs):
        r = _rb(rs * jnp.sum(xc * mrow(VW, n), axis=-1, keepdims=True) + mrow(VC, n)[:, 0:128])
        b = lax.bitcast_convert_type(r, I32)
        b = jnp.where(b < 0, b ^ 0x7FFFFFFF, b) & (-65536)
        return b | (65535 - r0 - lax.broadcasted_iota(I32, (n, 128), 0))

    def put_stats(r0, n, mu, rs):
        st_v[0, pl.ds(r0, n), :] = jnp.broadcast_to(mu, (n, 128))
        st_v[1, pl.ds(r0, n), :] = jnp.broadcast_to(rs, (n, 128))

    def put_out(r0, n, x2, xc, rs):
        hox_v[pl.ds(OO + r0, n), :] = (x2 + mrow(VB, n) + (xc * rs) * mrow(VA, n)).astype(BF)

    def epi(p, half, r, n, valid):
        r0 = pl.multiple_of(p * RP + half * HR + r, 8)
        x2 = resid(r0, n, attn_rows(p, half, pl.multiple_of(r, 8), n))
        mu, xc, rs = _center(x2)
        put_out(r0, n, x2, xc, rs)
        put_stats(r0, n, mu, rs)
        k1, k2 = _fold(keys(r0, n, xc, rs))
        k1, k2 = _merge((top_v[0], top_v[1]), (jnp.where(valid, k1, IMIN), jnp.where(valid, k2, IMIN)))
        top_v[0] = k1
        top_v[1] = k2

    def wq_head(g, u):
        return wq_v[g, :, u * DH:(u + 1) * DH]

    def qk(q, hd, k0=0, k1=S):
        return lax.dot_general(q, k_v[hd, k0:k1, :], NT_DIMS, preferred_element_type=F32)

    def probs(s):
        p = jnp.exp2(s - jnp.max(s, axis=-1, keepdims=True)).astype(BF)
        return p, p.astype(F32)

    def pv(s, hd):
        p, pf = probs(s)
        l = jnp.sum(pf, axis=-1, keepdims=True)
        o = jnp.dot(p, v_v[hd], preferred_element_type=F32)
        return o * _recip(l), o

    def pv_carry(s, hd):
        p, pf = probs(s)
        lp = pf[:, 0:128]
        for j in range(1, S // 128):
            lp = lp + pf[:, j * 128:(j + 1) * 128]
        of_v[0] = jnp.dot(p, v_v[hd], preferred_element_type=F32)
        of_v[1] = lp

    def carried_o():
        return of_v[0] * _recip(jnp.sum(of_v[1], axis=-1, keepdims=True))

    def oprod(o, i, p, hd):
        blk = lambda r, c: wo_v[hd + r, :, c * DK:(c + 1) * DK]
        w = blk(*RHS[i][0][1:]) if len(RHS[i]) == 1 else _comb(RHS[i], lambda r, c: blk(r, c).astype(F32)).astype(BF)
        rows = pl.ds(pl.multiple_of(p * HR, HR), HR)
        lhs = _comb(LHS[i], lambda r, c: o[c][r * HR:(r + 1) * HR]).astype(BF)
        acc_v[i, rows, :] = acc_v[i, rows, :] + jnp.dot(lhs, w, preferred_element_type=F32)

    start(cp_small())
    start(cp_x(0))
    for i in range(len(CA_CHUNKS)):
        start(cp_ca(i))
    for i in range(len(Q_BATCHES)):
        if Q_BATCHES[i][:2] == (1, 0):
            start(cp_cb())
        start(cp_qb(i))
    start(cp_sa())
    start(cp_k0())
    start(cp_v0())
    for h in range(1, NH0):
        start(cp_head(h))
        if h == 3:
            start(cp_x(1))
    start(cp_wo_last())
    start(cp_x(2))
    start(cp_group(T0))

    def clear(i, carry):
        acc_v[:, pl.ds(pl.multiple_of(i * 32, 32), 32), :] = jnp.zeros((7, 32, DK), F32)
        return carry

    lax.fori_loop(0, 22, clear, 0)
    top_v[...] = jnp.full(top_v.shape, IMIN, I32)
    mod_v[...] = jnp.zeros_like(mod_v)

    wait(cp_small())
    c = c_v[...].astype(F32)
    sc = (c * jax.nn.sigmoid(c)).astype(BF)
    scb_v[...] = jnp.broadcast_to(sc, (16, D))
    hox_v[ZO:ZO + 16, :] = jnp.zeros((16, D), BF)
    wait(cp_x(0))
    _, xc0, rs0 = _center(hox_v[pl.ds(XO, RP), :].astype(F32))
    xn_v[...] = xc0 * rs0
    lax.fori_loop(22, NP * HR // 32, clear, 0)

    def put_s1(half, m):
        s1 = _rb(1.0 + _rb(m[0:1]))
        mod_v[S1, :, half * DK:(half + 1) * DK] = jnp.broadcast_to(s1, (8, DK))
        return s1

    for i, (r0, n) in enumerate(CA_CHUNKS):
        wait(cp_ca(i))
        part_v[i] = jnp.dot(scb_v[:, r0:r0 + n], wgu_v[r0:r0 + n, D:D + DK], preferred_element_type=F32)
    s1 = put_s1(0, part_v[0] + part_v[1])

    hs = None
    for i, (half, h0, n) in enumerate(Q_BATCHES):
        wait(cp_qb(i))
        if (half, h0) == (1, 0):
            wait(cp_cb())
            s1 = put_s1(1, jnp.dot(scb_v[...], wgu_v[:, D + DK:2 * D], preferred_element_type=F32))
        if i == 1:
            sc_v[...] = jnp.broadcast_to(scb_v[0:1, :].astype(F32), (128, D)).T
        if h0 == 0:
            hs = (xn_v[:, half * DK:(half + 1) * DK] * s1).astype(BF)
        for h in range(h0, h0 + n):
            w = wq_v[h // G, half * DK:(half + 1) * DK, (h % G) * DH:(h % G + 1) * DH]
            if half == 0:
                qf_v[h] = jnp.dot(hs, w, preferred_element_type=F32)
            else:
                qf_v[h] = (qf_v[h] + jnp.dot(hs, w, preferred_element_type=F32)) * QSCALE
    wait(cp_sa())
    sab = jnp.dot(scb_v[...], wgu_v[:, 0:D], preferred_element_type=F32).astype(BF)
    put_mod(SA, sab[0:1].astype(F32))
    for h in range(NH0):
        qb_v[h] = jnp.dot(sab, wq_head(h // G, h % G), preferred_element_type=F32) * QSCALE

    def q_first(h):
        return (qf_v[h] + qb_v[h, 0:1, :]).astype(BF)

    for g in range(T0 + 1, NG):
        start(cp_group(g))
        if g == T0 + 1:
            start(cp_m2())
    wait(cp_k0())
    q = q_first(0)
    s_a = qk(q, 0, 0, 1536)
    wait(cp_v0())
    pv_carry(jnp.concatenate([s_a, qk(q, 0, 1536, S)], axis=1), 0)

    wait(cp_head(1))
    of_v[2] = carried_o()
    pv_carry(qk(q_first(1), 1), 1)

    def double(i, carry):
        h = 2 * i
        wait(cp_head(h))
        wait(cp_head(h + 1))

        @pl.when(i == 1)
        def _():
            wait(cp_x(1))

        q = q_first(h)
        hox_v[QO:QO + RP, 0:DH] = q
        ops = (of_v[2], carried_o())
        parts = [qk(q, h, 0, 512)]
        for j in (2, 5, 0, 3, 6):
            oprod(ops, j, 0, h - 2)
        parts.append(qk(q, h, 512, 1536))
        rl = jnp.minimum(i - 1, 1) * 16
        for j in range(2):
            ln1(1, rl + j * 8, 8, False)
        rh = jnp.minimum((i - 1) * 48, QR - 48)
        for j in range(6):
            r = pl.multiple_of(rh + j * 8, 8)
            put_h(0, r, 8, lambda u: xn_v[pl.ds(u * QR + r, 8), :] * mrow(S1, 8) + mrow(SA, 8))
        parts.append(qk(hox_v[QO:QO + RP, 0:DH], h, 1536, S))
        o0, _ = pv(jnp.concatenate(parts, axis=1), h)
        s = qk(q_first(h + 1), h + 1)
        for j in (1, 4):
            oprod(ops, j, 0, h - 2)
        pv_carry(s, h + 1)
        of_v[2] = o0
        return carry

    lax.fori_loop(1, NH0 // 2, double, 0)

    def block(t, carry):
        p = lax.shift_right_logical(t, LNG)
        g = t & (NG - 1)

        @pl.when(jnp.logical_or(t <= NG, g == 1))
        def _():
            @pl.when(t < NG)
            def _():
                wait(cp_group(t))

            @pl.when(t == T0)
            def _():
                wait(cp_wo_last())
                wait(cp_x(2))

            @pl.when(t == TM)
            def _():
                wait(cp_m2())

            @pl.when(t == NG)
            def _():
                m2 = _rb(jnp.concatenate([jnp.sum(mp_v[i], axis=0, keepdims=True) for i in range(4)], axis=1))
                sb = m2[:, D:2 * D]
                s2 = _rb(1.0 + m2[:, 2 * D:3 * D])
                gb = m2[:, 3 * D:4 * D]
                wr = wr_v[...].astype(F32).reshape(1, D)
                put_mod(GA, m2[:, 0:D])
                put_mod(SB, sb)
                put_mod(S2, s2)
                put_mod(GB, gb)
                put_mod(VA, gb * s2)
                put_mod(VB, gb * sb)
                put_mod(VW, s2 * wr)
                put_mod(VC, jnp.broadcast_to(jnp.sum(sb * wr, axis=-1, keepdims=True), (1, D)))
                start(cp_ffn(0))

            @pl.when(t == 2 * NG + 1)
            def _():
                wait(cp_ffn(0))
                start(cp_ffn(1))

            @pl.when(jnp.logical_and(g == 1, p >= 2))
            def _():
                start(cp_out(p - 2))

            @pl.when(t == NT - NG + 1)
            def _():
                wait(cp_ffn(1))

        h0 = g * G

        mq = {}

        def qprods(i, js=(1, 4, 3, 0, 6, 2, 5)):
            blk = lambda R, C, r, c: wq_v[g, R * DK + r * 256:R * DK + (r + 1) * 256,
                                          C * 256 + c * DH:C * 256 + (c + 1) * DH]
            lvl1 = _memo(lambda r, c: _comb(RHS[i], lambda R, C: blk(R, C, r, c).astype(F32)))
            for j in js:
                if len(RHS[i]) == 1 and len(RHS[j]) == 1:
                    w = blk(*RHS[i][0][1:], *RHS[j][0][1:])
                else:
                    w = _comb(RHS[j], lvl1).astype(BF)
                k = HPOS.index((i, j))
                base = pl.multiple_of(HO + (p & 1) * HROWS + (k // 4) * QR, QR)
                a = hox_v[pl.ds(base, QR), (k % 4) * 256:(k % 4 + 1) * 256]
                if len(js) == 1:
                    mq[i, j] = jnp.concatenate([jnp.dot(a[z:z + QR // 2], w, preferred_element_type=F32)
                                                for z in (0, QR // 2)], axis=0)
                else:
                    mq[i, j] = jnp.dot(a, w, preferred_element_type=F32)

        mq1 = _memo(lambda i, d, c: _comb(OUT[d, c], lambda j: mq[i, j]))

        def q_of(u):
            rows = [_comb(OUT[r, u // 2], lambda i: mq1(i, d, u % 2)) for r in range(2) for d in range(2)]
            return (jnp.concatenate(rows, axis=0) * QSCALE).astype(BF)

        def mod_quarter():
            live = jnp.logical_and(t >= TM, t < TM + 4)
            c0 = jnp.where(live, 2 * D + (t - TM) * D, jnp.where(t <= 2 * NG, 0, 4 * D))
            slot = jnp.where(live, t - TM, 4)
            link = hox_v[ZO:ZO + 16, 0:128].astype(F32)[0:8]
            for j in range(D // 128):
                a = link
                wv = wgu_v.at[:, pl.ds(pl.multiple_of(c0, D), D)]
                prod = wv[:, j * 128:(j + 1) * 128].astype(F32) * sc_v[...]
                for k in range(0, D, 8):
                    a = a + prod[k:k + 8]
                mp_v[slot, :, j * 128:(j + 1) * 128] = a
                link = jnp.minimum(jnp.abs(a), 0.0)
            for i in range(7):
                acc_v[i, pl.ds(pl.multiple_of(NP * HR + 8 * (t & 1), 8), 8), 0:128] = link

        def ln_next(i):
            tn = jnp.minimum(t + NG, NT - 1)
            ln1(lax.shift_right_logical(tn, LNG), (tn & (NG - 1)) * (SL // 4) + i * PC, PC, True)

        def epi_half(half):
            te = jnp.maximum(t - NG, 0)
            for i in range(SL // PC // 2):
                epi(lax.shift_right_logical(te, LNG), half, (te & (NG - 1)) * (SL // 2) + i * PC, PC, t >= NG)

        def gate(raw):
            hox_v[pl.ds(pl.multiple_of(GO + 16 * (t & 1), 16), 16), 0:DH] = raw[RP - 16:RP].astype(BF)

        tp = t - 1
        ops = (of_v[2], carried_o())
        for i in (1, 4, 0, 3, 6):
            qprods(i)
        q0, q1 = q_of(0), q_of(1)
        ln_next(0)
        for i in (2, 5, 1, 4, 0, 3, 6):
            oprod(ops, i, lax.shift_right_logical(tp, LNG), (tp & (NG - 1)) * G + G - 2)
        epi_half(0)
        s = qk(q0, h0)
        qprods(2)
        o0, raw = pv(s, h0)
        gate(raw)
        epi_half(1)
        s = jnp.concatenate([qk(q1[:HR], h0 + 1), qk(q1[HR:], h0 + 1)], axis=0)
        qprods(5, (1, 4, 0, 2, 3, 6))
        q2 = q_of(2)
        o1, raw = pv(s, h0 + 1)
        gate(raw)
        ln_next(1)
        s = qk(q2, h0 + 2)
        ops = (o0, o1)
        for i in (2, 5):
            oprod(ops, i, p, h0)
        qprods(5, (5,))
        q3 = q_of(3)
        o2, _ = pv(s, h0 + 2)
        for i in (0, 6):
            oprod(ops, i, p, h0)
        s = qk(q3, h0 + 3)
        for i in (1, 3):
            oprod(ops, i, p, h0)
        mod_quarter()
        pv_carry(s, h0 + 3)
        oprod(ops, 4, p, h0)
        of_v[2] = o2
        return carry

    lax.fori_loop(T0, NT, block, 0)

    RL = S - RP
    o_last = jnp.concatenate([of_v[2], carried_o()], axis=1).astype(BF)
    w_last = jnp.concatenate([wo_v[H - 2], wo_v[H - 1]], axis=0)
    pair = (top_v[0], top_v[1])
    start(cp_out(NP - 2))
    for r, EC in [(sum(ECS[:i]), n) for i, n in enumerate(ECS)]:
        a = attn_rows(NP - 1, r // HR, r % HR, EC) + jnp.dot(o_last[r:r + EC], w_last, preferred_element_type=F32)
        x2 = resid(RL + r, EC, a)
        xn_v[r:r + EC, :] = x2
        mu, xc, rs = _center(x2)
        put_stats(RL + r, EC, mu, rs)
        pair = _merge(pair, _fold(keys(RL + r, EC, xc, rs)))
        put_out(RL + r, EC, x2, xc, rs)
    start(cp_out(NP - 1))
    for sh in (4, 2, 1):
        pair = _merge(pair, (pltpu.roll(pair[0], sh, 0), pltpu.roll(pair[1], sh, 0)))
    k1, k2 = pair

    def score(k):
        b = jnp.where(k < 0, k ^ 0x7FFFFFFF, k) & (-65536)
        return lax.bitcast_convert_type(b, F32)[0:1, 0:1]

    def row_of(k):
        i = 65535 - (k[0, 0] & 65535)
        return i, pl.multiple_of(jnp.clip(i >> 3, 0, S // 8 - 1) * 8, 8)

    i1, t1 = row_of(k1)
    i2, t2 = row_of(k2)

    def post(t0):
        pt, rt = t0 >> 9, pl.multiple_of(t0 & (HR - 1), 8)
        x2 = resid(t0, 8, jnp.where((t0 & HR) == 0, attn_rows(pt, 0, rt, 8), attn_rows(pt, 1, rt, 8)))
        tl = pl.multiple_of(jnp.maximum(t0 - RL, 0), 8)
        mu = jnp.concatenate([st_v[0, pl.ds(t0, 8), :]] * (D // 128), axis=1)
        rs = jnp.concatenate([st_v[1, pl.ds(t0, 8), :]] * (D // 128), axis=1)
        x2 = jnp.where(t0 >= RL, xn_v[pl.ds(tl, 8), :], x2)
        return x2, ((x2 - mu) * rs) * mrow(S2, 8) + mrow(SB, 8)

    x2a, h2a = post(t1)
    x2b, h2b = post(t2)
    row = lax.broadcasted_iota(I32, (8, D), 0)
    sel1 = jnp.sum(jnp.where(row == i1 - t1, h2a, 0.0), axis=0, keepdims=True)
    sel2 = jnp.sum(jnp.where(row == i2 - t2, h2b, 0.0), axis=0, keepdims=True)
    row8 = lax.broadcasted_iota(I32, (8, D), 0)
    xs = jnp.where(row8 == 0, sel1, jnp.where(row8 == 1, sel2, 0.0)).astype(BF)

    wait(cp_out(0))
    gt = jnp.dot(xs, wgu_v[:, 0:F], preferred_element_type=F32)
    up = jnp.dot(xs, wgu_v[:, F:2 * F], preferred_element_type=F32)
    act = (gt * jax.nn.sigmoid(gt) * up).astype(BF)
    y = jnp.dot(act, wd_v[:, 0:D], preferred_element_type=F32)
    y1 = y[0:1, :] * jax.nn.sigmoid(score(k1))
    y2 = y[1:2, :] * jax.nn.sigmoid(score(k2))

    def upd(t0):
        return jnp.where(row == i1 - t0, y1, 0.0) + jnp.where(row == i2 - t0, y2, 0.0)

    patch_v[0] = (x2a + mrow(GB, 8) * (h2a + upd(t1))).astype(BF)
    patch_v[1] = (x2b + mrow(GB, 8) * (h2b + upd(t2))).astype(BF)
    for p in range(1, NP):
        wait(cp_out(p))
    pa = cp(patch_v.at[0], out_hbm.at[pl.ds(t1, 8)], SP)
    pb = cp(patch_v.at[1], out_hbm.at[pl.ds(t2, 8)], SP + 1)
    pa.start()

    @pl.when(t1 != t2)
    def _():
        pb.start()
        pb.wait()

    pa.wait()


@jax.jit
def pallas_adaLN_cond__mha_block_cached__moe_arch_mod__prompt_kernel(
    A_x: jax.Array,
    A_k_cache: jax.Array,
    A_v_cache: jax.Array,
    A_wq: jax.Array,
    A_wo: jax.Array,
    B_x: jax.Array,
    B_w_r: jax.Array,
    B_w_gate: jax.Array,
    B_w_up: jax.Array,
    B_w_down: jax.Array,
    c: jax.Array,
    w_mod: jax.Array,
):
    hbm = pl.BlockSpec(memory_space=pl.ANY)
    out = pl.pallas_call(
        _kernel,
        in_specs=[hbm] * 11,
        out_specs=hbm,
        out_shape=jax.ShapeDtypeStruct((S, D), BF),
        scratch_shapes=[
            pltpu.VMEM((H, S, DH), BF),
            pltpu.VMEM((H, S, DH), BF),
            pltpu.VMEM((NG, D, G * DH), BF),
            pltpu.VMEM((H, DH, D), BF),
            pltpu.VMEM((D, 2 * F + 128), BF),
            pltpu.VMEM((F, D + 128), BF),
            pltpu.VMEM((ZO + 16, D), BF),
            pltpu.VMEM((7, NP * HR + 16, DK), F32),
            pltpu.VMEM((10, 8, D), F32),
            pltpu.VMEM((2, 8, 128), I32),
            pltpu.VMEM((2, 8, D), BF),
            pltpu.VMEM((3, RP, DH), F32),
            pltpu.VMEM((RP, D), F32),
            pltpu.VMEM((2, S, 128), F32),
            pltpu.VMEM((len(CA_CHUNKS), 16, DK), F32),
            pltpu.VMEM((NH0, RP, DH), F32),
            pltpu.VMEM((NH0, 16, DH), F32),
            pltpu.VMEM((D, 128), F32),
            pltpu.VMEM((16, D), BF),
            pltpu.VMEM((5, 8, D), F32),
            pltpu.VMEM((1, D), BF),
            pltpu.VMEM((D,), BF),
            pltpu.SemaphoreType.DMA((NSEM,)),
        ],
        compiler_params=pltpu.CompilerParams(vmem_limit_bytes=124 << 20, disable_bounds_checks=True,
                                             disable_semaphore_checks=True),
        name="adaln_mha_moe",
    )(A_x.reshape(S, D), A_k_cache.reshape(H, S, DH), A_v_cache.reshape(H, S, DH), A_wq,
      A_wo.reshape(H, DH, D), B_w_r, B_w_gate, B_w_up, B_w_down, c, w_mod)
    return out.reshape(1, S, D)
```
